```python
import jax
import jax.numpy as jnp

def _softmax(x, axis=-1):
    return jax.nn.softmax(x, axis=axis)

def _gelu(x):
    return jax.nn.gelu(x, approximate=True)

def _silu(x):
    return jax.nn.silu(x)

def _sigmoid(x):
    return jax.nn.sigmoid(x)

def _layernorm(x, axis=-1, eps=1e-05):
    m = jnp.mean(x, axis=axis, keepdims=True)
    v = jnp.var(x, axis=axis, keepdims=True)
    return (x - m) / jnp.sqrt(v + eps)

def _scatter_add(tgt, idx, src, axis=0):
    return tgt.at[idx].add(src)

def _segment_sum(src, seg, n):
    return jax.ops.segment_sum(src, seg, n)

class _Rng:

    def __init__(self, key):
        self._k = key

    def _next(self):
        self._k, sub = jax.random.split(self._k)
        return sub

    def normal(self, shape):
        return jax.random.normal(self._next(), shape, dtype=jnp.bfloat16)

    def randint(self, lo, hi, shape):
        return jax.random.randint(self._next(), shape, lo, hi, dtype=jnp.int32)

    def uniform(self, shape, lo=0.0, hi=1.0):
        return jax.random.uniform(self._next(), shape, jnp.bfloat16, lo, hi)

    def permutation(self, n):
        return jax.random.permutation(self._next(), n)
kernel_name = 'standalone__window_attn_davit__vision'

def setup_inputs():
    _rng = _Rng(jax.random.key(int.from_bytes(__import__("os").urandom(4), "little")))
    _w = lambda a: (lambda t: t.astype(jnp.bfloat16) if jnp.issubdtype(t.dtype, jnp.floating) else t)(jnp.asarray(a))
    HW = 512
    C0 = 192
    ws = 7
    nh = 4
    H = W = max(HW // ws * ws, ws)
    C = max(C0 // nh * nh, nh)
    k = 3
    return {'x': _w((lambda *s: _rng.normal(s) * 0.05)(1, H, W, C)), 'dw_pe': _w((lambda *s: _rng.normal(s) * 0.05)(k, k, C) * 0.1), 'w_qkv': _w((lambda *s: _rng.normal(s) * 0.05)(C, 3 * C) * C ** (-0.5)), 'w_o': _w((lambda *s: _rng.normal(s) * 0.05)(C, C) * C ** (-0.5))}

def reference(x, dw_pe, w_qkv, w_o):
    B, H, W, C = x.shape
    ws = 7
    nh = 4
    dh = C // nh
    kk = dw_pe.shape[0]
    pad = kk // 2
    xp = jnp.pad(x, ((0, 0), (pad, pad), (pad, pad), (0, 0)))
    pe = jnp.zeros_like(x)
    for i in range(kk):
        for j in range(kk):
            pe = pe + xp[:, i:i + H, j:j + W, :] * dw_pe[i, j][None, None, None, :]
    x0 = x + pe
    h = _layernorm(x0, axis=-1)
    hw = h.reshape(B, H // ws, ws, W // ws, ws, C)
    hw = (lambda x, *d: x.transpose(*d))(hw, 0, 1, 3, 2, 4, 5)
    hw = hw.reshape(-1, ws * ws, C)
    qkv = (hw @ w_qkv).reshape(-1, ws * ws, 3, nh, dh)
    q = qkv[:, :, 0].copy()
    k = qkv[:, :, 1].copy()
    v = qkv[:, :, 2].copy()
    scale = dh ** (-0.5)
    attn = jnp.einsum('wnhd,wmhd->whnm', q, k) * scale
    attn = _softmax(attn, axis=-1)
    out = jnp.einsum('whnm,wmhd->wnhd', attn, v)
    out = out.reshape(-1, ws * ws, C) @ w_o
    out = out.reshape(B, H // ws, W // ws, ws, ws, C)
    out = (lambda x, *d: x.transpose(*d))(out, 0, 1, 3, 2, 4, 5)
    out = out.reshape(B, H, W, C)
    return x0 + out
```

```python
import functools
import math

import jax
import jax.numpy as jnp
from jax import lax
import jax.experimental.pallas as pl
import jax.experimental.pallas.tpu as pltpu

WS = 7
NH = 4
EPS = 1e-05
LANES = 128
F32 = jnp.float32
BF16 = jnp.bfloat16
U32 = jnp.uint32


def _iota(shape, dim):
    return lax.broadcasted_iota(jnp.int32, shape, dim)


def _kernel(xm_ref, xt_ref, xb_ref, dw_ref, wqkv_ref, wo_ref, o_ref,
            x0_s, qkv_s, o_s, wq_s, wo_s, dw_s, *, C, W, WP, NWIN):
    i = pl.program_id(0)
    nsteps = pl.num_programs(0)
    dh = C // NH
    CW = C // 2
    NT = WP // LANES
    G = WS * 8

    @pl.when(i == 0)
    def _():
        qscale = (dh ** -0.5) * math.log2(math.e)
        wq_s[0:C, :] = (wqkv_ref[0:C, :].astype(F32) * qscale).astype(BF16)
        wq_s[C:3 * C, :] = wqkv_ref[C:3 * C, :]
        wo_s[...] = wo_ref[...]
        for tap in range(9):
            w = dw_ref[tap].astype(F32)
            if tap == 4:
                w = w + 1.0
            dw_s[tap] = w
        qkv_s[...] = jnp.zeros(qkv_s.shape, U32)
        o_s[...] = jnp.zeros(o_s.shape, U32)

    lane8 = _iota((8, LANES), 1)
    top_ok = i > 0
    bot_ok = i < nsteps - 1

    last_valid = W - (NT - 1) * LANES
    for c in range(C // 16):
        cs = slice(16 * c, 16 * c + 16)
        acc = {}
        for rho in range(WS + 2):
            if rho == 0:
                xb = xt_ref[0, cs, :]
            elif rho == WS + 1:
                xb = xb_ref[0, cs, :]
            else:
                xb = xm_ref[rho - 1, cs, :]
            u = pltpu.bitcast(xb, U32)
            tiles = [u[:, LANES * t:LANES * (t + 1)] for t in range(NT)]
            tiles[NT - 1] = jnp.where(lane8 < last_valid, tiles[NT - 1], jnp.uint32(0))
            if rho == 0:
                tiles = [jnp.where(top_ok, tt, jnp.uint32(0)) for tt in tiles]
            if rho == WS + 1:
                tiles = [jnp.where(bot_ok, tt, jnp.uint32(0)) for tt in tiles]
            rr = [pltpu.roll(tt, 1, 1) for tt in tiles]
            rl = [pltpu.roll(tt, LANES - 1, 1) for tt in tiles]
            for t in range(NT):
                left = jnp.where(lane8 == 0, rr[t - 1], rr[t])
                right = jnp.where(lane8 == LANES - 1, rl[(t + 1) % NT], rl[t])
                sh = [pltpu.bitcast(v, BF16).astype(F32) for v in (left, tiles[t], right)]
                for ki in range(3):
                    r = rho - ki
                    if 0 <= r < WS:
                        part = (sh[0] * dw_s[3 * ki + 0, cs, :] + sh[1] * dw_s[3 * ki + 1, cs, :]
                                + sh[2] * dw_s[3 * ki + 2, cs, :])
                        if ki == 0:
                            acc[(r, t)] = part
                        else:
                            acc[(r, t)] = acc[(r, t)] + part
                        if ki == 2:
                            x0_s[r, cs, LANES * t:LANES * (t + 1)] = acc.pop((r, t))

    for r in range(WS):
        for tp in range(NT // 2):
            ls = slice(2 * LANES * tp, 2 * LANES * (tp + 1))
            x0 = x0_s[r, :, ls]
            m = jnp.sum(x0, axis=0, keepdims=True) * (1.0 / C)
            xc = x0 - m
            var = jnp.sum(xc * xc, axis=0, keepdims=True) * (1.0 / C)
            h = (xc * lax.rsqrt(var + EPS)).astype(BF16)
            qkv = jnp.dot(wq_s[...], h, preferred_element_type=F32)
            words = pltpu.bitcast(qkv.astype(BF16), U32)
            for k in range(3):
                for tt in range(2):
                    t = 2 * tp + tt
                    blk = words[CW * k:CW * (k + 1), LANES * tt:LANES * (tt + 1)]
                    qkv_s[k, r, LANES * t:LANES * (t + 1), 0:CW] = blk.T

    laneG = _iota((G, LANES), 1)
    hi = jnp.uint32(0xFFFF0000)
    full = jnp.uint32(0xFFFFFFFF)
    zero = jnp.uint32(0)
    m_a = jnp.where(laneG < dh, full, zero)
    m_b = jnp.where((laneG >= dh) & (laneG < 2 * dh), full, zero)
    m_a_hi = m_a & hi
    m_b_hi = m_b & hi
    sub8 = _iota((8, 2 * G), 0)
    junk8 = sub8 == WS
    lane8g = _iota((8, 2 * G), 1)
    prow = _iota((G, 2 * G), 0)
    plane = _iota((G, 2 * G), 1)
    keep = jnp.where(prow % 4 == 3, jnp.uint32(0x0000FFFF), full)
    same = (prow < G // 2) == (plane < G)
    pm_same = jnp.where(same, keep, zero)
    pm_diff = jnp.where(same, zero, keep)
    lane8w = _iota((8, CW), 1)
    even_head = (lane8w // (dh // 2)) % 2 == 0

    def gather(k, w):
        return jnp.concatenate([qkv_s[k, r, pl.ds(WS * w, 8), :] for r in range(WS)], axis=0)

    def f(u):
        return pltpu.bitcast(u, F32)

    for p in range((NWIN + 1) // 2):
        wa = 2 * p
        wb = min(2 * p + 1, NWIN - 1)
        dup = wb == wa
        pts = []
        rinv = []
        for w, swap in ((wa, False), (wb, True)):
            qw = gather(0, w)
            kw = gather(1, w)
            qlo = qw << 16
            for tile in range(2):
                if tile == 0:
                    kk = f(kw << 16)
                    qa, qb = f(qlo & m_a), f(qlo & m_b)
                else:
                    kk = f(kw & hi)
                    qa, qb = f(qw & m_a_hi), f(qw & m_b_hi)
                qst = jnp.concatenate([qb, qa] if swap else [qa, qb], axis=0)
                st = lax.dot_general(kk, qst, (((1,), (1,)), ((), ())),
                                     preferred_element_type=F32)
                sg = [st[8 * r:8 * r + 8, :] for r in range(WS)]
                m8 = functools.reduce(jnp.maximum, sg)
                mx = jnp.max(jnp.where(junk8, -jnp.inf, m8), axis=0, keepdims=True)
                mv = jnp.where(junk8, m8, mx)
                eg = [jnp.exp2(s - mv) for s in sg]
                s8 = functools.reduce(lambda a, b: a + b, eg)
                den = jnp.sum(jnp.where(junk8, 0.0, s8), axis=0, keepdims=True)
                rinv.append(pl.reciprocal(den, approx=False))
                pts.append(jnp.concatenate(eg, axis=0))
        vw = jnp.concatenate([gather(2, wa), gather(2, wb)], axis=0)
        vt = pltpu.bitcast(vw[:, 0:CW].T, BF16)
        outs = []
        for tile in range(2):
            pp = jnp.concatenate([pts[tile], pts[2 + tile]], axis=0).astype(BF16)
            pw = pltpu.bitcast(pp, U32)
            ra, rb = rinv[tile], rinv[2 + tile]
            for hh in range(2):
                h = 2 * tile + hh
                stn = pltpu.bitcast(pw & (pm_same if hh == 0 else pm_diff), BF16)
                ot = jnp.dot(vt[dh * h:dh * (h + 1), :], stn, preferred_element_type=F32)
                rr_ = jnp.where(lane8g[0:1] < G, ra, rb) if hh == 0 else jnp.where(lane8g[0:1] < G, rb, ra)
                outs.append(ot * rr_)
        ow = pltpu.bitcast(jnp.concatenate(outs, axis=0).astype(BF16), U32)
        tw = ow.T
        for r in range(WS):
            ga = tw[8 * r:8 * r + 8, :]
            gb = tw[G + 8 * r:G + 8 * r + 8, :]
            o_s[r, pl.ds(WS * wa, WS), 0:CW] = jnp.where(even_head, ga, gb)[0:WS]
            if not dup:
                o_s[r, pl.ds(WS * wb, WS), 0:CW] = jnp.where(even_head, gb, ga)[0:WS]

    for r in range(WS):
        for tp in range(NT // 2):
            ls = slice(2 * LANES * tp, 2 * LANES * (tp + 1))
            ot = jnp.concatenate(
                [o_s[r, LANES * t:LANES * (t + 1), 0:CW].T for t in (2 * tp, 2 * tp + 1)], axis=1)
            ot = pltpu.bitcast(ot, BF16)
            res = jnp.dot(wo_s[...], ot, preferred_element_type=F32)
            o_ref[r, :, ls] = (x0_s[r, :, ls] + res).astype(o_ref.dtype)


@jax.jit
def pallas_standalone__window_attn_davit__vision_kernel(
    x: jax.Array,
    dw_pe: jax.Array,
    w_qkv: jax.Array,
    w_o: jax.Array,
):
    B, H, W, C = x.shape
    assert B == 1 and H % WS == 0 and W % WS == 0 and C % (16 * NH) == 0
    WP = -(-(W + 1) // (2 * LANES)) * (2 * LANES)
    NWIN = W // WS
    CW = C // 2

    xt = jnp.transpose(x[0], (0, 2, 1))
    dwb = jnp.broadcast_to(dw_pe.reshape(9, C, 1), (9, C, LANES))

    def inter(w):
        return jnp.transpose(w.reshape(C, 2, CW), (2, 1, 0)).reshape(C, C)

    wqkv_t = jnp.concatenate(
        [inter(w_qkv[:, 0:C]), inter(w_qkv[:, C:2 * C]), w_qkv[:, 2 * C:].T], axis=0)
    wo_t = w_o.T

    kern = functools.partial(_kernel, C=C, W=W, WP=WP, NWIN=NWIN)
    out = pl.pallas_call(
        kern,
        grid=(H // WS,),
        in_specs=[
            pl.BlockSpec((WS, C, WP), lambda i: (i, 0, 0)),
            pl.BlockSpec((1, C, WP), lambda i: (jnp.maximum(WS * i - 1, 0), 0, 0)),
            pl.BlockSpec((1, C, WP), lambda i: (jnp.minimum(WS * i + WS, H - 1), 0, 0)),
            pl.BlockSpec((9, C, LANES), lambda i: (0, 0, 0)),
            pl.BlockSpec((3 * C, C), lambda i: (0, 0)),
            pl.BlockSpec((C, C), lambda i: (0, 0)),
        ],
        out_specs=pl.BlockSpec((WS, C, WP), lambda i: (i, 0, 0)),
        out_shape=jax.ShapeDtypeStruct((H, C, W), x.dtype),
        scratch_shapes=[
            pltpu.VMEM((WS, C, WP), F32),
            pltpu.VMEM((3, WS, WP, LANES), U32),
            pltpu.VMEM((WS, WP, LANES), U32),
            pltpu.VMEM((3 * C, C), BF16),
            pltpu.VMEM((C, C), BF16),
            pltpu.VMEM((9, C, LANES), F32),
        ],
        compiler_params=pltpu.CompilerParams(
            dimension_semantics=("arbitrary",),
            vmem_limit_bytes=64 * 1024 * 1024,
        ),
        name="davit_window_attn",
    )(xt, xt, xt, dwb, wqkv_t, wo_t)
    return jnp.transpose(out, (0, 2, 1))[None]
```

```python
import functools
import math
import os

import jax
import jax.numpy as jnp
from jax import lax
import jax.experimental.pallas as pl
import jax.experimental.pallas.tpu as pltpu

WS = 7
NH = 4
EPS = 1e-05
LANES = 128
F32 = jnp.float32
BF16 = jnp.bfloat16
U32 = jnp.uint32

P = lambda k, d: int(os.environ.get(k, d))
DL_A = P('DL_A', 440)
LAT_QK = P('LAT_QK', 300)
DL_PV = P('DL_PV', 520)
DL_C = P('DL_C', 170)
CP = P('CP', 4)
PRE_C = P('PRE_C', 350)
TAIL = P('TAIL', 1400)
CLEAD = P('CLEAD', 1)
PRE_LN = P('PRE_LN', 200)
DA, DC, DQ, DP = 288, 192, 56, 48


def _iota(shape, dim):
    return lax.broadcasted_iota(jnp.int32, shape, dim)


def _plan(npair, n0, nt):
    a_q = [(t, r) for t in range(nt) for r in range(WS)]
    c_q = [(h, r) for h in range(2) for r in range(WS)]
    pairs = list(range(n0, npair)) + list(range(n0))
    total = len(a_q) * DA + len(c_q) * DC + npair * (DQ + DP)
    t = 0
    ia = ic = iq = ip = 0
    out = []
    tq, tp, ta = {}, {}, {}
    last = None
    while ia < len(a_q) or ic < len(c_q) or ip < npair:
        cands = []
        if ip < iq and t >= tq[ip] + LAT_QK:
            cands.append((-1e9, 'pv'))
        if iq < npair and iq - ip < 2 and last != 'qk':
            ok = True
            if iq >= npair - n0:
                need = (2 * WS * pairs[iq] + 2 * WS) // LANES * WS + WS - 1
                ok = ia > need and t >= ta[need] + DA + DL_A + 60 and ic >= WS
            if ok:
                cands.append((iq * (total - TAIL) / npair - t - 200, 'qk'))
        if ia < len(a_q):
            cands.append((ia * (total - 700) / len(a_q) - t, 'a'))
        if ic < len(c_q):
            need = 0 if ic < WS else npair - n0 - 1
            if ip > need and t >= tp[need] + DL_PV + PRE_C:
                tc = 1000 + ic * 900 if ic < WS else total - DC - (2 * WS - 1 - ic) * 950
                cands.append((tc - t, 'c'))
        if not cands:
            t += 16
            last = None
            continue
        kind = min(cands)[1]
        last = kind
        if kind == 'pv':
            tp[ip] = t; out.append((t, 'pv', pairs[ip])); ip += 1; t += DP
        elif kind == 'qk':
            tq[iq] = t; out.append((t, 'qk', pairs[iq])); iq += 1; t += DQ
        elif kind == 'a':
            ta[ia] = t; out.append((t, 'a', a_q[ia])); ia += 1; t += DA
        else:
            out.append((t, 'c', c_q[ic])); ic += 1; t += DC
    return out, t


def _tree_sum(xs):
    while len(xs) > 1:
        xs = [xs[j] + xs[j + 1] if j + 1 < len(xs) else xs[j] for j in range(0, len(xs), 2)]
    return xs[0]


def _kernel(xn_ref, xt_ref, xb_ref, xf_ref, dw_ref, wqkv_ref, wo_ref, o_ref,
            x0_s, q_s, k_s, v_s, o_s, wq_s, wo_s, *, C, W, WP, NWIN, NBLK):
    i = pl.program_id(0)
    dh = C // NH
    CW = C // 2
    NT = WP // LANES
    G = WS * 8
    HW = WP // 2
    DW0 = 3 * WS
    lane8 = _iota((8, LANES), 1)
    last_valid = W - (NT - 1) * LANES
    zero = jnp.uint32(0)
    qkv_s = (q_s, k_s, v_s)
    zx = i >> 10
    zvec = jnp.full((8, LANES), zx, jnp.int32).astype(U32)

    def shifted_rows(load_row):
        sh = []
        for rho in range(WS + 2):
            u = load_row(rho)
            if u is None:
                sh.append(None)
                continue
            tiles = [u[:, LANES * t:LANES * (t + 1)] for t in range(NT)]
            tiles[NT - 1] = jnp.where(lane8 < last_valid, tiles[NT - 1], zero)
            rr = [pltpu.roll(tt, 1, 1) for tt in tiles]
            rl = [pltpu.roll(tt, LANES - 1, 1) for tt in tiles]
            row = []
            for t in range(NT):
                left = jnp.where(lane8 == 0, rr[t - 1] if t > 0 else zero, rr[t])
                right = jnp.where(lane8 == LANES - 1, rl[t + 1], rl[t]) if t < NT - 1 else rl[t]
                row.append((left, tiles[t], right))
            sh.append(row)
        return sh

    def conv_column(sh, t, cs, buf):
        un = [None if s is None else [pltpu.bitcast(v, BF16).astype(F32) for v in s[t]] for s in sh]

        def taps():
            return [x0_s[zx + (DW0 + tap // NT), cs, LANES * (tap % NT):LANES * (tap % NT + 1)]
                    for tap in range(9)]
        w = [taps() for _ in range(CLEAD)]
        for r in range(WS):
            if len(w) < WS:
                w.append(taps())
            terms = [un[r + ki][kj] * w[r][3 * ki + kj]
                     for ki in range(3) for kj in range(3) if un[r + ki] is not None]
            x0_s[buf * WS + r, cs, LANES * t:LANES * (t + 1)] = _tree_sum(terms)

    @pl.when(i == 0)
    def _():
        qscale = (dh ** -0.5) * math.log2(math.e)
        for j in range(3 * C // 16):
            blk = wqkv_ref[16 * j:16 * j + 16, :]
            if j < C // 16:
                blk = (blk.astype(F32) * qscale).astype(BF16)
            wq_s[j % 2, 8 * (j // 2):8 * (j // 2) + 8, :] = pltpu.bitcast(blk, U32)
        wo_s[...] = pltpu.bitcast(wo_ref[...], U32)

        def zrow(r, carry):
            for ref in (q_s, k_s, v_s, o_s):
                ref[r] = jnp.zeros(ref.shape[1:], U32)
            x0_s[2 * WS + r] = jnp.zeros(x0_s.shape[1:], F32)
            return carry
        lax.fori_loop(0, WS, zrow, 0)
        for tap in range(9):
            w = dw_ref[tap].astype(F32)
            if tap == 4:
                w = w + 1.0
            x0_s[DW0 + tap // NT, :, LANES * (tap % NT):LANES * (tap % NT + 1)] = w

        def conv0(c, carry):
            cs = pl.ds(pl.multiple_of(16 * c, 16), 16)
            sh = shifted_rows(lambda rho: None if rho == 0 else pltpu.bitcast(xf_ref[rho - 1, cs, :], U32))
            for t in range(NT):
                conv_column(sh, t, cs, 0)
            return carry
        lax.fori_loop(0, C // 16, conv0, 0)

    b_cur = i % 3
    b_next = (i + 1) % 3
    b_prev = (i + 2) % 3
    bot_ok = i + 1 < NBLK - 1

    hi = jnp.uint32(0xFFFF0000)
    head_a = lane8 < dh
    head_b = (lane8 >= dh) & (lane8 < 2 * dh)
    junk8 = _iota((8, 2 * G), 0) == WS
    lo_ok = (_iota((8, 2 * G), 1) < G) & ~junk8
    hi_ok = (_iota((8, 2 * G), 1) >= G) & ~junk8
    first_half = _iota((1, 2 * G), 1) < G
    even_head = (_iota((8, CW), 1) // (dh // 2)) % 2 == 0

    def gather(ref, w):
        return [ref[r, pl.ds(WS * w, 8), :] for r in range(WS)]

    def f(u):
        return pltpu.bitcast(u, F32)

    def cat(xs, axis=0):
        return jnp.concatenate(xs, axis=axis)

    st = {}
    toks = []

    def lhs(ref, t0):
        nblk = ref.shape[0] // 8
        inj = {}
        for d, tok in list(toks):
            j = max(0, -(-(d - t0) // 16))
            if j < nblk:
                inj[j] = tok if j not in inj else inj[j] | tok
                toks[:] = [x for x in toks if x[1] is not tok]
        parts, s = [], 0
        for j in sorted(inj):
            if j > s:
                parts.append(ref[8 * s:8 * j, :])
            parts.append(cat([ref[8 * j:8 * j + 8, 0:LANES] | (inj[j] & zvec), ref[8 * j:8 * j + 8, LANES:]], axis=1))
            s = j + 1
        if s < nblk:
            parts.append(ref[8 * s:8 * nblk, :])
        return pltpu.bitcast(cat(parts) if len(parts) > 1 else parts[0], BF16)

    def ln(t, r):
        x0 = x0_s[b_cur * WS + r, :, LANES * t:LANES * (t + 1)]
        m = jnp.sum(x0, axis=0, keepdims=True) * (1.0 / C)
        xc = x0 - m
        var = jnp.sum(xc * xc, axis=0, keepdims=True) * (1.0 / C)
        st['h', t, r] = (xc * lax.rsqrt(var + EPS)).astype(BF16)

    def a_dot(t0, t, r):
        h = st.pop(('h', t, r))
        res = [jnp.dot(lhs(wq_s.at[0], t0), h, preferred_element_type=F32),
               jnp.dot(pltpu.bitcast(wq_s[1], BF16), h, preferred_element_type=F32)]
        nb = C // 16
        for k in range(3):
            blk = cat([res[j % 2][16 * (j // 2):16 * (j // 2) + 16, :] for j in range(nb * k, nb * (k + 1))])
            qkv_s[k][r, LANES * t:LANES * (t + 1), 0:CW] = pltpu.bitcast(blk.astype(BF16), U32).T
            toks.append((t0 + 96 * (k + 1) + DL_A, qkv_s[k][zx, 0:8, :]))

    def wins(p):
        return 2 * p, min(2 * p + 1, NWIN - 1)

    def b_qk(t0, p):
        wa, wb = wins(p)
        pts = []
        rinv = []
        for w, swap in ((wa, False), (wb, True)):
            qw = gather(q_s, w)
            kw = cat(gather(k_s, w))
            for tile in range(2):
                if tile == 0:
                    kk = f(kw << 16)
                    qq = [f(g << 16) for g in qw]
                else:
                    kk = f(kw & hi)
                    qq = [f(g & hi) for g in qw]
                qa = [jnp.where(head_a, g, 0.0) for g in qq]
                qb = [jnp.where(head_b, g, 0.0) for g in qq]
                qst = cat(qb + qa if swap else qa + qb)
                s_t = lax.dot_general(kk, qst, (((1,), (1,)), ((), ())),
                                      preferred_element_type=F32)
                sg = [s_t[8 * r:8 * r + 8, :] for r in range(WS)]
                m8 = functools.reduce(jnp.maximum, sg)
                mx = jnp.max(jnp.where(junk8, -jnp.inf, m8), axis=0, keepdims=True)
                mv = jnp.where(junk8, m8, mx)
                eg = [jnp.exp2(s - mv) for s in sg]
                den = jnp.sum(jnp.where(junk8, 0.0, _tree_sum(eg)), axis=0, keepdims=True)
                r0 = pl.reciprocal(den, approx=True)
                rinv.append(r0 * (2.0 - den * r0))
                pts.append(eg)
        vw = cat(gather(v_s, wa) + gather(v_s, wb))
        vt = pltpu.bitcast(vw[:, 0:CW].T, BF16)
        st['b', p] = (pts, rinv, vt)

    def b_pv(t0, p):
        wa, wb = wins(p)
        pts, rinv, vt = st.pop(('b', p))
        outs = []
        for tile in range(2):
            ra, rb = rinv[tile], rinv[2 + tile]
            for hh in range(2):
                h = 2 * tile + hh
                ma, mb = (lo_ok, hi_ok) if hh == 0 else (hi_ok, lo_ok)
                stn = cat([jnp.where(ma, e, 0.0) for e in pts[tile]]
                          + [jnp.where(mb, e, 0.0) for e in pts[2 + tile]]).astype(BF16)
                ot = jnp.dot(vt[dh * h:dh * (h + 1), :], stn, preferred_element_type=F32)
                rr_ = jnp.where(first_half, ra, rb) if hh == 0 else jnp.where(first_half, rb, ra)
                outs.append(ot * rr_)
        tw = pltpu.bitcast(cat(outs).astype(BF16), U32).T
        for r in range(WS):
            ga = tw[8 * r:8 * r + 8, :]
            gb = tw[G + 8 * r:G + 8 * r + 8, :]
            o_s[r, pl.ds(WS * wa, WS), 0:CW] = jnp.where(even_head, ga, gb)[0:WS]
            if wb != wa:
                o_s[r, pl.ds(WS * wb, WS), 0:CW] = jnp.where(even_head, gb, ga)[0:WS]
        toks.append((t0 + DL_PV, o_s[zx, 0:8, :]))

    def c_dot(t0, h, r):
        ot = cat([o_s[r, LANES * t:LANES * (t + 1), 0:CW].T for t in (2 * h, 2 * h + 1)], axis=1)
        res = jnp.dot(lhs(wo_s, t0), pltpu.bitcast(ot, BF16), preferred_element_type=F32)
        ls = slice(HW * h, HW * (h + 1))
        n = C // CP
        for q in range(CP):
            rs = slice(n * q, n * (q + 1))
            o_ref[r, rs, ls] = (x0_s[b_prev * WS + r, rs, ls] + res[rs]).astype(o_ref.dtype)
            toks.append((t0 + n * (q + 1) + DL_C,
                         pltpu.bitcast(o_ref[zx + r, n * q:n * q + 16, HW * h:HW * h + LANES], U32)))

    def conv_prep(c):
        cs = slice(16 * c, 16 * c + 16)

        def load_row(rho):
            if rho == 0:
                return pltpu.bitcast(xt_ref[0, cs, :], U32)
            if rho == WS + 1:
                return jnp.where(bot_ok, pltpu.bitcast(xb_ref[0, cs, :], U32), zero)
            return pltpu.bitcast(xn_ref[rho - 1, cs, :], U32)
        st['sh', c] = shifted_rows(load_row)

    def conv_col(c, t):
        conv_column(st['sh', c], t, slice(16 * c, 16 * c + 16), b_next)

    npair = (NWIN + 1) // 2
    n0 = (HW - 1) // WS // 2
    plan, total = _plan(npair, n0, NT)
    ev = []

    def at(t, fn, *a):
        ev.append((t, len(ev), fn, a))

    for t, kind, idx in plan:
        if kind == 'a':
            at(t - PRE_LN, ln, *idx)
            at(t, a_dot, t, *idx)
        elif kind == 'qk':
            at(t, b_qk, t, idx)
        elif kind == 'pv':
            at(t, b_pv, t, idx)
        else:
            at(t, c_dot, t, *idx)
    ncol = (C // 16) * NT
    for c in range(C // 16):
        for t in range(NT):
            tt = 150 + (c * NT + t) * (total - 150) // ncol
            if t == 0:
                at(tt - 1, conv_prep, c)
            at(tt, conv_col, c, t)
    ev.sort(key=lambda e: (e[0], e[1]))
    a_done, pv_done = set(), set()
    for _, _, fn, a in ev:
        if fn is a_dot:
            a_done.add(a[1:])
        elif fn is b_qk:
            tl = range(2 * WS * a[1] // LANES, min(2 * WS * a[1] + 2 * WS, WP - 1) // LANES + 1)
            need = [(t, r) in a_done for t in tl for r in range(WS)]
            assert all(need) if a[1] < n0 else not any(need)
        elif fn is b_pv:
            pv_done.add(a[1])
        elif fn is c_dot:
            ps = range(0, n0 + 1) if a[1] == 0 else range(n0, npair)
            assert all((p in pv_done) == (p >= n0) for p in ps)
    for _, _, fn, a in ev:
        fn(*a)


@jax.jit
def pallas_standalone__window_attn_davit__vision_kernel(
    x: jax.Array,
    dw_pe: jax.Array,
    w_qkv: jax.Array,
    w_o: jax.Array,
):
    B, H, W, C = x.shape
    assert B == 1 and H % WS == 0 and W % WS == 0 and C % (16 * NH) == 0
    WP = -(-(W + 1) // (2 * LANES)) * (2 * LANES)
    assert WP == 4 * LANES
    NWIN = W // WS
    NBLK = H // WS
    CW = C // 2

    xt = jnp.transpose(x[0], (0, 2, 1))
    dwb = jnp.broadcast_to(dw_pe.reshape(9, C, 1), (9, C, LANES))

    def inter(w):
        return jnp.transpose(w.reshape(C, 2, CW), (2, 1, 0)).reshape(C, C)

    wqkv_t = jnp.concatenate(
        [inter(w_qkv[:, 0:C]), inter(w_qkv[:, C:2 * C]), w_qkv[:, 2 * C:].T], axis=0)
    wo_t = w_o.T

    def nxt(i):
        return jnp.minimum(i + 1, NBLK - 1)

    kern = functools.partial(_kernel, C=C, W=W, WP=WP, NWIN=NWIN, NBLK=NBLK)
    out = pl.pallas_call(
        kern,
        grid=(NBLK + 1,),
        in_specs=[
            pl.BlockSpec((WS, C, WP), lambda i: (nxt(i), 0, 0)),
            pl.BlockSpec((1, C, WP), lambda i: (WS * nxt(i) - 1, 0, 0)),
            pl.BlockSpec((1, C, WP), lambda i: (jnp.minimum(WS * nxt(i) + WS, H - 1), 0, 0)),
            pl.BlockSpec((WS + 1, C, WP), lambda i: (0, 0, 0)),
            pl.BlockSpec((9, C, LANES), lambda i: (0, 0, 0)),
            pl.BlockSpec((3 * C, C), lambda i: (0, 0)),
            pl.BlockSpec((C, C), lambda i: (0, 0)),
        ],
        out_specs=pl.BlockSpec((WS, C, WP), lambda i: (jnp.maximum(i - 1, 0), 0, 0)),
        out_shape=jax.ShapeDtypeStruct((H, C, W), x.dtype),
        scratch_shapes=[
            pltpu.VMEM((3 * WS + 3, C, WP), F32),
            pltpu.VMEM((WS, WP, LANES), U32),
            pltpu.VMEM((WS, WP, LANES), U32),
            pltpu.VMEM((WS, WP, LANES), U32),
            pltpu.VMEM((WS, WP, LANES), U32),
            pltpu.VMEM((2, 3 * C // 4, C), U32),
            pltpu.VMEM((C // 2, C), U32),
        ],
        compiler_params=pltpu.CompilerParams(
            dimension_semantics=("arbitrary",),
            vmem_limit_bytes=64 * 1024 * 1024,
        ),
        name="davit_window_attn",
    )(xt, xt, xt, xt, dwb, wqkv_t, wo_t)
    return jnp.transpose(out, (0, 2, 1))[None]
```

```python
import functools
import math
import os

import jax
import jax.numpy as jnp
from jax import lax
import jax.experimental.pallas as pl
import jax.experimental.pallas.tpu as pltpu

WS = 7
NH = 4
EPS = 1e-05
LANES = 128
F32 = jnp.float32
BF16 = jnp.bfloat16
U32 = jnp.uint32

P = lambda k, d: int(os.environ.get(k, d))
DL_A = P('DL_A', 440)
LAT_QK = P('LAT_QK', 300)
DL_PV = P('DL_PV', 520)
DL_C = P('DL_C', 170)
CP = P('CP', 4)
PRE_C = P('PRE_C', 350)
TAIL = P('TAIL', 1400)
CLEAD = P('CLEAD', 1)
PRE_LN = P('PRE_LN', 200)
SYM = P('SYM', 1)
FAKE = P('FAKE', 0)
CVK = P('CVK', 1)
LN3 = P('LN3', 1)
LN1 = P('LN1', 190)
LN2 = P('LN2', 120)
SM0 = P('SM0', 200)
SMD = P('SMD', 16)
CV0 = P('CV0', 500)
STOK = P('STOK', 1)
COFF = P('COFF', 0)
SMB = P('SMB', 130)
ONE = P('ONE', 0)
LNZ = P('LNZ', 1)
LNS = P('LNS', 2)
LND = P('LND', 16)
PVI = P('PVI', 0)
CAP = P('CAP', 48)
SMO = P('SMO', 32)
CTOK = P('CTOK', 0)
DA, DC, DQ, DP = 288, 192, 56, 48


def _iota(shape, dim):
    return lax.broadcasted_iota(jnp.int32, shape, dim)


def _plan(npair, n0, nt):
    a_q = [(t, r) for t in range(nt) for r in range(WS)]
    c_q = [(h, r) for h in range(2) for r in range(WS)]
    pairs = list(range(n0, npair)) + list(range(n0))
    total = len(a_q) * DA + len(c_q) * DC + npair * (DQ + DP)
    t = 0
    ia = ic = iq = ip = 0
    out = []
    tq, tp, ta = {}, {}, {}
    last = None
    while ia < len(a_q) or ic < len(c_q) or ip < npair:
        cands = []
        if ip < iq and t >= tq[ip] + LAT_QK:
            cands.append((-1e9, 'pv'))
        if iq < npair and iq - ip < 2 and last != 'qk':
            ok = True
            if iq >= npair - n0:
                need = (2 * WS * pairs[iq] + 2 * WS) // LANES * WS + WS - 1
                ok = ia > need and t >= ta[need] + DA + DL_A + 60 and ic >= WS
            if ok:
                cands.append((iq * (total - TAIL) / npair - t - 200, 'qk'))
        if ia < len(a_q):
            cands.append((ia * (total - 700) / len(a_q) - t, 'a'))
        if ic < len(c_q):
            need = 0 if ic < WS else npair - n0 - 1
            if ip > need and t >= tp[need] + DL_PV + PRE_C:
                tc = 1000 + ic * 900 if ic < WS else total - DC - (2 * WS - 1 - ic) * 950
                cands.append((tc - t, 'c'))
        if not cands:
            t += 16
            last = None
            continue
        kind = min(cands)[1]
        last = kind
        if kind == 'pv':
            tp[ip] = t; out.append((t, 'pv', pairs[ip])); ip += 1; t += DP
        elif kind == 'qk':
            tq[iq] = t; out.append((t, 'qk', pairs[iq])); iq += 1; t += DQ
        elif kind == 'a':
            ta[ia] = t; out.append((t, 'a', a_q[ia])); ia += 1; t += DA
        else:
            out.append((t, 'c', c_q[ic])); ic += 1; t += DC
    return out, t


def _tree_sum(xs):
    while len(xs) > 1:
        xs = [xs[j] + xs[j + 1] if j + 1 < len(xs) else xs[j] for j in range(0, len(xs), 2)]
    return xs[0]


def _kernel(xn_ref, xt_ref, xb_ref, xf_ref, dw_ref, wqkv_ref, wo_ref, o_ref,
            xa_s, xb_s, xc_s, q_s, k_s, v_s, o_s, wq_s, wo_s, stg_s, dw_s, *, C, W, WP, NWIN, NBLK):
    i = pl.program_id(0)
    dh = C // NH
    CW = C // 2
    NT = WP // LANES
    G = WS * 8
    HW = WP // 2
    lane8 = _iota((8, LANES), 1)
    last_valid = W - (NT - 1) * LANES
    zero = jnp.uint32(0)
    qkv_s = (q_s, k_s, v_s)
    zx = i >> 10
    zvec = jnp.full((8, LANES), zx, jnp.int32).astype(U32)

    def shifted(u):
        tiles = [u[:, LANES * t:LANES * (t + 1)] for t in range(NT)]
        tiles[NT - 1] = jnp.where(lane8 < last_valid, tiles[NT - 1], zero)
        row = []
        for t in range(NT):
            left = jnp.where(lane8 == LANES - 1, tiles[t - 1] if t > 0 else zero, tiles[t])
            right = jnp.where(lane8 == 0, tiles[t + 1], tiles[t]) if t < NT - 1 else tiles[t]
            row.append((pltpu.roll(left, 1, 1), tiles[t], pltpu.roll(right, LANES - 1, 1)))
        return row

    def unpack(vs):
        return [pltpu.bitcast(v, BF16).astype(F32) for v in vs]

    def conv_row(un, t, r, cs, buf):
        w = [dw_s[tap, cs, :] for tap in range(9)]
        terms = [un[r + ki][kj] * w[3 * ki + kj]
                 for ki in range(3) for kj in range(3) if un[r + ki] is not None]
        acc = _tree_sum(terms)
        buf[r, cs, LANES * t:LANES * (t + 1)] = acc
        return acc

    @pl.when(i == 0)
    def _():
        qscale = (dh ** -0.5) * math.log2(math.e)
        for j in range(3 * C // 16):
            blk = wqkv_ref[16 * j:16 * j + 16, :]
            if j < C // 16:
                blk = (blk.astype(F32) * qscale).astype(BF16)
            wq_s[j % 2, 8 * (j // 2):8 * (j // 2) + 8, :] = pltpu.bitcast(blk, U32)
        wo_s[...] = pltpu.bitcast(wo_ref[...], U32)

        def zrow(r, carry):
            for ref in (q_s, k_s, v_s, o_s):
                ref[r] = jnp.zeros(ref.shape[1:], U32)
            xc_s[r] = jnp.zeros(xc_s.shape[1:], F32)
            return carry
        lax.fori_loop(0, WS, zrow, 0)
        stg_s[...] = jnp.zeros(stg_s.shape, U32)
        for tap in range(9):
            w = dw_ref[tap].astype(F32)
            if tap == 4:
                w = w + 1.0
            dw_s[tap] = w

        def conv0(c, carry):
            cs = pl.ds(pl.multiple_of(16 * c, 16), 16)
            sh = [shifted(pltpu.bitcast(xf_ref[rho, cs, :], U32)) for rho in range(WS + 1)]
            for t in range(NT):
                un = [None] + [unpack(row[t]) for row in sh]
                for r in range(WS):
                    conv_row(un, t, r, cs, xa_s)
            return carry
        lax.fori_loop(0, C // 16, conv0, 0)

    def step(x_cur, x_next, x_prev):
        bot_ok = i + 1 < NBLK - 1

        hi = jnp.uint32(0xFFFF0000)
        head_a = lane8 < dh
        head_b = (lane8 >= dh) & (lane8 < 2 * dh)
        junk8 = _iota((8, 2 * G), 0) == WS
        lo_ok = (_iota((8, 2 * G), 1) < G) & ~junk8
        hi_ok = (_iota((8, 2 * G), 1) >= G) & ~junk8
        first_half = _iota((1, 2 * G), 1) < G
        even_head = (_iota((8, CW), 1) // (dh // 2)) % 2 == 0

        def gather(ref, w):
            return [ref[r, pl.ds(WS * w, 8), :] for r in range(WS)]

        def f(u):
            return pltpu.bitcast(u, F32)

        def cat(xs, axis=0):
            return jnp.concatenate(xs, axis=axis)

        st = {}
        toks = []
        soft = []
        ticks = []

        def tick(t):
            c = [x for x in ticks if x[0] >= t]
            return (min(c, key=lambda x: x[0])[1] & zvec) if c else None

        def due(lst, nblk, t0, step=16):
            inj = {}
            for d, tok in list(lst):
                j = max(0, -(-(d - t0) // step))
                if j < nblk:
                    inj[j] = tok if j not in inj else inj[j] | tok
                    lst[:] = [x for x in lst if x[1] is not tok]
            return {j: v & zvec for j, v in inj.items()}

        def lhs(ref, inj, inj1):
            nblk = ref.shape[0] // 8
            parts, s = [], 0
            for j in sorted(set(inj) | set(inj1)):
                if j > s:
                    parts.append(ref[8 * s:8 * j, :])
                k0, k1 = ref[8 * j:8 * j + 8, 0:LANES], ref[8 * j:8 * j + 8, LANES:]
                if j in inj:
                    k0 = k0 | inj[j]
                    if SYM:
                        k1 = k1 | inj[j][:, 0:C - LANES]
                if j in inj1:
                    k0 = k0 | inj1[j]
                parts.append(cat([k0, k1], axis=1))
                s = j + 1
            if s < nblk:
                parts.append(ref[8 * s:8 * nblk, :])
            return pltpu.bitcast(cat(parts) if len(parts) > 1 else parts[0], BF16)

        def rows8(x):
            return [x[8 * j:8 * j + 8] for j in range(x.shape[0] // 8)]

        def bc8(v):
            return pltpu.bitcast(jnp.broadcast_to(v, (8, LANES)), U32)

        def x0_cur(t, r):
            return x_cur[r, :, LANES * t:LANES * (t + 1)]

        def ln1(d, t, r):
            s8 = _tree_sum(rows8(x0_cur(t, r)))
            soft.append((d, pltpu.bitcast(s8, U32)))
            st['m', t, r] = jnp.sum(s8, axis=0, keepdims=True) * (1.0 / C)

        def ln2(d, t, r, k):
            n = C // LNS
            xc = x_cur[(zx if LNZ else 0) + r, n * k:n * (k + 1), LANES * t:LANES * (t + 1)] - st['m', t, r]
            s8 = _tree_sum(rows8(xc * xc))
            soft.append((d, pltpu.bitcast(s8, U32)))
            st.setdefault(('xc', t, r), []).append(xc)
            st.setdefault(('sq', t, r), []).append(s8)

        def ln3(t, r):
            var = jnp.sum(_tree_sum(st.pop(('sq', t, r))), axis=0, keepdims=True) * (1.0 / C)
            xc = cat(st.pop(('xc', t, r)))
            if LN3:
                xc = x_cur[(i >> 11) + r, :, LANES * t:LANES * (t + 1)] - st['m', t, r]
            st['h', t, r] = (xc * lax.rsqrt(var + EPS)).astype(BF16)

        def a_dot(t0, t, r):
            h = st.pop(('h', t, r))
            inj = due(toks, DA // 16, t0)
            res = [jnp.dot(lhs(wq_s.at[0], inj, due(soft, DA // 16, t0)), h, preferred_element_type=F32),
                   jnp.dot(lhs(wq_s.at[1], inj if SYM else {}, {}), h, preferred_element_type=F32)]
            ticks.extend((t0 + 130 + 8 * j, pltpu.bitcast(res[0][8 * j:8 * j + 8], U32)) for j in range(DA // 8))
            nb = C // 16
            for k in range(3):
                blk = cat([res[j % 2][16 * (j // 2):16 * (j // 2) + 16, :] for j in range(nb * k, nb * (k + 1))])
                qkv_s[k][r, LANES * t:LANES * (t + 1), 0:CW] = pltpu.bitcast(blk.astype(BF16), U32).T
                toks.append((t0 + 96 * (k + 1) + DL_A, qkv_s[k][zx, 0:8, :]))

        def wins(p):
            return 2 * p, min(2 * p + 1, NWIN - 1)

        def b_qk(t0, p):
            wa, wb = wins(p)
            sts = []
            inj = due(soft, WS, t0, 8)
            for w, swap in ((wa, False), (wb, True)):
                qw = gather(q_s, w)
                kw = gather(k_s, w)
                if not swap:
                    kw = [g | inj[r] if r in inj else g for r, g in enumerate(kw)]
                kw = cat(kw)
                for tile in range(2):
                    if tile == 0:
                        kk = f(kw << 16)
                        qq = [f(g << 16) for g in qw]
                    else:
                        kk = f(kw & hi)
                        qq = [f(g & hi) for g in qw]
                    qa = [jnp.where(head_a, g, 0.0) for g in qq]
                    qb = [jnp.where(head_b, g, 0.0) for g in qq]
                    qst = cat(qb + qa if swap else qa + qb)
                    s_t = lax.dot_general(kk, qst, (((1,), (1,)), ((), ())),
                                          preferred_element_type=F32)
                    sts.append(s_t)
            vw = cat(gather(v_s, wa) + gather(v_s, wb))
            vt = vw[:, 0:CW].T
            st['s', p] = (t0, sts, vt)

        def b_sm(tg, p):
            t0, sts, vt = st.pop(('s', p))
            pts = []
            rinv = []
            for n, s_t in enumerate(sts):
                sg = rows8(s_t)
                m8 = functools.reduce(jnp.maximum, sg)
                mx = jnp.max(jnp.where(junk8, -jnp.inf, m8), axis=0, keepdims=True)
                mv = jnp.where(junk8, m8, mx)
                z = tick(tg + SMD * (3 - n)) if SMD else None
                if z is not None:
                    mv = f(pltpu.bitcast(mv, U32) | z[:, 0:2 * G])
                eg = [jnp.exp2(s - mv) for s in sg]
                den = jnp.sum(jnp.where(junk8, 0.0, _tree_sum(eg)), axis=0, keepdims=True)
                r0 = pl.reciprocal(den, approx=True)
                rinv.append(r0 * (2.0 - den * r0))
                pts.append(eg)
            st['b', p] = (pts, rinv, vt)

        def b_pv(t0, p):
            wa, wb = wins(p)
            pts, rinv, vt = st.pop(('b', p))
            inj = due(soft, 3, t0) if PVI else {}
            vt = pltpu.bitcast(cat([g | inj[j][:, 0:2 * G] if j in inj else g for j, g in enumerate(rows8(vt))]), BF16)
            outs = []
            for tile in range(2):
                ra, rb = rinv[tile], rinv[2 + tile]
                for hh in range(2):
                    h = 2 * tile + hh
                    ma, mb = (lo_ok, hi_ok) if hh == 0 else (hi_ok, lo_ok)
                    stn = cat([jnp.where(ma, e, 0.0) for e in pts[tile]]
                              + [jnp.where(mb, e, 0.0) for e in pts[2 + tile]]).astype(BF16)
                    ot = jnp.dot(vt[dh * h:dh * (h + 1), :], stn, preferred_element_type=F32)
                    rr_ = jnp.where(first_half, ra, rb) if hh == 0 else jnp.where(first_half, rb, ra)
                    outs.append(ot * rr_)
            tw = pltpu.bitcast(cat(outs).astype(BF16), U32).T
            for r in range(WS):
                ga = tw[8 * r:8 * r + 8, :]
                gb = tw[G + 8 * r:G + 8 * r + 8, :]
                o_s[r, pl.ds(WS * wa, WS), 0:CW] = jnp.where(even_head, ga, gb)[0:WS]
                if wb != wa:
                    o_s[r, pl.ds(WS * wb, WS), 0:CW] = jnp.where(even_head, gb, ga)[0:WS]
            toks.append((t0 + DL_PV, o_s[zx, 0:8, :]))

        def c_dot(t0, h, r):
            ot = cat([o_s[r, LANES * t:LANES * (t + 1), 0:CW].T for t in (2 * h, 2 * h + 1)], axis=1)
            res = jnp.dot(lhs(wo_s, due(toks, DC // 16, t0), due(soft, DC // 16, t0)),
                          pltpu.bitcast(ot, BF16), preferred_element_type=F32)
            st['c', h, r] = res
            ticks.extend((t0 + 130 + 8 * j, pltpu.bitcast(res[8 * j:8 * j + 8, 0:LANES], U32)) for j in range(DC // 8))

        def c_load(h, r, q):
            n = C // CP
            st['cx', h, r, q] = x_prev[r, n * q:n * (q + 1), HW * h:HW * (h + 1)]

        def c_out(h, r, q):
            n = C // CP
            rs = slice(n * q, n * (q + 1))
            o_ref[r, rs, HW * h:HW * (h + 1)] = (st.pop(('cx', h, r, q)) + st['c', h, r][rs]).astype(o_ref.dtype)

        NR = WS + 2

        def stage_row(d, c, rho):
            cs = slice(16 * c, 16 * c + 16)
            if rho == 0:
                u = pltpu.bitcast(xt_ref[0, cs, :], U32)
            elif rho == WS + 1:
                u = jnp.where(bot_ok, pltpu.bitcast(xb_ref[0, cs, :], U32), zero)
            else:
                u = pltpu.bitcast(xn_ref[rho - 1, cs, :], U32)
            for t, vs in enumerate(shifted(u)):
                for j, v in enumerate(vs):
                    stg_s[c % 2 * NR + rho, 8 * j:8 * j + 8, LANES * t:LANES * (t + 1)] = v
            if STOK:
                soft.append((d, stg_s[zx + 2 * NR, 8:16, 0:LANES]))

        def conv_step(d, c, t, r):
            if r == 0:
                if t == 0:
                    stg_s[zx + 2 * NR, 0:8, 0:LANES] = zvec
                st['un'] = {}
            un = st['un']
            for rho in range(r, r + 3):
                if rho not in un:
                    un[rho] = unpack([stg_s[c % 2 * NR + rho, 8 * j:8 * j + 8, LANES * t:LANES * (t + 1)]
                                      for j in range(3)])
            acc = pltpu.bitcast(conv_row(un, t, r, slice(16 * c, 16 * c + 16), x_next), U32)
            soft.append((d, acc[0:8] | acc[8:16]))

        npair = (NWIN + 1) // 2
        n0 = (HW - 1) // WS // 2
        plan, total = _plan(npair, n0, NT)
        ev = []

        starts = [t for t, _, _ in plan]

        def at(t, fn, *a):
            ev.append((t, t, len(ev), fn, a))

        def before(d, fn, *a):
            e = max([t for t in starts if t <= d], default=0) - 1
            ev.append((e, d, len(ev), fn, a))
            return e

        load = [0.0] * (total + 1000)
        tqk = {}

        def add(t0, t1, n):
            for t in range(max(t0, 0), max(t1, 0)):
                load[t] += n / (t1 - t0)

        for t, kind, idx in plan:
            if kind == 'a':
                before(t - LN1, ln1, t - LN1, *idx)
                for k in range(LNS):
                    d = t - LN2 - LND * (LNS - 1 - k)
                    before(d, ln2, d, *idx, k)
                    add(d - 16, d, 72 // LNS)
                before(t - 40, ln3, *idx)
                at(t, a_dot, t, *idx)
                add(t + 130, t + 130 + DA, 12 * DA // 16)
                add(t - LN1 - 16, t - LN1, 32); add(t - LN2, t - 40, 20); add(t - 40, t, 60 if LN3 else 36)
            elif kind == 'qk':
                at(t, b_qk, t, idx)
                tqk[idx] = t
                add(t - 64, t, 28); add(t, t + 56, 28); add(t + 130, t + 186, 24); add(t + 186, t + 202, 36)
            elif kind == 'pv':
                tg = max(tqk[idx] + SM0, t - SMB)
                at(t - 1, b_sm, tg, idx)
                at(t, b_pv, t, idx)
                add(tg, tg + 4 * SMD + 16, 80); add(t + 120, t + 136, 46); add(t + 130, t + 178, 36)
                add(t + 400, t + 460, 14)
            else:
                at(t, c_dot, t, *idx)
                add(t + 130, t + 130 + DC, 20 * DC // 16)
                for q in range(CP):
                    e = before(t + 130 + (C // CP) * q + COFF, c_load, *idx, q)
                    at(max(e, t) + 2, c_out, *idx, q)
        nc = C // 16
        nstep = nc * NT * WS
        sm = [sum(load[max(t - SMO, 0):t + SMO]) / (2 * SMO) for t in range(total)]
        free = [max(0.0, CAP / 16 - sm[t]) if t >= CV0 - 40 else 0.0 for t in range(total)]
        tot_free, acc, tstep = sum(free), 0.0, []
        for t in range(total):
            acc += free[t]
            while len(tstep) < nstep and acc >= (len(tstep) + 1) * tot_free / nstep - 1e-6:
                tstep.append(t)
        for n in range(nstep):
            before(tstep[n], conv_step, tstep[n], n // (NT * WS), n // WS % NT, n % WS)
        for c in range(nc):
            t1 = tstep[c * NT * WS] - 30
            t0 = tstep[(c - 1) * NT * WS] + 120 if c else 130
            for rho in range(NR):
                d = t0 + (t1 - t0) * rho // (NR - 1)
                before(d, stage_row, d, c, rho)
        ev.sort(key=lambda e: e[:3])
        ev = [e[1:] for e in ev]
        a_done, pv_done = set(), set()
        for _, _, fn, a in ev:
            if fn is a_dot:
                a_done.add(a[1:])
            elif fn is b_qk:
                tl = range(2 * WS * a[1] // LANES, min(2 * WS * a[1] + 2 * WS, WP - 1) // LANES + 1)
                need = [(t, r) in a_done for t in tl for r in range(WS)]
                assert all(need) if a[1] < n0 else not any(need)
            elif fn is b_pv:
                pv_done.add(a[1])
            elif fn is c_dot:
                ps = range(0, n0 + 1) if a[1] == 0 else range(n0, npair)
                assert all((p in pv_done) == (p >= n0) for p in ps)
        for _, _, fn, a in ev:
            fn(*a)

    bufs = (xa_s, xb_s, xc_s)
    for k in range(1 if ONE else 3):
        pl.when(i % 3 == k)(functools.partial(step, bufs[k], bufs[(k + 1) % 3], bufs[(k + 2) % 3]))


@jax.jit
def pallas_standalone__window_attn_davit__vision_kernel(
    x: jax.Array,
    dw_pe: jax.Array,
    w_qkv: jax.Array,
    w_o: jax.Array,
):
    B, H, W, C = x.shape
    assert B == 1 and H % WS == 0 and W % WS == 0 and C % (16 * NH) == 0
    WP = -(-(W + 1) // (2 * LANES)) * (2 * LANES)
    assert WP == 4 * LANES
    NWIN = W // WS
    NBLK = H // WS
    CW = C // 2

    xt = jnp.transpose(x[0], (0, 2, 1))
    dwb = jnp.broadcast_to(dw_pe.reshape(9, C, 1), (9, C, LANES))

    def inter(w):
        return jnp.transpose(w.reshape(C, 2, CW), (2, 1, 0)).reshape(C, C)

    wqkv_t = jnp.concatenate(
        [inter(w_qkv[:, 0:C]), inter(w_qkv[:, C:2 * C]), w_qkv[:, 2 * C:].T], axis=0)
    wo_t = w_o.T

    def nxt(i):
        return jnp.minimum(i + 1, NBLK - 1)

    kern = functools.partial(_kernel, C=C, W=W, WP=WP, NWIN=NWIN, NBLK=NBLK)
    out = pl.pallas_call(
        kern,
        grid=(NBLK + 1,),
        in_specs=[
            pl.BlockSpec((WS, C, WP), lambda i: (nxt(i), 0, 0)),
            pl.BlockSpec((1, C, WP), lambda i: (WS * nxt(i) - 1, 0, 0)),
            pl.BlockSpec((1, C, WP), lambda i: (jnp.minimum(WS * nxt(i) + WS, H - 1), 0, 0)),
            pl.BlockSpec((WS + 1, C, WP), lambda i: (0, 0, 0)),
            pl.BlockSpec((9, C, LANES), lambda i: (0, 0, 0)),
            pl.BlockSpec((3 * C, C), lambda i: (0, 0)),
            pl.BlockSpec((C, C), lambda i: (0, 0)),
        ],
        out_specs=pl.BlockSpec((WS, C, WP), lambda i: (jnp.maximum(i - 1, 0), 0, 0)),
        out_shape=jax.ShapeDtypeStruct((H, C, W), x.dtype),
        scratch_shapes=[
            pltpu.VMEM((WS, C, WP), F32),
            pltpu.VMEM((WS, C, WP), F32),
            pltpu.VMEM((WS, C, WP), F32),
            pltpu.VMEM((WS, WP, LANES), U32),
            pltpu.VMEM((WS, WP, LANES), U32),
            pltpu.VMEM((WS, WP, LANES), U32),
            pltpu.VMEM((WS, WP, LANES), U32),
            pltpu.VMEM((2, 3 * C // 4, C), U32),
            pltpu.VMEM((C // 2, C), U32),
            pltpu.VMEM((2 * (WS + 2) + 1, 3 * 8, WP), U32),
            pltpu.VMEM((9, C, LANES), F32),
        ],
        compiler_params=pltpu.CompilerParams(
            dimension_semantics=("arbitrary",),
            vmem_limit_bytes=64 * 1024 * 1024,
        ),
        name="davit_window_attn",
    )(xt, xt, xt, xt, dwb, wqkv_t, wo_t)
    return jnp.transpose(out, (0, 2, 1))[None]
```

```python
import functools
import math
import os

import jax
import jax.numpy as jnp
from jax import lax
import jax.experimental.pallas as pl
import jax.experimental.pallas.tpu as pltpu

WS = 7
NH = 4
EPS = 1e-05
LANES = 128
F32 = jnp.float32
BF16 = jnp.bfloat16
U32 = jnp.uint32

P = lambda k, d: int(os.environ.get(k, d))
DL_A = P('DL_A', 480)
LAT_QK = P('LAT_QK', 300)
DL_PV = P('DL_PV', 580)
DL_C = P('DL_C', 170)
CP = P('CP', 4)
PRE_C = P('PRE_C', 120)
TAIL = P('TAIL', 1400)
CLEAD = P('CLEAD', 1)
PRE_LN = P('PRE_LN', 200)
SYM = P('SYM', 1)
FAKE = P('FAKE', 0)
CVK = P('CVK', 1)
LN3 = P('LN3', 1)
LN1 = P('LN1', 190)
LN2 = P('LN2', 120)
SM0 = P('SM0', 200)
SMD = P('SMD', 16)
CV0 = P('CV0', 500)
STOK = P('STOK', 1)
COFF = P('COFF', 0)
SMB = P('SMB', 130)
ONE = P('ONE', 0)
TB = P('TB', 0)
LNZ = P('LNZ', 1)
LNS = P('LNS', 2)
LND = P('LND', 16)
PVI = P('PVI', 0)
CAP = P('CAP', 48)
SMO = P('SMO', 32)
CTOK = P('CTOK', 0)
DA, DC, DQ, DP = 288, 192, 56, 48


def _iota(shape, dim):
    return lax.broadcasted_iota(jnp.int32, shape, dim)


def _plan(npair, n0, nt):
    a_q = [(t, r) for t in range(nt) for r in range(WS)]
    c_q = [(h, r) for h in range(2) for r in range(WS)]
    pairs = list(range(n0, npair)) + list(range(n0))
    total = len(a_q) * DA + len(c_q) * DC + npair * (DQ + DP)
    t = 0
    ia = ic = iq = ip = 0
    out = []
    tq, tp, ta = {}, {}, {}
    last = None
    while ia < len(a_q) or ic < len(c_q) or ip < npair:
        cands = []
        if ip < iq and t >= tq[ip] + LAT_QK:
            cands.append((-1e9, 'pv'))
        if iq < npair and iq - ip < 2 and last != 'qk':
            ok = True
            if iq >= npair - n0:
                need = (2 * WS * pairs[iq] + 2 * WS) // LANES * WS + WS - 1
                ok = ia > need and t >= ta[need] + DA + DL_A + 60 and ic >= WS
            if ok:
                cands.append((iq * (total - TAIL) / npair - t - 200, 'qk'))
        if ia < len(a_q):
            cands.append((ia * (total - 700) / len(a_q) - t, 'a'))
        if ic < len(c_q):
            need = 0 if ic < WS else npair - n0 - 1
            if ip > need and t >= tp[need] + DL_PV + PRE_C:
                tc = 1000 + ic * 900 if ic < WS else total - DC - (2 * WS - 1 - ic) * 950
                cands.append((tc - t, 'c'))
        if not cands:
            t += 16
            last = None
            continue
        kind = min(cands)[1]
        last = kind
        if kind == 'pv':
            tp[ip] = t; out.append((t, 'pv', pairs[ip])); ip += 1; t += DP
        elif kind == 'qk':
            tq[iq] = t; out.append((t, 'qk', pairs[iq])); iq += 1; t += DQ
        elif kind == 'a':
            ta[ia] = t; out.append((t, 'a', a_q[ia])); ia += 1; t += DA
        else:
            out.append((t, 'c', c_q[ic])); ic += 1; t += DC
    return out, t


def _tree_sum(xs):
    while len(xs) > 1:
        xs = [xs[j] + xs[j + 1] if j + 1 < len(xs) else xs[j] for j in range(0, len(xs), 2)]
    return xs[0]


def _kernel(xn_ref, xt_ref, xb_ref, xf_ref, dw_ref, wqkv_ref, wo_ref, o_ref,
            xa_s, xb_s, xc_s, q_s, k_s, v_s, o_s, wq_s, wo_s, stg_s, dw_s, *, C, W, WP, NWIN, NBLK):
    i = pl.program_id(0)
    dh = C // NH
    CW = C // 2
    NT = WP // LANES
    G = WS * 8
    HW = WP // 2
    lane8 = _iota((8, LANES), 1)
    last_valid = W - (NT - 1) * LANES
    zero = jnp.uint32(0)
    qkv_s = (q_s, k_s, v_s)
    zx = i >> 10
    zvec = jnp.full((8, LANES), zx, jnp.int32).astype(U32)

    def shifted(u):
        tiles = [u[:, LANES * t:LANES * (t + 1)] for t in range(NT)]
        tiles[NT - 1] = jnp.where(lane8 < last_valid, tiles[NT - 1], zero)
        row = []
        for t in range(NT):
            left = jnp.where(lane8 == LANES - 1, tiles[t - 1] if t > 0 else zero, tiles[t])
            right = jnp.where(lane8 == 0, tiles[t + 1], tiles[t]) if t < NT - 1 else tiles[t]
            row.append((pltpu.roll(left, 1, 1), tiles[t], pltpu.roll(right, LANES - 1, 1)))
        return row

    def unpack(vs):
        return [pltpu.bitcast(v, BF16).astype(F32) for v in vs]

    def conv_row(un, t, r, cs, buf):
        w = [dw_s[tap, cs, :] for tap in range(9)]
        terms = [un[r + ki][kj] * w[3 * ki + kj]
                 for ki in range(3) for kj in range(3) if un[r + ki] is not None]
        acc = _tree_sum(terms)
        buf[r, cs, LANES * t:LANES * (t + 1)] = acc
        return acc

    @pl.when(i == 0)
    def _():
        qscale = (dh ** -0.5) * math.log2(math.e)
        for j in range(3 * C // 16):
            blk = wqkv_ref[16 * j:16 * j + 16, :]
            if j < C // 16:
                blk = (blk.astype(F32) * qscale).astype(BF16)
            wq_s[j % 2, 8 * (j // 2):8 * (j // 2) + 8, :] = pltpu.bitcast(blk, U32)
        wo_s[...] = pltpu.bitcast(wo_ref[...].astype(F32), U32)

        def zrow(r, carry):
            for ref in (q_s, k_s, v_s, o_s):
                ref[r] = jnp.zeros(ref.shape[1:], U32)
            xc_s[r] = jnp.zeros(xc_s.shape[1:], F32)
            return carry
        lax.fori_loop(0, WS, zrow, 0)
        stg_s[...] = jnp.zeros(stg_s.shape, U32)
        for tap in range(9):
            w = dw_ref[tap].astype(F32)
            if tap == 4:
                w = w + 1.0
            dw_s[tap] = w

        def conv0(c, carry):
            cs = pl.ds(pl.multiple_of(16 * c, 16), 16)
            sh = [shifted(pltpu.bitcast(xf_ref[rho, cs, :], U32)) for rho in range(WS + 1)]
            for t in range(NT):
                un = [None] + [unpack(row[t]) for row in sh]
                for r in range(WS):
                    conv_row(un, t, r, cs, xa_s)
            return carry
        lax.fori_loop(0, C // 16, conv0, 0)

    def step(x_cur, x_next, x_prev):
        bot_ok = i + 1 < NBLK - 1

        hi = jnp.uint32(0xFFFF0000)
        head_a = lane8 < dh
        head_b = (lane8 >= dh) & (lane8 < 2 * dh)
        junk8 = _iota((8, 2 * G), 0) == WS
        lo_ok = (_iota((8, 2 * G), 1) < G) & ~junk8
        hi_ok = (_iota((8, 2 * G), 1) >= G) & ~junk8
        first_half = _iota((1, 2 * G), 1) < G
        even_head = (_iota((8, CW), 1) // (dh // 2)) % 2 == 0

        def gather(ref, w):
            return [ref[r, pl.ds(WS * w, 8), :] for r in range(WS)]

        def f(u):
            return pltpu.bitcast(u, F32)

        def cat(xs, axis=0):
            return jnp.concatenate(xs, axis=axis)

        st = {}
        toks = []
        soft = []
        ticks = []

        def tick(t):
            c = [x for x in ticks if x[0] >= t]
            return (min(c, key=lambda x: x[0])[1] & zvec) if c else None

        def due(lst, nblk, t0, step=16):
            inj = {}
            for d, tok in list(lst):
                j = max(0, -(-(d - t0) // step))
                if j < nblk:
                    inj[j] = tok if j not in inj else inj[j] | tok
                    lst[:] = [x for x in lst if x[1] is not tok]
            return {j: v & zvec for j, v in inj.items()}

        def lhs(ref, inj, inj1, dt=BF16):
            nblk = ref.shape[0] // 8
            parts, s = [], 0
            for j in sorted(set(inj) | set(inj1)):
                if j > s:
                    parts.append(ref[8 * s:8 * j, :])
                k0, k1 = ref[8 * j:8 * j + 8, 0:LANES], ref[8 * j:8 * j + 8, LANES:]
                if j in inj:
                    k0 = k0 | inj[j]
                    if SYM:
                        k1 = k1 | inj[j][:, 0:k1.shape[1]]
                if j in inj1:
                    k0 = k0 | inj1[j]
                parts.append(cat([k0, k1], axis=1))
                s = j + 1
            if s < nblk:
                parts.append(ref[8 * s:8 * nblk, :])
            return pltpu.bitcast(cat(parts) if len(parts) > 1 else parts[0], dt)

        def rows8(x):
            return [x[8 * j:8 * j + 8] for j in range(x.shape[0] // 8)]

        def bc8(v):
            return pltpu.bitcast(jnp.broadcast_to(v, (8, LANES)), U32)

        def x0_cur(t, r):
            return x_cur[r, :, LANES * t:LANES * (t + 1)]

        def ln1(d, t, r):
            s8 = _tree_sum(rows8(x0_cur(t, r)))
            soft.append((d, pltpu.bitcast(s8, U32)))
            st['m', t, r] = jnp.sum(s8, axis=0, keepdims=True) * (1.0 / C)

        def ln2(d, t, r, k):
            n = C // LNS
            xc = x_cur[(zx if LNZ else 0) + r, n * k:n * (k + 1), LANES * t:LANES * (t + 1)] - st['m', t, r]
            s8 = _tree_sum(rows8(xc * xc))
            soft.append((d, pltpu.bitcast(s8, U32)))
            st.setdefault(('xc', t, r), []).append(xc)
            st.setdefault(('sq', t, r), []).append(s8)

        def ln3(t, r):
            var = jnp.sum(_tree_sum(st.pop(('sq', t, r))), axis=0, keepdims=True) * (1.0 / C)
            xc = cat(st.pop(('xc', t, r)))
            if LN3:
                xc = x_cur[(i >> 11) + r, :, LANES * t:LANES * (t + 1)] - st['m', t, r]
            st['h', t, r] = (xc * lax.rsqrt(var + EPS)).astype(BF16)

        def a_dot(t0, t, r):
            h = st.pop(('h', t, r))
            inj = due(toks, DA // 16, t0)
            res = [jnp.dot(lhs(wq_s.at[0], inj, due(soft, DA // 16, t0)), h, preferred_element_type=F32),
                   jnp.dot(lhs(wq_s.at[1], inj if SYM else {}, {}), h, preferred_element_type=F32)]
            ticks.extend((t0 + 130 + 8 * j, pltpu.bitcast(res[0][8 * j:8 * j + 8], U32)) for j in range(DA // 8))
            nb = C // 16
            for k in range(3):
                blk = cat([res[j % 2][16 * (j // 2):16 * (j // 2) + 16, :] for j in range(nb * k, nb * (k + 1))])
                qkv_s[k][r, LANES * t:LANES * (t + 1), 0:CW] = pltpu.bitcast(blk.astype(BF16), U32).T
                toks.append((t0 + 96 * (k + 1) + DL_A, qkv_s[k][zx, 0:8, :]))

        def wins(p):
            return 2 * p, min(2 * p + 1, NWIN - 1)

        def b_qk(t0, p):
            wa, wb = wins(p)
            sts = []
            inj = due(soft, WS, t0, 8)
            for w, swap in ((wa, False), (wb, True)):
                qw = gather(q_s, w)
                kw = gather(k_s, w)
                if not swap:
                    kw = [g | inj[r] if r in inj else g for r, g in enumerate(kw)]
                kw = cat(kw)
                for tile in range(2):
                    if tile == 0:
                        kk = f(kw << 16)
                        qq = [f(g << 16) for g in qw]
                    else:
                        kk = f(kw & hi)
                        qq = [f(g & hi) for g in qw]
                    qa = [jnp.where(head_a, g, 0.0) for g in qq]
                    qb = [jnp.where(head_b, g, 0.0) for g in qq]
                    qst = cat(qb + qa if swap else qa + qb)
                    s_t = lax.dot_general(kk, qst, (((1,), (1,)), ((), ())),
                                          preferred_element_type=F32)
                    sts.append(s_t)
            vw = cat(gather(v_s, wa) + gather(v_s, wb))
            vt = vw[:, 0:CW].T
            st['s', p] = (t0, sts, vt)

        def b_sm(tg, p):
            t0, sts, vt = st.pop(('s', p))
            pts = []
            rinv = []
            for n, s_t in enumerate(sts):
                sg = rows8(s_t)
                m8 = functools.reduce(jnp.maximum, sg)
                mx = jnp.max(jnp.where(junk8, -jnp.inf, m8), axis=0, keepdims=True)
                mv = jnp.where(junk8, m8, mx)
                z = tick(tg + SMD * (3 - n)) if SMD else None
                if z is not None:
                    mv = f(pltpu.bitcast(mv, U32) | z[:, 0:2 * G])
                eg = [jnp.exp2(s - mv) for s in sg]
                den = jnp.sum(jnp.where(junk8, 0.0, _tree_sum(eg)), axis=0, keepdims=True)
                r0 = pl.reciprocal(den, approx=True)
                rinv.append(r0 * (2.0 - den * r0))
                pts.append(eg)
            st['b', p] = (pts, rinv, vt)

        def b_pv(t0, p):
            wa, wb = wins(p)
            pts, rinv, vt = st.pop(('b', p))
            inj = due(soft, 3, t0) if PVI else {}
            vt = pltpu.bitcast(cat([g | inj[j][:, 0:2 * G] if j in inj else g for j, g in enumerate(rows8(vt))]), BF16)
            outs = []
            for tile in range(2):
                ra, rb = rinv[tile], rinv[2 + tile]
                for hh in range(2):
                    h = 2 * tile + hh
                    ma, mb = (lo_ok, hi_ok) if hh == 0 else (hi_ok, lo_ok)
                    stn = cat([jnp.where(ma, e, 0.0) for e in pts[tile]]
                              + [jnp.where(mb, e, 0.0) for e in pts[2 + tile]]).astype(BF16)
                    ot = jnp.dot(vt[dh * h:dh * (h + 1), :], stn, preferred_element_type=F32)
                    rr_ = jnp.where(first_half, ra, rb) if hh == 0 else jnp.where(first_half, rb, ra)
                    outs.append(ot * rr_)
            tw = pltpu.bitcast(cat(outs).astype(BF16), U32).T
            for r in range(WS):
                ga = tw[8 * r:8 * r + 8, :]
                gb = tw[G + 8 * r:G + 8 * r + 8, :]
                o_s[r, pl.ds(WS * wa, WS), 0:CW] = jnp.where(even_head, ga, gb)[0:WS]
                if wb != wa:
                    o_s[r, pl.ds(WS * wb, WS), 0:CW] = jnp.where(even_head, gb, ga)[0:WS]
            toks.append((t0 + DL_PV, o_s[zx, 0:8, :]))

        def c_dot(t0, h, r):
            ow = o_s[r, HW * h:HW * (h + 1), :]
            rhs = cat([f(ow << 16), f(ow & hi)], axis=1)
            res = lax.dot_general(lhs(wo_s, due(toks, DC // 8, t0, 8), due(soft, DC // 8, t0, 8), F32), rhs,
                                  (((1,), (1,)), ((), ())), preferred_element_type=F32)
            st['c', h, r] = res
            ticks.extend((t0 + 130 + 8 * j, pltpu.bitcast(res[8 * j:8 * j + 8, 0:LANES], U32)) for j in range(DC // 8))

        def c_load(h, r, q):
            n = C // CP
            st['cx', h, r, q] = x_prev[r, n * q:n * (q + 1), HW * h:HW * (h + 1)]

        def c_out(h, r, q):
            n = C // CP
            rs = slice(n * q, n * (q + 1))
            o_ref[r, rs, HW * h:HW * (h + 1)] = (st.pop(('cx', h, r, q)) + st['c', h, r][rs]).astype(o_ref.dtype)

        NR = WS + 2

        def stage_row(d, c, rho):
            cs = slice(16 * c, 16 * c + 16)
            if rho == 0:
                u = pltpu.bitcast(xt_ref[0, cs, :], U32)
            elif rho == WS + 1:
                u = jnp.where(bot_ok, pltpu.bitcast(xb_ref[0, cs, :], U32), zero)
            else:
                u = pltpu.bitcast(xn_ref[rho - 1, cs, :], U32)
            for t, vs in enumerate(shifted(u)):
                for j, v in enumerate(vs):
                    stg_s[c % 2 * NR + rho, 8 * j:8 * j + 8, LANES * t:LANES * (t + 1)] = v
            if STOK:
                soft.append((d, stg_s[zx + 2 * NR, 8:16, 0:LANES]))

        def conv_step(d, c, t, r):
            if r == 0:
                if t == 0:
                    stg_s[zx + 2 * NR, 0:8, 0:LANES] = zvec
                st['un'] = {}
            un = st['un']
            for rho in range(r, r + 3):
                if rho not in un:
                    un[rho] = unpack([stg_s[c % 2 * NR + rho, 8 * j:8 * j + 8, LANES * t:LANES * (t + 1)]
                                      for j in range(3)])
            acc = pltpu.bitcast(conv_row(un, t, r, slice(16 * c, 16 * c + 16), x_next), U32)
            tok = acc[0:8] | acc[8:16]
            soft.append((d, tok))
            if TB and (r + 1) % TB == 0:
                dw_s[zx + 9, 0:8, :] = f(tok)

        npair = (NWIN + 1) // 2
        n0 = (HW - 1) // WS // 2
        plan, total = _plan(npair, n0, NT)
        ev = []

        starts = [t for t, _, _ in plan]

        def at(t, fn, *a):
            ev.append((t, t, len(ev), fn, a))

        def before(d, fn, *a):
            e = max([t for t in starts if t <= d], default=0) - 1
            ev.append((e, d, len(ev), fn, a))
            return e

        load = [0.0] * (total + 1000)
        tqk = {}

        def add(t0, t1, n):
            for t in range(max(t0, 0), max(t1, 0)):
                load[t] += n / (t1 - t0)

        for t, kind, idx in plan:
            if kind == 'a':
                before(t - LN1, ln1, t - LN1, *idx)
                for k in range(LNS):
                    d = t - LN2 - LND * (LNS - 1 - k)
                    before(d, ln2, d, *idx, k)
                    add(d - 16, d, 72 // LNS)
                before(t - 40, ln3, *idx)
                at(t, a_dot, t, *idx)
                add(t + 130, t + 130 + DA, 12 * DA // 16)
                add(t - LN1 - 16, t - LN1, 32); add(t - LN2, t - 40, 20); add(t - 40, t, 60 if LN3 else 36)
            elif kind == 'qk':
                at(t, b_qk, t, idx)
                tqk[idx] = t
                add(t - 64, t, 28); add(t, t + 56, 28); add(t + 130, t + 186, 24); add(t + 186, t + 202, 36)
            elif kind == 'pv':
                tg = max(tqk[idx] + SM0, t - SMB)
                at(t - 1, b_sm, tg, idx)
                at(t, b_pv, t, idx)
                add(tg, tg + 4 * SMD + 16, 80); add(t + 120, t + 136, 46); add(t + 130, t + 178, 36)
                add(t + 400, t + 460, 14)
            else:
                at(t, c_dot, t, *idx)
                add(t + 130, t + 130 + DC, 20 * DC // 16)
                add(t - 70, t, 64)
                for q in range(CP):
                    e = before(t + 130 + (C // CP) * q + COFF, c_load, *idx, q)
                    at(max(e, t) + 2, c_out, *idx, q)
        nc = C // 16
        nstep = nc * NT * WS
        sm = [sum(load[max(t - SMO, 0):t + SMO]) / (2 * SMO) for t in range(total)]
        free = [max(0.0, CAP / 16 - sm[t]) if t >= CV0 - 40 else 0.0 for t in range(total)]
        tot_free, acc, tstep = sum(free), 0.0, []
        for t in range(total):
            acc += free[t]
            while len(tstep) < nstep and acc >= (len(tstep) + 1) * tot_free / nstep - 1e-6:
                tstep.append(t)
        for n in range(nstep):
            before(tstep[n], conv_step, tstep[n], n // (NT * WS), n // WS % NT, n % WS)
        for c in range(nc):
            t1 = tstep[c * NT * WS] - 30
            t0 = tstep[(c - 1) * NT * WS] + 120 if c else 130
            for rho in range(NR):
                d = t0 + (t1 - t0) * rho // (NR - 1)
                before(d, stage_row, d, c, rho)
        ev.sort(key=lambda e: e[:3])
        ev = [e[1:] for e in ev]
        a_done, pv_done = set(), set()
        for _, _, fn, a in ev:
            if fn is a_dot:
                a_done.add(a[1:])
            elif fn is b_qk:
                tl = range(2 * WS * a[1] // LANES, min(2 * WS * a[1] + 2 * WS, WP - 1) // LANES + 1)
                need = [(t, r) in a_done for t in tl for r in range(WS)]
                assert all(need) if a[1] < n0 else not any(need)
            elif fn is b_pv:
                pv_done.add(a[1])
            elif fn is c_dot:
                ps = range(0, n0 + 1) if a[1] == 0 else range(n0, npair)
                assert all((p in pv_done) == (p >= n0) for p in ps)
        for _, _, fn, a in ev:
            fn(*a)

    bufs = (xa_s, xb_s, xc_s)
    if ONE:
        @pl.when(i == 1000)
        def _():
            lax.fori_loop(0, WS, lambda r, c: o_ref.__setitem__(r, xb_s[r].astype(o_ref.dtype)) or c, 0)
    for k in range(1 if ONE else 3):
        pl.when(i % 3 == k)(functools.partial(step, bufs[k], bufs[(k + 1) % 3], bufs[(k + 2) % 3]))


@jax.jit
def pallas_standalone__window_attn_davit__vision_kernel(
    x: jax.Array,
    dw_pe: jax.Array,
    w_qkv: jax.Array,
    w_o: jax.Array,
):
    B, H, W, C = x.shape
    assert B == 1 and H % WS == 0 and W % WS == 0 and C % (16 * NH) == 0
    WP = -(-(W + 1) // (2 * LANES)) * (2 * LANES)
    assert WP == 4 * LANES
    NWIN = W // WS
    NBLK = H // WS
    CW = C // 2

    xt = jnp.transpose(x[0], (0, 2, 1))
    dwb = jnp.broadcast_to(dw_pe.reshape(9, C, 1), (9, C, LANES))

    def inter(w):
        return jnp.transpose(w.reshape(C, 2, CW), (2, 1, 0)).reshape(C, C)

    wqkv_t = jnp.concatenate(
        [inter(w_qkv[:, 0:C]), inter(w_qkv[:, C:2 * C]), w_qkv[:, 2 * C:].T], axis=0)
    wo_t = jnp.pad(jnp.transpose(w_o.reshape(CW, 2, C), (2, 1, 0)), ((0, 0), (0, 0), (0, LANES - CW)))
    wo_t = wo_t.reshape(C, 2 * LANES)

    def nxt(i):
        return jnp.minimum(i + 1, NBLK - 1)

    kern = functools.partial(_kernel, C=C, W=W, WP=WP, NWIN=NWIN, NBLK=NBLK)
    out = pl.pallas_call(
        kern,
        grid=(NBLK + 1,),
        in_specs=[
            pl.BlockSpec((WS, C, WP), lambda i: (nxt(i), 0, 0)),
            pl.BlockSpec((1, C, WP), lambda i: (WS * nxt(i) - 1, 0, 0)),
            pl.BlockSpec((1, C, WP), lambda i: (jnp.minimum(WS * nxt(i) + WS, H - 1), 0, 0)),
            pl.BlockSpec((WS + 1, C, WP), lambda i: (0, 0, 0)),
            pl.BlockSpec((9, C, LANES), lambda i: (0, 0, 0)),
            pl.BlockSpec((3 * C, C), lambda i: (0, 0)),
            pl.BlockSpec((C, 2 * LANES), lambda i: (0, 0)),
        ],
        out_specs=pl.BlockSpec((WS, C, WP), lambda i: (jnp.maximum(i - 1, 0), 0, 0)),
        out_shape=jax.ShapeDtypeStruct((H, C, W), x.dtype),
        scratch_shapes=[
            pltpu.VMEM((WS, C, WP), F32),
            pltpu.VMEM((WS, C, WP), F32),
            pltpu.VMEM((WS, C, WP), F32),
            pltpu.VMEM((WS, WP, LANES), U32),
            pltpu.VMEM((WS, WP, LANES), U32),
            pltpu.VMEM((WS, WP, LANES), U32),
            pltpu.VMEM((WS, WP, LANES), U32),
            pltpu.VMEM((2, 3 * C // 4, C), U32),
            pltpu.VMEM((C, 2 * LANES), U32),
            pltpu.VMEM((2 * (WS + 2) + 1, 3 * 8, WP), U32),
            pltpu.VMEM((10, C, LANES), F32),
        ],
        compiler_params=pltpu.CompilerParams(
            dimension_semantics=("arbitrary",),
            vmem_limit_bytes=64 * 1024 * 1024,
        ),
        name="davit_window_attn",
    )(xt, xt, xt, xt, dwb, wqkv_t, wo_t)
    return jnp.transpose(out, (0, 2, 1))[None]
```

```python
import functools
import math
import os

import jax
import jax.numpy as jnp
from jax import lax
import jax.experimental.pallas as pl
import jax.experimental.pallas.tpu as pltpu

WS = 7
NH = 4
EPS = 1e-05
LANES = 128
F32 = jnp.float32
BF16 = jnp.bfloat16
U32 = jnp.uint32

P = lambda k, d: int(os.environ.get(k, d))
DL_A = P('DL_A', 480)
LAT_QK = P('LAT_QK', 300)
DL_PV = P('DL_PV', 580)
DL_C = P('DL_C', 170)
CP = P('CP', 4)
PRE_C = P('PRE_C', 120)
TAIL = P('TAIL', 1400)
CLEAD = P('CLEAD', 1)
PRE_LN = P('PRE_LN', 200)
SYM = P('SYM', 1)
FAKE = P('FAKE', 0)
CVK = P('CVK', 1)
LN3 = P('LN3', 0)
LN1 = P('LN1', 190)
LN2 = P('LN2', 120)
SM0 = P('SM0', 200)
SMD = P('SMD', 16)
CV0 = P('CV0', 500)
STOK = P('STOK', 1)
COFF = P('COFF', 0)
SMB = P('SMB', 130)
ONE = P('ONE', 0)
VG = P('VG', 0)
LNB = P('LNB', 0)
TB = P('TB', 0)
LNZ = P('LNZ', 0)
LNS = P('LNS', 2)
LND = P('LND', 16)
PVI = P('PVI', 0)
CAP = P('CAP', 42)
SMO = P('SMO', 32)
CTOK = P('CTOK', 0)
DA, DC, DQ, DP = 288, 192, 56, 48


def _iota(shape, dim):
    return lax.broadcasted_iota(jnp.int32, shape, dim)


def _plan(npair, n0, nt):
    a_q = [(t, r) for t in range(nt) for r in range(WS)]
    c_q = [(h, r) for h in range(2) for r in range(WS)]
    pairs = list(range(n0, npair)) + list(range(n0))
    total = len(a_q) * DA + len(c_q) * DC + npair * (DQ + DP)
    t = 0
    ia = ic = iq = ip = 0
    out = []
    tq, tp, ta = {}, {}, {}
    last = None
    while ia < len(a_q) or ic < len(c_q) or ip < npair:
        cands = []
        if ip < iq and t >= tq[ip] + LAT_QK:
            cands.append((-1e9, 'pv'))
        if iq < npair and iq - ip < 2 and last != 'qk':
            ok = True
            if iq >= npair - n0:
                need = (2 * WS * pairs[iq] + 2 * WS) // LANES * WS + WS - 1
                ok = ia > need and t >= ta[need] + DA + DL_A + 60 and ic >= WS
            if ok:
                cands.append((iq * (total - TAIL) / npair - t - 200, 'qk'))
        if ia < len(a_q):
            cands.append((ia * (total - 700) / len(a_q) - t, 'a'))
        if ic < len(c_q):
            need = 0 if ic < WS else npair - n0 - 1
            if ip > need and t >= tp[need] + DL_PV + PRE_C:
                tc = 1000 + ic * 900 if ic < WS else total - DC - (2 * WS - 1 - ic) * 950
                cands.append((tc - t, 'c'))
        if not cands:
            t += 16
            last = None
            continue
        kind = min(cands)[1]
        last = kind
        if kind == 'pv':
            tp[ip] = t; out.append((t, 'pv', pairs[ip])); ip += 1; t += DP
        elif kind == 'qk':
            tq[iq] = t; out.append((t, 'qk', pairs[iq])); iq += 1; t += DQ
        elif kind == 'a':
            ta[ia] = t; out.append((t, 'a', a_q[ia])); ia += 1; t += DA
        else:
            out.append((t, 'c', c_q[ic])); ic += 1; t += DC
    return out, t


def _tree_sum(xs):
    while len(xs) > 1:
        xs = [xs[j] + xs[j + 1] if j + 1 < len(xs) else xs[j] for j in range(0, len(xs), 2)]
    return xs[0]


def _kernel(xn_ref, xt_ref, xb_ref, xf_ref, dw_ref, wqkv_ref, wo_ref, o_ref,
            xa_s, xb_s, xc_s, q_s, k_s, v_s, o_s, wq_s, wo_s, sa_s, sb_s, dw_s, *, C, W, WP, NWIN, NBLK):
    i = pl.program_id(0)
    dh = C // NH
    CW = C // 2
    NT = WP // LANES
    G = WS * 8
    HW = WP // 2
    lane8 = _iota((8, LANES), 1)
    last_valid = W - (NT - 1) * LANES
    zero = jnp.uint32(0)
    qkv_s = (q_s, k_s, v_s)
    zx = i >> 10
    zvec = jnp.full((8, LANES), zx, jnp.int32).astype(U32)

    def shifted(u):
        tiles = [u[:, LANES * t:LANES * (t + 1)] for t in range(NT)]
        tiles[NT - 1] = jnp.where(lane8 < last_valid, tiles[NT - 1], zero)
        row = []
        for t in range(NT):
            left = jnp.where(lane8 == LANES - 1, tiles[t - 1] if t > 0 else zero, tiles[t])
            right = jnp.where(lane8 == 0, tiles[t + 1], tiles[t]) if t < NT - 1 else tiles[t]
            row.append((pltpu.roll(left, 1, 1), tiles[t], pltpu.roll(right, LANES - 1, 1)))
        return row

    def unpack(vs):
        return [pltpu.bitcast(v, BF16).astype(F32) for v in vs]

    def conv_row(un, t, r, cs, buf):
        w = [dw_s[tap, cs, :] for tap in range(9)]
        terms = [un[r + ki][kj] * w[3 * ki + kj]
                 for ki in range(3) for kj in range(3) if un[r + ki] is not None]
        acc = _tree_sum(terms)
        buf[r, cs, LANES * t:LANES * (t + 1)] = acc
        return acc

    @pl.when(i == 0)
    def _():
        qscale = (dh ** -0.5) * math.log2(math.e)
        for j in range(3 * C // 16):
            blk = wqkv_ref[16 * j:16 * j + 16, :]
            if j < C // 16:
                blk = (blk.astype(F32) * qscale).astype(BF16)
            wq_s[j % 2, 8 * (j // 2):8 * (j // 2) + 8, :] = pltpu.bitcast(blk, U32)
        wo_s[...] = pltpu.bitcast(wo_ref[...].astype(F32), U32)

        def zrow(r, carry):
            for ref in (q_s, k_s, v_s, o_s):
                ref[r] = jnp.zeros(ref.shape[1:], U32)
            xc_s[r] = jnp.zeros(xc_s.shape[1:], F32)
            return carry
        lax.fori_loop(0, WS, zrow, 0)
        for ref in (sa_s, sb_s):
            ref[WS + 2] = jnp.zeros(ref.shape[1:], U32)
        for tap in range(9):
            w = dw_ref[tap].astype(F32)
            if tap == 4:
                w = w + 1.0
            dw_s[tap] = w

        def conv0(c, carry):
            cs = pl.ds(pl.multiple_of(16 * c, 16), 16)
            sh = [shifted(pltpu.bitcast(xf_ref[rho, cs, :], U32)) for rho in range(WS + 1)]
            for t in range(NT):
                un = [None] + [unpack(row[t]) for row in sh]
                for r in range(WS):
                    conv_row(un, t, r, cs, xa_s)
            return carry
        lax.fori_loop(0, C // 16, conv0, 0)

    def step(x_cur, x_next, x_prev):
        bot_ok = i + 1 < NBLK - 1

        hi = jnp.uint32(0xFFFF0000)
        head_a = lane8 < dh
        head_b = (lane8 >= dh) & (lane8 < 2 * dh)
        junk8 = _iota((8, 2 * G), 0) == WS
        lo_ok = (_iota((8, 2 * G), 1) < G) & ~junk8
        hi_ok = (_iota((8, 2 * G), 1) >= G) & ~junk8
        first_half = _iota((1, 2 * G), 1) < G
        even_head = (_iota((8, CW), 1) // (dh // 2)) % 2 == 0

        def gather(ref, w):
            return [ref[r, pl.ds(WS * w, 8), :] for r in range(WS)]

        def f(u):
            return pltpu.bitcast(u, F32)

        def cat(xs, axis=0):
            return jnp.concatenate(xs, axis=axis)

        st = {}
        toks = []
        soft = []
        ticks = []

        def tick(t, before=False):
            if before:
                c = [x for x in ticks if x[0] <= t]
                return (max(c, key=lambda x: x[0])[1] & zvec) if c else None
            c = [x for x in ticks if x[0] >= t]
            return (min(c, key=lambda x: x[0])[1] & zvec) if c else None

        def due(lst, nblk, t0, step=16):
            inj = {}
            for d, tok in list(lst):
                j = max(0, -(-(d - t0) // step))
                if j < nblk:
                    inj[j] = tok if j not in inj else inj[j] | tok
                    lst[:] = [x for x in lst if x[1] is not tok]
            return {j: v & zvec for j, v in inj.items()}

        def lhs(ref, inj, inj1, dt=BF16):
            nblk = ref.shape[0] // 8
            parts, s = [], 0
            for j in sorted(set(inj) | set(inj1)):
                if j > s:
                    parts.append(ref[8 * s:8 * j, :])
                k0, k1 = ref[8 * j:8 * j + 8, 0:LANES], ref[8 * j:8 * j + 8, LANES:]
                if j in inj:
                    k0 = k0 | inj[j]
                    if SYM:
                        k1 = k1 | inj[j][:, 0:k1.shape[1]]
                if j in inj1:
                    k0 = k0 | inj1[j]
                parts.append(cat([k0, k1], axis=1))
                s = j + 1
            if s < nblk:
                parts.append(ref[8 * s:8 * nblk, :])
            return pltpu.bitcast(cat(parts) if len(parts) > 1 else parts[0], dt)

        def rows8(x):
            return [x[8 * j:8 * j + 8] for j in range(x.shape[0] // 8)]

        def bc8(v):
            return pltpu.bitcast(jnp.broadcast_to(v, (8, LANES)), U32)

        def x0_cur(t, r):
            return x_cur[r, :, LANES * t:LANES * (t + 1)]

        def ln1(d, t, r):
            s8 = _tree_sum(rows8(x0_cur(t, r)))
            soft.append((d, pltpu.bitcast(s8, U32)))
            st['s8', t, r] = s8
            st['m', t, r] = jnp.sum(s8, axis=0, keepdims=True) * (1.0 / C)

        def ln2(d, t, r, k):
            n = C // LNS
            if LNB and k == 0:
                x_cur[zx + WS, 0:8, 0:LANES] = st['s8', t, r]
            xc = x_cur[(zx if LNZ and not LNB else 0) + r, n * k:n * (k + 1), LANES * t:LANES * (t + 1)] - st['m', t, r]
            s8 = _tree_sum(rows8(xc * xc))
            soft.append((d, pltpu.bitcast(s8, U32)))
            st.setdefault(('xc', t, r), []).append(xc)
            st.setdefault(('sq', t, r), []).append(s8)

        def ln3(t, r):
            sq = _tree_sum(st.pop(('sq', t, r)))
            var = jnp.sum(sq, axis=0, keepdims=True) * (1.0 / C)
            xc = cat(st.pop(('xc', t, r)))
            if LN3:
                if LNB:
                    x_cur[zx + WS, 0:8, 0:LANES] = sq
                xc = x_cur[(0 if LNB else i >> 11) + r, :, LANES * t:LANES * (t + 1)] - st['m', t, r]
            st['h', t, r] = (xc * lax.rsqrt(var + EPS)).astype(BF16)

        def a_dot(t0, t, r):
            h = st.pop(('h', t, r))
            inj = due(toks, DA // 16, t0)
            res = [jnp.dot(lhs(wq_s.at[0], inj, due(soft, DA // 16, t0)), h, preferred_element_type=F32),
                   jnp.dot(lhs(wq_s.at[1], inj if SYM else {}, {}), h, preferred_element_type=F32)]
            ticks.extend((t0 + 130 + 8 * j, pltpu.bitcast(res[0][8 * j:8 * j + 8], U32)) for j in range(DA // 8))
            nb = C // 16
            for k in range(3):
                blk = cat([res[j % 2][16 * (j // 2):16 * (j // 2) + 16, :] for j in range(nb * k, nb * (k + 1))])
                qkv_s[k][r, LANES * t:LANES * (t + 1), 0:CW] = pltpu.bitcast(blk.astype(BF16), U32).T
                toks.append((t0 + 96 * (k + 1) + DL_A, qkv_s[k][zx, 0:8, :]))

        def wins(p):
            return 2 * p, min(2 * p + 1, NWIN - 1)

        def b_qk(t0, p):
            wa, wb = wins(p)
            sts = []
            inj = due(soft, WS, t0, 8)
            for w, swap in ((wa, False), (wb, True)):
                qw = gather(q_s, w)
                kw = gather(k_s, w)
                if not swap:
                    kw = [g | inj[r] if r in inj else g for r, g in enumerate(kw)]
                kw = cat(kw)
                for tile in range(2):
                    if tile == 0:
                        kk = f(kw << 16)
                        qq = [f(g << 16) for g in qw]
                    else:
                        kk = f(kw & hi)
                        qq = [f(g & hi) for g in qw]
                    qa = [jnp.where(head_a, g, 0.0) for g in qq]
                    qb = [jnp.where(head_b, g, 0.0) for g in qq]
                    qst = cat(qb + qa if swap else qa + qb)
                    s_t = lax.dot_general(kk, qst, (((1,), (1,)), ((), ())),
                                          preferred_element_type=F32)
                    sts.append(s_t)
            st['s', p] = (t0, sts, gather(v_s, wa) + gather(v_s, wb))

        def b_sm(tg, tv, p):
            t0, sts, vw = st.pop(('s', p))
            z = tick(tv, True) if VG else None
            if z is not None:
                vw[0] = vw[0] | z
            vt = cat(vw)[:, 0:CW].T
            pts = []
            rinv = []
            for n, s_t in enumerate(sts):
                sg = rows8(s_t)
                m8 = functools.reduce(jnp.maximum, sg)
                mx = jnp.max(jnp.where(junk8, -jnp.inf, m8), axis=0, keepdims=True)
                mv = jnp.where(junk8, m8, mx)
                z = tick(tg + SMD * (3 - n)) if SMD else None
                if z is not None:
                    mv = f(pltpu.bitcast(mv, U32) | z[:, 0:2 * G])
                eg = [jnp.exp2(s - mv) for s in sg]
                den = jnp.sum(jnp.where(junk8, 0.0, _tree_sum(eg)), axis=0, keepdims=True)
                r0 = pl.reciprocal(den, approx=True)
                rinv.append(r0 * (2.0 - den * r0))
                pts.append(eg)
            st['b', p] = (pts, rinv, vt)

        def b_pv(t0, p):
            wa, wb = wins(p)
            pts, rinv, vt = st.pop(('b', p))
            inj = due(soft, 3, t0) if PVI else {}
            vt = pltpu.bitcast(cat([g | inj[j][:, 0:2 * G] if j in inj else g for j, g in enumerate(rows8(vt))]), BF16)
            outs = []
            for tile in range(2):
                ra, rb = rinv[tile], rinv[2 + tile]
                for hh in range(2):
                    h = 2 * tile + hh
                    ma, mb = (lo_ok, hi_ok) if hh == 0 else (hi_ok, lo_ok)
                    stn = cat([jnp.where(ma, e, 0.0) for e in pts[tile]]
                              + [jnp.where(mb, e, 0.0) for e in pts[2 + tile]]).astype(BF16)
                    ot = jnp.dot(vt[dh * h:dh * (h + 1), :], stn, preferred_element_type=F32)
                    rr_ = jnp.where(first_half, ra, rb) if hh == 0 else jnp.where(first_half, rb, ra)
                    outs.append(ot * rr_)
            tw = pltpu.bitcast(cat(outs).astype(BF16), U32).T
            for r in range(WS):
                ga = tw[8 * r:8 * r + 8, :]
                gb = tw[G + 8 * r:G + 8 * r + 8, :]
                o_s[r, pl.ds(WS * wa, WS), 0:CW] = jnp.where(even_head, ga, gb)[0:WS]
                if wb != wa:
                    o_s[r, pl.ds(WS * wb, WS), 0:CW] = jnp.where(even_head, gb, ga)[0:WS]
            toks.append((t0 + DL_PV, o_s[zx, 0:8, :]))

        def c_dot(t0, h, r):
            ow = o_s[r, HW * h:HW * (h + 1), :]
            rhs = cat([f(ow << 16), f(ow & hi)], axis=1)
            res = lax.dot_general(lhs(wo_s, due(toks, DC // 8, t0, 8), due(soft, DC // 8, t0, 8), F32), rhs,
                                  (((1,), (1,)), ((), ())), preferred_element_type=F32)
            st['c', h, r] = res
            ticks.extend((t0 + 130 + 8 * j, pltpu.bitcast(res[8 * j:8 * j + 8, 0:LANES], U32)) for j in range(DC // 8))

        def c_load(h, r, q):
            n = C // CP
            st['cx', h, r, q] = x_prev[r, n * q:n * (q + 1), HW * h:HW * (h + 1)]

        def c_out(h, r, q):
            n = C // CP
            rs = slice(n * q, n * (q + 1))
            o_ref[r, rs, HW * h:HW * (h + 1)] = (st.pop(('cx', h, r, q)) + st['c', h, r][rs]).astype(o_ref.dtype)

        NR = WS + 2
        stg = (sa_s, sb_s)

        def stage_row(d, c, rho):
            cs = slice(16 * c, 16 * c + 16)
            if rho == 0:
                u = pltpu.bitcast(xt_ref[0, cs, :], U32)
            elif rho == WS + 1:
                u = jnp.where(bot_ok, pltpu.bitcast(xb_ref[0, cs, :], U32), zero)
            else:
                u = pltpu.bitcast(xn_ref[rho - 1, cs, :], U32)
            for t, vs in enumerate(shifted(u)):
                for j, v in enumerate(vs):
                    stg[c % 2][rho, 8 * j:8 * j + 8, LANES * t:LANES * (t + 1)] = v
            if STOK:
                soft.append((d, stg[c % 2][zx + NR, 8:16, 0:LANES]))

        def conv_step(d, c, hf, t, r):
            if r == 0:
                if t == 0:
                    stg[c % 2][zx + NR, 0:8, 0:LANES] = zvec
                st['un'] = {}
            un = st['un']
            for rho in range(r, r + 3):
                if rho not in un:
                    un[rho] = [v[8 * hf:8 * hf + 8] for v in unpack(
                        [stg[c % 2][rho, 8 * j:8 * j + 8, LANES * t:LANES * (t + 1)] for j in range(3)])]
            tok = pltpu.bitcast(conv_row(un, t, r, slice(16 * c + 8 * hf, 16 * c + 8 * hf + 8), x_next), U32)
            soft.append((d, tok))

        npair = (NWIN + 1) // 2
        n0 = (HW - 1) // WS // 2
        plan, total = _plan(npair, n0, NT)
        ev = []

        starts = [t for t, _, _ in plan]

        def at(t, fn, *a):
            ev.append((t, t, len(ev), fn, a))

        def before(d, fn, *a):
            e = max([t for t in starts if t <= d], default=0) - 1
            ev.append((e, d, len(ev), fn, a))
            return e

        load = [0.0] * (total + 1000)
        tqk = {}

        def add(t0, t1, n):
            for t in range(max(t0, 0), max(t1, 0)):
                load[t] += n / (t1 - t0)

        for t, kind, idx in plan:
            if kind == 'a':
                before(t - LN1, ln1, t - LN1, *idx)
                for k in range(LNS):
                    d = t - LN2 - LND * (LNS - 1 - k)
                    before(d, ln2, d, *idx, k)
                    add(d - 16, d, 72 // LNS)
                before(t - 40, ln3, *idx)
                at(t, a_dot, t, *idx)
                add(t + 130, t + 130 + DA, 12 * DA // 16)
                add(t - LN1 - 16, t - LN1, 32); add(t - LN2, t - 40, 20); add(t - 40, t, 60 if LN3 else 36)
            elif kind == 'qk':
                at(t, b_qk, t, idx)
                tqk[idx] = t
                add(t - 64, t, 28); add(t, t + 56, 28); add(t + 130, t + 186, 24); add(t + 186, t + 202, 36)
            elif kind == 'pv':
                tg = max(tqk[idx] + SM0, t - SMB)
                at(t - 1, b_sm, tg, t - VG, idx)
                at(t, b_pv, t, idx)
                add(tg, tg + 4 * SMD + 16, 80); add(t + 120, t + 136, 46); add(t + 130, t + 178, 36)
                add(t + 400, t + 460, 14)
            else:
                at(t, c_dot, t, *idx)
                add(t + 130, t + 130 + DC, 20 * DC // 16)
                add(t - 70, t, 64)
                for q in range(CP):
                    e = before(t + 130 + (C // CP) * q + COFF, c_load, *idx, q)
                    at(max(e, t) + 2, c_out, *idx, q)
        nc = C // 16
        nstep = nc * 2 * NT * WS
        sm = [sum(load[max(t - SMO, 0):t + SMO]) / (2 * SMO) for t in range(total)]
        free = [max(0.0, CAP / 16 - sm[t]) if t >= CV0 - 40 else 0.0 for t in range(total)]
        tot_free, acc, tstep = sum(free), 0.0, []
        for t in range(total):
            acc += free[t]
            while len(tstep) < nstep and acc >= (len(tstep) + 1) * tot_free / nstep - 1e-6:
                tstep.append(t)
        for n in range(nstep):
            before(tstep[n], conv_step, tstep[n], n // (2 * NT * WS), n // (NT * WS) % 2, n // WS % NT, n % WS)
        for c in range(nc):
            t1 = tstep[c * 2 * NT * WS] - 30
            t0 = tstep[(c - 1) * 2 * NT * WS] + 120 if c else 130
            for rho in range(NR):
                d = t0 + (t1 - t0) * rho // (NR - 1)
                before(d, stage_row, d, c, rho)
        ev.sort(key=lambda e: e[:3])
        ev = [e[1:] for e in ev]
        a_done, pv_done = set(), set()
        for _, _, fn, a in ev:
            if fn is a_dot:
                a_done.add(a[1:])
            elif fn is b_qk:
                tl = range(2 * WS * a[1] // LANES, min(2 * WS * a[1] + 2 * WS, WP - 1) // LANES + 1)
                need = [(t, r) in a_done for t in tl for r in range(WS)]
                assert all(need) if a[1] < n0 else not any(need)
            elif fn is b_pv:
                pv_done.add(a[1])
            elif fn is c_dot:
                ps = range(0, n0 + 1) if a[1] == 0 else range(n0, npair)
                assert all((p in pv_done) == (p >= n0) for p in ps)
        for _, _, fn, a in ev:
            fn(*a)

    bufs = (xa_s, xb_s, xc_s)
    if ONE:
        @pl.when(i == 1000)
        def _():
            lax.fori_loop(0, WS, lambda r, c: o_ref.__setitem__(r, xb_s[r].astype(o_ref.dtype)) or c, 0)
    for k in range(1 if ONE else 3):
        pl.when(i % 3 == k)(functools.partial(step, bufs[k], bufs[(k + 1) % 3], bufs[(k + 2) % 3]))


@jax.jit
def pallas_standalone__window_attn_davit__vision_kernel(
    x: jax.Array,
    dw_pe: jax.Array,
    w_qkv: jax.Array,
    w_o: jax.Array,
):
    B, H, W, C = x.shape
    assert B == 1 and H % WS == 0 and W % WS == 0 and C % (16 * NH) == 0
    WP = -(-(W + 1) // (2 * LANES)) * (2 * LANES)
    assert WP == 4 * LANES
    NWIN = W // WS
    NBLK = H // WS
    CW = C // 2

    xt = jnp.transpose(x[0], (0, 2, 1))
    dwb = jnp.broadcast_to(dw_pe.reshape(9, C, 1), (9, C, LANES))

    def inter(w):
        return jnp.transpose(w.reshape(C, 2, CW), (2, 1, 0)).reshape(C, C)

    wqkv_t = jnp.concatenate(
        [inter(w_qkv[:, 0:C]), inter(w_qkv[:, C:2 * C]), w_qkv[:, 2 * C:].T], axis=0)
    wo_t = jnp.pad(jnp.transpose(w_o.reshape(CW, 2, C), (2, 1, 0)), ((0, 0), (0, 0), (0, LANES - CW)))
    wo_t = wo_t.reshape(C, 2 * LANES)

    def nxt(i):
        return jnp.minimum(i + 1, NBLK - 1)

    kern = functools.partial(_kernel, C=C, W=W, WP=WP, NWIN=NWIN, NBLK=NBLK)
    out = pl.pallas_call(
        kern,
        grid=(NBLK + 1,),
        in_specs=[
            pl.BlockSpec((WS, C, WP), lambda i: (nxt(i), 0, 0)),
            pl.BlockSpec((1, C, WP), lambda i: (WS * nxt(i) - 1, 0, 0)),
            pl.BlockSpec((1, C, WP), lambda i: (jnp.minimum(WS * nxt(i) + WS, H - 1), 0, 0)),
            pl.BlockSpec((WS + 1, C, WP), lambda i: (0, 0, 0)),
            pl.BlockSpec((9, C, LANES), lambda i: (0, 0, 0)),
            pl.BlockSpec((3 * C, C), lambda i: (0, 0)),
            pl.BlockSpec((C, 2 * LANES), lambda i: (0, 0)),
        ],
        out_specs=pl.BlockSpec((WS, C, WP), lambda i: (jnp.maximum(i - 1, 0), 0, 0)),
        out_shape=jax.ShapeDtypeStruct((H, C, W), x.dtype),
        scratch_shapes=[
            pltpu.VMEM((WS + 1, C, WP), F32),
            pltpu.VMEM((WS + 1, C, WP), F32),
            pltpu.VMEM((WS + 1, C, WP), F32),
            pltpu.VMEM((WS, WP, LANES), U32),
            pltpu.VMEM((WS, WP, LANES), U32),
            pltpu.VMEM((WS, WP, LANES), U32),
            pltpu.VMEM((WS, WP, LANES), U32),
            pltpu.VMEM((2, 3 * C // 4, C), U32),
            pltpu.VMEM((C, 2 * LANES), U32),
            pltpu.VMEM((WS + 3, 3 * 8, WP), U32),
            pltpu.VMEM((WS + 3, 3 * 8, WP), U32),
            pltpu.VMEM((10, C, LANES), F32),
        ],
        compiler_params=pltpu.CompilerParams(
            dimension_semantics=("arbitrary",),
            vmem_limit_bytes=64 * 1024 * 1024,
        ),
        name="davit_window_attn",
    )(xt, xt, xt, xt, dwb, wqkv_t, wo_t)
    return jnp.transpose(out, (0, 2, 1))[None]
```

```python
import functools
import math
import os

import jax
import jax.numpy as jnp
from jax import lax
import jax.experimental.pallas as pl
import jax.experimental.pallas.tpu as pltpu

WS = 7
NH = 4
EPS = 1e-05
LANES = 128
F32 = jnp.float32
BF16 = jnp.bfloat16
U32 = jnp.uint32

P = lambda k, d: int(os.environ.get(k, d))
DL_A = P('DL_A', 480)
LAT_QK = P('LAT_QK', 300)
DL_PV = P('DL_PV', 580)
PRE_C = P('PRE_C', 120)
TAIL = P('TAIL', 1400)
LN1 = P('LN1', 170)
LN2 = P('LN2', 110)
LNS = P('LNS', 2)
LND = P('LND', 16)
SM0 = P('SM0', 200)
SMD = P('SMD', 16)
SMB = P('SMB', 130)
CV0 = P('CV0', 450)
CVI = P('CVI', 170)
CVE = P('CVE', 60)
CVX = P('CVX', 200)
ORD = P('ORD', 0)
CAP = P('CAP', 42)
SMO = P('SMO', 32)
ONLY = P('ONLY', 0)
NOBC = P('NOBC', 1)
DA, DC, DQ, DP = 288, 192, 56, 48
MXU_LAT = 130
NSUB = 3


def _iota(shape, dim):
    return lax.broadcasted_iota(jnp.int32, shape, dim)


def _plan(npair, n0, nt, cur, prev):
    a_q = [(t, r) for t in range(nt) for r in range(WS)] if cur else []
    c_q = [(h, r) for h in range(2) for r in range(WS)] if prev else []
    n1 = npair - n0 if prev else 0
    pairs = list(range(n0, n0 + n1)) + (list(range(n0)) if cur else [])
    total = len(a_q) * DA + len(c_q) * DC + len(pairs) * (DQ + DP)
    q0 = 0 if prev else total // 3
    t = 0
    ia = ic = iq = ip = 0
    out = []
    tq, tp, ta = {}, {}, {}
    last = None
    while ia < len(a_q) or ic < len(c_q) or ip < len(pairs):
        cands = []
        if ip < iq and t >= tq[ip] + LAT_QK:
            cands.append((-1e6, 'pv'))
        if iq < len(pairs) and (not cur or (iq - ip < 2 and last != 'qk' and not (ORD and last == 'pv'))):
            ok = iq - ip < 4
            if iq >= n1:
                need = (2 * WS * pairs[iq] + 2 * WS) // LANES * WS + WS - 1
                ok = ia > need and t >= ta[need] + DA + DL_A + 60 and ic >= len(c_q) // 2
            if ok:
                pr = q0 + iq * (total - q0 - TAIL) / len(pairs) - t - 200
                cands.append((-2e6 if ORD and pr <= 0 else pr, 'qk'))
        if ia < len(a_q):
            cands.append((ia * (total - 700) / len(a_q) - t, 'a'))
        if ic < len(c_q):
            need = 0 if ic < WS else n1 - 1
            if ip > need and t >= tp[need] + DL_PV + PRE_C:
                if cur:
                    tc = 1000 + ic * 900 if ic < WS else total - DC - (2 * WS - 1 - ic) * 950
                else:
                    tc = 1500 + ic * 400
                cands.append((tc - t, 'c'))
        if not cands:
            t += 8
            last = None
            continue
        kind = min(cands)[1]
        last = kind
        if kind == 'pv':
            tp[ip] = t; out.append((t, 'pv', pairs[ip])); ip += 1; t += DP
        elif kind == 'qk':
            tq[iq] = t; out.append((t, 'qk', pairs[iq])); iq += 1; t += DQ
        elif kind == 'a':
            ta[ia] = t; out.append((t, 'a', a_q[ia])); ia += 1; t += DA
        else:
            out.append((t, 'c', c_q[ic])); ic += 1; t += DC
    return out, t


def _tree_sum(xs):
    while len(xs) > 1:
        xs = [xs[j] + xs[j + 1] if j + 1 < len(xs) else xs[j] for j in range(0, len(xs), 2)]
    return xs[0]


def _rows8(x):
    return [x[8 * j:8 * j + 8] for j in range(x.shape[0] // 8)]


def _cat(xs, axis=0):
    return jnp.concatenate(xs, axis=axis) if len(xs) > 1 else xs[0]


def _f32(u):
    return pltpu.bitcast(u, F32)


def _u32(x):
    return pltpu.bitcast(x, U32)


def _kernel(x0_ref, x1_ref, x2_ref, x3_ref, dw_ref, wqkv_ref, wo_ref, o_ref,
            xa_s, xb_s, xc_s, q_s, k_s, v_s, o_s, wq_s, wo_s, sa_s, sb_s, dw_s, *, C, W, WP, NWIN, NBLK):
    g = pl.program_id(0)
    ng = pl.num_programs(0)
    dh = C // NH
    CW = C // 2
    NT = WP // LANES
    G = WS * 8
    HW = WP // 2
    NC = C // 16
    NR = WS + 2
    lane8 = _iota((8, LANES), 1)
    last_valid = W - (NT - 1) * LANES
    zero = jnp.uint32(0)
    hi = jnp.uint32(0xFFFF0000)
    qkv_s = (q_s, k_s, v_s)
    xbuf = (xa_s, xb_s, xc_s)
    xin = (x0_ref, x1_ref, x2_ref, x3_ref)
    stg = (sa_s, sb_s)
    SPARE = sa_s.shape[0] - 1
    zx = g >> 10
    zvec = jnp.full((8, LANES), zx, jnp.int32).astype(U32)

    def stg_row(j, c2, rho):
        if 2 <= rho < WS:
            return rho - 2
        slot = j % NSUB if rho >= WS else (j - 1) % NSUB
        return WS - 2 + (slot * (NC // 2) + c2) * 2 + rho % WS

    def shifted(u):
        tiles = [u[:, LANES * t:LANES * (t + 1)] for t in range(NT)]
        tiles[NT - 1] = jnp.where(lane8 < last_valid, tiles[NT - 1], zero)
        row = []
        for t in range(NT):
            left = jnp.where(lane8 == LANES - 1, tiles[t - 1] if t > 0 else zero, tiles[t])
            right = jnp.where(lane8 == 0, tiles[t + 1], tiles[t]) if t < NT - 1 else tiles[t]
            row.append((pltpu.roll(left, 1, 1), tiles[t], pltpu.roll(right, LANES - 1, 1)))
        return row

    def put_row(ref, idx, row):
        for t, vs in enumerate(row):
            for j, v in enumerate(vs):
                ref[idx, 8 * j:8 * j + 8, LANES * t:LANES * (t + 1)] = v

    def unpack(vs):
        return [pltpu.bitcast(v, BF16).astype(F32) for v in vs]

    def conv_row(un, t, r, cs, buf):
        w = [dw_s[tap, cs, :] for tap in range(9)]
        terms = [un[r + ki][kj] * w[3 * ki + kj]
                 for ki in range(3) for kj in range(3) if un[r + ki] is not None]
        acc = _tree_sum(terms)
        buf[r, cs, LANES * t:LANES * (t + 1)] = acc
        return acc

    def setup():
        qscale = (dh ** -0.5) * math.log2(math.e)
        wt = wqkv_ref[...].astype(F32).T
        wq = (wt[0:C] * qscale).astype(BF16).astype(F32)
        words = [(_u32(w[0:CW]) >> 16) | (_u32(w[CW:C]) & hi) for w in (wq, wt[C:2 * C])]
        words = _rows8(_cat(words + [_u32(wt[2 * C:].astype(BF16))]))
        for par in range(2):
            wq_s[par] = _cat(words[par::2])
        wo = _u32(wo_ref[...])
        wo_s[...] = jnp.zeros(wo_s.shape, U32)
        wo_s[:, 0:CW] = (wo << 16).T
        wo_s[:, LANES:LANES + CW] = (wo & hi).T

        def zrow(r, carry):
            rs = pl.ds(pl.multiple_of(r % 4 * LANES, LANES), LANES)
            for ref in (q_s, k_s, v_s, o_s):
                ref[r // 4, rs, :] = jnp.zeros((LANES, LANES), U32)
            return carry
        lax.fori_loop(0, WS * NT, zrow, 0)
        for ref in stg:
            ref[SPARE] = jnp.zeros(ref.shape[1:], U32)

        def taps(ki, carry):
            w3 = dw_ref[ki].astype(F32)
            for kj in range(3):
                w = w3[kj:kj + 1]
                if kj == 1:
                    w = w + jnp.where(ki == 1, 1.0, 0.0)
                dw_s[3 * ki + kj] = jnp.broadcast_to(w, (LANES, C)).T
            return carry
        lax.fori_loop(0, 3, taps, 0)

        def conv0(c2, carry):
            for par in range(2):
                cs = pl.ds(pl.multiple_of(32 * c2 + 16 * par, 16), 16)
                sh = [shifted(_u32(x1_ref[r, cs, :])) for r in range(WS)] + [shifted(_u32(x2_ref[0, cs, :]))]
                for rho in (WS, WS + 1):
                    put_row(stg[par], stg_row(-1, c2, rho), sh[rho - 1])
                for t in range(NT):
                    un = [None] + [unpack(row[t]) for row in sh]
                    for r in range(WS):
                        conv_row(un, t, r, cs, xbuf[0])
            return carry
        lax.fori_loop(0, NC // 2, conv0, 0)

    def body(subs):
        head_a = lane8 < dh
        head_b = (lane8 >= dh) & (lane8 < 2 * dh)
        junk8 = _iota((8, 2 * G), 0) == WS
        lo_ok = (_iota((8, 2 * G), 1) < G) & ~junk8
        hi_ok = (_iota((8, 2 * G), 1) >= G) & ~junk8
        first_half = _iota((1, 2 * G), 1) < G
        even_head = (_iota((8, CW), 1) // (dh // 2)) % 2 == 0
        npair = (NWIN + 1) // 2
        n0 = (HW - 1) // WS // 2

        st = {}
        toks = []
        soft = []
        ticks = []
        j0 = subs[0][0]
        tag = {('qkv', t, r): -1 for t in range(NT) for r in range(WS)}
        tag.update({('o', p): (-1 if p < n0 else -2) for p in range(npair)})
        for b, blk in ((j0 % 3, 0), ((j0 + 2) % 3, -1)):
            tag.update({('x', b, c, t, r): blk for c in range(2 * NC) for t in range(NT) for r in range(WS)})
        tag.update({('s', c % 2, stg_row(j0, c // 2, rho)): (0, c, rho) for c in range(NC) for rho in (0, 1)})

        def gather(ref, w):
            return [ref[r, pl.ds(WS * w, 8), :] for r in range(WS)]

        def tick(t):
            c = [x for x in ticks if t <= x[0] <= t + 40]
            if not c:
                return None
            _, res, j = min(c, key=lambda x: x[0])
            return _u32(res[8 * j:8 * j + 8, 0:LANES]) & zvec

        def due(lst, nblk, t0, step):
            inj = {}
            for d, tok in list(lst):
                j = max(0, -(-(d - t0) // step))
                if j < nblk:
                    inj[j] = tok if j not in inj else inj[j] | tok
            lst[:] = [x for x in lst if x[0] > t0 + (nblk - 1) * step]
            return {j: v & zvec for j, v in inj.items()}

        def lhs(ref, inj, inj1, dt):
            nblk = ref.shape[0] // 8
            parts, s = [], 0
            for j in sorted(set(inj) | set(inj1)):
                if j > s:
                    parts.append(ref[8 * s:8 * j, :])
                k0, k1 = ref[8 * j:8 * j + 8, 0:LANES], ref[8 * j:8 * j + 8, LANES:]
                if j in inj:
                    k0 = k0 | inj[j]
                    k1 = k1 | inj[j][:, 0:k1.shape[1]]
                if j in inj1:
                    k0 = k0 | inj1[j]
                parts.append(_cat([k0, k1], axis=1))
                s = j + 1
            if s < nblk:
                parts.append(ref[8 * s:8 * nblk, :])
            return pltpu.bitcast(_cat(parts), dt)

        def fence(d, b):
            _, res, j = max([x for x in ticks if x[0] <= d], key=lambda x: x[0])
            xbuf[b][zx + WS, 0:8, 0:LANES] = res[8 * j:8 * j + 8, 0:LANES]

        def ln1(d, k, t, r):
            b = subs[k][0] % 3
            assert all(tag['x', b, c, t, r] == k for c in range(2 * NC))
            x0 = xbuf[b][r, :, LANES * t:LANES * (t + 1)]
            s8 = _tree_sum(_rows8(x0))
            soft.append((d, _u32(s8)))
            xc = x0 - jnp.sum(s8, axis=0, keepdims=True) * (1.0 / C)
            st['ln', k, t, r] = (xc, [])

        def ln2(d, n, *key):
            m = C // LNS
            xc = st[('ln',) + key][0][m * n:m * (n + 1)]
            s8 = _tree_sum(_rows8(xc * xc))
            soft.append((d, _u32(s8)))
            st[('ln',) + key][1].append(s8)

        def a_dot(t0, k, t, r):
            xc, sq = st.pop(('ln', k, t, r))
            var = jnp.sum(_tree_sum(sq), axis=0, keepdims=True) * (1.0 / C)
            h = (xc * lax.rsqrt(var + EPS)).astype(BF16)
            inj = due(toks, DA // 16, t0, 16)
            res = [jnp.dot(lhs(wq_s.at[0], inj, due(soft, DA // 16, t0, 16), BF16), h, preferred_element_type=F32),
                   jnp.dot(lhs(wq_s.at[1], inj, {}, BF16), h, preferred_element_type=F32)]
            ticks.extend((t0 + MXU_LAT + 8 * j, res[0], j) for j in range(DA // 8))
            for m in range(3):
                blk = _cat([res[j % 2][16 * (j // 2):16 * (j // 2) + 16, :] for j in range(NC * m, NC * (m + 1))])
                qkv_s[m][r, LANES * t:LANES * (t + 1), 0:CW] = _u32(blk.astype(BF16)).T
                toks.append((t0 + 96 * (m + 1) + DL_A, qkv_s[m][zx, 0:8, :]))
            tag['qkv', t, r] = k

        def wins(p):
            return 2 * p, min(2 * p + 1, NWIN - 1)

        def b_qk(t0, k, p):
            wa, wb = wins(p)
            blk = k if p < n0 else k - 1
            assert all(tag['qkv', t, r] == blk for r in range(WS)
                       for t in range(WS * wa // LANES, (WS * wb + WS) // LANES + 1))
            sts = []
            inj = due(soft, WS, t0, 8)
            for w, swap in ((wa, False), (wb, True)):
                qw = gather(q_s, w)
                kw = gather(k_s, w)
                if not swap:
                    kw = [v | inj[r] if r in inj else v for r, v in enumerate(kw)]
                kw = _cat(kw)
                for tile in range(2):
                    if tile == 0:
                        kk = _f32(kw << 16)
                        qq = [_f32(v << 16) for v in qw]
                    else:
                        kk = _f32(kw & hi)
                        qq = [_f32(v & hi) for v in qw]
                    qa = [jnp.where(head_a, v, 0.0) for v in qq]
                    qb = [jnp.where(head_b, v, 0.0) for v in qq]
                    qst = _cat(qb + qa if swap else qa + qb)
                    sts.append(lax.dot_general(kk, qst, (((1,), (1,)), ((), ())),
                                               preferred_element_type=F32))
            vt = pltpu.bitcast(_cat(gather(v_s, wa) + gather(v_s, wb))[:, 0:CW].T, BF16)
            st['s', p] = (sts, vt)

        def b_pv(t0, tg, k, p):
            wa, wb = wins(p)
            sts, vt = st.pop(('s', p))
            pts = []
            rinv = []
            for n, s_t in enumerate(sts):
                sg = _rows8(s_t)
                m8 = functools.reduce(jnp.maximum, sg)
                mx = jnp.max(jnp.where(junk8, -jnp.inf, m8), axis=0, keepdims=True)
                mv = jnp.where(junk8, m8, mx)
                z = tick(tg + SMD * (3 - n))
                if z is not None:
                    mv = _f32(_u32(mv) | z[:, 0:2 * G])
                eg = [jnp.exp2(s - mv) for s in sg]
                den = jnp.sum(jnp.where(junk8, 0.0, _tree_sum(eg)), axis=0, keepdims=True)
                r0 = pl.reciprocal(den, approx=True)
                rinv.append(r0 * (2.0 - den * r0))
                pts.append(eg)
            outs = []
            for tile in range(2):
                ra, rb = rinv[tile], rinv[2 + tile]
                for hh in range(2):
                    h = 2 * tile + hh
                    ma, mb = (lo_ok, hi_ok) if hh == 0 else (hi_ok, lo_ok)
                    stn = _cat([jnp.where(ma, e, 0.0) for e in pts[tile]]
                               + [jnp.where(mb, e, 0.0) for e in pts[2 + tile]]).astype(BF16)
                    ot = jnp.dot(vt[dh * h:dh * (h + 1), :], stn, preferred_element_type=F32)
                    rr = jnp.where(first_half, ra, rb) if hh == 0 else jnp.where(first_half, rb, ra)
                    outs.append(ot * rr)
            tw = _u32(_cat(outs).astype(BF16)).T
            for r in range(WS):
                ga = tw[8 * r:8 * r + 8, :]
                gb = tw[G + 8 * r:G + 8 * r + 8, :]
                o_s[r, pl.ds(WS * wa, WS), 0:CW] = jnp.where(even_head, ga, gb)[0:WS]
                if wb != wa:
                    o_s[r, pl.ds(WS * wb, WS), 0:CW] = jnp.where(even_head, gb, ga)[0:WS]
            toks.append((t0 + DL_PV, o_s[zx, 0:8, :]))
            tag['o', p] = k if p < n0 else k - 1

        def c_dot(t0, k, h, r):
            b = (subs[k][0] + 2) % 3
            assert all(tag['o', p] == k - 1 for p in (range(n0 + 1) if h == 0 else range(n0, npair)))
            assert all(tag['x', b, c, t, r] == k - 1 for c in range(2 * NC) for t in (2 * h, 2 * h + 1))
            ls = slice(HW * h, HW * (h + 1))
            ow = o_s[r, ls, :]
            rhs = _cat([_f32(ow << 16), _f32(ow & hi)], axis=1)
            res = lax.dot_general(lhs(wo_s, due(toks, DC // 8, t0, 8), due(soft, DC // 8, t0, 8), F32), rhs,
                                  (((1,), (1,)), ((), ())), preferred_element_type=F32)
            ticks.extend((t0 + MXU_LAT + 8 * j, res, j) for j in range(DC // 8))
            o_ref[subs[k][2] + r, :, ls] = (xbuf[b][r, :, ls] + res).astype(o_ref.dtype)

        def stage_row(d, k, c, rho):
            j, slot = subs[k][0:2]
            cs = slice(16 * c, 16 * c + 16)
            if rho == WS + 1:
                u = _u32(xin[slot + 1][0, cs, :])
                if slot == 1:
                    u = jnp.where(g < ng - 2, u, zero)
            else:
                u = _u32(xin[slot][rho - 1, cs, :])
            idx = stg_row(j, c // 2, rho)
            put_row(stg[c % 2], idx, shifted(u))
            soft.append((d, stg[c % 2][zx + SPARE, 8:16, 0:LANES]))
            tag['s', c % 2, idx] = (k, c, rho)

        def conv_step(d, k, c, hf, t, r):
            j = subs[k][0]
            if r == 0:
                if t == 0:
                    stg[c % 2][zx + SPARE, 0:8, 0:LANES] = zvec
                st['un'] = {}
            un = st['un']
            for rho in range(r, r + 3):
                if rho not in un:
                    idx = stg_row(j, c // 2, rho)
                    assert tag['s', c % 2, idx] in ((k, c, rho), (k - 1, c, rho + WS))
                    un[rho] = [v[8 * hf:8 * hf + 8] for v in unpack(
                        [stg[c % 2][idx, 8 * m:8 * m + 8, LANES * t:LANES * (t + 1)] for m in range(3)])]
            cs = slice(16 * c + 8 * hf, 16 * c + 8 * hf + 8)
            soft.append((d, _u32(conv_row(un, t, r, cs, xbuf[(j + 1) % 3]))))
            tag['x', (j + 1) % 3, 2 * c + hf, t, r] = k + 1

        plan, offs = [], [0]
        for k, sub in enumerate(subs):
            pk, tk = _plan(npair, n0, NT, sub[3], sub[4])
            plan += [(offs[k] + t, kind, k, idx) for t, kind, idx in pk]
            offs.append(offs[k] + tk)
        total = offs[-1]
        starts = [e[0] for e in plan]
        ev = []

        def at(t, fn, *a):
            ev.append((t, t, len(ev), fn, a))

        def before(d, fn, *a):
            ev.append((max([t for t in starts if t <= d], default=0) - 1, d, len(ev), fn, a))

        load = [0.0] * (total + 1000)
        tqk = {}

        def add(t0, t1, n):
            for t in range(max(t0, 0), max(t1, 0)):
                load[t] += n / (t1 - t0)

        for t, kind, k, idx in plan:
            tr = t + MXU_LAT
            if kind == 'a':
                if idx == (0, 0) and k > 0:
                    before(t - LN1 - 1, fence, t - LN1 - 40, subs[k][0] % 3)
                before(t - LN1, ln1, t - LN1, k, *idx)
                for n in range(LNS):
                    d = t - LN2 - LND * (LNS - 1 - n)
                    before(d, ln2, d, n, k, *idx)
                    add(d - 16, d, 72 // LNS)
                at(t, a_dot, t, k, *idx)
                add(tr, tr + DA, 12 * DA // 16)
                add(t - LN1 - 16, t - LN1, 32); add(t - LN2, t - 40, 20); add(t - 40, t, 36)
            elif kind == 'qk':
                at(t, b_qk, t, k, idx)
                tqk[idx] = t
                add(t - 64, t, 28); add(t, t + DQ, 28); add(tr, tr + DQ, 24); add(tr + DQ, tr + DQ + 16, 36)
            elif kind == 'pv':
                tg = max(tqk[idx] + SM0, t - SMB)
                at(t, b_pv, t, tg, k, idx)
                add(tg, tg + 4 * SMD + 16, 80); add(tr - 10, tr + 6, 46); add(tr, tr + DP, 36)
                add(t + 400, t + 460, 14)
            else:
                if idx == (0, 0) and k > 0:
                    at(t - 1, fence, t - 100, (subs[k][0] + 2) % 3)
                at(t, c_dot, t, k, *idx)
                add(tr, tr + DC, 20 * DC // 16)
                add(t - 70, t, 64)
        pre = [0.0]
        for v in load:
            pre.append(pre[-1] + v)
        nstep = NC * 2 * NT * WS
        prev_chunk = 10
        for k, sub in enumerate(subs):
            if not sub[3]:
                continue
            ta = offs[k] + (CVI if k else CV0) - 20
            tb = offs[k + 1] - (CVE if k == len(subs) - 1 else CVX)
            cap = CAP if sub[4] else 64
            free = [max(0.02, cap / 16 - (pre[t + SMO] - pre[max(t - SMO, 0)]) / (2 * SMO)) for t in range(ta, tb)]
            tot_free, acc, tstep = sum(free), 0.0, []
            for t, v in enumerate(free):
                acc += v
                while len(tstep) < nstep and acc >= (len(tstep) + 1) * tot_free / nstep - 1e-6:
                    tstep.append(ta + t)
            for n in range(nstep):
                before(tstep[n], conv_step, tstep[n], k, n // (2 * NT * WS), n // (NT * WS) % 2, n // WS % NT, n % WS)
            for c in range(NC):
                t1 = tstep[c * 2 * NT * WS] - 30
                t0 = prev_chunk + 120
                prev_chunk = t1 + 30
                for rho in range(2, NR):
                    d = t0 + (t1 - t0) * (rho - 2) // (NR - 3)
                    before(d, stage_row, d, k, c, rho)
        ev.sort(key=lambda e: e[:3])
        for e in ev:
            e[3](*e[4])
        if subs[-1][3]:
            n = len(subs)
            assert all(tag['qkv', t, r] == n - 1 for t in range(NT) for r in range(WS))
            assert all(tag['o', p] == n - 1 for p in range(n0))

    if ONLY in (0, 1):
        @pl.when(g == 0)
        def _():
            setup()
            body([(0, 2, 0, True, False)])

    if ONLY in (0, 2):
        @pl.when((g > 0) & (g < ng - 1))
        def _():
            body([(1 + k, k, WS * k, True, True) for k in range(NSUB)])

    if ONLY in (0, 3):
        @pl.when(g == ng - 1)
        def _():
            body([(1, 0, 0, False, True)])


@jax.jit
def pallas_standalone__window_attn_davit__vision_kernel(
    x: jax.Array,
    dw_pe: jax.Array,
    w_qkv: jax.Array,
    w_o: jax.Array,
):
    B, H, W, C = x.shape
    assert B == 1 and H % WS == 0 and W % WS == 0 and C % (16 * NH) == 0
    WP = -(-(W + 1) // (2 * LANES)) * (2 * LANES)
    assert WP == 4 * LANES
    NWIN = W // WS
    NBLK = H // WS
    assert (NBLK - 1) % NSUB == 0
    NM = (NBLK - 1) // NSUB

    xt = jnp.transpose(x[0], (0, 2, 1))

    def blk(k):
        return lambda g: (jnp.clip(NSUB * g - 1 + k, 0, NBLK - 1), 0, 0)

    nstg = WS - 2 + NSUB * (C // 32) * 2 + 1
    kern = functools.partial(_kernel, C=C, W=W, WP=WP, NWIN=NWIN, NBLK=NBLK)
    out = pl.pallas_call(
        kern,
        grid=(NM + 2,),
        in_specs=[
            pl.BlockSpec((WS, C, WP), blk(0)),
            pl.BlockSpec((WS, C, WP), blk(1)),
            pl.BlockSpec((WS, C, WP), blk(2)),
            pl.BlockSpec((1, C, WP), lambda g: (jnp.minimum(WS * (NSUB * g + 2), H - 1), 0, 0)),
            pl.BlockSpec((3, 3, C), lambda g: (0, 0, 0)),
            pl.BlockSpec((C, 3 * C), lambda g: (0, 0)),
            pl.BlockSpec((C, C), lambda g: (0, 0)),
        ],
        out_specs=pl.BlockSpec((NSUB * WS, C, WP), lambda g: (jnp.maximum(g - 1, 0), 0, 0)),
        out_shape=jax.ShapeDtypeStruct((H, C, W), x.dtype),
        scratch_shapes=[
            pltpu.VMEM((WS + 1, C, WP), F32),
            pltpu.VMEM((WS + 1, C, WP), F32),
            pltpu.VMEM((WS + 1, C, WP), F32),
            pltpu.VMEM((WS, WP, LANES), U32),
            pltpu.VMEM((WS, WP, LANES), U32),
            pltpu.VMEM((WS, WP, LANES), U32),
            pltpu.VMEM((WS, WP, LANES), U32),
            pltpu.VMEM((2, 3 * C // 4, C), U32),
            pltpu.VMEM((C, 2 * LANES), U32),
            pltpu.VMEM((nstg, 3 * 8, WP), U32),
            pltpu.VMEM((nstg, 3 * 8, WP), U32),
            pltpu.VMEM((9, C, LANES), F32),
        ],
        compiler_params=pltpu.CompilerParams(
            dimension_semantics=("arbitrary",),
            vmem_limit_bytes=96 * 1024 * 1024,
            disable_bounds_checks=bool(NOBC),
        ),
        name="davit_window_attn",
    )(xt, xt, xt, xt, dw_pe, w_qkv, w_o)
    return jnp.transpose(out, (0, 2, 1))[None]
```

```python
import functools
import math
import os

import jax
import jax.numpy as jnp
from jax import lax
import jax.experimental.pallas as pl
import jax.experimental.pallas.tpu as pltpu

WS = 7
NH = 4
EPS = 1e-05
LANES = 128
F32 = jnp.float32
BF16 = jnp.bfloat16
U32 = jnp.uint32

P = lambda k, d: int(os.environ.get(k, d))
DL_A = P('DL_A', 480)
LAT_QK = P('LAT_QK', 300)
DL_PV = P('DL_PV', 580)
PRE_C = P('PRE_C', 120)
TAIL = P('TAIL', 1400)
LN1 = P('LN1', 200)
LN2 = P('LN2', 130)
LNS = P('LNS', 2)
LND = P('LND', 16)
SM0 = P('SM0', 200)
SMD = P('SMD', 16)
SMB = P('SMB', 130)
CV0 = P('CV0', 450)
CVI = P('CVI', 170)
CVE = P('CVE', 60)
CVX = P('CVX', 200)
ORD = P('ORD', 0)
CAP = P('CAP', 42)
SMO = P('SMO', 32)
ONLY = P('ONLY', 0)
PVP = P('PVP', 0)
LNF = P('LNF', 3)
LN3 = P('LN3', 50)
LNG = P('LNG', 0)
NOBC = P('NOBC', 1)
DA, DC, DQ, DP = 288, 192, 56, 48
MXU_LAT = 130
NSUB = 3


def _iota(shape, dim):
    return lax.broadcasted_iota(jnp.int32, shape, dim)


def _plan(npair, n0, nt, cur, prev):
    a_q = [(t, r) for t in range(nt) for r in range(WS)] if cur else []
    c_q = [(h, r) for h in range(2) for r in range(WS)] if prev else []
    n1 = npair - n0 if prev else 0
    pairs = list(range(n0, n0 + n1)) + (list(range(n0)) if cur else [])
    total = len(a_q) * DA + len(c_q) * DC + len(pairs) * (DQ + DP)
    q0 = 0 if prev else total // 3
    t = 0
    ia = ic = iq = ip = 0
    out = []
    tq, tp, ta = {}, {}, {}
    last = None
    while ia < len(a_q) or ic < len(c_q) or ip < len(pairs):
        cands = []
        if ip < iq and t >= tq[ip] + LAT_QK:
            cands.append((-1e6, 'pv'))
        if iq < len(pairs) and (not cur or (iq - ip < 2 and last != 'qk' and not (ORD and last == 'pv'))):
            ok = iq - ip < 4
            if iq >= n1:
                need = (2 * WS * pairs[iq] + 2 * WS) // LANES * WS + WS - 1
                ok = ia > need and t >= ta[need] + DA + DL_A + 60 and ic >= len(c_q) // 2
            if ok:
                pr = q0 + iq * (total - q0 - TAIL) / len(pairs) - t - 200
                cands.append((-2e6 if ORD and pr <= 0 else pr, 'qk'))
        if ia < len(a_q):
            cands.append((ia * (total - 700) / len(a_q) - t, 'a'))
        if ic < len(c_q):
            need = 0 if ic < WS else n1 - 1
            if ip > need and t >= tp[need] + DL_PV + PRE_C:
                if cur:
                    tc = 1000 + ic * 900 if ic < WS else total - DC - (2 * WS - 1 - ic) * 950
                else:
                    tc = 1500 + ic * 400
                cands.append((tc - t, 'c'))
        if not cands:
            t += 8
            last = None
            continue
        kind = min(cands)[1]
        last = kind
        if kind == 'pv':
            tp[ip] = t; out.append((t, 'pv', pairs[ip])); ip += 1; t += DP
        elif kind == 'qk':
            tq[iq] = t; out.append((t, 'qk', pairs[iq])); iq += 1; t += DQ
        elif kind == 'a':
            ta[ia] = t; out.append((t, 'a', a_q[ia])); ia += 1; t += DA
        else:
            out.append((t, 'c', c_q[ic])); ic += 1; t += DC
    return out, t


def _tree_sum(xs):
    while len(xs) > 1:
        xs = [xs[j] + xs[j + 1] if j + 1 < len(xs) else xs[j] for j in range(0, len(xs), 2)]
    return xs[0]


def _sum8(x):
    while x.shape[0] % 16 == 0:
        x = x[:x.shape[0] // 2] + x[x.shape[0] // 2:]
    return _tree_sum(_rows8(x))


def _fold7(op, x):
    t = op(x[0:24], x[24:48])
    return op(op(t[0:8], t[8:16]), op(t[16:24], x[48:56]))


def _all8(op, x):
    for sh in (4, 2, 1):
        x = op(x, pltpu.roll(x, sh, 0))
    return x


def _rows8(x):
    return [x[8 * j:8 * j + 8] for j in range(x.shape[0] // 8)]


def _cat(xs, axis=0):
    return jnp.concatenate(xs, axis=axis) if len(xs) > 1 else xs[0]


def _f32(u):
    return pltpu.bitcast(u, F32)


def _u32(x):
    return pltpu.bitcast(x, U32)


def _kernel(x0_ref, x1_ref, x2_ref, x3_ref, dw_ref, wqkv_ref, wo_ref, o_ref,
            xa_s, xb_s, xc_s, q_s, k_s, v_s, o_s, wq_s, wo_s, sa_s, sb_s, dw_s, *, C, W, WP, NWIN, NBLK):
    g = pl.program_id(0)
    ng = pl.num_programs(0)
    dh = C // NH
    CW = C // 2
    NT = WP // LANES
    G = WS * 8
    HW = WP // 2
    NC = C // 16
    NR = WS + 2
    lane8 = _iota((8, LANES), 1)
    last_valid = W - (NT - 1) * LANES
    zero = jnp.uint32(0)
    hi = jnp.uint32(0xFFFF0000)
    qkv_s = (q_s, k_s, v_s)
    xbuf = (xa_s, xb_s, xc_s)
    xin = (x0_ref, x1_ref, x2_ref, x3_ref)
    stg = (sa_s, sb_s)
    SPARE = sa_s.shape[0] - 1
    zx = g >> 10
    never = lane8 < zx

    def tie(x, toks):
        for tok in toks:
            n = x.shape[1]
            x = lax.select(never[:, 0:n], tok[:, 0:n], x) if n < LANES else lax.select(never, tok, x)
        return x

    def stg_row(j, c2, rho):
        if 2 <= rho < WS:
            return rho - 2
        slot = j % NSUB if rho >= WS else (j - 1) % NSUB
        return WS - 2 + (slot * (NC // 2) + c2) * 2 + rho % WS

    zt = jnp.zeros((8, LANES), U32)
    is_first, is_last = lane8 == 0, lane8 == LANES - 1
    assert last_valid == LANES - 1

    def shifted(u):
        tiles = [u[:, LANES * t:LANES * (t + 1)] for t in range(NT)]
        tiles[NT - 1] = lax.select(is_last, zt, tiles[NT - 1])
        left = [pltpu.roll(lax.select(is_last, tiles[t - 1] if t > 0 else zt, tiles[t]), 1, 1)
                for t in range(NT)]
        right = [pltpu.roll(lax.select(is_first, tiles[t + 1], tiles[t]) if t < NT - 1 else tiles[t], LANES - 1, 1)
                 for t in range(NT)]
        return _cat([_cat(v, axis=1) for v in (left, tiles, right)])

    def unpack(v, hf):
        return pltpu.bitcast(v, BF16).astype(F32).reshape(3, 2, 8, LANES)[:, hf]

    def conv_row(un, w, r):
        return jnp.sum(_tree_sum([un[r + ki] * w[ki] for ki in range(3) if un[r + ki] is not None]), axis=0)

    def setup():
        qscale = (dh ** -0.5) * math.log2(math.e)
        wt = wqkv_ref[...].astype(F32).T
        wq = (wt[0:C] * qscale).astype(BF16).astype(F32)
        words = [(_u32(w[0:CW]) >> 16) | (_u32(w[CW:C]) & hi) for w in (wq, wt[C:2 * C])]
        words = _rows8(_cat(words + [_u32(wt[2 * C:].astype(BF16))]))
        for par in range(2):
            wpar = _cat(words[par::2])
            wq_s[par, :, 0:CW] = wpar[:, 0:CW]
            wq_s[par, :, LANES:LANES + CW] = wpar[:, CW:C]
        wo = _u32(wo_ref[...])
        wo_s[...] = jnp.zeros(wo_s.shape, U32)
        wo_s[:, 0:CW] = (wo << 16).T
        wo_s[:, LANES:LANES + CW] = (wo & hi).T

        def zrow(r, carry):
            rs = pl.ds(pl.multiple_of(r % 4 * LANES, LANES), LANES)
            for ref in (q_s, k_s, v_s, o_s):
                ref[r // 4, rs, :] = jnp.zeros((LANES, LANES), U32)
            return carry
        lax.fori_loop(0, WS * NT, zrow, 0)
        for ref in stg:
            ref[SPARE] = jnp.zeros(ref.shape[1:], U32)

        def taps(ki, carry):
            w3 = dw_ref[ki].astype(F32)
            for kj in range(3):
                w = w3[kj:kj + 1]
                if kj == 1:
                    w = w + jnp.where(ki == 1, 1.0, 0.0)
                dw_s[:, ki, kj] = jnp.broadcast_to(w, (LANES, C)).T.reshape(C // 8, 8, LANES)
            return carry
        lax.fori_loop(0, 3, taps, 0)

        def conv0(c2, carry):
            for par in range(2):
                cs = pl.ds(pl.multiple_of(32 * c2 + 16 * par, 16), 16)
                sh = [shifted(_u32(x1_ref[r, cs, :])) for r in range(WS)] + [shifted(_u32(x2_ref[0, cs, :]))]
                for rho in (WS, WS + 1):
                    stg[par][stg_row(-1, c2, rho)] = sh[rho - 1]
                for hf in range(2):
                    c8 = 4 * c2 + 2 * par + hf
                    w = [dw_s[c8, ki] for ki in range(3)]
                    for t in range(NT):
                        ls = slice(LANES * t, LANES * (t + 1))
                        un = [None] + [unpack(row[:, ls], hf) for row in sh]
                        for r in range(WS):
                            xbuf[0][r, pl.ds(pl.multiple_of(8 * c8, 8), 8), ls] = conv_row(un, w, r)
            return carry
        lax.fori_loop(0, NC // 2, conv0, 0)

    def body(subs):
        lane3 = _iota((WS, 8, LANES), 2)
        head = (lane3 < dh, (lane3 >= dh) & (lane3 < 2 * dh))
        zq = jnp.zeros((WS, 8, LANES), F32)
        junk8 = _iota((8, 2 * G), 0) == WS
        ninf8 = jnp.full((8, 2 * G), -jnp.inf, F32)
        zero8 = jnp.zeros((8, 2 * G), F32)
        ngr = WS + PVP
        real3 = _iota((ngr, 8, 2 * G), 1) < WS
        key_ok = tuple(((_iota((ngr, 8, 2 * G), 2) & 8) == 8 * hh) & real3 for hh in range(2))
        zp = jnp.zeros((ngr, 8, 2 * G), F32)
        first_half = (_iota((8, 2 * G), 1) & 8) == 0
        even_head = (_iota((WS, 8, CW), 2) // (dh // 2)) % 2 == 0
        npair = (NWIN + 1) // 2
        n0 = (HW - 1) // WS // 2

        st = {}
        toks = []
        soft = []
        ticks = []
        j0 = subs[0][0]
        tag = {('qkv', t, r): -1 for t in range(NT) for r in range(WS)}
        tag.update({('o', p): (-1 if p < n0 else None) for p in range(npair)})
        for b, blk in ((j0 % 3, 0), ((j0 + 2) % 3, -1)):
            tag.update({('x', b, c, t, r): blk for c in range(2 * NC) for t in range(NT) for r in range(WS)})
        tag.update({('s', c % 2, stg_row(j0, c // 2, rho)): (0, c, rho) for c in range(NC) for rho in (0, 1)})

        def gather(ref, w):
            return ref[:, pl.ds(WS * w, 8), :]

        def tick(t):
            c = [x for x in ticks if t <= x[0] <= t + 40]
            if not c:
                return None
            _, res, j = min(c, key=lambda x: x[0])
            return res[8 * j:8 * j + 8, 0:LANES]

        def due(lst, nblk, t0, step):
            inj = {}
            for d, tok in list(lst):
                j = max(0, -(-(d - t0) // step))
                if j < nblk:
                    inj.setdefault(j, []).append(tok)
            lst[:] = [x for x in lst if x[0] > t0 + (nblk - 1) * step]
            return inj

        def lhs(ref, ls, inj, dt):
            nblk = ref.shape[0] // 8
            parts, s = [], 0
            for j in sorted(inj):
                if j > s:
                    parts.append(ref[8 * s:8 * j, ls])
                parts.append(tie(ref[8 * j:8 * j + 8, ls], inj[j]))
                s = j + 1
            if s < nblk:
                parts.append(ref[8 * s:8 * nblk, ls])
            return pltpu.bitcast(_cat(parts), dt)

        def merged(a, b):
            return {j: a.get(j, []) + b.get(j, []) for j in set(a) | set(b)}

        def fence(d, b):
            c = [x for x in ticks if x[0] <= d]
            if c:
                _, res, j = max(c, key=lambda x: x[0])
                xbuf[b][zx + WS, 0:8, 0:LANES] = res[8 * j:8 * j + 8, 0:LANES]

        def ln1(d, k, t, r):
            b = subs[k][0] % 3
            assert all(tag['x', b, c, t, r] == k for c in range(2 * NC))
            x0 = xbuf[b][r, :, LANES * t:LANES * (t + 1)]
            s8 = _sum8(x0)
            soft.append((d, _u32(s8)))
            mean = jnp.sum(s8, axis=0, keepdims=True) * (1.0 / C)
            if LNF & 2:
                fence(d + LNG, b)
                x0 = xbuf[b][r, :, LANES * t:LANES * (t + 1)]
            st['ln', k, t, r] = [x0 - mean, [], mean]

        def ln3(d, k, t, r):
            b = subs[k][0] % 3
            fence(d, b)
            st['ln', k, t, r][0] = xbuf[b][r, :, LANES * t:LANES * (t + 1)] - st['ln', k, t, r][2]

        def ln2(d, n, *key):
            m = C // LNS
            xc = st[('ln',) + key][0][m * n:m * (n + 1)]
            s8 = _sum8(xc * xc)
            soft.append((d, _u32(s8)))
            st[('ln',) + key][1].append(s8)

        def a_dot(t0, k, t, r):
            xc, sq, _ = st.pop(('ln', k, t, r))
            var = jnp.sum(_tree_sum(sq), axis=0, keepdims=True) * (1.0 / C)
            h = xc * lax.rsqrt(var + EPS)
            h = [h[CW * kt:CW * (kt + 1)].astype(BF16) for kt in range(2)]
            inj = due(toks, DA // 16, t0, 16)
            inj0 = merged(inj, due(soft, DA // 16, t0, 16))
            part = [jnp.dot(lhs(wq_s.at[par], slice(LANES * kt, LANES * kt + CW), inj if par or kt else inj0, BF16),
                            h[kt], preferred_element_type=F32)
                    for par in range(2) for kt in range(2)]
            res = [part[0] + part[1], part[2] + part[3]]
            ticks.extend((t0 + MXU_LAT + 8 * j, res[0], j) for j in range(DA // 8))
            qkv = jnp.stack([v.reshape(-1, 16, LANES) for v in res], axis=1).reshape(3 * C, LANES)
            for m in range(3):
                qkv_s[m][r, LANES * t:LANES * (t + 1), 0:CW] = _u32(qkv[C * m:C * (m + 1)].astype(BF16)).T
                toks.append((t0 + 96 * (m + 1) + DL_A, qkv_s[m][zx, 0:8, :]))
            tag['qkv', t, r] = k

        def wins(p):
            return 2 * p, min(2 * p + 1, NWIN - 1)

        def b_qk(t0, k, p):
            wa, wb = wins(p)
            blk = k if p < n0 else k - 1
            assert all(tag['qkv', t, r] == blk for r in range(WS)
                       for t in range(WS * wa // LANES, (WS * wb + WS) // LANES + 1))
            sts = []
            inj = due(soft, WS, t0, 8)
            for w, swap in ((wa, 0), (wb, 1)):
                qw = gather(q_s, w)
                kw = gather(k_s, w).reshape(G, LANES)
                if not swap and inj:
                    kw = _cat([tie(v, inj.get(r, [])) for r, v in enumerate(_rows8(kw))])
                for tile in range(2):
                    kk = _f32(kw & hi if tile else kw << 16)
                    qq = _f32(qw & hi if tile else qw << 16)
                    qst = jnp.stack([lax.select(head[swap], qq, zq), lax.select(head[1 - swap], qq, zq)], axis=1)
                    sts.append(lax.dot_general(kk, qst.reshape(2 * G, LANES), (((1,), (1,)), ((), ())),
                                               preferred_element_type=F32))
            if PVP:
                vw = _cat([gather(v_s, wa), zt[None], gather(v_s, wb), zt[None]]).reshape(LANES, LANES)
            else:
                vw = _cat([gather(v_s, wa), gather(v_s, wb)]).reshape(2 * G, LANES)
            st['s', p] = (sts, pltpu.bitcast(vw[:, 0:CW].T, BF16))

        def b_pv(t0, tg, k, p):
            wa, wb = wins(p)
            sts, vt = st.pop(('s', p))
            pts = []
            rinv = []
            for n, s_t in enumerate(sts):
                m8 = _fold7(jnp.maximum, s_t)
                mx = _all8(jnp.maximum, lax.select(junk8, ninf8, m8))
                mv = lax.select(junk8, m8, mx)
                z = tick(tg + SMD * (3 - n))
                if z is not None:
                    mv = tie(mv, [z])
                eg = jnp.exp2(s_t.reshape(WS, 8, 2 * G) - mv)
                den = _all8(jnp.add, lax.select(junk8, zero8, _fold7(jnp.add, eg.reshape(G, 2 * G))))
                r0 = pl.reciprocal(den, approx=True)
                rinv.append(r0 * (2.0 - den * r0))
                pts.append(_cat([eg, eg[WS - 1:WS]]) if PVP else eg)
            outs = []
            for tile in range(2):
                for hh in range(2):
                    h = 2 * tile + hh
                    stn = _cat([lax.select(key_ok[hh], pts[tile], zp), lax.select(key_ok[1 - hh], pts[2 + tile], zp)])
                    ot = jnp.dot(vt[dh * h:dh * (h + 1), :], stn.reshape(-1, 2 * G).astype(BF16),
                                 preferred_element_type=F32)
                    rr = lax.select(first_half, rinv[2 * hh + tile], rinv[2 - 2 * hh + tile])
                    outs.append(ot.reshape(dh // 8, 8, 2 * G) * rr)
            tw = _u32(_cat(outs).reshape(C, 2 * G).astype(BF16)).T.reshape(WS, 2, 8, CW)
            tw = (tw[:, 0], tw[:, 1])
            o_s[:, pl.ds(WS * wa, 8), 0:CW] = lax.select(even_head, tw[0], tw[1])
            if wb != wa:
                o_s[:, pl.ds(WS * wb, 8), 0:CW] = lax.select(even_head, tw[1], tw[0])
                tag['o', p + 1] = None
            toks.append((t0 + DL_PV, o_s[zx, 0:8, :]))
            tag['o', p] = k if p < n0 else k - 1
            if p == n0:
                tag['o2'] = k - 1

        def c_dot(t0, k, h, r):
            b = (subs[k][0] + 2) % 3
            assert all(tag['o', p] == k - 1 for p in (range(n0 + 1) if h == 0 else range(n0 + 1, npair)))
            assert tag['o2'] == k - 1 and 2 * WS * n0 < HW
            assert all(tag['x', b, c, t, r] == k - 1 for c in range(2 * NC) for t in (2 * h, 2 * h + 1))
            ls = slice(HW * h, HW * (h + 1))
            ow = o_s[r, ls, :]
            rhs = _cat([_f32(ow << 16), _f32(ow & hi)], axis=1)
            inj = due(toks, DC // 8, t0, 8)
            wo = _cat([lhs(wo_s, slice(0, LANES), merged(inj, due(soft, DC // 8, t0, 8)), F32),
                       lhs(wo_s, slice(LANES, 2 * LANES), inj, F32)], axis=1)
            res = lax.dot_general(wo, rhs, (((1,), (1,)), ((), ())), preferred_element_type=F32)
            ticks.extend((t0 + MXU_LAT + 8 * j, res, j) for j in range(DC // 8))
            o_ref[subs[k][2] + r, :, ls] = (xbuf[b][r, :, ls] + res).astype(o_ref.dtype)

        def stage_row(d, k, c, rho):
            j, slot = subs[k][0:2]
            cs = slice(16 * c, 16 * c + 16)
            if rho == WS + 1:
                u = _u32(xin[slot + 1][0, cs, :])
                if slot == 1:
                    u = jnp.where(g < ng - 2, u, zero)
            else:
                u = _u32(xin[slot][rho - 1, cs, :])
            idx = stg_row(j, c // 2, rho)
            stg[c % 2][idx] = shifted(u)
            soft.append((d, stg[c % 2][zx + SPARE, 8:16, 0:LANES]))
            tag['s', c % 2, idx] = (k, c, rho)

        def conv_step(d, k, c, hf, t, r):
            j = subs[k][0]
            if r == 0:
                if t == 0:
                    stg[c % 2][zx + SPARE, 0:8, 0:LANES] = zt
                    st['w'] = [dw_s[2 * c + hf, ki] for ki in range(3)]
                st['un'] = {}
            un = st['un']
            for rho in range(r, r + 3):
                if rho not in un:
                    idx = stg_row(j, c // 2, rho)
                    assert tag['s', c % 2, idx] in ((k, c, rho), (k - 1, c, rho + WS))
                    un[rho] = unpack(stg[c % 2][idx, :, LANES * t:LANES * (t + 1)], hf)
            acc = conv_row(un, st['w'], r)
            xbuf[(j + 1) % 3][r, 16 * c + 8 * hf:16 * c + 8 * hf + 8, LANES * t:LANES * (t + 1)] = acc
            soft.append((d, _u32(acc)))
            tag['x', (j + 1) % 3, 2 * c + hf, t, r] = k + 1

        plan, offs = [], [0]
        for k, sub in enumerate(subs):
            pk, tk = _plan(npair, n0, NT, sub[3], sub[4])
            plan += [(offs[k] + t, kind, k, idx) for t, kind, idx in pk]
            offs.append(offs[k] + tk)
        total = offs[-1]
        starts = [e[0] for e in plan]
        ev = []

        def at(t, fn, *a):
            ev.append((t, t, len(ev), fn, a))

        def before(d, fn, *a):
            ev.append((max([t for t in starts if t <= d], default=0) - 1, d, len(ev), fn, a))

        load = [0.0] * (total + 1000)
        tqk = {}

        def add(t0, t1, n):
            for t in range(max(t0, 0), max(t1, 0)):
                load[t] += n / (t1 - t0)

        for t, kind, k, idx in plan:
            tr = t + MXU_LAT
            if kind == 'a':
                if idx == (0, 0) and k > 0:
                    before(t - LN1 - 1, fence, t - LN1 - 40, subs[k][0] % 3)
                before(t - LN1, ln1, t - LN1, k, *idx)
                for n in range(LNS):
                    d = t - LN2 - LND * (LNS - 1 - n)
                    before(d, ln2, d, n, k, *idx)
                    add(d - 16, d, 72 // LNS)
                if LNF & 1:
                    before(t - LN3, ln3, t - LN3, k, *idx)
                    add(t - 40, t, 24)
                at(t, a_dot, t, k, *idx)
                add(tr, tr + DA, 12 * DA // 16)
                add(t - LN1 - 16, t - LN1, 32); add(t - LN2, t - 40, 20); add(t - 40, t, 36)
            elif kind == 'qk':
                at(t, b_qk, t, k, idx)
                tqk[idx] = t
                add(t - 64, t, 28); add(t, t + DQ, 28); add(tr, tr + DQ, 24); add(tr + DQ, tr + DQ + 16, 36)
            elif kind == 'pv':
                tg = max(tqk[idx] + SM0, t - SMB)
                at(t, b_pv, t, tg, k, idx)
                add(tg, tg + 4 * SMD + 16, 80); add(tr - 10, tr + 6, 46); add(tr, tr + DP, 36)
                add(t + 400, t + 460, 14)
            else:
                if idx == (0, 0) and k > 0:
                    at(t - 1, fence, t - 100, (subs[k][0] + 2) % 3)
                at(t, c_dot, t, k, *idx)
                add(tr, tr + DC, 20 * DC // 16)
                add(t - 70, t, 64)
        pre = [0.0]
        for v in load:
            pre.append(pre[-1] + v)
        nstep = NC * 2 * NT * WS
        prev_chunk = 10
        for k, sub in enumerate(subs):
            if not sub[3]:
                continue
            ta = offs[k] + (CVI if k else CV0) - 20
            tb = offs[k + 1] - (CVE if k == len(subs) - 1 else CVX)
            cap = CAP if sub[4] else 64
            free = [max(0.02, cap / 16 - (pre[t + SMO] - pre[max(t - SMO, 0)]) / (2 * SMO)) for t in range(ta, tb)]
            tot_free, acc, tstep = sum(free), 0.0, []
            for t, v in enumerate(free):
                acc += v
                while len(tstep) < nstep and acc >= (len(tstep) + 1) * tot_free / nstep - 1e-6:
                    tstep.append(ta + t)
            for n in range(nstep):
                before(tstep[n], conv_step, tstep[n], k, n // (2 * NT * WS), n // (NT * WS) % 2, n // WS % NT, n % WS)
            for c in range(NC):
                t1 = tstep[c * 2 * NT * WS] - 30
                t0 = prev_chunk + 120
                prev_chunk = t1 + 30
                for rho in range(2, NR):
                    d = t0 + (t1 - t0) * (rho - 2) // (NR - 3)
                    before(d, stage_row, d, k, c, rho)
        ev.sort(key=lambda e: e[:3])
        for e in ev:
            e[3](*e[4])
        if subs[-1][3]:
            n = len(subs)
            assert all(tag['qkv', t, r] == n - 1 for t in range(NT) for r in range(WS))
            assert all(tag['o', p] == n - 1 for p in range(n0))

    if ONLY in (0, 1):
        @pl.when(g == 0)
        def _():
            setup()
            body([(0, 2, 0, True, False)])

    if ONLY in (0, 2):
        @pl.when((g > 0) & (g < ng - 1))
        def _():
            body([(1 + k, k, WS * k, True, True) for k in range(NSUB)])

    if ONLY in (0, 3):
        @pl.when(g == ng - 1)
        def _():
            body([(1, 0, 0, False, True)])


@jax.jit
def pallas_standalone__window_attn_davit__vision_kernel(
    x: jax.Array,
    dw_pe: jax.Array,
    w_qkv: jax.Array,
    w_o: jax.Array,
):
    B, H, W, C = x.shape
    assert B == 1 and H % WS == 0 and W % WS == 0 and C % (16 * NH) == 0
    WP = -(-(W + 1) // (2 * LANES)) * (2 * LANES)
    assert WP == 4 * LANES
    NWIN = W // WS
    NBLK = H // WS
    assert (NBLK - 1) % NSUB == 0
    NM = (NBLK - 1) // NSUB

    xt = jnp.transpose(x[0], (0, 2, 1))

    def blk(k):
        return lambda g: (jnp.clip(NSUB * g - 1 + k, 0, NBLK - 1), 0, 0)

    nstg = WS - 2 + NSUB * (C // 32) * 2 + 1
    kern = functools.partial(_kernel, C=C, W=W, WP=WP, NWIN=NWIN, NBLK=NBLK)
    out = pl.pallas_call(
        kern,
        grid=(NM + 2,),
        in_specs=[
            pl.BlockSpec((WS, C, WP), blk(0)),
            pl.BlockSpec((WS, C, WP), blk(1)),
            pl.BlockSpec((WS, C, WP), blk(2)),
            pl.BlockSpec((1, C, WP), lambda g: (jnp.minimum(WS * (NSUB * g + 2), H - 1), 0, 0)),
            pl.BlockSpec((3, 3, C), lambda g: (0, 0, 0)),
            pl.BlockSpec((C, 3 * C), lambda g: (0, 0)),
            pl.BlockSpec((C, C), lambda g: (0, 0)),
        ],
        out_specs=pl.BlockSpec((NSUB * WS, C, WP), lambda g: (jnp.maximum(g - 1, 0), 0, 0)),
        out_shape=jax.ShapeDtypeStruct((H, C, W), x.dtype),
        scratch_shapes=[
            pltpu.VMEM((WS + 1, C, WP), F32),
            pltpu.VMEM((WS + 1, C, WP), F32),
            pltpu.VMEM((WS + 1, C, WP), F32),
            pltpu.VMEM((WS, WP, LANES), U32),
            pltpu.VMEM((WS, WP, LANES), U32),
            pltpu.VMEM((WS, WP, LANES), U32),
            pltpu.VMEM((WS, WP, LANES), U32),
            pltpu.VMEM((2, 3 * C // 4, 2 * LANES), U32),
            pltpu.VMEM((C, 2 * LANES), U32),
            pltpu.VMEM((nstg, 3 * 8, WP), U32),
            pltpu.VMEM((nstg, 3 * 8, WP), U32),
            pltpu.VMEM((C // 8, 3, 3, 8, LANES), F32),
        ],
        compiler_params=pltpu.CompilerParams(
            dimension_semantics=("arbitrary",),
            vmem_limit_bytes=96 * 1024 * 1024,
            disable_bounds_checks=bool(NOBC),
        ),
        name="davit_window_attn",
    )(xt, xt, xt, xt, dw_pe, w_qkv, w_o)
    return jnp.transpose(out, (0, 2, 1))[None]
```

```python
import functools
import math
import os

import jax
import jax.numpy as jnp
from jax import lax
import jax.experimental.pallas as pl
import jax.experimental.pallas.tpu as pltpu

WS = 7
NH = 4
EPS = 1e-05
LANES = 128
F32 = jnp.float32
BF16 = jnp.bfloat16
U32 = jnp.uint32

P = lambda k, d: int(os.environ.get(k, d))
DL_A = P('DL_A', 500)
LAT_QK = P('LAT_QK', 280)
DL_PV = P('DL_PV', 580)
PRE_C = P('PRE_C', 120)
TAIL = P('TAIL', 1000)
LN1 = P('LN1', 200)
LN2 = P('LN2', 130)
LNS = P('LNS', 3)
LND = P('LND', 16)
SM0 = P('SM0', 200)
SMD = P('SMD', 16)
SMB = P('SMB', 110)
CV0 = P('CV0', 400)
CVI = P('CVI', 170)
CVE = P('CVE', 60)
CVX = P('CVX', 200)
ORD = P('ORD', 0)
CAP = P('CAP', 42)
SMO = P('SMO', 32)
ONLY = P('ONLY', 0)
DL_D = P('DL_D', 100)
PVP = P('PVP', 0)
LNF = P('LNF', 3)
LN3 = P('LN3', 50)
LNG = P('LNG', 16)
NOBC = P('NOBC', 1)
DA, DC, DQ, DP = 288, 192, 56, 48
MXU_LAT = 130
NSUB = 3


def _iota(shape, dim):
    return lax.broadcasted_iota(jnp.int32, shape, dim)


def _plan(npair, n0, nt, cur, prev):
    a_q = [(t, r) for t in range(nt) for r in range(WS)] if cur else []
    c_q = [(h, r) for h in range(2) for r in range(WS)] if prev else []
    n1 = npair - n0 if prev else 0
    pairs = list(range(n0, n0 + n1)) + (list(range(n0)) if cur else [])
    total = len(a_q) * DA + len(c_q) * DC + len(pairs) * (DQ + DP)
    q0 = 0 if prev else total // 3
    t = 0
    ia = ic = iq = ip = 0
    out = []
    tq, tp, ta = {}, {}, {}
    last = None
    while ia < len(a_q) or ic < len(c_q) or ip < len(pairs):
        cands = []
        if ip < iq and t >= tq[ip] + LAT_QK:
            cands.append((-1e6, 'pv'))
        if iq < len(pairs) and (not cur or (iq - ip < 2 and last != 'qk' and not (ORD and last == 'pv'))):
            ok = iq - ip < 4
            if iq >= n1:
                need = (2 * WS * pairs[iq] + 2 * WS) // LANES * WS + WS - 1
                ok = ia > need and t >= ta[need] + DA + DL_A + 60 and ic >= len(c_q) // 2
            if ok:
                pr = q0 + iq * (total - q0 - TAIL) / len(pairs) - t - 200
                cands.append((-2e6 if ORD and pr <= 0 else pr, 'qk'))
        if ia < len(a_q):
            cands.append((ia * (total - 700) / len(a_q) - t, 'a'))
        if ic < len(c_q):
            need = 0 if ic < WS else n1 - 1
            if ip > need and t >= tp[need] + DL_PV + PRE_C:
                if cur:
                    tc = 1000 + ic * 900 if ic < WS else total - DC - (2 * WS - 1 - ic) * 950
                else:
                    tc = 1500 + ic * 400
                cands.append((tc - t, 'c'))
        if not cands:
            t += 8
            last = None
            continue
        kind = min(cands)[1]
        last = kind
        if kind == 'pv':
            tp[ip] = t; out.append((t, 'pv', pairs[ip])); ip += 1; t += DP
        elif kind == 'qk':
            tq[iq] = t; out.append((t, 'qk', pairs[iq])); iq += 1; t += DQ
        elif kind == 'a':
            ta[ia] = t; out.append((t, 'a', a_q[ia])); ia += 1; t += DA
        else:
            out.append((t, 'c', c_q[ic])); ic += 1; t += DC
    return out, t


def _tree_sum(xs):
    while len(xs) > 1:
        xs = [xs[j] + xs[j + 1] if j + 1 < len(xs) else xs[j] for j in range(0, len(xs), 2)]
    return xs[0]


def _sum8(x):
    while x.shape[0] % 16 == 0:
        x = x[:x.shape[0] // 2] + x[x.shape[0] // 2:]
    return _tree_sum(_rows8(x))


def _fold7(op, x):
    t = op(x[0:24], x[24:48])
    return op(op(t[0:8], t[8:16]), op(t[16:24], x[48:56]))


def _all8(op, x):
    for sh in (4, 2, 1):
        x = op(x, pltpu.roll(x, sh, 0))
    return x


def _rows8(x):
    return [x[8 * j:8 * j + 8] for j in range(x.shape[0] // 8)]


def _cat(xs, axis=0):
    return jnp.concatenate(xs, axis=axis) if len(xs) > 1 else xs[0]


def _f32(u):
    return pltpu.bitcast(u, F32)


def _u32(x):
    return pltpu.bitcast(x, U32)


def _kernel(x_hbm, dw_hbm, wqkv_hbm, wo_hbm, o_hbm,
            xa_s, xb_s, xc_s, q_s, k_s, v_s, o_s, wq_s, wo_s, sa_s, sb_s, dw_s,
            i0_s, i1_s, i2_s, o0_s, o1_s, o2_s, dw_ref, wqkv_ref, wo_ref, in_sem, out_sem, w_sem,
            *, C, H, W, WP, NWIN):
    g = pl.program_id(0)
    ng = pl.num_programs(0)
    dh = C // NH
    CW = C // 2
    NT = WP // LANES
    G = WS * 8
    HW = WP // 2
    NC = C // 16
    NR = WS + 2
    lane8 = _iota((8, LANES), 1)
    last_valid = W - (NT - 1) * LANES
    zero = jnp.uint32(0)
    hi = jnp.uint32(0xFFFF0000)
    qkv_s = (q_s, k_s, v_s)
    xbuf = (xa_s, xb_s, xc_s)
    xin = (i0_s, i1_s, i2_s)
    xout = (o0_s, o1_s, o2_s)

    def row0(k, m):
        return (m & 1) * WS if k == NSUB - 1 else 0

    def in_copies(k, m):
        r = WS * (NSUB * m - 1 + k) + 1
        return [pltpu.make_async_copy(x_hbm.at[pl.ds(jnp.minimum(r + o, H - n), n)],
                                      xin[k].at[pl.ds(row0(k, m) + o, n)], in_sem.at[2 * k + e])
                for e, (o, n) in enumerate(((0, WS - 1), (WS - 1, 1)))]

    def out_copy(k, m, o=0, n=WS):
        return pltpu.make_async_copy(xout[k].at[pl.ds(row0(k, m) + o, n)],
                                     o_hbm.at[pl.ds(WS * (NSUB * (m - 1) + k) + o, n)],
                                     out_sem.at[k + (m & 1) if k == NSUB - 1 else k])

    stg = (sa_s, sb_s)
    SPARE = sa_s.shape[0] - 1
    zx = g >> 10
    zy = g >> 11
    never = lane8 < zx

    def tie(x, toks):
        if not toks:
            return x
        tok = functools.reduce(lax.bitwise_or, toks)
        n = x.shape[1]
        return lax.select(never[:, 0:n], tok[:, 0:n], x) if n < LANES else lax.select(never, tok, x)

    def stg_row(j, c2, rho):
        if 2 <= rho < WS:
            return rho - 2
        slot = j % NSUB if rho >= WS else (j - 1) % NSUB
        return WS - 2 + (slot * (NC // 2) + c2) * 2 + rho % WS

    zt = jnp.zeros((8, LANES), U32)
    is_first, is_last = lane8 == 0, lane8 == LANES - 1

    def shifted(u):
        tiles = [u[:, LANES * t:LANES * (t + 1)] for t in range(NT)]
        tiles[NT - 1] = _cat([tiles[NT - 1], zt[:, last_valid:]], axis=1)
        left = [pltpu.roll(lax.select(is_last, tiles[t - 1] if t > 0 else zt, tiles[t]), 1, 1)
                for t in range(NT)]
        right = [pltpu.roll(lax.select(is_first, tiles[t + 1], tiles[t]) if t < NT - 1 else tiles[t], LANES - 1, 1)
                 for t in range(NT)]
        return _cat([_cat(v, axis=1) for v in (left, tiles, right)])

    def unpack(v, hf):
        return pltpu.bitcast(v, BF16).astype(F32).reshape(3, 2, 8, LANES)[:, hf]

    def conv_row(un, w, r):
        return jnp.sum(_tree_sum([un[r + ki] * w[ki] for ki in range(3) if un[r + ki] is not None]), axis=0)

    def setup():
        wcp = [pltpu.make_async_copy(src, dst, w_sem.at[n])
               for n, (src, dst) in enumerate(((wqkv_hbm, wqkv_ref), (wo_hbm, wo_ref), (dw_hbm, dw_ref)))]
        top = [pltpu.make_async_copy(x_hbm.at[pl.ds(0, 1)], i0_s.at[pl.ds(0, 1)], in_sem.at[1])] + in_copies(1, 0)
        for cp in wcp + top + in_copies(2, 0):
            cp.start()

        def zrow(r, carry):
            rs = pl.ds(pl.multiple_of(r % 4 * LANES, LANES), LANES)
            for ref in (q_s, k_s, v_s, o_s):
                ref[r // 4, rs, :] = jnp.zeros((LANES, LANES), U32)
            return carry
        lax.fori_loop(0, WS * NT, zrow, 0)
        for ref in stg:
            ref[SPARE] = jnp.zeros(ref.shape[1:], U32)

        for ref in xin + xout:
            ref[ref.shape[0] - 1, 0:16, 0:LANES] = jnp.zeros((16, LANES), BF16)
        for cp in wcp:
            cp.wait()
        qscale = (dh ** -0.5) * math.log2(math.e)
        wt = wqkv_ref[...].astype(F32).T
        wq = (wt[0:C] * qscale).astype(BF16).astype(F32)
        words = [(_u32(w[0:CW]) >> 16) | (_u32(w[CW:C]) & hi) for w in (wq, wt[C:2 * C])]
        words = _rows8(_cat(words + [_u32(wt[2 * C:].astype(BF16))]))
        for par in range(2):
            wpar = _cat(words[par::2])
            wq_s[par, :, 0:CW] = wpar[:, 0:CW]
            wq_s[par, :, LANES:LANES + CW] = wpar[:, CW:C]
        wo = _u32(wo_ref[...])
        wo_s[...] = jnp.zeros(wo_s.shape, U32)
        wo_s[:, 0:CW] = (wo << 16).T
        wo_s[:, LANES:LANES + CW] = (wo & hi).T

        def taps(ki, carry):
            w3 = dw_ref[ki].astype(F32)
            for kj in range(3):
                w = w3[kj:kj + 1]
                if kj == 1:
                    w = w + jnp.where(ki == 1, 1.0, 0.0)
                dw_s[:, ki, kj] = jnp.broadcast_to(w, (LANES, C)).T.reshape(C // 8, 8, LANES)
            return carry
        lax.fori_loop(0, 3, taps, 0)

        for cp in top:
            cp.wait()

        def conv0(c2, carry):
            for par in range(2):
                cs = pl.ds(pl.multiple_of(32 * c2 + 16 * par, 16), 16)
                sh = [shifted(_u32(i0_s[0, cs, :]))] + [shifted(_u32(i1_s[r, cs, :])) for r in range(WS)]
                for rho in (WS, WS + 1):
                    stg[par][stg_row(-1, c2, rho)] = sh[rho - 1]
                for hf in range(2):
                    c8 = 4 * c2 + 2 * par + hf
                    w = [dw_s[c8, ki] for ki in range(3)]
                    for t in range(NT):
                        ls = slice(LANES * t, LANES * (t + 1))
                        un = [None] + [unpack(row[:, ls], hf) for row in sh]
                        for r in range(WS):
                            xbuf[0][r, pl.ds(pl.multiple_of(8 * c8, 8), 8), ls] = conv_row(un, w, r)
            return carry
        lax.fori_loop(0, NC // 2, conv0, 0)
        for cp in in_copies(0, 1) + in_copies(1, 1):
            cp.start()
        for cp in in_copies(2, 0):
            cp.wait()
        for cp in in_copies(2, 1):
            cp.start()

    def body(subs):
        lane3 = _iota((WS, 8, LANES), 2)
        head = (lane3 < dh, (lane3 >= dh) & (lane3 < 2 * dh))
        zq = jnp.zeros((WS, 8, LANES), F32)
        junk8 = _iota((8, 2 * G), 0) == WS
        ninf8 = jnp.full((8, 2 * G), -jnp.inf, F32)
        zero8 = jnp.zeros((8, 2 * G), F32)
        ngr = WS + PVP
        real3 = _iota((ngr, 8, 2 * G), 1) < WS
        key_ok = tuple(((_iota((ngr, 8, 2 * G), 2) & 8) == 8 * hh) & real3 for hh in range(2))
        zp = jnp.zeros((ngr, 8, 2 * G), F32)
        first_half = (_iota((8, 2 * G), 1) & 8) == 0
        even_head = (_iota((WS, 8, CW), 2) // (dh // 2)) % 2 == 0
        npair = (NWIN + 1) // 2
        n0 = (HW - 1) // WS // 2

        st = {}
        toks = []
        soft = []
        ticks = []
        j0 = subs[0][0]
        tag = {('qkv', t, r): -1 for t in range(NT) for r in range(WS)}
        tag.update({('o', p): (-1 if p < n0 else None) for p in range(npair)})
        for b, blk in ((j0 % 3, 0), ((j0 + 2) % 3, -1)):
            tag.update({('x', b, c, t, r): blk for c in range(2 * NC) for t in range(NT) for r in range(WS)})
        tag.update({('s', c % 2, stg_row(j0, c // 2, rho)): (0, c, rho) for c in range(NC) for rho in (0, 1)})

        def gather(ref, w):
            return ref[:, pl.ds(WS * w, 8), :]

        def tick(t):
            c = [x for x in ticks if t <= x[0] <= t + 40]
            if not c:
                return None
            _, res, j = min(c, key=lambda x: x[0])
            return res[8 * j:8 * j + 8, 0:LANES]

        def due(lst, nblk, t0, step):
            inj = {}
            for d, tok in list(lst):
                j = max(0, -(-(d - t0) // step))
                if j < nblk:
                    inj.setdefault(j, []).append(tok)
            lst[:] = [x for x in lst if x[0] > t0 + (nblk - 1) * step]
            return inj

        def lhs(ref, ls, inj, dt):
            nblk = ref.shape[0] // 8
            parts, s = [], 0
            for j in sorted(inj):
                if j > s:
                    parts.append(ref[8 * s:8 * j, ls])
                parts.append(tie(ref[8 * j:8 * j + 8, ls], inj[j]))
                s = j + 1
            if s < nblk:
                parts.append(ref[8 * s:8 * nblk, ls])
            return pltpu.bitcast(_cat(parts), dt)

        def merged(a, b):
            return {j: a.get(j, []) + b.get(j, []) for j in set(a) | set(b)}

        def fence(d, b):
            c = [x for x in ticks if x[0] <= d]
            if c:
                _, res, j = max(c, key=lambda x: x[0])
                xbuf[b][zx + WS, 0:8, 0:LANES] = res[8 * j:8 * j + 8, 0:LANES]

        def ln1(d, k, t, r):
            b = subs[k][0] % 3
            assert all(tag['x', b, c, t, r] == k for c in range(2 * NC))
            x0 = xbuf[b][r, :, LANES * t:LANES * (t + 1)]
            s8 = _sum8(x0)
            soft.append((d, _u32(s8)))
            mean = jnp.sum(s8, axis=0, keepdims=True) * (1.0 / C)
            if LNF & 2:
                fence(d + LNG, b)
                x0 = xbuf[b][r, :, LANES * t:LANES * (t + 1)]
            st['ln', k, t, r] = [x0 - mean, [], mean]

        def ln3(d, k, t, r):
            b = subs[k][0] % 3
            fence(d, b)
            st['ln', k, t, r][0] = xbuf[b][r, :, LANES * t:LANES * (t + 1)] - st['ln', k, t, r][2]

        def ln2(d, n, *key):
            m = C // LNS
            xc = st[('ln',) + key][0][m * n:m * (n + 1)]
            s8 = _sum8(xc * xc)
            soft.append((d, _u32(s8)))
            st[('ln',) + key][1].append(s8)

        def a_dot(t0, k, t, r):
            xc, sq, _ = st.pop(('ln', k, t, r))
            var = jnp.sum(_tree_sum(sq), axis=0, keepdims=True) * (1.0 / C)
            h = xc * lax.rsqrt(var + EPS)
            h = [h[CW * kt:CW * (kt + 1)].astype(BF16) for kt in range(2)]
            inj = due(toks, DA // 16, t0, 16)
            inj0 = merged(inj, due(soft, DA // 16, t0, 16))
            part = [jnp.dot(lhs(wq_s.at[par], slice(LANES * kt, LANES * kt + CW), inj if par or kt else inj0, BF16),
                            h[kt], preferred_element_type=F32)
                    for par in range(2) for kt in range(2)]
            res = [part[0] + part[1], part[2] + part[3]]
            ticks.extend((t0 + MXU_LAT + 8 * j, res[0], j) for j in range(DA // 8))
            qkv = jnp.stack([v.reshape(-1, 16, LANES) for v in res], axis=1).reshape(3 * C, LANES)
            for m in range(3):
                qkv_s[m][r, LANES * t:LANES * (t + 1), 0:CW] = _u32(qkv[C * m:C * (m + 1)].astype(BF16)).T
                toks.append((t0 + 96 * (m + 1) + DL_A, qkv_s[m][zx, 0:8, :]))
            tag['qkv', t, r] = k

        def wins(p):
            return 2 * p, min(2 * p + 1, NWIN - 1)

        def b_qk(t0, k, p):
            wa, wb = wins(p)
            blk = k if p < n0 else k - 1
            assert all(tag['qkv', t, r] == blk for r in range(WS)
                       for t in range(WS * wa // LANES, (WS * wb + WS) // LANES + 1))
            sts = []
            inj = due(soft, WS, t0, 8)
            for w, swap in ((wa, 0), (wb, 1)):
                qw = gather(q_s, w)
                kw = gather(k_s, w).reshape(G, LANES)
                if not swap and inj:
                    kw = _cat([tie(v, inj.get(r, [])) for r, v in enumerate(_rows8(kw))])
                for tile in range(2):
                    kk = _f32(kw & hi if tile else kw << 16)
                    qq = _f32(qw & hi if tile else qw << 16)
                    qst = jnp.stack([lax.select(head[swap], qq, zq), lax.select(head[1 - swap], qq, zq)], axis=1)
                    sts.append(lax.dot_general(kk, qst.reshape(2 * G, LANES), (((1,), (1,)), ((), ())),
                                               preferred_element_type=F32))
            if PVP:
                vw = _cat([gather(v_s, wa), zt[None], gather(v_s, wb), zt[None]]).reshape(LANES, LANES)
            else:
                vw = _cat([gather(v_s, wa), gather(v_s, wb)]).reshape(2 * G, LANES)
            st['s', p] = (sts, pltpu.bitcast(vw[:, 0:CW].T, BF16))

        def b_pv(t0, tg, k, p):
            wa, wb = wins(p)
            sts, vt = st.pop(('s', p))
            pts = []
            rinv = []
            for n, s_t in enumerate(sts):
                m8 = _fold7(jnp.maximum, s_t)
                mx = _all8(jnp.maximum, lax.select(junk8, ninf8, m8))
                mv = lax.select(junk8, m8, mx)
                z = tick(tg + SMD * (3 - n))
                if z is not None:
                    mv = tie(mv, [z])
                eg = jnp.exp2(s_t.reshape(WS, 8, 2 * G) - mv)
                den = _all8(jnp.add, lax.select(junk8, zero8, _fold7(jnp.add, eg.reshape(G, 2 * G))))
                r0 = pl.reciprocal(den, approx=True)
                rinv.append(r0 * (2.0 - den * r0))
                pts.append(_cat([eg, eg[WS - 1:WS]]) if PVP else eg)
            outs = []
            for tile in range(2):
                for hh in range(2):
                    h = 2 * tile + hh
                    stn = _cat([lax.select(key_ok[hh], pts[tile], zp), lax.select(key_ok[1 - hh], pts[2 + tile], zp)])
                    ot = jnp.dot(vt[dh * h:dh * (h + 1), :], stn.reshape(-1, 2 * G).astype(BF16),
                                 preferred_element_type=F32)
                    rr = lax.select(first_half, rinv[2 * hh + tile], rinv[2 - 2 * hh + tile])
                    outs.append(ot.reshape(dh // 8, 8, 2 * G) * rr)
            tw = _u32(_cat(outs).reshape(C, 2 * G).astype(BF16)).T.reshape(WS, 2, 8, CW)
            tw = (tw[:, 0], tw[:, 1])
            o_s[:, pl.ds(WS * wa, 8), 0:CW] = lax.select(even_head, tw[0], tw[1])
            if wb != wa:
                o_s[:, pl.ds(WS * wb, 8), 0:CW] = lax.select(even_head, tw[1], tw[0])
                tag['o', p + 1] = None
            toks.append((t0 + DL_PV, o_s[zx, 0:8, :]))
            tag['o', p] = k if p < n0 else k - 1
            if p == n0:
                tag['o2'] = k - 1

        def c_dot(t0, k, h, r):
            b = (subs[k][0] + 2) % 3
            assert all(tag['o', p] == k - 1 for p in (range(n0 + 1) if h == 0 else range(n0 + 1, npair)))
            assert tag['o2'] == k - 1 and 2 * WS * n0 < HW
            assert all(tag['x', b, c, t, r] == k - 1 for c in range(2 * NC) for t in (2 * h, 2 * h + 1))
            ls = slice(HW * h, HW * (h + 1))
            ow = o_s[r, ls, :]
            rhs = _cat([_f32(ow << 16), _f32(ow & hi)], axis=1)
            inj = due(toks, DC // 8, t0, 8)
            wo = _cat([lhs(wo_s, slice(0, LANES), merged(inj, due(soft, DC // 8, t0, 8)), F32),
                       lhs(wo_s, slice(LANES, 2 * LANES), inj, F32)], axis=1)
            res = lax.dot_general(wo, rhs, (((1,), (1,)), ((), ())), preferred_element_type=F32)
            ticks.extend((t0 + MXU_LAT + 8 * j, res, j) for j in range(DC // 8))
            slot = subs[k][2]
            n = min(HW, W - HW * h)
            xout[slot][row0(slot, g) + r, :, HW * h:HW * h + n] = (xbuf[b][r, :, ls] + res)[:, 0:n].astype(BF16)
            if h == 1 and not subs[k][3]:
                out_copy(slot, g, r, 1).start()
            elif h == 1 and r == WS - 1:
                out_copy(slot, g).start()
                xout[slot][zx + xout[slot].shape[0] - 1, 0:16, 0:LANES] = jnp.zeros((16, LANES), BF16)
                soft.append((t0 + MXU_LAT + DC + DL_D, _u32(xout[slot][zy + xout[slot].shape[0] - 1, 0:16, 0:LANES])))

        def stage_row(d, k, c, rho):
            j, slot = subs[k][0:2]
            cs = slice(16 * c, 16 * c + 16)
            u = _u32(xin[slot][row0(slot, g) + rho - 2, cs, :])
            if rho == WS + 1 and slot == 1:
                u = jnp.where(g < ng - 2, u, zero)
            idx = stg_row(j, c // 2, rho)
            stg[c % 2][idx] = shifted(u)
            soft.append((d, stg[c % 2][zx + SPARE, 8:16, 0:LANES]))
            tag['s', c % 2, idx] = (k, c, rho)
            if c == NC - 1 and rho == WS + 1 and slot < NSUB - 1:
                for cp in in_copies(slot, g + 1):
                    cp.start()
                xin[slot][zx + WS, 0:16, 0:LANES] = jnp.zeros((16, LANES), BF16)
                soft.append((d + DL_D, _u32(xin[slot][zy + WS, 0:16, 0:LANES])))

        def conv_step(d, k, c, hf, t, r):
            j = subs[k][0]
            if r == 0:
                if t == 0:
                    stg[c % 2][zx + SPARE, 0:8, 0:LANES] = zt
                    st['w'] = [dw_s[2 * c + hf, ki] for ki in range(3)]
                st['un'] = {}
            un = st['un']
            for rho in range(r, r + 3):
                if rho not in un:
                    idx = stg_row(j, c // 2, rho)
                    assert tag['s', c % 2, idx] in ((k, c, rho), (k - 1, c, rho + WS))
                    un[rho] = unpack(stg[c % 2][idx, :, LANES * t:LANES * (t + 1)], hf)
            acc = conv_row(un, st['w'], r)
            xbuf[(j + 1) % 3][r, 16 * c + 8 * hf:16 * c + 8 * hf + 8, LANES * t:LANES * (t + 1)] = acc
            soft.append((d, _u32(acc)))
            tag['x', (j + 1) % 3, 2 * c + hf, t, r] = k + 1

        plan, offs = [], [0]
        for k, sub in enumerate(subs):
            pk, tk = _plan(npair, n0, NT, sub[3], sub[4])
            plan += [(offs[k] + t, kind, k, idx) for t, kind, idx in pk]
            offs.append(offs[k] + tk)
        total = offs[-1]
        starts = [e[0] for e in plan]
        ev = []

        def at(t, fn, *a):
            ev.append((t, t, len(ev), fn, a))

        def before(d, fn, *a):
            ev.append((max([t for t in starts if t <= d], default=0) - 1, d, len(ev), fn, a))

        load = [0.0] * (total + 1000)
        tqk = {}

        def add(t0, t1, n):
            for t in range(max(t0, 0), max(t1, 0)):
                load[t] += n / (t1 - t0)

        for t, kind, k, idx in plan:
            tr = t + MXU_LAT
            if kind == 'a':
                if idx == (0, 0) and k > 0:
                    before(t - LN1 - 1, fence, t - LN1 - 40, subs[k][0] % 3)
                before(t - LN1, ln1, t - LN1, k, *idx)
                for n in range(LNS):
                    d = t - LN2 - LND * (LNS - 1 - n)
                    before(d, ln2, d, n, k, *idx)
                    add(d - 16, d, 72 // LNS)
                if LNF & 1:
                    before(t - LN3, ln3, t - LN3, k, *idx)
                    add(t - 40, t, 24)
                at(t, a_dot, t, k, *idx)
                add(tr, tr + DA, 12 * DA // 16)
                add(t - LN1 - 16, t - LN1, 32); add(t - LN2, t - 40, 20); add(t - 40, t, 36)
            elif kind == 'qk':
                at(t, b_qk, t, k, idx)
                tqk[idx] = t
                add(t - 64, t, 28); add(t, t + DQ, 28); add(tr, tr + DQ, 24); add(tr + DQ, tr + DQ + 16, 36)
            elif kind == 'pv':
                tg = max(tqk[idx] + SM0, t - SMB)
                at(t, b_pv, t, tg, k, idx)
                add(tg, tg + 4 * SMD + 16, 80); add(tr - 10, tr + 6, 46); add(tr, tr + DP, 36)
                add(t + 400, t + 460, 14)
            else:
                if idx == (0, 0) and k > 0:
                    at(t - 1, fence, t - 100, (subs[k][0] + 2) % 3)
                at(t, c_dot, t, k, *idx)
                add(tr, tr + DC, 20 * DC // 16)
                add(t - 70, t, 64)
        pre = [0.0]
        for v in load:
            pre.append(pre[-1] + v)
        nstep = NC * 2 * NT * WS
        prev_chunk = 10
        for k, sub in enumerate(subs):
            if not sub[3]:
                continue
            ta = offs[k] + (CVI if k else CV0) - 20
            tb = offs[k + 1] - (CVE if k == len(subs) - 1 else CVX)
            cap = CAP if sub[4] else 64
            free = [max(0.02, cap / 16 - (pre[t + SMO] - pre[max(t - SMO, 0)]) / (2 * SMO)) for t in range(ta, tb)]
            tot_free, acc, tstep = sum(free), 0.0, []
            for t, v in enumerate(free):
                acc += v
                while len(tstep) < nstep and acc >= (len(tstep) + 1) * tot_free / nstep - 1e-6:
                    tstep.append(ta + t)
            for n in range(nstep):
                before(tstep[n], conv_step, tstep[n], k, n // (2 * NT * WS), n // (NT * WS) % 2, n // WS % NT, n % WS)
            for c in range(NC):
                t1 = tstep[c * 2 * NT * WS] - 30
                t0 = prev_chunk + 120
                prev_chunk = t1 + 30
                for rho in range(2, NR):
                    d = t0 + (t1 - t0) * (rho - 2) // (NR - 3)
                    before(d, stage_row, d, k, c, rho)
        ev.sort(key=lambda e: e[:3])
        for e in ev:
            e[3](*e[4])
        if subs[-1][3]:
            n = len(subs)
            assert all(tag['qkv', t, r] == n - 1 for t in range(NT) for r in range(WS))
            assert all(tag['o', p] == n - 1 for p in range(n0))

    if ONLY in (0, 1):
        @pl.when(g == 0)
        def _():
            setup()
            body([(0, 2, 0, True, False)])

    @pl.when(g > 0)
    def _():
        for k in range(NSUB):
            for cp in in_copies(k, g):
                cp.wait()

    @pl.when((g > 0) & (g < ng - 1))
    def _():
        for cp in in_copies(NSUB - 1, g + 1):
            cp.start()

    @pl.when(g > 1)
    def _():
        for k in range(NSUB - 1):
            out_copy(k, g - 1).wait()

    @pl.when(g > 2)
    def _():
        out_copy(NSUB - 1, g - 2).wait()

    if ONLY in (0, 2):
        @pl.when((g > 0) & (g < ng - 1))
        def _():
            body([(1 + k, k, k, True, True) for k in range(NSUB)])

    if ONLY in (0, 3):
        @pl.when(g == ng - 1)
        def _():
            body([(1, 0, 0, False, True)])
            out_copy(NSUB - 1, g - 1).wait()
            out_copy(0, g).wait()


@jax.jit
def pallas_standalone__window_attn_davit__vision_kernel(
    x: jax.Array,
    dw_pe: jax.Array,
    w_qkv: jax.Array,
    w_o: jax.Array,
):
    B, H, W, C = x.shape
    assert B == 1 and H % WS == 0 and W % WS == 0 and C % (16 * NH) == 0
    WP = -(-(W + 1) // (2 * LANES)) * (2 * LANES)
    assert WP == 4 * LANES
    NWIN = W // WS
    NBLK = H // WS
    assert (NBLK - 1) % NSUB == 0
    NM = (NBLK - 1) // NSUB

    xt = jnp.transpose(x[0], (0, 2, 1))

    nstg = WS - 2 + NSUB * (C // 32) * 2 + 1
    kern = functools.partial(_kernel, C=C, H=H, W=W, WP=WP, NWIN=NWIN)
    out = pl.pallas_call(
        kern,
        grid=(NM + 2,),
        in_specs=[pl.BlockSpec(memory_space=pl.ANY)] * 4,
        out_specs=pl.BlockSpec(memory_space=pl.ANY),
        out_shape=jax.ShapeDtypeStruct((H, C, W), x.dtype),
        scratch_shapes=[
            pltpu.VMEM((WS + 1, C, WP), F32),
            pltpu.VMEM((WS + 1, C, WP), F32),
            pltpu.VMEM((WS + 1, C, WP), F32),
            pltpu.VMEM((WS, WP, LANES), U32),
            pltpu.VMEM((WS, WP, LANES), U32),
            pltpu.VMEM((WS, WP, LANES), U32),
            pltpu.VMEM((WS, WP, LANES), U32),
            pltpu.VMEM((2, 3 * C // 4, 2 * LANES), U32),
            pltpu.VMEM((C, 2 * LANES), U32),
            pltpu.VMEM((nstg, 3 * 8, WP), U32),
            pltpu.VMEM((nstg, 3 * 8, WP), U32),
            pltpu.VMEM((C // 8, 3, 3, 8, LANES), F32),
            pltpu.VMEM((WS + 1, C, W), BF16),
            pltpu.VMEM((WS + 1, C, W), BF16),
            pltpu.VMEM((2 * WS + 1, C, W), BF16),
            pltpu.VMEM((WS + 1, C, W), BF16),
            pltpu.VMEM((WS + 1, C, W), BF16),
            pltpu.VMEM((2 * WS + 1, C, W), BF16),
            pltpu.VMEM(dw_pe.shape, BF16),
            pltpu.VMEM(w_qkv.shape, BF16),
            pltpu.VMEM(w_o.shape, BF16),
            pltpu.SemaphoreType.DMA((2 * NSUB,)),
            pltpu.SemaphoreType.DMA((NSUB + 1,)),
            pltpu.SemaphoreType.DMA((3,)),
        ],
        compiler_params=pltpu.CompilerParams(
            dimension_semantics=("arbitrary",),
            vmem_limit_bytes=96 * 1024 * 1024,
            disable_bounds_checks=bool(NOBC),
        ),
        name="davit_window_attn",
    )(xt, dw_pe, w_qkv, w_o)
    return jnp.transpose(out, (0, 2, 1))[None]
```

```python
import functools
import math
import os

import jax
import jax.numpy as jnp
from jax import lax
import jax.experimental.pallas as pl
import jax.experimental.pallas.tpu as pltpu

WS = 7
NH = 4
EPS = 1e-05
LANES = 128
F32 = jnp.float32
BF16 = jnp.bfloat16
U32 = jnp.uint32

P = lambda k, d: int(os.environ.get(k, d))
DL_A = P('DL_A', 500)
LAT_QK = P('LAT_QK', 280)
DL_PV = P('DL_PV', 580)
PRE_C = P('PRE_C', 120)
TAIL = P('TAIL', 1000)
LN1 = P('LN1', 200)
LN2 = P('LN2', 130)
LNS = P('LNS', 3)
LND = P('LND', 16)
SM0 = P('SM0', 200)
SMD = P('SMD', 16)
SMB = P('SMB', 110)
CV0 = P('CV0', 400)
CVI = P('CVI', 170)
CVE = P('CVE', 60)
CVX = P('CVX', 200)
ORD = P('ORD', 0)
CAP = P('CAP', 42)
SMO = P('SMO', 32)
ONLY = P('ONLY', 0)
MRG = P('MRG', 0)
DL_D = P('DL_D', 100)
PVP = P('PVP', 0)
LNF = P('LNF', 3)
LN3 = P('LN3', 50)
LNG = P('LNG', 16)
NOBC = P('NOBC', 1)
DA, DC, DQ, DP = 288, 192, 56, 48
MXU_LAT = 130
NSUB = 3


def _iota(shape, dim):
    return lax.broadcasted_iota(jnp.int32, shape, dim)


def _plan(npair, n0, nt, cur, prev):
    a_q = [(t, r) for t in range(nt) for r in range(WS)] if cur else []
    c_q = [(h, r) for h in range(2) for r in range(WS)] if prev else []
    n1 = npair - n0 if prev else 0
    pairs = list(range(n0, n0 + n1)) + (list(range(n0)) if cur else [])
    total = len(a_q) * DA + len(c_q) * DC + len(pairs) * (DQ + DP)
    q0 = 0 if prev else total // 3
    t = 0
    ia = ic = iq = ip = 0
    out = []
    tq, tp, ta = {}, {}, {}
    last = None
    while ia < len(a_q) or ic < len(c_q) or ip < len(pairs):
        cands = []
        if ip < iq and t >= tq[ip] + LAT_QK:
            cands.append((-1e6, 'pv'))
        if iq < len(pairs) and (not cur or (iq - ip < 2 and last != 'qk' and not (ORD and last == 'pv'))):
            ok = iq - ip < 4
            if iq >= n1:
                need = (2 * WS * pairs[iq] + 2 * WS) // LANES * WS + WS - 1
                ok = ia > need and t >= ta[need] + DA + DL_A + 60 and ic >= len(c_q) // 2
            if ok:
                pr = q0 + iq * (total - q0 - TAIL) / len(pairs) - t - 200
                cands.append((-2e6 if ORD and pr <= 0 else pr, 'qk'))
        if ia < len(a_q):
            cands.append((ia * (total - 700) / len(a_q) - t, 'a'))
        if ic < len(c_q):
            need = 0 if ic < WS else n1 - 1
            if ip > need and t >= tp[need] + DL_PV + PRE_C:
                if cur:
                    tc = 1000 + ic * 900 if ic < WS else total - DC - (2 * WS - 1 - ic) * 950
                else:
                    tc = 1500 + ic * 400
                cands.append((tc - t, 'c'))
        if not cands:
            t += 8
            last = None
            continue
        kind = min(cands)[1]
        last = kind
        if kind == 'pv':
            tp[ip] = t; out.append((t, 'pv', pairs[ip])); ip += 1; t += DP
        elif kind == 'qk':
            tq[iq] = t; out.append((t, 'qk', pairs[iq])); iq += 1; t += DQ
        elif kind == 'a':
            ta[ia] = t; out.append((t, 'a', a_q[ia])); ia += 1; t += DA
        else:
            out.append((t, 'c', c_q[ic])); ic += 1; t += DC
    return out, t


def _tree_sum(xs):
    while len(xs) > 1:
        xs = [xs[j] + xs[j + 1] if j + 1 < len(xs) else xs[j] for j in range(0, len(xs), 2)]
    return xs[0]


def _sum8(x):
    while x.shape[0] % 16 == 0:
        x = x[:x.shape[0] // 2] + x[x.shape[0] // 2:]
    return _tree_sum(_rows8(x))


def _fold7(op, x):
    t = op(x[0:24], x[24:48])
    return op(op(t[0:8], t[8:16]), op(t[16:24], x[48:56]))


def _all8(op, x):
    for sh in (4, 2, 1):
        x = op(x, pltpu.roll(x, sh, 0))
    return x


def _rows8(x):
    return [x[8 * j:8 * j + 8] for j in range(x.shape[0] // 8)]


def _cat(xs, axis=0):
    return jnp.concatenate(xs, axis=axis) if len(xs) > 1 else xs[0]


def _f32(u):
    return pltpu.bitcast(u, F32)


def _u32(x):
    return pltpu.bitcast(x, U32)


def _kernel(x_hbm, dw_hbm, wqkv_hbm, wo_hbm, o_hbm,
            xa_s, xb_s, xc_s, q_s, k_s, v_s, o_s, wq_s, wo_s, sa_s, sb_s, dw_s,
            i0_s, i1_s, i2_s, o0_s, o1_s, o2_s, dw_ref, wqkv_ref, wo_ref, in_sem, out_sem, w_sem,
            *, C, H, W, WP, NWIN):
    g = pl.program_id(0)
    ng = pl.num_programs(0)
    dh = C // NH
    CW = C // 2
    NT = WP // LANES
    G = WS * 8
    HW = WP // 2
    NC = C // 16
    NR = WS + 2
    lane8 = _iota((8, LANES), 1)
    last_valid = W - (NT - 1) * LANES
    zero = jnp.uint32(0)
    hi = jnp.uint32(0xFFFF0000)
    qkv_s = (q_s, k_s, v_s)
    xbuf = (xa_s, xb_s, xc_s)
    xin = (i0_s, i1_s, i2_s)
    xout = (o0_s, o1_s, o2_s)

    def row0(k, m):
        return (m & 1) * WS if k == NSUB - 1 else 0

    def in_copies(k, m):
        r = WS * (NSUB * m - 1 + k) + 1
        return [pltpu.make_async_copy(x_hbm.at[pl.ds(jnp.minimum(r + o, H - n), n)],
                                      xin[k].at[pl.ds(row0(k, m) + o, n)], in_sem.at[2 * k + e])
                for e, (o, n) in enumerate(((0, WS - 1), (WS - 1, 1)))]

    def out_copy(k, m, o=0, n=WS):
        return pltpu.make_async_copy(xout[k].at[pl.ds(row0(k, m) + o, n)],
                                     o_hbm.at[pl.ds(WS * (NSUB * (m - 1) + k) + o, n)],
                                     out_sem.at[k + (m & 1) if k == NSUB - 1 else k])

    stg = (sa_s, sb_s)
    SPARE = sa_s.shape[0] - 1
    zx = g >> 10
    zy = g >> 11
    never = lane8 < zx

    def tie(x, toks):
        if not toks:
            return x
        tok = functools.reduce(lax.bitwise_or, toks)
        n = x.shape[1]
        return lax.select(never[:, 0:n], tok[:, 0:n], x) if n < LANES else lax.select(never, tok, x)

    def stg_row(j, c2, rho):
        if 2 <= rho < WS:
            return rho - 2
        slot = j % NSUB if rho >= WS else (j - 1) % NSUB
        return WS - 2 + (slot * (NC // 2) + c2) * 2 + rho % WS

    zt = jnp.zeros((8, LANES), U32)
    is_first, is_last = lane8 == 0, lane8 == LANES - 1

    def shifted(u):
        tiles = [u[:, LANES * t:LANES * (t + 1)] for t in range(NT)]
        tiles[NT - 1] = _cat([tiles[NT - 1], zt[:, last_valid:]], axis=1)
        left = [pltpu.roll(lax.select(is_last, tiles[t - 1] if t > 0 else zt, tiles[t]), 1, 1)
                for t in range(NT)]
        right = [pltpu.roll(lax.select(is_first, tiles[t + 1], tiles[t]) if t < NT - 1 else tiles[t], LANES - 1, 1)
                 for t in range(NT)]
        return _cat([v[t] for t in range(NT) for v in (left, tiles, right)])

    def unpack(v, hf):
        return pltpu.bitcast(v, BF16).astype(F32).reshape(3, 2, 8, LANES)[:, hf]

    def conv_row(un, w, r):
        return jnp.sum(_tree_sum([un[r + ki] * w[ki] for ki in range(3) if un[r + ki] is not None]), axis=0)

    def setup():
        wcp = [pltpu.make_async_copy(src, dst, w_sem.at[n])
               for n, (src, dst) in enumerate(((wqkv_hbm, wqkv_ref), (wo_hbm, wo_ref), (dw_hbm, dw_ref)))]
        top = [pltpu.make_async_copy(x_hbm.at[pl.ds(0, 1)], i0_s.at[pl.ds(0, 1)], in_sem.at[1])] + in_copies(1, 0)
        for cp in wcp + top + in_copies(2, 0):
            cp.start()

        def zrow(r, carry):
            rs = pl.ds(pl.multiple_of(r % 4 * LANES, LANES), LANES)
            for ref in (q_s, k_s, v_s, o_s):
                ref[r // 4, rs, :] = jnp.zeros((LANES, LANES), U32)
            return carry
        lax.fori_loop(0, WS * NT, zrow, 0)
        for ref in stg:
            ref[SPARE] = jnp.zeros(ref.shape[1:], U32)

        for ref in xin + xout:
            ref[ref.shape[0] - 1, 0:16, 0:LANES] = jnp.zeros((16, LANES), BF16)
        for cp in wcp:
            cp.wait()
        qscale = (dh ** -0.5) * math.log2(math.e)
        wt = wqkv_ref[...].astype(F32).T
        wq = (wt[0:C] * qscale).astype(BF16).astype(F32)
        words = [(_u32(w[0:CW]) >> 16) | (_u32(w[CW:C]) & hi) for w in (wq, wt[C:2 * C])]
        words = _rows8(_cat(words + [_u32(wt[2 * C:].astype(BF16))]))
        for par in range(2):
            wpar = _cat(words[par::2])
            wq_s[par, :, 0:CW] = wpar[:, 0:CW]
            wq_s[par, :, LANES:LANES + CW] = wpar[:, CW:C]
        wo = _u32(wo_ref[...])
        wo_s[...] = jnp.zeros(wo_s.shape, U32)
        wo_s[:, 0:CW] = (wo << 16).T
        wo_s[:, LANES:LANES + CW] = (wo & hi).T

        def taps(ki, carry):
            w3 = dw_ref[ki].astype(F32)
            for kj in range(3):
                w = w3[kj:kj + 1]
                if kj == 1:
                    w = w + jnp.where(ki == 1, 1.0, 0.0)
                dw_s[:, ki, kj] = jnp.broadcast_to(w, (LANES, C)).T.reshape(C // 8, 8, LANES)
            return carry
        lax.fori_loop(0, 3, taps, 0)

        for cp in top:
            cp.wait()

        def conv0(c2, carry):
            for par in range(2):
                cs = pl.ds(pl.multiple_of(32 * c2 + 16 * par, 16), 16)
                sh = [shifted(_u32(i0_s[0, cs, :]))] + [shifted(_u32(i1_s[r, cs, :])) for r in range(WS)]
                for rho in (WS, WS + 1):
                    stg[par][stg_row(-1, c2, rho)] = sh[rho - 1]
                for hf in range(2):
                    c8 = 4 * c2 + 2 * par + hf
                    w = [dw_s[c8, ki] for ki in range(3)]
                    for t in range(NT):
                        un = [None] + [unpack(row[24 * t:24 * t + 24], hf) for row in sh]
                        for r in range(WS):
                            xbuf[0][r, t, pl.ds(pl.multiple_of(8 * c8, 8), 8), :] = conv_row(un, w, r)
            return carry
        lax.fori_loop(0, NC // 2, conv0, 0)
        for cp in in_copies(0, 1) + in_copies(1, 1):
            cp.start()
        for cp in in_copies(2, 0):
            cp.wait()
        for cp in in_copies(2, 1):
            cp.start()

    def body(subs):
        lane3 = _iota((WS, 8, LANES), 2)
        head = (lane3 < dh, (lane3 >= dh) & (lane3 < 2 * dh))
        zq = jnp.zeros((WS, 8, LANES), F32)
        junk8 = _iota((8, 2 * G), 0) == WS
        ninf8 = jnp.full((8, 2 * G), -jnp.inf, F32)
        ngr = WS + PVP
        key_ok = tuple((_iota((ngr, 8, 2 * G), 2) & 8) == 8 * hh for hh in range(2))
        sub1 = (_iota((8, 2 * G), 0) & 1) == 0
        sub2 = (_iota((8, 2 * G), 0) & 2) == 0
        zp = jnp.zeros((ngr, 8, 2 * G), F32)
        first_half = (_iota((8, 2 * G), 1) & 8) == 0
        even_head = (_iota((WS, 8, CW), 2) // (dh // 2)) % 2 == 0
        npair = (NWIN + 1) // 2
        n0 = (HW - 1) // WS // 2

        st = {}
        toks = []
        soft = []
        ticks = []
        j0 = subs[0][0]
        tag = {('qkv', t, r): -1 for t in range(NT) for r in range(WS)}
        tag.update({('o', p): (-1 if p < n0 else None) for p in range(npair)})
        for b, blk in ((j0 % 3, 0), ((j0 + 2) % 3, -1)):
            tag.update({('x', b, c, t, r): blk for c in range(2 * NC) for t in range(NT) for r in range(WS)})
        tag.update({('s', c % 2, stg_row(j0, c // 2, rho)): (0, c, rho) for c in range(NC) for rho in (0, 1)})

        def gather(ref, w):
            return ref[:, pl.ds(WS * w, 8), :]

        def tick(t):
            c = [x for x in ticks if t <= x[0] <= t + 40]
            if not c:
                return None
            _, res, j = min(c, key=lambda x: x[0])
            return res[8 * j:8 * j + 8, 0:LANES]

        def due(lst, nblk, t0, step):
            inj = {}
            for d, tok in list(lst):
                j = max(0, -(-(d - t0) // step))
                if j < nblk:
                    inj.setdefault(j, []).append(tok)
            lst[:] = [x for x in lst if x[0] > t0 + (nblk - 1) * step]
            return inj

        def lhs(ref, ls, inj, dt):
            nblk = ref.shape[0] // 8
            parts, s = [], 0
            for j in sorted(inj):
                if j > s:
                    parts.append(ref[8 * s:8 * j, ls])
                parts.append(tie(ref[8 * j:8 * j + 8, ls], inj[j]))
                s = j + 1
            if s < nblk:
                parts.append(ref[8 * s:8 * nblk, ls])
            return pltpu.bitcast(_cat(parts), dt)

        def merged(a, b):
            return {j: a.get(j, []) + b.get(j, []) for j in set(a) | set(b)}

        def fence(d, b):
            c = [x for x in ticks if x[0] <= d]
            if c:
                _, res, j = max(c, key=lambda x: x[0])
                xbuf[b][zx + WS, 0, 0:8, :] = res[8 * j:8 * j + 8, 0:LANES]

        def ln1(d, k, t, r):
            b = subs[k][0] % 3
            assert all(tag['x', b, c, t, r] == k for c in range(2 * NC))
            x0 = xbuf[b][r, t, 0:C, :]
            s8 = _sum8(x0)
            soft.append((d, _u32(s8)))
            mean = jnp.sum(s8, axis=0, keepdims=True) * (1.0 / C)
            if LNF & 2:
                fence(d + LNG, b)
                x0 = xbuf[b][r, t, 0:C, :]
            st['ln', k, t, r] = [x0 - mean, [], mean]

        def ln3(d, k, t, r):
            b = subs[k][0] % 3
            fence(d, b)
            st['ln', k, t, r][0] = xbuf[b][r, t, 0:C, :] - st['ln', k, t, r][2]

        def ln2(d, n, *key):
            m = C // LNS
            xc = st[('ln',) + key][0][m * n:m * (n + 1)]
            s8 = _sum8(xc * xc)
            soft.append((d, _u32(s8)))
            st[('ln',) + key][1].append(s8)

        def a_dot(t0, k, t, r):
            xc, sq, _ = st.pop(('ln', k, t, r))
            var = jnp.sum(_tree_sum(sq), axis=0, keepdims=True) * (1.0 / C)
            h = xc * lax.rsqrt(var + EPS)
            h = [h[CW * kt:CW * (kt + 1)].astype(BF16) for kt in range(2)]
            inj = due(toks, DA // 16, t0, 16)
            inj0 = merged(inj, due(soft, DA // 16, t0, 16))
            part = [jnp.dot(lhs(wq_s.at[par], slice(LANES * kt, LANES * kt + CW), inj if par or kt else inj0, BF16),
                            h[kt], preferred_element_type=F32)
                    for par in range(2) for kt in range(2)]
            res = [part[0] + part[1], part[2] + part[3]]
            ticks.extend((t0 + MXU_LAT + 8 * j, res[0], j) for j in range(DA // 8))
            qkv = jnp.stack([v.reshape(-1, 16, LANES) for v in res], axis=1).reshape(3 * C, LANES)
            for m in range(3):
                qkv_s[m][r, LANES * t:LANES * (t + 1), 0:CW] = _u32(qkv[C * m:C * (m + 1)].astype(BF16)).T
                toks.append((t0 + 96 * (m + 1) + DL_A, qkv_s[m][zx, 0:8, :]))
            tag['qkv', t, r] = k

        def wins(p):
            return 2 * p, min(2 * p + 1, NWIN - 1)

        def b_qk(t0, k, p):
            wa, wb = wins(p)
            blk = k if p < n0 else k - 1
            assert all(tag['qkv', t, r] == blk for r in range(WS)
                       for t in range(WS * wa // LANES, (WS * wb + WS) // LANES + 1))
            sts = []
            inj = due(soft, WS, t0, 8)
            for w, swap in ((wa, 0), (wb, 1)):
                qw = gather(q_s, w)
                kw = gather(k_s, w).reshape(G, LANES)
                if not swap and inj:
                    kw = _cat([tie(v, inj.get(r, [])) for r, v in enumerate(_rows8(kw))])
                for tile in range(2):
                    kk = _f32(kw & hi if tile else kw << 16)
                    qq = _f32(qw & hi if tile else qw << 16)
                    qst = jnp.stack([lax.select(head[swap], qq, zq), lax.select(head[1 - swap], qq, zq)], axis=1)
                    sts.append(lax.dot_general(kk, qst.reshape(2 * G, LANES), (((1,), (1,)), ((), ())),
                                               preferred_element_type=F32))
            if PVP:
                vw = _cat([gather(v_s, wa), zt[None], gather(v_s, wb), zt[None]]).reshape(LANES, LANES)
            else:
                vw = _cat([gather(v_s, wa), gather(v_s, wb)]).reshape(2 * G, LANES)
            st['s', p] = (sts, pltpu.bitcast(vw[:, 0:CW].T, BF16))

        def b_pv(t0, tg, k, p):
            wa, wb = wins(p)
            sts, vt = st.pop(('s', p))
            pts = []
            dens = []
            for n, s_t in enumerate(sts):
                m8 = _fold7(jnp.maximum, s_t)
                mx = _all8(jnp.maximum, lax.select(junk8, ninf8, m8))
                mv = lax.select(junk8, -ninf8, mx)
                z = tick(tg + SMD * (3 - n))
                if z is not None:
                    mv = tie(mv, [z])
                eg = jnp.exp2(s_t.reshape(WS, 8, 2 * G) - mv)
                dens.append(_fold7(jnp.add, eg.reshape(G, 2 * G)))
                pts.append(_cat([eg, eg[WS - 1:WS]]) if PVP else eg)
            if MRG:
                def mix(m, sh, a, b):
                    return lax.select(m, a, b) + pltpu.roll(lax.select(m, b, a), sh, 0)
                den = mix(sub2, 2, mix(sub1, 1, dens[0], dens[1]), mix(sub1, 1, dens[2], dens[3]))
                den = den + pltpu.roll(den, 4, 0)
                r0 = pl.reciprocal(den, approx=True)
                r0 = r0 * (2.0 - den * r0)
                r0 = lax.select(first_half, r0, pltpu.roll(r0, 2, 0))
                rsel = [jnp.broadcast_to(r0[n:n + 1], r0.shape) for n in range(4)]
            else:
                rinv = []
                for den in dens:
                    den = _all8(jnp.add, den)
                    r0 = pl.reciprocal(den, approx=True)
                    rinv.append(r0 * (2.0 - den * r0))
                rsel = [lax.select(first_half, rinv[n], rinv[(n + 2) % 4]) for n in range(4)]
            outs = []
            for tile in range(2):
                for hh in range(2):
                    h = 2 * tile + hh
                    stn = _cat([lax.select(key_ok[hh], pts[tile], zp), lax.select(key_ok[1 - hh], pts[2 + tile], zp)])
                    ot = jnp.dot(vt[dh * h:dh * (h + 1), :], stn.reshape(-1, 2 * G).astype(BF16),
                                 preferred_element_type=F32)
                    outs.append(ot.reshape(dh // 8, 8, 2 * G) * rsel[2 * hh + tile])
            tw = _u32(_cat(outs).reshape(C, 2 * G).astype(BF16)).T.reshape(WS, 2, 8, CW)
            tw = (tw[:, 0], tw[:, 1])
            o_s[:, pl.ds(WS * wa, 8), 0:CW] = lax.select(even_head, tw[0], tw[1])
            if wb != wa:
                o_s[:, pl.ds(WS * wb, 8), 0:CW] = lax.select(even_head, tw[1], tw[0])
                tag['o', p + 1] = None
            toks.append((t0 + DL_PV, o_s[zx, 0:8, :]))
            tag['o', p] = k if p < n0 else k - 1
            if p == n0:
                tag['o2'] = k - 1

        def c_dot(t0, k, h, r):
            b = (subs[k][0] + 2) % 3
            assert all(tag['o', p] == k - 1 for p in (range(n0 + 1) if h == 0 else range(n0 + 1, npair)))
            assert tag['o2'] == k - 1 and 2 * WS * n0 < HW
            assert all(tag['x', b, c, t, r] == k - 1 for c in range(2 * NC) for t in (2 * h, 2 * h + 1))
            ls = slice(HW * h, HW * (h + 1))
            ow = o_s[r, ls, :]
            rhs = _cat([_f32(ow << 16), _f32(ow & hi)], axis=1)
            inj = due(toks, DC // 8, t0, 8)
            wo = _cat([lhs(wo_s, slice(0, LANES), merged(inj, due(soft, DC // 8, t0, 8)), F32),
                       lhs(wo_s, slice(LANES, 2 * LANES), inj, F32)], axis=1)
            res = lax.dot_general(wo, rhs, (((1,), (1,)), ((), ())), preferred_element_type=F32)
            ticks.extend((t0 + MXU_LAT + 8 * j, res, j) for j in range(DC // 8))
            slot = subs[k][2]
            n = min(HW, W - HW * h)
            xout[slot][row0(slot, g) + r, :, HW * h:HW * h + n] = (_cat([xbuf[b][r, t, 0:C, :] for t in (2 * h, 2 * h + 1)], axis=1) + res)[:, 0:n].astype(BF16)
            if h == 1 and not subs[k][3]:
                out_copy(slot, g, r, 1).start()
            elif h == 1 and r == WS - 1:
                out_copy(slot, g).start()
                xout[slot][zx + xout[slot].shape[0] - 1, 0:16, 0:LANES] = jnp.zeros((16, LANES), BF16)
                soft.append((t0 + MXU_LAT + DC + DL_D, _u32(xout[slot][zy + xout[slot].shape[0] - 1, 0:16, 0:LANES])))

        def stage_row(d, k, c, rho):
            j, slot = subs[k][0:2]
            cs = slice(16 * c, 16 * c + 16)
            u = _u32(xin[slot][row0(slot, g) + rho - 2, cs, :])
            if rho == WS + 1 and slot == 1:
                u = jnp.where(g < ng - 2, u, zero)
            idx = stg_row(j, c // 2, rho)
            stg[c % 2][idx] = shifted(u)
            soft.append((d, stg[c % 2][zx + SPARE, 8:16, 0:LANES]))
            tag['s', c % 2, idx] = (k, c, rho)
            if c == NC - 1 and rho == WS + 1 and slot < NSUB - 1:
                for cp in in_copies(slot, g + 1):
                    cp.start()
                xin[slot][zx + WS, 0:16, 0:LANES] = jnp.zeros((16, LANES), BF16)
                soft.append((d + DL_D, _u32(xin[slot][zy + WS, 0:16, 0:LANES])))

        def conv_step(d, k, c, hf, t, r):
            j = subs[k][0]
            if r == 0:
                if t == 0:
                    stg[c % 2][zx + SPARE, 0:8, 0:LANES] = zt
                    st['w'] = [dw_s[2 * c + hf, ki] for ki in range(3)]
                st['un'] = {}
            un = st['un']
            for rho in range(r, r + 3):
                if rho not in un:
                    idx = stg_row(j, c // 2, rho)
                    assert tag['s', c % 2, idx] in ((k, c, rho), (k - 1, c, rho + WS))
                    un[rho] = unpack(stg[c % 2][idx, 24 * t:24 * t + 24, :], hf)
            acc = conv_row(un, st['w'], r)
            xbuf[(j + 1) % 3][r, t, 16 * c + 8 * hf:16 * c + 8 * hf + 8, :] = acc
            soft.append((d, _u32(acc)))
            tag['x', (j + 1) % 3, 2 * c + hf, t, r] = k + 1

        plan, offs = [], [0]
        for k, sub in enumerate(subs):
            pk, tk = _plan(npair, n0, NT, sub[3], sub[4])
            plan += [(offs[k] + t, kind, k, idx) for t, kind, idx in pk]
            offs.append(offs[k] + tk)
        total = offs[-1]
        starts = [e[0] for e in plan]
        ev = []

        def at(t, fn, *a):
            ev.append((t, t, len(ev), fn, a))

        def before(d, fn, *a):
            ev.append((max([t for t in starts if t <= d], default=0) - 1, d, len(ev), fn, a))

        load = [0.0] * (total + 1000)
        tqk = {}

        def add(t0, t1, n):
            for t in range(max(t0, 0), max(t1, 0)):
                load[t] += n / (t1 - t0)

        for t, kind, k, idx in plan:
            tr = t + MXU_LAT
            if kind == 'a':
                if idx == (0, 0) and k > 0:
                    before(t - LN1 - 1, fence, t - LN1 - 40, subs[k][0] % 3)
                before(t - LN1, ln1, t - LN1, k, *idx)
                for n in range(LNS):
                    d = t - LN2 - LND * (LNS - 1 - n)
                    before(d, ln2, d, n, k, *idx)
                    add(d - 16, d, 72 // LNS)
                if LNF & 1:
                    before(t - LN3, ln3, t - LN3, k, *idx)
                    add(t - 40, t, 24)
                at(t, a_dot, t, k, *idx)
                add(tr, tr + DA, 12 * DA // 16)
                add(t - LN1 - 16, t - LN1, 32); add(t - LN2, t - 40, 20); add(t - 40, t, 36)
            elif kind == 'qk':
                at(t, b_qk, t, k, idx)
                tqk[idx] = t
                add(t - 64, t, 28); add(t, t + DQ, 28); add(tr, tr + DQ, 24); add(tr + DQ, tr + DQ + 16, 36)
            elif kind == 'pv':
                tg = max(tqk[idx] + SM0, t - SMB)
                at(t, b_pv, t, tg, k, idx)
                add(tg, tg + 4 * SMD + 16, 80); add(tr - 10, tr + 6, 46); add(tr, tr + DP, 36)
                add(t + 400, t + 460, 14)
            else:
                if idx == (0, 0) and k > 0:
                    at(t - 1, fence, t - 100, (subs[k][0] + 2) % 3)
                at(t, c_dot, t, k, *idx)
                add(tr, tr + DC, 20 * DC // 16)
                add(t - 70, t, 64)
        pre = [0.0]
        for v in load:
            pre.append(pre[-1] + v)
        nstep = NC * 2 * NT * WS
        prev_chunk = 10
        for k, sub in enumerate(subs):
            if not sub[3]:
                continue
            ta = offs[k] + (CVI if k else CV0) - 20
            tb = offs[k + 1] - (CVE if k == len(subs) - 1 else CVX)
            cap = CAP if sub[4] else 64
            free = [max(0.02, cap / 16 - (pre[t + SMO] - pre[max(t - SMO, 0)]) / (2 * SMO)) for t in range(ta, tb)]
            tot_free, acc, tstep = sum(free), 0.0, []
            for t, v in enumerate(free):
                acc += v
                while len(tstep) < nstep and acc >= (len(tstep) + 1) * tot_free / nstep - 1e-6:
                    tstep.append(ta + t)
            for n in range(nstep):
                before(tstep[n], conv_step, tstep[n], k, n // (2 * NT * WS), n // (NT * WS) % 2, n // WS % NT, n % WS)
            for c in range(NC):
                t1 = tstep[c * 2 * NT * WS] - 30
                t0 = prev_chunk + 120
                prev_chunk = t1 + 30
                for rho in range(2, NR):
                    d = t0 + (t1 - t0) * (rho - 2) // (NR - 3)
                    before(d, stage_row, d, k, c, rho)
        ev.sort(key=lambda e: e[:3])
        for e in ev:
            e[3](*e[4])
        if subs[-1][3]:
            n = len(subs)
            assert all(tag['qkv', t, r] == n - 1 for t in range(NT) for r in range(WS))
            assert all(tag['o', p] == n - 1 for p in range(n0))

    if ONLY in (0, 1):
        @pl.when(g == 0)
        def _():
            setup()
            body([(0, 2, 0, True, False)])

    @pl.when(g > 0)
    def _():
        for k in range(NSUB):
            for cp in in_copies(k, g):
                cp.wait()

    @pl.when((g > 0) & (g < ng - 1))
    def _():
        for cp in in_copies(NSUB - 1, g + 1):
            cp.start()

    @pl.when(g > 1)
    def _():
        for k in range(NSUB - 1):
            out_copy(k, g - 1).wait()

    @pl.when(g > 2)
    def _():
        out_copy(NSUB - 1, g - 2).wait()

    if ONLY in (0, 2):
        @pl.when((g > 0) & (g < ng - 1))
        def _():
            body([(1 + k, k, k, True, True) for k in range(NSUB)])

    if ONLY in (0, 3):
        @pl.when(g == ng - 1)
        def _():
            body([(1, 0, 0, False, True)])
            out_copy(NSUB - 1, g - 1).wait()
            out_copy(0, g).wait()


@jax.jit
def pallas_standalone__window_attn_davit__vision_kernel(
    x: jax.Array,
    dw_pe: jax.Array,
    w_qkv: jax.Array,
    w_o: jax.Array,
):
    B, H, W, C = x.shape
    assert B == 1 and H % WS == 0 and W % WS == 0 and C % (16 * NH) == 0
    WP = -(-(W + 1) // (2 * LANES)) * (2 * LANES)
    assert WP == 4 * LANES
    NWIN = W // WS
    NBLK = H // WS
    assert (NBLK - 1) % NSUB == 0
    NM = (NBLK - 1) // NSUB

    xt = jnp.transpose(x[0], (0, 2, 1))

    nstg = WS - 2 + NSUB * (C // 32) * 2 + 1
    kern = functools.partial(_kernel, C=C, H=H, W=W, WP=WP, NWIN=NWIN)
    out = pl.pallas_call(
        kern,
        grid=(NM + 2,),
        in_specs=[pl.BlockSpec(memory_space=pl.ANY)] * 4,
        out_specs=pl.BlockSpec(memory_space=pl.ANY),
        out_shape=jax.ShapeDtypeStruct((H, C, W), x.dtype),
        scratch_shapes=[
            pltpu.VMEM((WS + 1, WP // LANES, C + 8, LANES), F32),
            pltpu.VMEM((WS + 1, WP // LANES, C + 8, LANES), F32),
            pltpu.VMEM((WS + 1, WP // LANES, C + 8, LANES), F32),
            pltpu.VMEM((WS, WP + 8, LANES), U32),
            pltpu.VMEM((WS, WP + 8, LANES), U32),
            pltpu.VMEM((WS, WP + 8, LANES), U32),
            pltpu.VMEM((WS, WP + 8, LANES), U32),
            pltpu.VMEM((2, 3 * C // 4, 2 * LANES), U32),
            pltpu.VMEM((C, 2 * LANES), U32),
            pltpu.VMEM((nstg, WP // LANES * 24, LANES), U32),
            pltpu.VMEM((nstg, WP // LANES * 24, LANES), U32),
            pltpu.VMEM((C // 8, 3, 3, 8, LANES), F32),
            pltpu.VMEM((WS + 1, C, W), BF16),
            pltpu.VMEM((WS + 1, C, W), BF16),
            pltpu.VMEM((2 * WS + 1, C, W), BF16),
            pltpu.VMEM((WS + 1, C, W), BF16),
            pltpu.VMEM((WS + 1, C, W), BF16),
            pltpu.VMEM((2 * WS + 1, C, W), BF16),
            pltpu.VMEM(dw_pe.shape, BF16),
            pltpu.VMEM(w_qkv.shape, BF16),
            pltpu.VMEM(w_o.shape, BF16),
            pltpu.SemaphoreType.DMA((2 * NSUB,)),
            pltpu.SemaphoreType.DMA((NSUB + 1,)),
            pltpu.SemaphoreType.DMA((3,)),
        ],
        compiler_params=pltpu.CompilerParams(
            dimension_semantics=("arbitrary",),
            vmem_limit_bytes=96 * 1024 * 1024,
            disable_bounds_checks=bool(NOBC),
        ),
        name="davit_window_attn",
    )(xt, dw_pe, w_qkv, w_o)
    return jnp.transpose(out, (0, 2, 1))[None]
```

```python
import functools
import math
import os

import jax
import jax.numpy as jnp
from jax import lax
import jax.experimental.pallas as pl
import jax.experimental.pallas.tpu as pltpu

WS = 7
NH = 4
EPS = 1e-05
LANES = 128
F32 = jnp.float32
BF16 = jnp.bfloat16
U32 = jnp.uint32

P = lambda k, d: int(os.environ.get(k, d))
DL_A = P('DL_A', 500)
LAT_QK = P('LAT_QK', 280)
DL_PV = P('DL_PV', 580)
PRE_C = P('PRE_C', 120)
TAIL = P('TAIL', 1000)
LN1 = P('LN1', 200)
LN2 = P('LN2', 130)
LNS = P('LNS', 3)
LND = P('LND', 16)
SM0 = P('SM0', 200)
SMD = P('SMD', 16)
SMB = P('SMB', 110)
CV0 = P('CV0', 400)
CVI = P('CVI', 170)
CVE = P('CVE', 60)
CVX = P('CVX', 180)
ORD = P('ORD', 0)
CAP = P('CAP', 42)
SMO = P('SMO', 32)
ONLY = P('ONLY', 0)
ZK = P('ZK', 0)
EC0 = P('EC0', 1500)
ECD = P('ECD', 900)
PVI = P('PVI', 1)
SST = P('SST', 0)
VST = P('VST', 1)
VDL = P('VDL', 60)
MRG = P('MRG', 0)
DL_D = P('DL_D', 100)
PVP = P('PVP', 0)
LNF = P('LNF', 3)
LN3 = P('LN3', 50)
LNG = P('LNG', 16)
NOBC = P('NOBC', 1)
DA, DC, DQ, DP = 288, 192, 56, 48
MXU_LAT = 130
NSUB = 3


def _iota(shape, dim):
    return lax.broadcasted_iota(jnp.int32, shape, dim)


def _plan(npair, n0, nt, cur, prev):
    a_q = [(t, r) for t in range(nt) for r in range(WS)] if cur else []
    c_q = [(h, r) for h in range(2) for r in range(WS)] if prev else []
    n1 = npair - n0 if prev else 0
    pairs = list(range(n0, n0 + n1)) + (list(range(n0)) if cur else [])
    total = len(a_q) * DA + len(c_q) * DC + len(pairs) * (DQ + DP)
    q0 = 0 if prev else total // 3
    t = 0
    ia = ic = iq = ip = 0
    out = []
    tq, tp, ta = {}, {}, {}
    last = None
    while ia < len(a_q) or ic < len(c_q) or ip < len(pairs):
        cands = []
        if ip < iq and t >= tq[ip] + LAT_QK:
            cands.append((-1e6, 'pv'))
        if iq < len(pairs) and (not cur or (iq - ip < 2 and last != 'qk' and not (ORD and last == 'pv'))):
            ok = iq - ip < 4
            if iq >= n1:
                need = (2 * WS * pairs[iq] + 2 * WS) // LANES * WS + WS - 1
                ok = ia > need and t >= ta[need] + DA + DL_A + 60 and ic >= len(c_q) // 2
            if ok:
                pr = q0 + iq * (total - q0 - TAIL) / len(pairs) - t - 200
                cands.append((-2e6 if ORD and pr <= 0 else pr, 'qk'))
        if ia < len(a_q):
            cands.append((ia * (total - 700) / len(a_q) - t, 'a'))
        if ic < len(c_q):
            need = 0 if ic < WS else n1 - 1
            if ip > need and t >= tp[need] + DL_PV + PRE_C:
                if cur:
                    tc = 1000 + ic * 900 if ic < WS else total - DC - (2 * WS - 1 - ic) * 950
                else:
                    tc = EC0 + ic * ECD
                cands.append((tc - t, 'c'))
        if not cands:
            t += 8
            last = None
            continue
        kind = min(cands)[1]
        last = kind
        if kind == 'pv':
            tp[ip] = t; out.append((t, 'pv', pairs[ip])); ip += 1; t += DP
        elif kind == 'qk':
            tq[iq] = t; out.append((t, 'qk', pairs[iq])); iq += 1; t += DQ
        elif kind == 'a':
            ta[ia] = t; out.append((t, 'a', a_q[ia])); ia += 1; t += DA
        else:
            out.append((t, 'c', c_q[ic])); ic += 1; t += DC
    return out, t


def _tree_sum(xs):
    while len(xs) > 1:
        xs = [xs[j] + xs[j + 1] if j + 1 < len(xs) else xs[j] for j in range(0, len(xs), 2)]
    return xs[0]


def _sum8(x):
    while x.shape[0] % 16 == 0:
        x = x[:x.shape[0] // 2] + x[x.shape[0] // 2:]
    return _tree_sum(_rows8(x))


def _fold7(op, x):
    t = op(x[0:24], x[24:48])
    return op(op(t[0:8], t[8:16]), op(t[16:24], x[48:56]))


def _all8(op, x):
    for sh in (4, 2, 1):
        x = op(x, pltpu.roll(x, sh, 0))
    return x


def _rows8(x):
    return [x[8 * j:8 * j + 8] for j in range(x.shape[0] // 8)]


def _cat(xs, axis=0):
    return jnp.concatenate(xs, axis=axis) if len(xs) > 1 else xs[0]


def _f32(u):
    return pltpu.bitcast(u, F32)


def _u32(x):
    return pltpu.bitcast(x, U32)


def _kernel(x_hbm, dw_hbm, wqkv_hbm, wo_hbm, o_hbm,
            xa_s, xb_s, xc_s, q_s, k_s, v_s, o_s, wq_s, wo_s, sa_s, sb_s, dw_s,
            i0_s, i1_s, i2_s, o0_s, o1_s, o2_s, va_s, vb_s, vc_s, vd_s, ta_s, tb_s, tc_s, td_s, dw_ref, wqkv_ref, wo_ref, in_sem, out_sem, w_sem,
            *, C, H, W, WP, NWIN):
    g = pl.program_id(0)
    ng = pl.num_programs(0)
    dh = C // NH
    CW = C // 2
    NT = WP // LANES
    G = WS * 8
    HW = WP // 2
    NC = C // 16
    NR = WS + 2
    lane8 = _iota((8, LANES), 1)
    last_valid = W - (NT - 1) * LANES
    zero = jnp.uint32(0)
    hi = jnp.uint32(0xFFFF0000)
    qkv_s = (q_s, k_s, v_s)
    xbuf = (xa_s, xb_s, xc_s)
    xin = (i0_s, i1_s, i2_s)
    xout = (o0_s, o1_s, o2_s)

    def row0(k, m):
        return (m & 1) * WS if k == NSUB - 1 else 0

    def in_copies(k, m):
        r = WS * (NSUB * m - 1 + k) + 1
        return [pltpu.make_async_copy(x_hbm.at[pl.ds(jnp.minimum(r + o, H - n), n)],
                                      xin[k].at[pl.ds(row0(k, m) + o, n)], in_sem.at[2 * k + e])
                for e, (o, n) in enumerate(((0, WS - 1), (WS - 1, 1)))]

    def out_copy(k, m, o=0, n=WS):
        return pltpu.make_async_copy(xout[k].at[pl.ds(row0(k, m) + o, n)],
                                     o_hbm.at[pl.ds(WS * (NSUB * (m - 1) + k) + o, n)],
                                     out_sem.at[k + (m & 1) if k == NSUB - 1 else k])

    stg = (sa_s, sb_s)
    vts = (va_s, vb_s, vc_s, vd_s)
    sts_s = (ta_s, tb_s, tc_s, td_s)
    SPARE = sa_s.shape[0] - 1
    zx = g >> 10
    zy = g >> 11
    never = lane8 < zx

    def tie(x, toks):
        if not toks:
            return x
        tok = functools.reduce(lax.bitwise_or, toks)
        n = x.shape[1]
        return lax.select(never[:, 0:n], tok[:, 0:n], x) if n < LANES else lax.select(never, tok, x)

    def stg_row(j, c2, rho):
        if 2 <= rho < WS:
            return rho - 2
        slot = j % NSUB if rho >= WS else (j - 1) % NSUB
        return WS - 2 + (slot * (NC // 2) + c2) * 2 + rho % WS

    zt = jnp.zeros((8, LANES), U32)
    is_first, is_last = lane8 == 0, lane8 == LANES - 1

    def shifted(u):
        tiles = [u[:, LANES * t:LANES * (t + 1)] for t in range(NT)]
        tiles[NT - 1] = _cat([tiles[NT - 1], zt[:, last_valid:]], axis=1)
        left = [pltpu.roll(lax.select(is_last, tiles[t - 1] if t > 0 else zt, tiles[t]), 1, 1)
                for t in range(NT)]
        right = [pltpu.roll(lax.select(is_first, tiles[t + 1], tiles[t]) if t < NT - 1 else tiles[t], LANES - 1, 1)
                 for t in range(NT)]
        return _cat([v[t] for t in range(NT) for v in (left, tiles, right)])

    def unpack(v, hf):
        return pltpu.bitcast(v, BF16).astype(F32).reshape(3, 2, 8, LANES)[:, hf]

    def conv_row(un, w, r):
        return jnp.sum(_tree_sum([un[r + ki] * w[ki] for ki in range(3) if un[r + ki] is not None]), axis=0)

    def setup():
        wcp = [pltpu.make_async_copy(src, dst, w_sem.at[n])
               for n, (src, dst) in enumerate(((dw_hbm, dw_ref), (wqkv_hbm, wqkv_ref), (wo_hbm, wo_ref)))]
        top = [pltpu.make_async_copy(x_hbm.at[pl.ds(0, 1)], i0_s.at[pl.ds(0, 1)], in_sem.at[1])] + in_copies(1, 0)
        for cp in wcp + top + in_copies(2, 0):
            cp.start()

        def zrow(r, carry):
            for ref in ((k_s, o_s) if ZK else (q_s, k_s, v_s, o_s)):
                ref[r, 0:WP, :] = jnp.zeros((WP, LANES), U32)
            return carry
        lax.fori_loop(0, WS, zrow, 0)
        for ref in (q_s, v_s):
            ref[0, 0:8, :] = zt
        for ref in stg:
            ref[SPARE, 0:16, :] = jnp.zeros((16, LANES), U32)
        for ref in vts:
            ref[1, 0:8, :] = zt
        for ref in xin + xout:
            ref[ref.shape[0] - 1, 0:16, 0:LANES] = jnp.zeros((16, LANES), BF16)
        wo_s[...] = jnp.zeros(wo_s.shape, U32)
        for cp in wcp:
            cp.wait()
        for ki in range(3):
            w3 = dw_ref[ki].astype(F32)
            for kj in range(3):
                w = w3[kj:kj + 1] + 1.0 if ki == kj == 1 else w3[kj:kj + 1]
                dw_s[:, ki, kj] = jnp.broadcast_to(w, (LANES, C)).T.reshape(C // 8, 8, LANES)
        qscale = (dh ** -0.5) * math.log2(math.e)
        for kt in range(2):
            wt = wqkv_ref[CW * kt:CW * (kt + 1), :].astype(F32).T
            wq = (wt[0:C] * qscale).astype(BF16).astype(F32)
            words = [(_u32(w[0:CW]) >> 16) | (_u32(w[CW:C]) & hi) for w in (wq, wt[C:2 * C])]
            words = _rows8(_cat(words + [_u32(wt[2 * C:].astype(BF16))]))
            for par in range(2):
                wq_s[par, :, LANES * kt:LANES * kt + CW] = _cat(words[par::2])
        wo = _u32(wo_ref[...])
        wo_s[:, 0:CW] = (wo << 16).T
        wo_s[:, LANES:LANES + CW] = (wo & hi).T

        for cp in top:
            cp.wait()

        def conv0(c2, carry):
            for par in range(2):
                cs = pl.ds(pl.multiple_of(32 * c2 + 16 * par, 16), 16)
                sh = [shifted(_u32(i0_s[0, cs, :]))] + [shifted(_u32(i1_s[r, cs, :])) for r in range(WS)]
                for rho in (WS, WS + 1):
                    stg[par][stg_row(-1, c2, rho)] = sh[rho - 1]
                for hf in range(2):
                    c8 = 4 * c2 + 2 * par + hf
                    w = [dw_s[c8, ki] for ki in range(3)]
                    for t in range(NT):
                        un = [None] + [unpack(row[24 * t:24 * t + 24], hf) for row in sh]
                        for r in range(WS):
                            xbuf[0][r, t, pl.ds(pl.multiple_of(8 * c8, 8), 8), :] = conv_row(un, w, r)
            return carry
        lax.fori_loop(0, NC // 2, conv0, 0)
        for cp in in_copies(0, 1) + in_copies(1, 1):
            cp.start()
        for cp in in_copies(2, 0):
            cp.wait()
        for cp in in_copies(2, 1):
            cp.start()

    def body(subs):
        lane3 = _iota((WS, 8, LANES), 2)
        head = (lane3 < dh, (lane3 >= dh) & (lane3 < 2 * dh))
        zq = jnp.zeros((WS, 8, LANES), F32)
        junk8 = _iota((8, 2 * G), 0) == WS
        ninf8 = jnp.full((8, 2 * G), -jnp.inf, F32)
        ngr = WS + PVP
        key_ok = tuple((_iota((ngr, 8, 2 * G), 2) & 8) == 8 * hh for hh in range(2))
        sub1 = (_iota((8, 2 * G), 0) & 1) == 0
        sub2 = (_iota((8, 2 * G), 0) & 2) == 0
        zp = jnp.zeros((ngr, 8, 2 * G), F32)
        first_half = (_iota((8, 2 * G), 1) & 8) == 0
        even_head = (_iota((WS, 8, CW), 2) // (dh // 2)) % 2 == 0
        npair = (NWIN + 1) // 2
        n0 = (HW - 1) // WS // 2

        st = {}
        toks = []
        soft = []
        ticks = []
        j0 = subs[0][0]
        tag = {('qkv', t, r): -1 for t in range(NT) for r in range(WS)}
        tag.update({('o', p): (-1 if p < n0 else None) for p in range(npair)})
        for b, blk in ((j0 % 3, 0), ((j0 + 2) % 3, -1)):
            tag.update({('x', b, c, t, r): blk for c in range(2 * NC) for t in range(NT) for r in range(WS)})
        tag.update({('s', c % 2, stg_row(j0, c // 2, rho)): (0, c, rho) for c in range(NC) for rho in (0, 1)})

        def gather(ref, w):
            return ref[:, pl.ds(WS * w, 8), :]

        def tick(t):
            c = [x for x in ticks if t <= x[0] <= t + 40]
            if not c:
                return None
            _, res, j = min(c, key=lambda x: x[0])
            return res[8 * j:8 * j + 8, 0:LANES]

        def due(lst, nblk, t0, step):
            inj = {}
            for d, tok in list(lst):
                j = max(0, -(-(d - t0) // step))
                if j < nblk:
                    inj.setdefault(j, []).append(tok)
            lst[:] = [x for x in lst if x[0] > t0 + (nblk - 1) * step]
            return inj

        def lhs(ref, ls, inj, dt):
            nblk = ref.shape[0] // 8
            parts, s = [], 0
            for j in sorted(inj):
                if j > s:
                    parts.append(ref[8 * s:8 * j, ls])
                parts.append(tie(ref[8 * j:8 * j + 8, ls], inj[j]))
                s = j + 1
            if s < nblk:
                parts.append(ref[8 * s:8 * nblk, ls])
            return pltpu.bitcast(_cat(parts), dt)

        def merged(a, b):
            return {j: a.get(j, []) + b.get(j, []) for j in set(a) | set(b)}

        def fence(d, b):
            c = [x for x in ticks if x[0] <= d]
            if c:
                _, res, j = max(c, key=lambda x: x[0])
                xbuf[b][zx + WS, 0, 0:8, :] = res[8 * j:8 * j + 8, 0:LANES]

        def ln1(d, k, t, r):
            b = subs[k][0] % 3
            assert all(tag['x', b, c, t, r] == k for c in range(2 * NC))
            x0 = xbuf[b][r, t, 0:C, :]
            s8 = _sum8(x0)
            soft.append((d, _u32(s8)))
            mean = jnp.sum(s8, axis=0, keepdims=True) * (1.0 / C)
            if LNF & 2:
                fence(d + LNG, b)
                x0 = xbuf[b][r, t, 0:C, :]
            st['ln', k, t, r] = [x0 - mean, [], mean]

        def ln3(d, k, t, r):
            b = subs[k][0] % 3
            fence(d, b)
            st['ln', k, t, r][0] = xbuf[b][r, t, 0:C, :] - st['ln', k, t, r][2]

        def ln2(d, n, *key):
            m = C // LNS
            xc = st[('ln',) + key][0][m * n:m * (n + 1)]
            s8 = _sum8(xc * xc)
            soft.append((d, _u32(s8)))
            st[('ln',) + key][1].append(s8)

        def a_dot(t0, k, t, r):
            xc, sq, _ = st.pop(('ln', k, t, r))
            var = jnp.sum(_tree_sum(sq), axis=0, keepdims=True) * (1.0 / C)
            h = xc * lax.rsqrt(var + EPS)
            h = [h[CW * kt:CW * (kt + 1)].astype(BF16) for kt in range(2)]
            inj = due(toks, DA // 16, t0, 16)
            inj0 = merged(inj, due(soft, DA // 16, t0, 16))
            part = [jnp.dot(lhs(wq_s.at[par], slice(LANES * kt, LANES * kt + CW), inj if par or kt else inj0, BF16),
                            h[kt], preferred_element_type=F32)
                    for par in range(2) for kt in range(2)]
            res = [part[0] + part[1], part[2] + part[3]]
            ticks.extend((t0 + MXU_LAT + 8 * j, res[0], j) for j in range(DA // 8))
            qkv = jnp.stack([v.reshape(-1, 16, LANES) for v in res], axis=1).reshape(3 * C, LANES)
            for m in range(3):
                qkv_s[m][r, LANES * t:LANES * (t + 1), 0:CW] = _u32(qkv[C * m:C * (m + 1)].astype(BF16)).T
                toks.append((t0 + 96 * (m + 1) + DL_A, qkv_s[m][zx, 0:8, :]))
            tag['qkv', t, r] = k

        def wins(p):
            return 2 * p, min(2 * p + 1, NWIN - 1)

        def b_qk(t0, k, p):
            wa, wb = wins(p)
            blk = k if p < n0 else k - 1
            assert all(tag['qkv', t, r] == blk for r in range(WS)
                       for t in range(WS * wa // LANES, (WS * wb + WS) // LANES + 1))
            sts = []
            inj = due(soft, WS, t0, 8)
            for w, swap in ((wa, 0), (wb, 1)):
                qw = gather(q_s, w)
                kw = gather(k_s, w).reshape(G, LANES)
                if not swap and inj:
                    kw = _cat([tie(v, inj.get(r, [])) for r, v in enumerate(_rows8(kw))])
                for tile in range(2):
                    kk = _f32(kw & hi if tile else kw << 16)
                    qq = _f32(qw & hi if tile else qw << 16)
                    qst = jnp.stack([lax.select(head[swap], qq, zq), lax.select(head[1 - swap], qq, zq)], axis=1)
                    sts.append(lax.dot_general(kk, qst.reshape(2 * G, LANES), (((1,), (1,)), ((), ())),
                                               preferred_element_type=F32))
            if PVP:
                vw = _cat([gather(v_s, wa), zt[None], gather(v_s, wb), zt[None]]).reshape(LANES, LANES)
            else:
                vw = _cat([gather(v_s, wa), gather(v_s, wb)]).reshape(2 * G, LANES)
            vt = vw[:, 0:CW].T
            if VST:
                st['nv'] = st.get('nv', 0) + 1
                ref = vts[st['nv'] % len(vts)]
                st['nv', p] = st['nv']
                ref[0, :, 0:vt.shape[1]] = vt
                if VDL:
                    soft.append((tpv[k, p] - VDL, ref[zx + 1, 0:8, :]))
                vt = (ref, vt.shape[1])
            st['s', p] = (sts, vt)

        def b_pv(t0, tg, k, p):
            wa, wb = wins(p)
            sts, vt = st.pop(('s', p))
            if VST:
                vt[0][zx + 1, 8:16, :] = zt
                vt = lhs(vt[0].at[0], slice(0, vt[1]), due(soft, 3, t0, 16) if PVI else {}, BF16)
            else:
                vt = pltpu.bitcast(vt, BF16)
            if SST:
                sref = sts_s[st['nv', p] % len(sts_s)]
                for n, s_t in enumerate(sts):
                    sref[n, 0:G, 0:2 * G] = s_t
                c = [x for x in ticks if x[0] <= tg]
                _, res, j = max(c, key=lambda x: x[0]) if c else (0, _f32(zt), 0)
                sref[zx + 4, 0:8, :] = res[8 * j:8 * j + 8, 0:LANES]
            pts = []
            dens = []
            for n, s_t in enumerate(sts):
                m8 = _fold7(jnp.maximum, s_t)
                mx = _all8(jnp.maximum, lax.select(junk8, ninf8, m8))
                mv = lax.select(junk8, -ninf8, mx)
                z = tick(tg + SMD * (3 - n)) if SST != 1 else None
                if z is not None:
                    mv = tie(mv, [z])
                if SST:
                    s_t = sref[n, 0:G, 0:2 * G]
                eg = jnp.exp2(s_t.reshape(WS, 8, 2 * G) - mv)
                dens.append(_fold7(jnp.add, eg.reshape(G, 2 * G)))
                pts.append(_cat([eg, eg[WS - 1:WS]]) if PVP else eg)
            if MRG:
                def mix(m, sh, a, b):
                    return lax.select(m, a, b) + pltpu.roll(lax.select(m, b, a), sh, 0)
                den = mix(sub2, 2, mix(sub1, 1, dens[0], dens[1]), mix(sub1, 1, dens[2], dens[3]))
                den = den + pltpu.roll(den, 4, 0)
                r0 = pl.reciprocal(den, approx=True)
                r0 = r0 * (2.0 - den * r0)
                r0 = lax.select(first_half, r0, pltpu.roll(r0, 2, 0))
                rsel = [jnp.broadcast_to(r0[n:n + 1], r0.shape) for n in range(4)]
            else:
                rinv = []
                for den in dens:
                    den = _all8(jnp.add, den)
                    r0 = pl.reciprocal(den, approx=True)
                    rinv.append(r0 * (2.0 - den * r0))
                rsel = [lax.select(first_half, rinv[n], rinv[(n + 2) % 4]) for n in range(4)]
            outs = []
            for tile in range(2):
                for hh in range(2):
                    h = 2 * tile + hh
                    stn = _cat([lax.select(key_ok[hh], pts[tile], zp), lax.select(key_ok[1 - hh], pts[2 + tile], zp)])
                    ot = jnp.dot(vt[dh * h:dh * (h + 1), :], stn.reshape(-1, 2 * G).astype(BF16),
                                 preferred_element_type=F32)
                    outs.append(ot.reshape(dh // 8, 8, 2 * G) * rsel[2 * hh + tile])
            tw = _u32(_cat(outs).reshape(C, 2 * G).astype(BF16)).T.reshape(WS, 2, 8, CW)
            tw = (tw[:, 0], tw[:, 1])
            o_s[:, pl.ds(WS * wa, 8), 0:CW] = lax.select(even_head, tw[0], tw[1])
            if wb != wa:
                o_s[:, pl.ds(WS * wb, 8), 0:CW] = lax.select(even_head, tw[1], tw[0])
                tag['o', p + 1] = None
            toks.append((t0 + DL_PV, o_s[zx, 0:8, :]))
            tag['o', p] = k if p < n0 else k - 1
            if p == n0:
                tag['o2'] = k - 1

        def c_dot(t0, k, h, r):
            b = (subs[k][0] + 2) % 3
            assert all(tag['o', p] == k - 1 for p in (range(n0 + 1) if h == 0 else range(n0 + 1, npair)))
            assert tag['o2'] == k - 1 and 2 * WS * n0 < HW
            assert all(tag['x', b, c, t, r] == k - 1 for c in range(2 * NC) for t in (2 * h, 2 * h + 1))
            ls = slice(HW * h, HW * (h + 1))
            ow = o_s[r, ls, :]
            rhs = _cat([_f32(ow << 16), _f32(ow & hi)], axis=1)
            inj = due(toks, DC // 8, t0, 8)
            wo = _cat([lhs(wo_s, slice(0, LANES), merged(inj, due(soft, DC // 8, t0, 8)), F32),
                       lhs(wo_s, slice(LANES, 2 * LANES), inj, F32)], axis=1)
            res = lax.dot_general(wo, rhs, (((1,), (1,)), ((), ())), preferred_element_type=F32)
            ticks.extend((t0 + MXU_LAT + 8 * j, res, j) for j in range(DC // 8))
            slot = subs[k][2]
            n = min(HW, W - HW * h)
            xout[slot][row0(slot, g) + r, :, HW * h:HW * h + n] = (_cat([xbuf[b][r, t, 0:C, :] for t in (2 * h, 2 * h + 1)], axis=1) + res)[:, 0:n].astype(BF16)
            if h == 1 and not subs[k][3]:
                out_copy(slot, g, r, 1).start()
            elif h == 1 and r == WS - 1:
                out_copy(slot, g).start()
                xout[slot][zx + xout[slot].shape[0] - 1, 0:16, 0:LANES] = jnp.zeros((16, LANES), BF16)
                soft.append((t0 + MXU_LAT + DC + DL_D, _u32(xout[slot][zy + xout[slot].shape[0] - 1, 0:16, 0:LANES])))

        def stage_row(d, k, c, rho):
            j, slot = subs[k][0:2]
            cs = slice(16 * c, 16 * c + 16)
            u = _u32(xin[slot][row0(slot, g) + rho - 2, cs, :])
            if rho == WS + 1 and slot == 1:
                u = jnp.where(g < ng - 2, u, zero)
            idx = stg_row(j, c // 2, rho)
            stg[c % 2][idx] = shifted(u)
            soft.append((d, stg[c % 2][zx + SPARE, 8:16, 0:LANES]))
            tag['s', c % 2, idx] = (k, c, rho)
            if c == NC - 1 and rho == WS + 1 and slot < NSUB - 1:
                for cp in in_copies(slot, g + 1):
                    cp.start()
                xin[slot][zx + WS, 0:16, 0:LANES] = jnp.zeros((16, LANES), BF16)
                soft.append((d + DL_D, _u32(xin[slot][zy + WS, 0:16, 0:LANES])))

        def conv_step(d, k, c, hf, t, r):
            j = subs[k][0]
            if r == 0:
                if t == 0:
                    stg[c % 2][zx + SPARE, 0:8, 0:LANES] = zt
                    st['w'] = [dw_s[2 * c + hf, ki] for ki in range(3)]
                st['un'] = {}
            un = st['un']
            for rho in range(r, r + 3):
                if rho not in un:
                    idx = stg_row(j, c // 2, rho)
                    assert tag['s', c % 2, idx] in ((k, c, rho), (k - 1, c, rho + WS))
                    un[rho] = unpack(stg[c % 2][idx, 24 * t:24 * t + 24, :], hf)
            acc = conv_row(un, st['w'], r)
            xbuf[(j + 1) % 3][r, t, 16 * c + 8 * hf:16 * c + 8 * hf + 8, :] = acc
            soft.append((d, _u32(acc)))
            tag['x', (j + 1) % 3, 2 * c + hf, t, r] = k + 1

        plan, offs = [], [0]
        for k, sub in enumerate(subs):
            pk, tk = _plan(npair, n0, NT, sub[3], sub[4])
            plan += [(offs[k] + t, kind, k, idx) for t, kind, idx in pk]
            offs.append(offs[k] + tk)
        total = offs[-1]
        starts = [e[0] for e in plan]
        ev = []

        def at(t, fn, *a):
            ev.append((t, t, len(ev), fn, a))

        def before(d, fn, *a):
            ev.append((max([t for t in starts if t <= d], default=0) - 1, d, len(ev), fn, a))

        load = [0.0] * (total + 1000)
        tqk = {}
        tpv = {(k, idx): t for t, kind, k, idx in plan if kind == 'pv'}

        def add(t0, t1, n):
            for t in range(max(t0, 0), max(t1, 0)):
                load[t] += n / (t1 - t0)

        for t, kind, k, idx in plan:
            tr = t + MXU_LAT
            if kind == 'a':
                if idx == (0, 0) and k > 0:
                    before(t - LN1 - 1, fence, t - LN1 - 40, subs[k][0] % 3)
                before(t - LN1, ln1, t - LN1, k, *idx)
                for n in range(LNS):
                    d = t - LN2 - LND * (LNS - 1 - n)
                    before(d, ln2, d, n, k, *idx)
                    add(d - 16, d, 72 // LNS)
                if LNF & 1:
                    before(t - LN3, ln3, t - LN3, k, *idx)
                    add(t - 40, t, 24)
                at(t, a_dot, t, k, *idx)
                add(tr, tr + DA, 12 * DA // 16)
                add(t - LN1 - 16, t - LN1, 32); add(t - LN2, t - 40, 20); add(t - 40, t, 36)
            elif kind == 'qk':
                at(t, b_qk, t, k, idx)
                tqk[idx] = t
                add(t - 64, t, 28); add(t, t + DQ, 28); add(tr, tr + DQ, 24); add(tr + DQ, tr + DQ + 16, 36)
            elif kind == 'pv':
                tg = max(tqk[idx] + SM0, t - SMB)
                at(t, b_pv, t, tg, k, idx)
                add(tg, tg + 4 * SMD + 16, 80); add(tr - 10, tr + 6, 46); add(tr, tr + DP, 36)
                add(t + 400, t + 460, 14)
            else:
                if idx == (0, 0) and k > 0:
                    at(t - 1, fence, t - 100, (subs[k][0] + 2) % 3)
                at(t, c_dot, t, k, *idx)
                add(tr, tr + DC, 20 * DC // 16)
                add(t - 70, t, 64)
        pre = [0.0]
        for v in load:
            pre.append(pre[-1] + v)
        nstep = NC * 2 * NT * WS
        prev_chunk = 10
        for k, sub in enumerate(subs):
            if not sub[3]:
                continue
            ta = offs[k] + (CVI if k else CV0) - 20
            tb = offs[k + 1] - (CVE if k == len(subs) - 1 else CVX)
            cap = CAP if sub[4] else 64
            free = [max(0.02, cap / 16 - (pre[t + SMO] - pre[max(t - SMO, 0)]) / (2 * SMO)) for t in range(ta, tb)]
            tot_free, acc, tstep = sum(free), 0.0, []
            for t, v in enumerate(free):
                acc += v
                while len(tstep) < nstep and acc >= (len(tstep) + 1) * tot_free / nstep - 1e-6:
                    tstep.append(ta + t)
            for n in range(nstep):
                before(tstep[n], conv_step, tstep[n], k, n // (2 * NT * WS), n // (NT * WS) % 2, n // WS % NT, n % WS)
            for c in range(NC):
                t1 = tstep[c * 2 * NT * WS] - 30
                t0 = prev_chunk + 120
                prev_chunk = t1 + 30
                for rho in range(2, NR):
                    d = t0 + (t1 - t0) * (rho - 2) // (NR - 3)
                    before(d, stage_row, d, k, c, rho)
        ev.sort(key=lambda e: e[:3])
        for e in ev:
            e[3](*e[4])
        if subs[-1][3]:
            n = len(subs)
            assert all(tag['qkv', t, r] == n - 1 for t in range(NT) for r in range(WS))
            assert all(tag['o', p] == n - 1 for p in range(n0))

    if ONLY in (0, 1):
        @pl.when(g == 0)
        def _():
            setup()
            body([(0, 2, 0, True, False)])

    @pl.when(g > 0)
    def _():
        for k in range(NSUB):
            for cp in in_copies(k, g):
                cp.wait()

    @pl.when((g > 0) & (g < ng - 1))
    def _():
        for cp in in_copies(NSUB - 1, g + 1):
            cp.start()

    @pl.when(g > 1)
    def _():
        for k in range(NSUB - 1):
            out_copy(k, g - 1).wait()

    @pl.when(g > 2)
    def _():
        out_copy(NSUB - 1, g - 2).wait()

    if ONLY in (0, 2):
        @pl.when((g > 0) & (g < ng - 1))
        def _():
            body([(1 + k, k, k, True, True) for k in range(NSUB)])

    if ONLY in (0, 3):
        @pl.when(g == ng - 1)
        def _():
            body([(1, 0, 0, False, True)])
            out_copy(NSUB - 1, g - 1).wait()
            out_copy(0, g).wait()


@jax.jit
def pallas_standalone__window_attn_davit__vision_kernel(
    x: jax.Array,
    dw_pe: jax.Array,
    w_qkv: jax.Array,
    w_o: jax.Array,
):
    B, H, W, C = x.shape
    assert B == 1 and H % WS == 0 and W % WS == 0 and C % (16 * NH) == 0
    WP = -(-(W + 1) // (2 * LANES)) * (2 * LANES)
    assert WP == 4 * LANES
    NWIN = W // WS
    NBLK = H // WS
    assert (NBLK - 1) % NSUB == 0
    NM = (NBLK - 1) // NSUB

    xt = jnp.transpose(x[0], (0, 2, 1))

    nstg = WS - 2 + NSUB * (C // 32) * 2 + 1
    kern = functools.partial(_kernel, C=C, H=H, W=W, WP=WP, NWIN=NWIN)
    out = pl.pallas_call(
        kern,
        grid=(NM + 2,),
        in_specs=[pl.BlockSpec(memory_space=pl.ANY)] * 4,
        out_specs=pl.BlockSpec(memory_space=pl.ANY),
        out_shape=jax.ShapeDtypeStruct((H, C, W), x.dtype),
        scratch_shapes=[
            pltpu.VMEM((WS + 1, WP // LANES, C + 8, LANES), F32),
            pltpu.VMEM((WS + 1, WP // LANES, C + 8, LANES), F32),
            pltpu.VMEM((WS + 1, WP // LANES, C + 8, LANES), F32),
            pltpu.VMEM((WS, WP + 8, LANES), U32),
            pltpu.VMEM((WS, WP + 8, LANES), U32),
            pltpu.VMEM((WS, WP + 8, LANES), U32),
            pltpu.VMEM((WS, WP + 8, LANES), U32),
            pltpu.VMEM((2, 3 * C // 4, 2 * LANES), U32),
            pltpu.VMEM((C, 2 * LANES), U32),
            pltpu.VMEM((nstg, WP // LANES * 24, LANES), U32),
            pltpu.VMEM((nstg, WP // LANES * 24, LANES), U32),
            pltpu.VMEM((C // 8, 3, 3, 8, LANES), F32),
            pltpu.VMEM((WS + 1, C, W), BF16),
            pltpu.VMEM((WS + 1, C, W), BF16),
            pltpu.VMEM((2 * WS + 1, C, W), BF16),
            pltpu.VMEM((WS + 1, C, W), BF16),
            pltpu.VMEM((WS + 1, C, W), BF16),
            pltpu.VMEM((2 * WS + 1, C, W), BF16),
            pltpu.VMEM((2, C // 2, LANES), U32),
            pltpu.VMEM((2, C // 2, LANES), U32),
            pltpu.VMEM((2, C // 2, LANES), U32),
            pltpu.VMEM((2, C // 2, LANES), U32),
            pltpu.VMEM((5, 8 * WS + 16, LANES), F32),
            pltpu.VMEM((5, 8 * WS + 16, LANES), F32),
            pltpu.VMEM((5, 8 * WS + 16, LANES), F32),
            pltpu.VMEM((5, 8 * WS + 16, LANES), F32),
            pltpu.VMEM(dw_pe.shape, BF16),
            pltpu.VMEM(w_qkv.shape, BF16),
            pltpu.VMEM(w_o.shape, BF16),
            pltpu.SemaphoreType.DMA((2 * NSUB,)),
            pltpu.SemaphoreType.DMA((NSUB + 1,)),
            pltpu.SemaphoreType.DMA((3,)),
        ],
        compiler_params=pltpu.CompilerParams(
            dimension_semantics=("arbitrary",),
            vmem_limit_bytes=96 * 1024 * 1024,
            disable_bounds_checks=bool(NOBC),
        ),
        name="davit_window_attn",
    )(xt, dw_pe, w_qkv, w_o)
    return jnp.transpose(out, (0, 2, 1))[None]
```

```python
import functools
import math
import os

import jax
import jax.numpy as jnp
from jax import lax
import jax.experimental.pallas as pl
import jax.experimental.pallas.tpu as pltpu

WS = 7
NH = 4
EPS = 1e-05
LANES = 128
F32 = jnp.float32
BF16 = jnp.bfloat16
U32 = jnp.uint32

P = lambda k, d: int(os.environ.get(k, d))
DL_A = P('DL_A', 500)
LAT_QK = P('LAT_QK', 280)
DL_PV = P('DL_PV', 580)
PRE_C = P('PRE_C', 120)
TAIL = P('TAIL', 1000)
LN1 = P('LN1', 200)
LN2 = P('LN2', 130)
LNS = P('LNS', 3)
LND = P('LND', 16)
SM0 = P('SM0', 200)
SMD = P('SMD', 16)
SMB = P('SMB', 110)
CV0 = P('CV0', 400)
CVI = P('CVI', 170)
CVE = P('CVE', 60)
CVX = P('CVX', 180)
ORD = P('ORD', 0)
CAP = P('CAP', 42)
SMO = P('SMO', 32)
ONLY = P('ONLY', 0)
ZK = P('ZK', 1)
EC0 = P('EC0', 1500)
ECD = P('ECD', 900)
PVI = P('PVI', 1)
SST = P('SST', 0)
VST = P('VST', 1)
VDL = P('VDL', 60)
MRG = P('MRG', 0)
DL_D = P('DL_D', 100)
PVP = P('PVP', 0)
LNF = P('LNF', 3)
LN3 = P('LN3', 50)
LNG = P('LNG', 16)
NOBC = P('NOBC', 1)
DA, DC, DQ, DP = 288, 192, 56, 48
MXU_LAT = 130
NSUB = 3


def _iota(shape, dim):
    return lax.broadcasted_iota(jnp.int32, shape, dim)


def _plan(npair, n0, nt, cur, prev):
    a_q = [(t, r) for t in range(nt) for r in range(WS)] if cur else []
    c_q = [(h, r) for h in range(2) for r in range(WS)] if prev else []
    n1 = npair - n0 if prev else 0
    pairs = list(range(n0, n0 + n1)) + (list(range(n0)) if cur else [])
    total = len(a_q) * DA + len(c_q) * DC + len(pairs) * (DQ + DP)
    q0 = 0 if prev else total // 3
    t = 0
    ia = ic = iq = ip = 0
    out = []
    tq, tp, ta = {}, {}, {}
    last = None
    while ia < len(a_q) or ic < len(c_q) or ip < len(pairs):
        cands = []
        if ip < iq and t >= tq[ip] + LAT_QK:
            cands.append((-1e6, 'pv'))
        if iq < len(pairs) and (not cur or (iq - ip < 2 and last != 'qk' and not (ORD and last == 'pv'))):
            ok = iq - ip < 4
            if iq >= n1:
                need = (2 * WS * pairs[iq] + 2 * WS) // LANES * WS + WS - 1
                ok = ia > need and t >= ta[need] + DA + DL_A + 60 and ic >= len(c_q) // 2
            if ok:
                pr = q0 + iq * (total - q0 - TAIL) / len(pairs) - t - 200
                cands.append((-2e6 if ORD and pr <= 0 else pr, 'qk'))
        if ia < len(a_q):
            cands.append((ia * (total - 700) / len(a_q) - t, 'a'))
        if ic < len(c_q):
            need = 0 if ic < WS else n1 - 1
            if ip > need and t >= tp[need] + DL_PV + PRE_C:
                if cur:
                    tc = 1000 + ic * 900 if ic < WS else total - DC - (2 * WS - 1 - ic) * 950
                else:
                    tc = EC0 + ic * ECD
                cands.append((tc - t, 'c'))
        if not cands:
            t += 8
            last = None
            continue
        kind = min(cands)[1]
        last = kind
        if kind == 'pv':
            tp[ip] = t; out.append((t, 'pv', pairs[ip])); ip += 1; t += DP
        elif kind == 'qk':
            tq[iq] = t; out.append((t, 'qk', pairs[iq])); iq += 1; t += DQ
        elif kind == 'a':
            ta[ia] = t; out.append((t, 'a', a_q[ia])); ia += 1; t += DA
        else:
            out.append((t, 'c', c_q[ic])); ic += 1; t += DC
    return out, t


def _tree_sum(xs):
    while len(xs) > 1:
        xs = [xs[j] + xs[j + 1] if j + 1 < len(xs) else xs[j] for j in range(0, len(xs), 2)]
    return xs[0]


def _sum8(x):
    while x.shape[0] % 16 == 0:
        x = x[:x.shape[0] // 2] + x[x.shape[0] // 2:]
    return _tree_sum(_rows8(x))


def _fold7(op, x):
    t = op(x[0:24], x[24:48])
    return op(op(t[0:8], t[8:16]), op(t[16:24], x[48:56]))


def _all8(op, x):
    for sh in (4, 2, 1):
        x = op(x, pltpu.roll(x, sh, 0))
    return x


def _rows8(x):
    return [x[8 * j:8 * j + 8] for j in range(x.shape[0] // 8)]


def _cat(xs, axis=0):
    return jnp.concatenate(xs, axis=axis) if len(xs) > 1 else xs[0]


def _f32(u):
    return pltpu.bitcast(u, F32)


def _u32(x):
    return pltpu.bitcast(x, U32)


def _kernel(x_hbm, dw_hbm, wqkv_hbm, wo_hbm, o_hbm,
            xa_s, xb_s, xc_s, q_s, k_s, v_s, o_s, wq_s, wo_s, sa_s, sb_s, dw_s,
            i0_s, i1_s, i2_s, o0_s, o1_s, o2_s, va_s, vb_s, vc_s, vd_s, ta_s, tb_s, tc_s, td_s, dw_ref, wqkv_ref, wo_ref, in_sem, out_sem, w_sem,
            *, C, H, W, WP, NWIN):
    g = pl.program_id(0)
    ng = pl.num_programs(0)
    dh = C // NH
    CW = C // 2
    NT = WP // LANES
    G = WS * 8
    HW = WP // 2
    NC = C // 16
    NR = WS + 2
    lane8 = _iota((8, LANES), 1)
    last_valid = W - (NT - 1) * LANES
    zero = jnp.uint32(0)
    hi = jnp.uint32(0xFFFF0000)
    qkv_s = (q_s, k_s, v_s)
    xbuf = (xa_s, xb_s, xc_s)
    xin = (i0_s, i1_s, i2_s)
    xout = (o0_s, o1_s, o2_s)

    def row0(k, m):
        return (m & 1) * WS if k == NSUB - 1 else 0

    def in_copies(k, m):
        r = WS * (NSUB * m - 1 + k) + 1
        return [pltpu.make_async_copy(x_hbm.at[pl.ds(jnp.minimum(r + o, H - n), n)],
                                      xin[k].at[pl.ds(row0(k, m) + o, n)], in_sem.at[2 * k + e])
                for e, (o, n) in enumerate(((0, WS - 1), (WS - 1, 1)))]

    def out_copy(k, m, o=0, n=WS):
        return pltpu.make_async_copy(xout[k].at[pl.ds(row0(k, m) + o, n)],
                                     o_hbm.at[pl.ds(WS * (NSUB * (m - 1) + k) + o, n)],
                                     out_sem.at[k + (m & 1) if k == NSUB - 1 else k])

    stg = (sa_s, sb_s)
    vts = (va_s, vb_s, vc_s, vd_s)
    sts_s = (ta_s, tb_s, tc_s, td_s)
    SPARE = sa_s.shape[0] - 1
    zx = g >> 10
    zy = g >> 11
    never = lane8 < zx

    def tie(x, toks):
        if not toks:
            return x
        tok = functools.reduce(lax.bitwise_or, toks)
        n = x.shape[1]
        return lax.select(never[:, 0:n], tok[:, 0:n], x) if n < LANES else lax.select(never, tok, x)

    def stg_row(j, c2, rho):
        if 2 <= rho < WS:
            return rho - 2
        slot = j % NSUB if rho >= WS else (j - 1) % NSUB
        return WS - 2 + (slot * (NC // 2) + c2) * 2 + rho % WS

    zt = jnp.zeros((8, LANES), U32)
    is_first, is_last = lane8 == 0, lane8 == LANES - 1

    def shifted(u):
        tiles = [u[:, LANES * t:LANES * (t + 1)] for t in range(NT)]
        tiles[NT - 1] = _cat([tiles[NT - 1], zt[:, last_valid:]], axis=1)
        left = [pltpu.roll(lax.select(is_last, tiles[t - 1] if t > 0 else zt, tiles[t]), 1, 1)
                for t in range(NT)]
        right = [pltpu.roll(lax.select(is_first, tiles[t + 1], tiles[t]) if t < NT - 1 else tiles[t], LANES - 1, 1)
                 for t in range(NT)]
        return _cat([v[t] for t in range(NT) for v in (left, tiles, right)])

    def unpack(v, hf):
        return pltpu.bitcast(v, BF16).astype(F32).reshape(3, 2, 8, LANES)[:, hf]

    def conv_row(un, w, r):
        return jnp.sum(_tree_sum([un[r + ki] * w[ki] for ki in range(3) if un[r + ki] is not None]), axis=0)

    def setup():
        wcp = [pltpu.make_async_copy(src, dst, w_sem.at[n])
               for n, (src, dst) in enumerate(((dw_hbm, dw_ref), (wqkv_hbm, wqkv_ref), (wo_hbm, wo_ref)))]
        def top(c2):
            cs = pl.ds(pl.multiple_of(32 * c2, 32), 32)
            return pltpu.make_async_copy(x_hbm.at[pl.ds(0, WS + 1), cs], i1_s.at[:, cs], w_sem.at[3 + c2])
        for cp in wcp + [top(c2) for c2 in range(NC // 2)]:
            cp.start()

        def zrow(r, carry):
            for ref in ((k_s, o_s) if ZK else (q_s, k_s, v_s, o_s)):
                ref[r, 0:WP, :] = jnp.zeros((WP, LANES), U32)
            return carry
        lax.fori_loop(0, WS, zrow, 0)
        for ref in (q_s, v_s):
            ref[0, 0:8, :] = zt
        for ref in stg:
            ref[SPARE, 0:16, :] = jnp.zeros((16, LANES), U32)
        for ref in vts:
            ref[1, 0:8, :] = zt
        for ref in (i0_s,) + xout:
            ref[ref.shape[0] - 1, 0:16, 0:LANES] = jnp.zeros((16, LANES), BF16)
        wo_s[...] = jnp.zeros(wo_s.shape, U32)
        for cp in wcp:
            cp.wait()
        for ki in range(3):
            w3 = dw_ref[ki].astype(F32)
            for kj in range(3):
                w = w3[kj:kj + 1] + 1.0 if ki == kj == 1 else w3[kj:kj + 1]
                dw_s[:, ki, kj] = jnp.broadcast_to(w, (LANES, C)).T.reshape(C // 8, 8, LANES)
        qscale = (dh ** -0.5) * math.log2(math.e)
        for kt in range(2):
            wt = wqkv_ref[CW * kt:CW * (kt + 1), :].astype(F32).T
            wq = (wt[0:C] * qscale).astype(BF16).astype(F32)
            words = [(_u32(w[0:CW]) >> 16) | (_u32(w[CW:C]) & hi) for w in (wq, wt[C:2 * C])]
            words = _rows8(_cat(words + [_u32(wt[2 * C:].astype(BF16))]))
            for par in range(2):
                wq_s[par, :, LANES * kt:LANES * kt + CW] = _cat(words[par::2])
        wo = _u32(wo_ref[...])
        wo_s[:, 0:CW] = (wo << 16).T
        wo_s[:, LANES:LANES + CW] = (wo & hi).T

        def conv0(c2, carry):
            top(c2).wait()

            @pl.when(c2 == 2)
            def _():
                for cp in in_copies(2, 0):
                    cp.start()
            for par in range(2):
                cs = pl.ds(pl.multiple_of(32 * c2 + 16 * par, 16), 16)
                sh = [shifted(_u32(i1_s[r, cs, :])) for r in range(WS + 1)]
                for rho in (WS, WS + 1):
                    stg[par][stg_row(-1, c2, rho)] = sh[rho - 1]
                for hf in range(2):
                    c8 = 4 * c2 + 2 * par + hf
                    w = [dw_s[c8, ki] for ki in range(3)]
                    for t in range(NT):
                        un = [None] + [unpack(row[24 * t:24 * t + 24], hf) for row in sh]
                        for r in range(WS):
                            xbuf[0][r, t, pl.ds(pl.multiple_of(8 * c8, 8), 8), :] = conv_row(un, w, r)
            return carry
        lax.fori_loop(0, NC // 2, conv0, 0)
        for cp in in_copies(0, 1) + in_copies(1, 1):
            cp.start()
        for cp in in_copies(2, 0):
            cp.wait()
        for cp in in_copies(2, 1):
            cp.start()

    def body(subs):
        lane3 = _iota((WS, 8, LANES), 2)
        head = (lane3 < dh, (lane3 >= dh) & (lane3 < 2 * dh))
        zq = jnp.zeros((WS, 8, LANES), F32)
        junk8 = _iota((8, 2 * G), 0) == WS
        ninf8 = jnp.full((8, 2 * G), -jnp.inf, F32)
        ngr = WS + PVP
        key_ok = tuple((_iota((ngr, 8, 2 * G), 2) & 8) == 8 * hh for hh in range(2))
        sub1 = (_iota((8, 2 * G), 0) & 1) == 0
        sub2 = (_iota((8, 2 * G), 0) & 2) == 0
        zp = jnp.zeros((ngr, 8, 2 * G), F32)
        first_half = (_iota((8, 2 * G), 1) & 8) == 0
        even_head = (_iota((WS, 8, CW), 2) // (dh // 2)) % 2 == 0
        npair = (NWIN + 1) // 2
        n0 = (HW - 1) // WS // 2

        st = {}
        toks = []
        soft = []
        ticks = []
        j0 = subs[0][0]
        tag = {('qkv', t, r): -1 for t in range(NT) for r in range(WS)}
        tag.update({('o', p): (-1 if p < n0 else None) for p in range(npair)})
        for b, blk in ((j0 % 3, 0), ((j0 + 2) % 3, -1)):
            tag.update({('x', b, c, t, r): blk for c in range(2 * NC) for t in range(NT) for r in range(WS)})
        tag.update({('s', c % 2, stg_row(j0, c // 2, rho)): (0, c, rho) for c in range(NC) for rho in (0, 1)})

        def gather(ref, w):
            return ref[:, pl.ds(WS * w, 8), :]

        def tick(t):
            c = [x for x in ticks if t <= x[0] <= t + 40]
            if not c:
                return None
            _, res, j = min(c, key=lambda x: x[0])
            return res[8 * j:8 * j + 8, 0:LANES]

        def due(lst, nblk, t0, step):
            inj = {}
            for d, tok in list(lst):
                j = max(0, -(-(d - t0) // step))
                if j < nblk:
                    inj.setdefault(j, []).append(tok)
            lst[:] = [x for x in lst if x[0] > t0 + (nblk - 1) * step]
            return inj

        def lhs(ref, ls, inj, dt):
            nblk = ref.shape[0] // 8
            parts, s = [], 0
            for j in sorted(inj):
                if j > s:
                    parts.append(ref[8 * s:8 * j, ls])
                parts.append(tie(ref[8 * j:8 * j + 8, ls], inj[j]))
                s = j + 1
            if s < nblk:
                parts.append(ref[8 * s:8 * nblk, ls])
            return pltpu.bitcast(_cat(parts), dt)

        def merged(a, b):
            return {j: a.get(j, []) + b.get(j, []) for j in set(a) | set(b)}

        def fence(d, b):
            c = [x for x in ticks if x[0] <= d]
            if c:
                _, res, j = max(c, key=lambda x: x[0])
                xbuf[b][zx + WS, 0, 0:8, :] = res[8 * j:8 * j + 8, 0:LANES]

        def ln1(d, k, t, r):
            b = subs[k][0] % 3
            assert all(tag['x', b, c, t, r] == k for c in range(2 * NC))
            x0 = xbuf[b][r, t, 0:C, :]
            s8 = _sum8(x0)
            soft.append((d, _u32(s8)))
            mean = jnp.sum(s8, axis=0, keepdims=True) * (1.0 / C)
            if LNF & 2:
                fence(d + LNG, b)
                x0 = xbuf[b][r, t, 0:C, :]
            st['ln', k, t, r] = [x0 - mean, [], mean]

        def ln3(d, k, t, r):
            b = subs[k][0] % 3
            fence(d, b)
            st['ln', k, t, r][0] = xbuf[b][r, t, 0:C, :] - st['ln', k, t, r][2]

        def ln2(d, n, *key):
            m = C // LNS
            xc = st[('ln',) + key][0][m * n:m * (n + 1)]
            s8 = _sum8(xc * xc)
            soft.append((d, _u32(s8)))
            st[('ln',) + key][1].append(s8)

        def a_dot(t0, k, t, r):
            xc, sq, _ = st.pop(('ln', k, t, r))
            var = jnp.sum(_tree_sum(sq), axis=0, keepdims=True) * (1.0 / C)
            h = xc * lax.rsqrt(var + EPS)
            h = [h[CW * kt:CW * (kt + 1)].astype(BF16) for kt in range(2)]
            inj = due(toks, DA // 16, t0, 16)
            inj0 = merged(inj, due(soft, DA // 16, t0, 16))
            part = [jnp.dot(lhs(wq_s.at[par], slice(LANES * kt, LANES * kt + CW), inj if par or kt else inj0, BF16),
                            h[kt], preferred_element_type=F32)
                    for par in range(2) for kt in range(2)]
            res = [part[0] + part[1], part[2] + part[3]]
            ticks.extend((t0 + MXU_LAT + 8 * j, res[0], j) for j in range(DA // 8))
            qkv = jnp.stack([v.reshape(-1, 16, LANES) for v in res], axis=1).reshape(3 * C, LANES)
            for m in range(3):
                qkv_s[m][r, LANES * t:LANES * (t + 1), 0:CW] = _u32(qkv[C * m:C * (m + 1)].astype(BF16)).T
                toks.append((t0 + 96 * (m + 1) + DL_A, qkv_s[m][zx, 0:8, :]))
            tag['qkv', t, r] = k

        def wins(p):
            return 2 * p, min(2 * p + 1, NWIN - 1)

        def b_qk(t0, k, p):
            wa, wb = wins(p)
            blk = k if p < n0 else k - 1
            assert all(tag['qkv', t, r] == blk for r in range(WS)
                       for t in range(WS * wa // LANES, (WS * wb + WS) // LANES + 1))
            sts = []
            inj = due(soft, WS, t0, 8)
            for w, swap in ((wa, 0), (wb, 1)):
                qw = gather(q_s, w)
                kw = gather(k_s, w).reshape(G, LANES)
                if not swap and inj:
                    kw = _cat([tie(v, inj.get(r, [])) for r, v in enumerate(_rows8(kw))])
                for tile in range(2):
                    kk = _f32(kw & hi if tile else kw << 16)
                    qq = _f32(qw & hi if tile else qw << 16)
                    qst = jnp.stack([lax.select(head[swap], qq, zq), lax.select(head[1 - swap], qq, zq)], axis=1)
                    sts.append(lax.dot_general(kk, qst.reshape(2 * G, LANES), (((1,), (1,)), ((), ())),
                                               preferred_element_type=F32))
            if PVP:
                vw = _cat([gather(v_s, wa), zt[None], gather(v_s, wb), zt[None]]).reshape(LANES, LANES)
            else:
                vw = _cat([gather(v_s, wa), gather(v_s, wb)]).reshape(2 * G, LANES)
            vt = vw[:, 0:CW].T
            if VST:
                st['nv'] = st.get('nv', 0) + 1
                ref = vts[st['nv'] % len(vts)]
                st['nv', p] = st['nv']
                ref[0, :, 0:vt.shape[1]] = vt
                if VDL:
                    soft.append((tpv[k, p] - VDL, ref[zx + 1, 0:8, :]))
                vt = (ref, vt.shape[1])
            st['s', p] = (sts, vt)

        def b_pv(t0, tg, k, p):
            wa, wb = wins(p)
            sts, vt = st.pop(('s', p))
            if VST:
                vt[0][zx + 1, 8:16, :] = zt
                vt = lhs(vt[0].at[0], slice(0, vt[1]), due(soft, 3, t0, 16) if PVI else {}, BF16)
            else:
                vt = pltpu.bitcast(vt, BF16)
            if SST:
                sref = sts_s[st['nv', p] % len(sts_s)]
                for n, s_t in enumerate(sts):
                    sref[n, 0:G, 0:2 * G] = s_t
                c = [x for x in ticks if x[0] <= tg]
                _, res, j = max(c, key=lambda x: x[0]) if c else (0, _f32(zt), 0)
                sref[zx + 4, 0:8, :] = res[8 * j:8 * j + 8, 0:LANES]
            pts = []
            dens = []
            for n, s_t in enumerate(sts):
                m8 = _fold7(jnp.maximum, s_t)
                mx = _all8(jnp.maximum, lax.select(junk8, ninf8, m8))
                mv = lax.select(junk8, -ninf8, mx)
                z = tick(tg + SMD * (3 - n)) if SST != 1 else None
                if z is not None:
                    mv = tie(mv, [z])
                if SST:
                    s_t = sref[n, 0:G, 0:2 * G]
                eg = jnp.exp2(s_t.reshape(WS, 8, 2 * G) - mv)
                dens.append(_fold7(jnp.add, eg.reshape(G, 2 * G)))
                pts.append(_cat([eg, eg[WS - 1:WS]]) if PVP else eg)
            if MRG:
                def mix(m, sh, a, b):
                    return lax.select(m, a, b) + pltpu.roll(lax.select(m, b, a), sh, 0)
                den = mix(sub2, 2, mix(sub1, 1, dens[0], dens[1]), mix(sub1, 1, dens[2], dens[3]))
                den = den + pltpu.roll(den, 4, 0)
                r0 = pl.reciprocal(den, approx=True)
                r0 = r0 * (2.0 - den * r0)
                r0 = lax.select(first_half, r0, pltpu.roll(r0, 2, 0))
                rsel = [jnp.broadcast_to(r0[n:n + 1], r0.shape) for n in range(4)]
            else:
                rinv = []
                for den in dens:
                    den = _all8(jnp.add, den)
                    r0 = pl.reciprocal(den, approx=True)
                    rinv.append(r0 * (2.0 - den * r0))
                rsel = [lax.select(first_half, rinv[n], rinv[(n + 2) % 4]) for n in range(4)]
            outs = []
            for tile in range(2):
                for hh in range(2):
                    h = 2 * tile + hh
                    stn = _cat([lax.select(key_ok[hh], pts[tile], zp), lax.select(key_ok[1 - hh], pts[2 + tile], zp)])
                    ot = jnp.dot(vt[dh * h:dh * (h + 1), :], stn.reshape(-1, 2 * G).astype(BF16),
                                 preferred_element_type=F32)
                    outs.append(ot.reshape(dh // 8, 8, 2 * G) * rsel[2 * hh + tile])
            tw = _u32(_cat(outs).reshape(C, 2 * G).astype(BF16)).T.reshape(WS, 2, 8, CW)
            tw = (tw[:, 0], tw[:, 1])
            o_s[:, pl.ds(WS * wa, 8), 0:CW] = lax.select(even_head, tw[0], tw[1])
            if wb != wa:
                o_s[:, pl.ds(WS * wb, 8), 0:CW] = lax.select(even_head, tw[1], tw[0])
                tag['o', p + 1] = None
            toks.append((t0 + DL_PV, o_s[zx, 0:8, :]))
            tag['o', p] = k if p < n0 else k - 1
            if p == n0:
                tag['o2'] = k - 1

        def c_dot(t0, k, h, r):
            b = (subs[k][0] + 2) % 3
            assert all(tag['o', p] == k - 1 for p in (range(n0 + 1) if h == 0 else range(n0 + 1, npair)))
            assert tag['o2'] == k - 1 and 2 * WS * n0 < HW
            assert all(tag['x', b, c, t, r] == k - 1 for c in range(2 * NC) for t in (2 * h, 2 * h + 1))
            ls = slice(HW * h, HW * (h + 1))
            ow = o_s[r, ls, :]
            rhs = _cat([_f32(ow << 16), _f32(ow & hi)], axis=1)
            inj = due(toks, DC // 8, t0, 8)
            wo = _cat([lhs(wo_s, slice(0, LANES), merged(inj, due(soft, DC // 8, t0, 8)), F32),
                       lhs(wo_s, slice(LANES, 2 * LANES), inj, F32)], axis=1)
            res = lax.dot_general(wo, rhs, (((1,), (1,)), ((), ())), preferred_element_type=F32)
            ticks.extend((t0 + MXU_LAT + 8 * j, res, j) for j in range(DC // 8))
            slot = subs[k][2]
            n = min(HW, W - HW * h)
            xout[slot][row0(slot, g) + r, :, HW * h:HW * h + n] = (_cat([xbuf[b][r, t, 0:C, :] for t in (2 * h, 2 * h + 1)], axis=1) + res)[:, 0:n].astype(BF16)
            if h == 1 and not subs[k][3]:
                out_copy(slot, g, r, 1).start()
            elif h == 1 and r == WS - 1:
                out_copy(slot, g).start()
                xout[slot][zx + xout[slot].shape[0] - 1, 0:16, 0:LANES] = jnp.zeros((16, LANES), BF16)
                soft.append((t0 + MXU_LAT + DC + DL_D, _u32(xout[slot][zy + xout[slot].shape[0] - 1, 0:16, 0:LANES])))

        def stage_row(d, k, c, rho):
            j, slot = subs[k][0:2]
            cs = slice(16 * c, 16 * c + 16)
            u = _u32(xin[slot][row0(slot, g) + rho - 2, cs, :])
            if rho == WS + 1 and slot == 1:
                u = jnp.where(g < ng - 2, u, zero)
            idx = stg_row(j, c // 2, rho)
            stg[c % 2][idx] = shifted(u)
            soft.append((d, stg[c % 2][zx + SPARE, 8:16, 0:LANES]))
            tag['s', c % 2, idx] = (k, c, rho)
            if c == NC - 1 and rho == WS + 1 and slot < NSUB - 1:
                for cp in in_copies(slot, g + 1):
                    cp.start()
                xin[slot][zx + WS, 0:16, 0:LANES] = jnp.zeros((16, LANES), BF16)
                soft.append((d + DL_D, _u32(xin[slot][zy + WS, 0:16, 0:LANES])))

        def conv_step(d, k, c, hf, t, r):
            j = subs[k][0]
            if r == 0:
                if t == 0:
                    stg[c % 2][zx + SPARE, 0:8, 0:LANES] = zt
                    st['w'] = [dw_s[2 * c + hf, ki] for ki in range(3)]
                st['un'] = {}
            un = st['un']
            for rho in range(r, r + 3):
                if rho not in un:
                    idx = stg_row(j, c // 2, rho)
                    assert tag['s', c % 2, idx] in ((k, c, rho), (k - 1, c, rho + WS))
                    un[rho] = unpack(stg[c % 2][idx, 24 * t:24 * t + 24, :], hf)
            acc = conv_row(un, st['w'], r)
            xbuf[(j + 1) % 3][r, t, 16 * c + 8 * hf:16 * c + 8 * hf + 8, :] = acc
            soft.append((d, _u32(acc)))
            tag['x', (j + 1) % 3, 2 * c + hf, t, r] = k + 1

        plan, offs = [], [0]
        for k, sub in enumerate(subs):
            pk, tk = _plan(npair, n0, NT, sub[3], sub[4])
            plan += [(offs[k] + t, kind, k, idx) for t, kind, idx in pk]
            offs.append(offs[k] + tk)
        total = offs[-1]
        starts = [e[0] for e in plan]
        ev = []

        def at(t, fn, *a):
            ev.append((t, t, len(ev), fn, a))

        def before(d, fn, *a):
            ev.append((max([t for t in starts if t <= d], default=0) - 1, d, len(ev), fn, a))

        load = [0.0] * (total + 1000)
        tqk = {}
        tpv = {(k, idx): t for t, kind, k, idx in plan if kind == 'pv'}

        def add(t0, t1, n):
            for t in range(max(t0, 0), max(t1, 0)):
                load[t] += n / (t1 - t0)

        for t, kind, k, idx in plan:
            tr = t + MXU_LAT
            if kind == 'a':
                if idx == (0, 0) and k > 0:
                    before(t - LN1 - 1, fence, t - LN1 - 40, subs[k][0] % 3)
                before(t - LN1, ln1, t - LN1, k, *idx)
                for n in range(LNS):
                    d = t - LN2 - LND * (LNS - 1 - n)
                    before(d, ln2, d, n, k, *idx)
                    add(d - 16, d, 72 // LNS)
                if LNF & 1:
                    before(t - LN3, ln3, t - LN3, k, *idx)
                    add(t - 40, t, 24)
                at(t, a_dot, t, k, *idx)
                add(tr, tr + DA, 12 * DA // 16)
                add(t - LN1 - 16, t - LN1, 32); add(t - LN2, t - 40, 20); add(t - 40, t, 36)
            elif kind == 'qk':
                at(t, b_qk, t, k, idx)
                tqk[idx] = t
                add(t - 64, t, 28); add(t, t + DQ, 28); add(tr, tr + DQ, 24); add(tr + DQ, tr + DQ + 16, 36)
            elif kind == 'pv':
                tg = max(tqk[idx] + SM0, t - SMB)
                at(t, b_pv, t, tg, k, idx)
                add(tg, tg + 4 * SMD + 16, 80); add(tr - 10, tr + 6, 46); add(tr, tr + DP, 36)
                add(t + 400, t + 460, 14)
            else:
                if idx == (0, 0) and k > 0:
                    at(t - 1, fence, t - 100, (subs[k][0] + 2) % 3)
                at(t, c_dot, t, k, *idx)
                add(tr, tr + DC, 20 * DC // 16)
                add(t - 70, t, 64)
        pre = [0.0]
        for v in load:
            pre.append(pre[-1] + v)
        nstep = NC * 2 * NT * WS
        prev_chunk = 10
        for k, sub in enumerate(subs):
            if not sub[3]:
                continue
            ta = offs[k] + (CVI if k else CV0) - 20
            tb = offs[k + 1] - (CVE if k == len(subs) - 1 else CVX)
            cap = CAP if sub[4] else 64
            free = [max(0.02, cap / 16 - (pre[t + SMO] - pre[max(t - SMO, 0)]) / (2 * SMO)) for t in range(ta, tb)]
            tot_free, acc, tstep = sum(free), 0.0, []
            for t, v in enumerate(free):
                acc += v
                while len(tstep) < nstep and acc >= (len(tstep) + 1) * tot_free / nstep - 1e-6:
                    tstep.append(ta + t)
            for n in range(nstep):
                before(tstep[n], conv_step, tstep[n], k, n // (2 * NT * WS), n // (NT * WS) % 2, n // WS % NT, n % WS)
            for c in range(NC):
                t1 = tstep[c * 2 * NT * WS] - 30
                t0 = prev_chunk + 120
                prev_chunk = t1 + 30
                for rho in range(2, NR):
                    d = t0 + (t1 - t0) * (rho - 2) // (NR - 3)
                    before(d, stage_row, d, k, c, rho)
        ev.sort(key=lambda e: e[:3])
        for e in ev:
            e[3](*e[4])
        if subs[-1][3]:
            n = len(subs)
            assert all(tag['qkv', t, r] == n - 1 for t in range(NT) for r in range(WS))
            assert all(tag['o', p] == n - 1 for p in range(n0))

    if ONLY in (0, 1):
        @pl.when(g == 0)
        def _():
            setup()
            body([(0, 2, 0, True, False)])

    @pl.when(g > 0)
    def _():
        for k in range(NSUB):
            for cp in in_copies(k, g):
                cp.wait()

    @pl.when((g > 0) & (g < ng - 1))
    def _():
        for cp in in_copies(NSUB - 1, g + 1):
            cp.start()

    @pl.when(g > 1)
    def _():
        for k in range(NSUB - 1):
            out_copy(k, g - 1).wait()

    @pl.when(g > 2)
    def _():
        out_copy(NSUB - 1, g - 2).wait()

    if ONLY in (0, 2):
        @pl.when((g > 0) & (g < ng - 1))
        def _():
            body([(1 + k, k, k, True, True) for k in range(NSUB)])

    if ONLY in (0, 3):
        @pl.when(g == ng - 1)
        def _():
            body([(1, 0, 0, False, True)])
            out_copy(NSUB - 1, g - 1).wait()
            out_copy(0, g).wait()


@jax.jit
def pallas_standalone__window_attn_davit__vision_kernel(
    x: jax.Array,
    dw_pe: jax.Array,
    w_qkv: jax.Array,
    w_o: jax.Array,
):
    B, H, W, C = x.shape
    assert B == 1 and H % WS == 0 and W % WS == 0 and C % (16 * NH) == 0
    WP = -(-(W + 1) // (2 * LANES)) * (2 * LANES)
    assert WP == 4 * LANES
    NWIN = W // WS
    NBLK = H // WS
    assert (NBLK - 1) % NSUB == 0
    NM = (NBLK - 1) // NSUB

    xt = jnp.transpose(x[0], (0, 2, 1))

    nstg = WS - 2 + NSUB * (C // 32) * 2 + 1
    kern = functools.partial(_kernel, C=C, H=H, W=W, WP=WP, NWIN=NWIN)
    out = pl.pallas_call(
        kern,
        grid=(NM + 2,),
        in_specs=[pl.BlockSpec(memory_space=pl.ANY)] * 4,
        out_specs=pl.BlockSpec(memory_space=pl.ANY),
        out_shape=jax.ShapeDtypeStruct((H, C, W), x.dtype),
        scratch_shapes=[
            pltpu.VMEM((WS + 1, WP // LANES, C + 8, LANES), F32),
            pltpu.VMEM((WS + 1, WP // LANES, C + 8, LANES), F32),
            pltpu.VMEM((WS + 1, WP // LANES, C + 8, LANES), F32),
            pltpu.VMEM((WS, WP + 8, LANES), U32),
            pltpu.VMEM((WS, WP + 8, LANES), U32),
            pltpu.VMEM((WS, WP + 8, LANES), U32),
            pltpu.VMEM((WS, WP + 8, LANES), U32),
            pltpu.VMEM((2, 3 * C // 4, 2 * LANES), U32),
            pltpu.VMEM((C, 2 * LANES), U32),
            pltpu.VMEM((nstg, WP // LANES * 24, LANES), U32),
            pltpu.VMEM((nstg, WP // LANES * 24, LANES), U32),
            pltpu.VMEM((C // 8, 3, 3, 8, LANES), F32),
            pltpu.VMEM((WS + 1, C, W), BF16),
            pltpu.VMEM((WS + 1, C, W), BF16),
            pltpu.VMEM((2 * WS + 1, C, W), BF16),
            pltpu.VMEM((WS + 1, C, W), BF16),
            pltpu.VMEM((WS + 1, C, W), BF16),
            pltpu.VMEM((2 * WS + 1, C, W), BF16),
            pltpu.VMEM((2, C // 2, LANES), U32),
            pltpu.VMEM((2, C // 2, LANES), U32),
            pltpu.VMEM((2, C // 2, LANES), U32),
            pltpu.VMEM((2, C // 2, LANES), U32),
            pltpu.VMEM((5, 8 * WS + 16, LANES), F32),
            pltpu.VMEM((5, 8 * WS + 16, LANES), F32),
            pltpu.VMEM((5, 8 * WS + 16, LANES), F32),
            pltpu.VMEM((5, 8 * WS + 16, LANES), F32),
            pltpu.VMEM(dw_pe.shape, BF16),
            pltpu.VMEM(w_qkv.shape, BF16),
            pltpu.VMEM(w_o.shape, BF16),
            pltpu.SemaphoreType.DMA((2 * NSUB,)),
            pltpu.SemaphoreType.DMA((NSUB + 1,)),
            pltpu.SemaphoreType.DMA((3 + C // 32,)),
        ],
        compiler_params=pltpu.CompilerParams(
            dimension_semantics=("arbitrary",),
            vmem_limit_bytes=96 * 1024 * 1024,
            disable_bounds_checks=bool(NOBC),
        ),
        name="davit_window_attn",
    )(xt, dw_pe, w_qkv, w_o)
    return jnp.transpose(out, (0, 2, 1))[None]
```

```python
import functools
import math
import os

import jax
import jax.numpy as jnp
from jax import lax
import jax.experimental.pallas as pl
import jax.experimental.pallas.tpu as pltpu

WS = 7
NH = 4
EPS = 1e-05
LANES = 128
F32 = jnp.float32
BF16 = jnp.bfloat16
U32 = jnp.uint32

P = lambda k, d: int(os.environ.get(k, d))
DL_A = P('DL_A', 500)
LAT_QK = P('LAT_QK', 280)
DL_PV = P('DL_PV', 580)
PRE_C = P('PRE_C', 120)
TAIL = P('TAIL', 1400)
LN1 = P('LN1', 200)
LN2 = P('LN2', 130)
LNS = P('LNS', 3)
LND = P('LND', 16)
SM0 = P('SM0', 200)
SMD = P('SMD', 16)
SMB = P('SMB', 140)
CV0 = P('CV0', 450)
CVI = P('CVI', 170)
CVE = P('CVE', 60)
CVX = P('CVX', 180)
ORD = P('ORD', 1)
CAP = P('CAP', 42)
SMO = P('SMO', 32)
ONLY = P('ONLY', 0)
CBF = P('CBF', 1)
WA = P('WA', 7)
WC = P('WC', 11)
WQ = P('WQ', 40)
MIX = P('MIX', 1)
ZK = P('ZK', 1)
EC0 = P('EC0', 1500)
ECD = P('ECD', 900)
PVI = P('PVI', 1)
SST = P('SST', 0)
VST = P('VST', 1)
VDL = P('VDL', 60)
MRG = P('MRG', 0)
DL_D = P('DL_D', 100)
PVP = P('PVP', 1)
LNF = P('LNF', 3)
LN3 = P('LN3', 60)
LNG = P('LNG', 16)
NOBC = P('NOBC', 1)
DA, DC, DQ, DP = 288, 192, 56, 48
MXU_LAT = 130
NSUB = 3


def _iota(shape, dim):
    return lax.broadcasted_iota(jnp.int32, shape, dim)


def _plan(nwin, w0, w1, nt, cur, prev):
    a_q = [(t, r) for t in range(nt) for r in range(WS)] if cur else []
    c_q = [(h, r) for h in range(2) for r in range(WS)] if prev else []
    old = [(-1, w) for w in range(w0, nwin)] if prev else []
    new = [(0, w) for w in range(w1)] if cur else []
    ws = old + old[-1:] * ((len(old) + len(new)) % 2) + new
    pairs = list(zip(ws[0::2], ws[1::2]))
    n1 = sum(a[0] < 0 for a, _ in pairs)
    nh = sum(a[0] < 0 and WS * a[1] < nt * LANES // 2 for a, _ in pairs)
    total = len(a_q) * DA + len(c_q) * DC + len(pairs) * (DQ + DP)
    q0 = 0 if prev else total // 3
    t = 0
    ia = ic = iq = ip = 0
    out = []
    tq, tp, ta = {}, {}, {}
    last = None
    while ia < len(a_q) or ic < len(c_q) or ip < len(pairs):
        cands = []
        if ip < iq and t >= tq[ip] + LAT_QK:
            cands.append((-1e6, 'pv'))
        if iq < len(pairs) and (not cur or (iq - ip < 2 and last != 'qk' and not (ORD and last == 'pv'))):
            ok = iq - ip < 4
            if pairs[iq][1][0] == 0:
                need = (WS * pairs[iq][1][1] + WS) // LANES * WS + WS - 1
                ok = ia > need and t >= ta[need] + DA + DL_A + 60 and ic >= len(c_q) // 2
            if ok:
                pr = q0 + iq * (total - q0 - TAIL) / len(pairs) - t - 200
                cands.append((-2e6 if ORD and pr <= 0 else pr, 'qk'))
        if ia < len(a_q):
            cands.append((ia * (total - 700) / len(a_q) - t, 'a'))
        if ic < len(c_q):
            need = nh - 1 if ic < WS else n1 - 1
            if ip > need and t >= tp[need] + DL_PV + PRE_C:
                if cur:
                    tc = 1000 + ic * 900 if ic < WS else total - DC - (2 * WS - 1 - ic) * 950
                else:
                    tc = EC0 + ic * ECD
                cands.append((tc - t, 'c'))
        if not cands:
            t += 8
            last = None
            continue
        kind = min(cands)[1]
        last = kind
        if kind == 'pv':
            tp[ip] = t; out.append((t, 'pv', pairs[ip])); ip += 1; t += DP
        elif kind == 'qk':
            tq[iq] = t; out.append((t, 'qk', pairs[iq])); iq += 1; t += DQ
        elif kind == 'a':
            ta[ia] = t; out.append((t, 'a', a_q[ia])); ia += 1; t += DA
        else:
            out.append((t, 'c', c_q[ic])); ic += 1; t += DC
    return out, t


def _tree_sum(xs):
    while len(xs) > 1:
        xs = [xs[j] + xs[j + 1] if j + 1 < len(xs) else xs[j] for j in range(0, len(xs), 2)]
    return xs[0]


def _sum8(x):
    while x.shape[0] % 16 == 0:
        x = x[:x.shape[0] // 2] + x[x.shape[0] // 2:]
    return _tree_sum(_rows8(x))


def _fold7(op, x):
    t = op(x[0:24], x[24:48])
    return op(op(t[0:8], t[8:16]), op(t[16:24], x[48:56]))


def _all8(op, x):
    for sh in (4, 2, 1):
        x = op(x, pltpu.roll(x, sh, 0))
    return x


def _rows8(x):
    return [x[8 * j:8 * j + 8] for j in range(x.shape[0] // 8)]


def _cat(xs, axis=0):
    return jnp.concatenate(xs, axis=axis) if len(xs) > 1 else xs[0]


def _f32(u):
    return pltpu.bitcast(u, F32)


def _u32(x):
    return pltpu.bitcast(x, U32)


def _kernel(x_hbm, dw_hbm, wqkv_hbm, wo_hbm, o_hbm,
            xa_s, xb_s, xc_s, q_s, k_s, v_s, o_s, wq_s, wo_s, sa_s, sb_s, dw_s,
            i0_s, i1_s, i2_s, o0_s, o1_s, o2_s, va_s, vb_s, vc_s, vd_s, ta_s, tb_s, tc_s, td_s, dw_ref, wqkv_ref, wo_ref, in_sem, out_sem, w_sem,
            *, C, H, W, WP, NWIN):
    g = pl.program_id(0)
    ng = pl.num_programs(0)
    dh = C // NH
    CW = C // 2
    NT = WP // LANES
    G = WS * 8
    HW = WP // 2
    NC = C // 16
    NR = WS + 2
    lane8 = _iota((8, LANES), 1)
    last_valid = W - (NT - 1) * LANES
    zero = jnp.uint32(0)
    hi = jnp.uint32(0xFFFF0000)
    qkv_s = (q_s, k_s, v_s)
    xbuf = (xa_s, xb_s, xc_s)
    xin = (i0_s, i1_s, i2_s)
    xout = (o0_s, o1_s, o2_s)

    def row0(k, m):
        return (m & 1) * WS if k == NSUB - 1 else 0

    def in_copies(k, m):
        r = WS * (NSUB * m - 1 + k) + 1
        return [pltpu.make_async_copy(x_hbm.at[pl.ds(jnp.minimum(r + o, H - n), n)],
                                      xin[k].at[pl.ds(row0(k, m) + o, n)], in_sem.at[2 * k + e])
                for e, (o, n) in enumerate(((0, WS - 1), (WS - 1, 1)))]

    def out_copy(k, m, o=0, n=WS):
        return pltpu.make_async_copy(xout[k].at[pl.ds(row0(k, m) + o, n)],
                                     o_hbm.at[pl.ds(WS * (NSUB * (m - 1) + k) + o, n)],
                                     out_sem.at[k + (m & 1) if k == NSUB - 1 else k])

    stg = (sa_s, sb_s)
    vts = (va_s, vb_s, vc_s, vd_s)
    sts_s = (ta_s, tb_s, tc_s, td_s)
    SPARE = sa_s.shape[0] - 1
    zx = g >> 10
    zy = g >> 11
    never = lane8 < zx

    def tie(x, toks):
        if not toks:
            return x
        tok = functools.reduce(lax.bitwise_or, toks)
        n = x.shape[1]
        return lax.select(never[:, 0:n], tok[:, 0:n], x) if n < LANES else lax.select(never, tok, x)

    def stg_row(j, c2, rho):
        if 2 <= rho < WS:
            return rho - 2
        slot = j % NSUB if rho >= WS else (j - 1) % NSUB
        return WS - 2 + (slot * (NC // 2) + c2) * 2 + rho % WS

    zt = jnp.zeros((8, LANES), U32)
    is_first, is_last = lane8 == 0, lane8 == LANES - 1

    def shifted(u):
        tiles = [u[:, LANES * t:LANES * (t + 1)] for t in range(NT)]
        tiles[NT - 1] = _cat([tiles[NT - 1], zt[:, last_valid:]], axis=1)
        left = [pltpu.roll(lax.select(is_last, tiles[t - 1] if t > 0 else zt, tiles[t]), 1, 1)
                for t in range(NT)]
        right = [pltpu.roll(lax.select(is_first, tiles[t + 1], tiles[t]) if t < NT - 1 else tiles[t], LANES - 1, 1)
                 for t in range(NT)]
        return _cat([v[t] for t in range(NT) for v in (left, tiles, right)])

    def unpack(v, hf):
        return pltpu.bitcast(v, BF16).astype(F32).reshape(3, 2, 8, LANES)[:, hf]

    def conv_row(un, w, r):
        return jnp.sum(_tree_sum([un[r + ki] * w[ki] for ki in range(3) if un[r + ki] is not None]), axis=0)

    def setup():
        wcp = [pltpu.make_async_copy(src, dst, w_sem.at[n])
               for n, (src, dst) in enumerate(((dw_hbm, dw_ref), (wqkv_hbm, wqkv_ref), (wo_hbm, wo_ref)))]
        def top(c2):
            cs = pl.ds(pl.multiple_of(32 * c2, 32), 32)
            return pltpu.make_async_copy(x_hbm.at[pl.ds(0, WS + 1), cs], i1_s.at[:, cs], w_sem.at[3 + c2])
        for cp in wcp + [top(c2) for c2 in range(NC // 2)]:
            cp.start()

        def zrow(r, carry):
            for ref in ((k_s, o_s) if ZK else (q_s, k_s, v_s, o_s)):
                ref[r, 0:WP, :] = jnp.zeros((WP, LANES), U32)
            return carry
        lax.fori_loop(0, WS, zrow, 0)
        for ref in (q_s, v_s):
            ref[0, 0:8, :] = zt
        for ref in stg:
            ref[SPARE, 0:16, :] = jnp.zeros((16, LANES), U32)
        for ref in vts:
            ref[1, 0:8, :] = zt
        for ref in (i0_s,) + xout:
            ref[ref.shape[0] - 1, 0:16, 0:LANES] = jnp.zeros((16, LANES), BF16)
        wo_s[...] = jnp.zeros(wo_s.shape, U32)
        for cp in wcp:
            cp.wait()
        for ki in range(3):
            w3 = dw_ref[ki].astype(F32)
            for kj in range(3):
                w = w3[kj:kj + 1] + 1.0 if ki == kj == 1 else w3[kj:kj + 1]
                dw_s[:, ki, kj] = jnp.broadcast_to(w, (LANES, C)).T.reshape(C // 8, 8, LANES)
        qscale = (dh ** -0.5) * math.log2(math.e)
        for kt in range(2):
            wt = wqkv_ref[CW * kt:CW * (kt + 1), :].astype(F32).T
            wq = (wt[0:C] * qscale).astype(BF16).astype(F32)
            words = [(_u32(w[0:CW]) >> 16) | (_u32(w[CW:C]) & hi) for w in (wq, wt[C:2 * C])]
            words = _rows8(_cat(words + [_u32(wt[2 * C:].astype(BF16))]))
            for par in range(2):
                wq_s[par, :, LANES * kt:LANES * kt + CW] = _cat(words[par::2])
        wo = _u32(wo_ref[...])
        for kt, w in enumerate((wo << 16, wo & hi)):
            wo_s[:, LANES * kt:LANES * kt + CW] = _u32(_f32(w.T).astype(BF16)) if CBF else w.T

        def conv0(c2, carry):
            top(c2).wait()

            @pl.when(c2 == 2)
            def _():
                for cp in in_copies(2, 0):
                    cp.start()
            for par in range(2):
                cs = pl.ds(pl.multiple_of(32 * c2 + 16 * par, 16), 16)
                sh = [shifted(_u32(i1_s[r, cs, :])) for r in range(WS + 1)]
                for rho in (WS, WS + 1):
                    stg[par][stg_row(-1, c2, rho)] = sh[rho - 1]
                for hf in range(2):
                    c8 = 4 * c2 + 2 * par + hf
                    w = [dw_s[c8, ki] for ki in range(3)]
                    for t in range(NT):
                        un = [None] + [unpack(row[24 * t:24 * t + 24], hf) for row in sh]
                        for r in range(WS):
                            xbuf[0][r, t, pl.ds(pl.multiple_of(8 * c8, 8), 8), :] = conv_row(un, w, r)
            return carry
        lax.fori_loop(0, NC // 2, conv0, 0)
        for cp in in_copies(0, 1) + in_copies(1, 1):
            cp.start()
        for cp in in_copies(2, 0):
            cp.wait()
        for cp in in_copies(2, 1):
            cp.start()

    def body(subs):
        lane3 = _iota((WS, 8, LANES), 2)
        head = (lane3 < dh, (lane3 >= dh) & (lane3 < 2 * dh))
        zq = jnp.zeros((WS, 8, LANES), F32)
        junk8 = _iota((8, 2 * G), 0) == WS
        ninf8 = jnp.full((8, 2 * G), -jnp.inf, F32)
        ngr = WS + PVP
        key_ok = tuple((_iota((ngr, 8, 2 * G), 2) & 8) == 8 * hh for hh in range(2))
        sub1 = (_iota((8, 2 * G), 0) & 1) == 0
        sub2 = (_iota((8, 2 * G), 0) & 2) == 0
        zp = jnp.zeros((ngr, 8, 2 * G), F32)
        first_half = (_iota((8, 2 * G), 1) & 8) == 0
        even_head = (_iota((WS, 8, CW), 2) // (dh // 2)) % 2 == 0
        wsp = (HW - 1) // WS

        st = {}
        toks = []
        soft = []
        ticks = []
        j0 = subs[0][0]
        tag = {('qkv', t, r): -1 for t in range(NT) for r in range(WS)}
        tag.update({('o', w): (-1 if w < wsp else None) for w in range(NWIN)})
        dirty = {wsp}
        for b, blk in ((j0 % 3, 0), ((j0 + 2) % 3, -1)):
            tag.update({('x', b, c, t, r): blk for c in range(2 * NC) for t in range(NT) for r in range(WS)})
        tag.update({('s', c % 2, stg_row(j0, c // 2, rho)): (0, c, rho) for c in range(NC) for rho in (0, 1)})

        def gather(ref, w):
            return ref[:, pl.ds(WS * w, 8), :]

        def tick(t):
            c = [x for x in ticks if t <= x[0] <= t + 40]
            if not c:
                return None
            _, res, j = min(c, key=lambda x: x[0])
            return res[8 * j:8 * j + 8, 0:LANES]

        def due(lst, nblk, t0, step):
            inj = {}
            for d, tok in list(lst):
                j = max(0, -(-(d - t0) // step))
                if j < nblk:
                    inj.setdefault(j, []).append(tok)
            lst[:] = [x for x in lst if x[0] > t0 + (nblk - 1) * step]
            return inj

        def lhs(ref, ls, inj, dt):
            nblk = ref.shape[0] // 8
            parts, s = [], 0
            for j in sorted(inj):
                if j > s:
                    parts.append(ref[8 * s:8 * j, ls])
                parts.append(tie(ref[8 * j:8 * j + 8, ls], inj[j]))
                s = j + 1
            if s < nblk:
                parts.append(ref[8 * s:8 * nblk, ls])
            return pltpu.bitcast(_cat(parts), dt)

        def merged(a, b):
            return {j: a.get(j, []) + b.get(j, []) for j in set(a) | set(b)}

        def fence(d, b):
            c = [x for x in ticks if x[0] <= d]
            if c:
                _, res, j = max(c, key=lambda x: x[0])
                xbuf[b][zx + WS, 0, 0:8, :] = res[8 * j:8 * j + 8, 0:LANES]

        def ln1(d, k, t, r):
            b = subs[k][0] % 3
            assert all(tag['x', b, c, t, r] == k for c in range(2 * NC))
            x0 = xbuf[b][r, t, 0:C, :]
            s8 = _sum8(x0)
            soft.append((d, _u32(s8)))
            mean = jnp.sum(s8, axis=0, keepdims=True) * (1.0 / C)
            if LNF & 2:
                fence(d + LNG, b)
                x0 = xbuf[b][r, t, 0:C, :]
            st['ln', k, t, r] = [x0 - mean, [], mean]

        def ln3(d, k, t, r):
            b = subs[k][0] % 3
            fence(d, b)
            st['ln', k, t, r][0] = xbuf[b][r, t, 0:C, :] - st['ln', k, t, r][2]

        def ln2(d, n, *key):
            m = C // LNS
            xc = st[('ln',) + key][0][m * n:m * (n + 1)]
            s8 = _sum8(xc * xc)
            soft.append((d, _u32(s8)))
            st[('ln',) + key][1].append(s8)

        def a_dot(t0, k, t, r):
            xc, sq, _ = st.pop(('ln', k, t, r))
            var = jnp.sum(_tree_sum(sq), axis=0, keepdims=True) * (1.0 / C)
            h = xc * lax.rsqrt(var + EPS)
            h = [h[CW * kt:CW * (kt + 1)].astype(BF16) for kt in range(2)]
            inj = due(toks, DA // 16, t0, 16)
            inj0 = merged(inj, due(soft, DA // 16, t0, 16))
            part = [jnp.dot(lhs(wq_s.at[par], slice(LANES * kt, LANES * kt + CW), inj if par or kt else inj0, BF16),
                            h[kt], preferred_element_type=F32)
                    for par in range(2) for kt in range(2)]
            res = [part[0] + part[1], part[2] + part[3]]
            ticks.extend((t0 + MXU_LAT + 8 * j, res[0], j) for j in range(DA // 8))
            qkv = jnp.stack([v.reshape(-1, 16, LANES) for v in res], axis=1).reshape(3 * C, LANES)
            for m in range(3):
                qkv_s[m][r, LANES * t:LANES * (t + 1), 0:CW] = _u32(qkv[C * m:C * (m + 1)].astype(BF16)).T
                toks.append((t0 + 96 * (m + 1) + DL_A, qkv_s[m][zx, 0:8, :]))
            tag['qkv', t, r] = k

        def b_qk(t0, k, p):
            (_, wa), (_, wb) = p
            assert all(tag['qkv', t, r] == k + rel for r in range(WS) for rel, w in p
                       for t in range(WS * w // LANES, min(WS * w + WS, WP - 1) // LANES + 1))
            sts = []
            inj = due(soft, WS, t0, 8)
            for w, swap in ((wa, 0), (wb, 1)):
                qw = gather(q_s, w)
                kw = gather(k_s, w).reshape(G, LANES)
                if not swap and inj:
                    kw = _cat([tie(v, inj.get(r, [])) for r, v in enumerate(_rows8(kw))])
                for tile in range(2):
                    kk = _f32(kw & hi if tile else kw << 16)
                    qq = _f32(qw & hi if tile else qw << 16)
                    qst = jnp.stack([lax.select(head[swap], qq, zq), lax.select(head[1 - swap], qq, zq)], axis=1)
                    sts.append(lax.dot_general(kk, qst.reshape(2 * G, LANES), (((1,), (1,)), ((), ())),
                                               preferred_element_type=F32))
            if PVP:
                vw = _cat([gather(v_s, wa), zt[None], gather(v_s, wb), zt[None]]).reshape(LANES, LANES)
            else:
                vw = _cat([gather(v_s, wa), gather(v_s, wb)]).reshape(2 * G, LANES)
            vt = vw[:, 0:CW].T
            if VST:
                st['nv'] = st.get('nv', 0) + 1
                ref = vts[st['nv'] % len(vts)]
                st['nv', p] = st['nv']
                ref[0, :, 0:vt.shape[1]] = vt
                if VDL:
                    soft.append((tpv[k, p] - VDL, ref[zx + 1, 0:8, :]))
                vt = (ref, vt.shape[1])
            st['s', p] = (sts, vt)

        def b_pv(t0, tg, k, p):
            (_, wa), (_, wb) = p
            sts, vt = st.pop(('s', p))
            if VST:
                vt[0][zx + 1, 8:16, :] = zt
                vt = lhs(vt[0].at[0], slice(0, vt[1]), due(soft, 3, t0, 16) if PVI else {}, BF16)
            else:
                vt = pltpu.bitcast(vt, BF16)
            if SST:
                sref = sts_s[st['nv', p] % len(sts_s)]
                for n, s_t in enumerate(sts):
                    sref[n, 0:G, 0:2 * G] = s_t
                c = [x for x in ticks if x[0] <= tg]
                _, res, j = max(c, key=lambda x: x[0]) if c else (0, _f32(zt), 0)
                sref[zx + 4, 0:8, :] = res[8 * j:8 * j + 8, 0:LANES]
            pts = []
            dens = []
            for n, s_t in enumerate(sts):
                m8 = _fold7(jnp.maximum, s_t)
                mx = _all8(jnp.maximum, lax.select(junk8, ninf8, m8))
                mv = lax.select(junk8, -ninf8, mx)
                z = tick(tg + SMD * (3 - n)) if SST != 1 else None
                if z is not None:
                    mv = tie(mv, [z])
                if SST:
                    s_t = sref[n, 0:G, 0:2 * G]
                eg = jnp.exp2(s_t.reshape(WS, 8, 2 * G) - mv)
                dens.append(_fold7(jnp.add, eg.reshape(G, 2 * G)))
                pts.append(_cat([eg, eg[WS - 1:WS]]) if PVP else eg)
            if MRG:
                def mix(m, sh, a, b):
                    return lax.select(m, a, b) + pltpu.roll(lax.select(m, b, a), sh, 0)
                den = mix(sub2, 2, mix(sub1, 1, dens[0], dens[1]), mix(sub1, 1, dens[2], dens[3]))
                den = den + pltpu.roll(den, 4, 0)
                r0 = pl.reciprocal(den, approx=True)
                r0 = r0 * (2.0 - den * r0)
                r0 = lax.select(first_half, r0, pltpu.roll(r0, 2, 0))
                rsel = [jnp.broadcast_to(r0[n:n + 1], r0.shape) for n in range(4)]
            else:
                rinv = []
                for den in dens:
                    den = _all8(jnp.add, den)
                    r0 = pl.reciprocal(den, approx=True)
                    rinv.append(r0 * (2.0 - den * r0))
                rsel = [lax.select(first_half, rinv[n], rinv[(n + 2) % 4]) for n in range(4)]
            outs = []
            for tile in range(2):
                for hh in range(2):
                    h = 2 * tile + hh
                    stn = _cat([lax.select(key_ok[hh], pts[tile], zp), lax.select(key_ok[1 - hh], pts[2 + tile], zp)])
                    ot = jnp.dot(vt[dh * h:dh * (h + 1), :], stn.reshape(-1, 2 * G).astype(BF16),
                                 preferred_element_type=F32)
                    outs.append(ot.reshape(dh // 8, 8, 2 * G) * rsel[2 * hh + tile])
            tw = _u32(_cat(outs).reshape(C, 2 * G).astype(BF16)).T.reshape(WS, 2, 8, CW)
            tw = (tw[:, 0], tw[:, 1])
            o_s[:, pl.ds(WS * wa, 8), 0:CW] = lax.select(even_head, tw[0], tw[1])
            if wb != wa:
                o_s[:, pl.ds(WS * wb, 8), 0:CW] = lax.select(even_head, tw[1], tw[0])
            toks.append((t0 + DL_PV, o_s[zx, 0:8, :]))
            for rel, w in p:
                tag['o', w] = k + rel
                dirty.discard(w)
                dirty.add(w + 1)

        def c_dot(t0, k, h, r):
            b = (subs[k][0] + 2) % 3
            assert all(tag['o', w] == k - 1 and not (w in dirty and WS * w >= HW * h)
                       for w in range(HW * h // WS, min((HW * h + HW - 1) // WS + 1, NWIN)))
            assert all(tag['x', b, c, t, r] == k - 1 for c in range(2 * NC) for t in (2 * h, 2 * h + 1))
            ls = slice(HW * h, HW * (h + 1))
            ow = o_s[r, ls, :]
            cdt, cst = (BF16, 16) if CBF else (F32, 8)
            inj = due(toks, DC // cst, t0, cst)
            inj = (merged(inj, due(soft, DC // cst, t0, cst)), inj)
            res = [lax.dot_general(lhs(wo_s, slice(LANES * kt, LANES * (kt + 1)), inj[kt], cdt),
                                   _f32(ow & hi if kt else ow << 16).astype(cdt),
                                   (((1,), (1,)), ((), ())), preferred_element_type=F32) for kt in range(2)]
            res = res[0] + res[1]
            ticks.extend((t0 + MXU_LAT + 8 * j, res, j) for j in range(DC // 8))
            slot = subs[k][2]
            n = min(HW, W - HW * h)
            xout[slot][row0(slot, g) + r, :, HW * h:HW * h + n] = (_cat([xbuf[b][r, t, 0:C, :] for t in (2 * h, 2 * h + 1)], axis=1) + res)[:, 0:n].astype(BF16)
            if h == 1 and not subs[k][3]:
                out_copy(slot, g, r, 1).start()
            elif h == 1 and r == WS - 1:
                out_copy(slot, g).start()
                xout[slot][zx + xout[slot].shape[0] - 1, 0:16, 0:LANES] = jnp.zeros((16, LANES), BF16)
                soft.append((t0 + MXU_LAT + DC + DL_D, _u32(xout[slot][zy + xout[slot].shape[0] - 1, 0:16, 0:LANES])))

        def stage_row(d, k, c, rho):
            j, slot = subs[k][0:2]
            cs = slice(16 * c, 16 * c + 16)
            u = _u32(xin[slot][row0(slot, g) + rho - 2, cs, :])
            if rho == WS + 1 and slot == 1:
                u = jnp.where(g < ng - 2, u, zero)
            idx = stg_row(j, c // 2, rho)
            stg[c % 2][idx] = shifted(u)
            soft.append((d, stg[c % 2][zx + SPARE, 8:16, 0:LANES]))
            tag['s', c % 2, idx] = (k, c, rho)
            if c == NC - 1 and rho == WS + 1 and slot < NSUB - 1:
                for cp in in_copies(slot, g + 1):
                    cp.start()
                xin[slot][zx + WS, 0:16, 0:LANES] = jnp.zeros((16, LANES), BF16)
                soft.append((d + DL_D, _u32(xin[slot][zy + WS, 0:16, 0:LANES])))

        def conv_step(d, k, c, hf, t, r):
            j = subs[k][0]
            if r == 0:
                if t == 0:
                    stg[c % 2][zx + SPARE, 0:8, 0:LANES] = zt
                    st['w'] = [dw_s[2 * c + hf, ki] for ki in range(3)]
                st['un'] = {}
            un = st['un']
            for rho in range(r, r + 3):
                if rho not in un:
                    idx = stg_row(j, c // 2, rho)
                    assert tag['s', c % 2, idx] in ((k, c, rho), (k - 1, c, rho + WS))
                    un[rho] = unpack(stg[c % 2][idx, 24 * t:24 * t + 24, :], hf)
            acc = conv_row(un, st['w'], r)
            xbuf[(j + 1) % 3][r, t, 16 * c + 8 * hf:16 * c + 8 * hf + 8, :] = acc
            soft.append((d, _u32(acc)))
            tag['x', (j + 1) % 3, 2 * c + hf, t, r] = k + 1

        plan, offs = [], [0]
        for k, sub in enumerate(subs):
            w0 = wsp - (MIX and k == 1)
            w1 = wsp - (MIX and k == 0 and len(subs) > 1)
            pk, tk = _plan(NWIN, w0, w1, NT, sub[3], sub[4])
            plan += [(offs[k] + t, kind, k, idx) for t, kind, idx in pk]
            offs.append(offs[k] + tk)
        total = offs[-1]
        starts = [e[0] for e in plan]
        ev = []

        def at(t, fn, *a):
            ev.append((t, t, len(ev), fn, a))

        def before(d, fn, *a):
            ev.append((max([t for t in starts if t <= d], default=0) - 1, d, len(ev), fn, a))

        load = [0.0] * (total + 1000)
        tqk = {}
        tpv = {(k, idx): t for t, kind, k, idx in plan if kind == 'pv'}

        def add(t0, t1, n):
            for t in range(max(t0, 0), max(t1, 0)):
                load[t] += n / (t1 - t0)

        pend = 0
        for n_op, (t, kind, k, idx) in enumerate(plan):
            tr = t + MXU_LAT
            tp0 = max(starts[n_op - 2] if n_op > 1 else t - 64, pend)
            if kind == 'a':
                if idx == (0, 0) and k > 0:
                    before(t - LN1 - 1, fence, t - LN1 - 40, subs[k][0] % 3)
                before(t - LN1, ln1, t - LN1, k, *idx)
                for n in range(LNS):
                    d = t - LN2 - LND * (LNS - 1 - n)
                    before(d, ln2, d, n, k, *idx)
                    add(d - 16, d, 72 // LNS)
                if LNF & 1:
                    before(t - LN3, ln3, t - LN3, k, *idx)
                at(t, a_dot, t, k, *idx)
                add(tr, tr + DA, WA * DA // 16)
                pend = t - LN3 + 32
                add(t - LN1 - 16, t - LN1, 32); add(t - LN2, t - LN3, 20); add(t - LN3, t - LN3 + 32, 60)
            elif kind == 'qk':
                at(t, b_qk, t, k, idx)
                tqk[idx] = t
                add(tp0, tp0 + 60, WQ); add(t - 8, t + DQ - 8, 28); pend = tp0 + 60; add(tr, tr + DQ, 24); add(tr + DQ, tr + DQ + 16, 36)
            elif kind == 'pv':
                tg = max(tqk[idx] + SM0, t - SMB)
                at(t, b_pv, t, tg, k, idx)
                add(tg, tg + 4 * SMD + 16, 80); add(tr - 10, tr + 6, 46); add(tr, tr + DP, 36)
                add(t + 400, t + 460, 14)
                pend = tg + 4 * SMD + 16
            else:
                if idx == (0, 0) and k > 0:
                    at(t - 1, fence, t - 100, (subs[k][0] + 2) % 3)
                at(t, c_dot, t, k, *idx)
                add(tr, tr + DC, WC * DC // 16)
                add(tp0, tp0 + 64, 96 if CBF else 64 + WQ - 28)
                pend = tp0 + 64
        pre = [0.0]
        for v in load:
            pre.append(pre[-1] + v)
        nstep = NC * 2 * NT * WS
        prev_chunk = 10
        for k, sub in enumerate(subs):
            if not sub[3]:
                continue
            ta = offs[k] + (CVI if k else CV0) - 20
            tb = offs[k + 1] - (CVE if k == len(subs) - 1 else CVX)
            cap = CAP if sub[4] else 64
            free = [max(0.02, cap / 16 - (pre[t + SMO] - pre[max(t - SMO, 0)]) / (2 * SMO)) for t in range(ta, tb)]
            tot_free, acc, tstep = sum(free), 0.0, []
            for t, v in enumerate(free):
                acc += v
                while len(tstep) < nstep and acc >= (len(tstep) + 1) * tot_free / nstep - 1e-6:
                    tstep.append(ta + t)
            for n in range(nstep):
                before(tstep[n], conv_step, tstep[n], k, n // (2 * NT * WS), n // (NT * WS) % 2, n // WS % NT, n % WS)
            for c in range(NC):
                t1 = tstep[c * 2 * NT * WS] - 30
                t0 = prev_chunk + 120
                prev_chunk = t1 + 30
                for rho in range(2, NR):
                    d = t0 + (t1 - t0) * (rho - 2) // (NR - 3)
                    before(d, stage_row, d, k, c, rho)
        ev.sort(key=lambda e: e[:3])
        for e in ev:
            e[3](*e[4])
        if subs[-1][3]:
            n = len(subs)
            assert all(tag['qkv', t, r] == n - 1 for t in range(NT) for r in range(WS))
            assert all(tag['o', w] == n - 1 and w not in dirty for w in range(wsp))

    if ONLY in (0, 1):
        @pl.when(g == 0)
        def _():
            setup()
            body([(0, 2, 0, True, False)])

    @pl.when(g > 0)
    def _():
        for k in range(NSUB):
            for cp in in_copies(k, g):
                cp.wait()

    @pl.when((g > 0) & (g < ng - 1))
    def _():
        for cp in in_copies(NSUB - 1, g + 1):
            cp.start()

    @pl.when(g > 1)
    def _():
        for k in range(NSUB - 1):
            out_copy(k, g - 1).wait()

    @pl.when(g > 2)
    def _():
        out_copy(NSUB - 1, g - 2).wait()

    if ONLY in (0, 2):
        @pl.when((g > 0) & (g < ng - 1))
        def _():
            body([(1 + k, k, k, True, True) for k in range(NSUB)])

    if ONLY in (0, 3):
        @pl.when(g == ng - 1)
        def _():
            body([(1, 0, 0, False, True)])
            out_copy(NSUB - 1, g - 1).wait()
            out_copy(0, g).wait()


@jax.jit
def pallas_standalone__window_attn_davit__vision_kernel(
    x: jax.Array,
    dw_pe: jax.Array,
    w_qkv: jax.Array,
    w_o: jax.Array,
):
    B, H, W, C = x.shape
    assert B == 1 and H % WS == 0 and W % WS == 0 and C % (16 * NH) == 0
    WP = -(-(W + 1) // (2 * LANES)) * (2 * LANES)
    assert WP == 4 * LANES
    NWIN = W // WS
    NBLK = H // WS
    assert (NBLK - 1) % NSUB == 0
    NM = (NBLK - 1) // NSUB

    xt = jnp.transpose(x[0], (0, 2, 1))

    nstg = WS - 2 + NSUB * (C // 32) * 2 + 1
    kern = functools.partial(_kernel, C=C, H=H, W=W, WP=WP, NWIN=NWIN)
    out = pl.pallas_call(
        kern,
        grid=(NM + 2,),
        in_specs=[pl.BlockSpec(memory_space=pl.ANY)] * 4,
        out_specs=pl.BlockSpec(memory_space=pl.ANY),
        out_shape=jax.ShapeDtypeStruct((H, C, W), x.dtype),
        scratch_shapes=[
            pltpu.VMEM((WS + 1, WP // LANES, C + 8, LANES), F32),
            pltpu.VMEM((WS + 1, WP // LANES, C + 8, LANES), F32),
            pltpu.VMEM((WS + 1, WP // LANES, C + 8, LANES), F32),
            pltpu.VMEM((WS, WP + 8, LANES), U32),
            pltpu.VMEM((WS, WP + 8, LANES), U32),
            pltpu.VMEM((WS, WP + 8, LANES), U32),
            pltpu.VMEM((WS, WP + 8, LANES), U32),
            pltpu.VMEM((2, 3 * C // 4, 2 * LANES), U32),
            pltpu.VMEM((C // 2 if CBF else C, 2 * LANES), U32),
            pltpu.VMEM((nstg, WP // LANES * 24, LANES), U32),
            pltpu.VMEM((nstg, WP // LANES * 24, LANES), U32),
            pltpu.VMEM((C // 8, 3, 3, 8, LANES), F32),
            pltpu.VMEM((WS + 1, C, W), BF16),
            pltpu.VMEM((WS + 1, C, W), BF16),
            pltpu.VMEM((2 * WS + 1, C, W), BF16),
            pltpu.VMEM((WS + 1, C, W), BF16),
            pltpu.VMEM((WS + 1, C, W), BF16),
            pltpu.VMEM((2 * WS + 1, C, W), BF16),
            pltpu.VMEM((2, C // 2, LANES), U32),
            pltpu.VMEM((2, C // 2, LANES), U32),
            pltpu.VMEM((2, C // 2, LANES), U32),
            pltpu.VMEM((2, C // 2, LANES), U32),
            pltpu.VMEM((5, 8 * WS + 16, LANES), F32),
            pltpu.VMEM((5, 8 * WS + 16, LANES), F32),
            pltpu.VMEM((5, 8 * WS + 16, LANES), F32),
            pltpu.VMEM((5, 8 * WS + 16, LANES), F32),
            pltpu.VMEM(dw_pe.shape, BF16),
            pltpu.VMEM(w_qkv.shape, BF16),
            pltpu.VMEM(w_o.shape, BF16),
            pltpu.SemaphoreType.DMA((2 * NSUB,)),
            pltpu.SemaphoreType.DMA((NSUB + 1,)),
            pltpu.SemaphoreType.DMA((3 + C // 32,)),
        ],
        compiler_params=pltpu.CompilerParams(
            dimension_semantics=("arbitrary",),
            vmem_limit_bytes=96 * 1024 * 1024,
            disable_bounds_checks=bool(NOBC),
        ),
        name="davit_window_attn",
    )(xt, dw_pe, w_qkv, w_o)
    return jnp.transpose(out, (0, 2, 1))[None]
```

```python
import functools
import math

import jax
import jax.numpy as jnp
from jax import lax
import jax.experimental.pallas as pl
import jax.experimental.pallas.tpu as pltpu

WS = 7
NH = 4
EPS = 1e-05
LANES = 128
F32 = jnp.float32
BF16 = jnp.bfloat16
U32 = jnp.uint32
NSUB = 3

DA, DC, DQ, DP = 288, 192, 56, 48
MXU_LAT = 130
DL_A = 500
LAT_QK = 280
DL_PV = 580
PRE_C = 120
TAIL = 1400
LN1 = 200
LN2 = 130
LNS = 3
LND = 16
LN3 = 60
LNG = 16
SM0 = 200
SMD = 16
SMB = 140
VDL = 60
DL_D = 100
CV0 = 450
CVI = 170
CVE = 30
CVX = 180
CAP = 42
SMO = 32
WA = 7
WC = 11
WQ = 40
EC0 = 1500
ECD = 900


def _iota(shape, dim):
    return lax.broadcasted_iota(jnp.int32, shape, dim)


def _plan(nwin, w0, w1, nt, cur, prev):
    a_q = [(t, r) for t in range(nt) for r in range(WS)] if cur else []
    c_q = [(h, r) for h in range(2) for r in range(WS)] if prev else []
    old = [(-1, w) for w in range(w0, nwin)] if prev else []
    new = [(0, w) for w in range(w1)] if cur else []
    ws = old + old[-1:] * ((len(old) + len(new)) % 2) + new
    pairs = list(zip(ws[0::2], ws[1::2]))
    n1 = sum(a[0] < 0 for a, _ in pairs)
    nh = sum(a[0] < 0 and WS * a[1] < nt * LANES // 2 for a, _ in pairs)
    total = len(a_q) * DA + len(c_q) * DC + len(pairs) * (DQ + DP)
    q0 = 0 if prev else total // 3
    t = 0
    ia = ic = iq = ip = 0
    out = []
    tq, tp, ta = {}, {}, {}
    last = None
    while ia < len(a_q) or ic < len(c_q) or ip < len(pairs):
        cands = []
        if ip < iq and t >= tq[ip] + LAT_QK:
            cands.append((-1e6, 'pv'))
        if iq < len(pairs) and (not cur or (iq - ip < 2 and last not in ('qk', 'pv'))):
            ok = iq - ip < 4
            if pairs[iq][1][0] == 0:
                need = (WS * pairs[iq][1][1] + WS) // LANES * WS + WS - 1
                ok = ia > need and t >= ta[need] + DA + DL_A + 60 and ic >= len(c_q) // 2
            if ok:
                pr = q0 + iq * (total - q0 - TAIL) / len(pairs) - t - 200
                cands.append((-2e6 if pr <= 0 else pr, 'qk'))
        if ia < len(a_q):
            cands.append((ia * (total - 700) / len(a_q) - t, 'a'))
        if ic < len(c_q):
            need = nh - 1 if ic < WS else n1 - 1
            if ip > need and t >= tp[need] + DL_PV + PRE_C:
                if cur:
                    tc = 1000 + ic * 900 if ic < WS else total - DC - (2 * WS - 1 - ic) * 950
                else:
                    tc = EC0 + ic * ECD
                cands.append((tc - t, 'c'))
        if not cands:
            t += 8
            last = None
            continue
        last = kind = min(cands)[1]
        if kind == 'pv':
            out.append((t, kind, pairs[ip]))
            tp[ip], ip, t = t, ip + 1, t + DP
        elif kind == 'qk':
            out.append((t, kind, pairs[iq]))
            tq[iq], iq, t = t, iq + 1, t + DQ
        elif kind == 'a':
            out.append((t, kind, a_q[ia]))
            ta[ia], ia, t = t, ia + 1, t + DA
        else:
            out.append((t, kind, c_q[ic]))
            ic, t = ic + 1, t + DC
    return out, t


def _tree_sum(xs):
    while len(xs) > 1:
        xs = [xs[j] + xs[j + 1] if j + 1 < len(xs) else xs[j] for j in range(0, len(xs), 2)]
    return xs[0]


def _sum8(x):
    while x.shape[0] % 16 == 0:
        x = x[:x.shape[0] // 2] + x[x.shape[0] // 2:]
    return _tree_sum(_rows8(x))


def _fold7(op, x):
    t = op(x[0:24], x[24:48])
    return op(op(t[0:8], t[8:16]), op(t[16:24], x[48:56]))


def _all8(op, x):
    for sh in (4, 2, 1):
        x = op(x, pltpu.roll(x, sh, 0))
    return x


def _rows8(x):
    return [x[8 * j:8 * j + 8] for j in range(x.shape[0] // 8)]


def _cat(xs, axis=0):
    return jnp.concatenate(xs, axis=axis) if len(xs) > 1 else xs[0]


def _f32(u):
    return pltpu.bitcast(u, F32)


def _u32(x):
    return pltpu.bitcast(x, U32)


def _kernel(x_hbm, dw_hbm, wqkv_hbm, wo_hbm, o_hbm,
            xa_s, xb_s, xc_s, q_s, k_s, v_s, o_s, wq_s, wo_s, sa_s, sb_s, dw_s,
            i0_s, i1_s, i2_s, o0_s, o1_s, o2_s, va_s, vb_s, vc_s, vd_s,
            dw_ref, wqkv_ref, wo_ref, in_sem, out_sem, w_sem, *, C, H, W, WP, NWIN):
    g = pl.program_id(0)
    ng = pl.num_programs(0)
    dh = C // NH
    CW = C // 2
    NT = WP // LANES
    G = WS * 8
    HW = WP // 2
    NC = C // 16
    NR = WS + 2
    lane8 = _iota((8, LANES), 1)
    last_valid = W - (NT - 1) * LANES
    zero = jnp.uint32(0)
    hi = jnp.uint32(0xFFFF0000)
    qkv_s = (q_s, k_s, v_s)
    xbuf = (xa_s, xb_s, xc_s)
    xin = (i0_s, i1_s, i2_s)
    xout = (o0_s, o1_s, o2_s)

    def row0(k, m):
        return (m & 1) * WS if k == NSUB - 1 else 0

    def in_copies(k, m):
        r = WS * (NSUB * m - 1 + k) + 1
        return [pltpu.make_async_copy(x_hbm.at[pl.ds(jnp.minimum(r + o, H - n), n)],
                                      xin[k].at[pl.ds(row0(k, m) + o, n)], in_sem.at[k])
                for o, n in ((0, WS - 1), (WS - 1, 1))]

    def in_wait(k, m):
        dst = xin[k].at[pl.ds(row0(k, m), WS)]
        pltpu.make_async_copy(dst, dst, in_sem.at[k]).wait()

    def out_copy(k, m, o=0, n=WS):
        return pltpu.make_async_copy(xout[k].at[pl.ds(row0(k, m) + o, n)],
                                     o_hbm.at[pl.ds(WS * (NSUB * (m - 1) + k) + o, n)],
                                     out_sem.at[k + (m & 1) if k == NSUB - 1 else k])

    stg = (sa_s, sb_s)
    vts = (va_s, vb_s, vc_s, vd_s)
    SPARE = sa_s.shape[0] - 1
    zx = g >> 10
    zy = g >> 11
    never = lane8 < zx

    def tie(x, toks):
        if not toks:
            return x
        tok = functools.reduce(lax.bitwise_or, toks)
        n = x.shape[1]
        return lax.select(never[:, 0:n], tok[:, 0:n], x) if n < LANES else lax.select(never, tok, x)

    def stg_row(j, c2, rho):
        if 2 <= rho < WS:
            return rho - 2
        slot = j % NSUB if rho >= WS else (j - 1) % NSUB
        return WS - 2 + (slot * (NC // 2) + c2) * 2 + rho % WS

    zt = jnp.zeros((8, LANES), U32)
    is_first, is_last = lane8 == 0, lane8 == LANES - 1

    def shifted(u):
        tiles = [u[:, LANES * t:LANES * (t + 1)] for t in range(NT)]
        tiles[NT - 1] = _cat([tiles[NT - 1], zt[:, last_valid:]], axis=1)
        left = [pltpu.roll(lax.select(is_last, tiles[t - 1] if t > 0 else zt, tiles[t]), 1, 1)
                for t in range(NT)]
        right = [pltpu.roll(lax.select(is_first, tiles[t + 1], tiles[t]) if t < NT - 1 else tiles[t], LANES - 1, 1)
                 for t in range(NT)]
        return _cat([v[t] for t in range(NT) for v in (left, tiles, right)])

    def unpack(v, hf):
        return pltpu.bitcast(v, BF16).astype(F32).reshape(3, 2, 8, LANES)[:, hf]

    def conv_row(un, w, r):
        return jnp.sum(_tree_sum([un[r + ki] * w[ki] for ki in range(3) if un[r + ki] is not None]), axis=0)

    def setup():
        wcp = [pltpu.make_async_copy(src, dst, w_sem.at[n])
               for n, (src, dst) in enumerate(((dw_hbm, dw_ref), (wqkv_hbm, wqkv_ref), (wo_hbm, wo_ref)))]

        def top(c2):
            cs = pl.ds(pl.multiple_of(32 * c2, 32), 32)
            return pltpu.make_async_copy(x_hbm.at[pl.ds(0, WS + 1), cs], i1_s.at[:, cs], w_sem.at[3 + c2])
        for cp in wcp + [top(c2) for c2 in range(NC // 2)]:
            cp.start()

        def zrow(r, carry):
            for ref in (k_s, o_s):
                ref[r, 0:WP, :] = jnp.zeros((WP, LANES), U32)
            return carry
        lax.fori_loop(0, WS, zrow, 0)
        for ref in (q_s, v_s):
            ref[0, 0:8, :] = zt
        for ref in stg:
            ref[SPARE, 0:16, :] = jnp.zeros((16, LANES), U32)
        for ref in vts:
            ref[1, 0:8, :] = zt
        wo_s[...] = jnp.zeros(wo_s.shape, U32)
        for cp in wcp:
            cp.wait()
        for ki in range(3):
            w3 = dw_ref[ki].astype(F32)
            for kj in range(3):
                w = w3[kj:kj + 1] + 1.0 if ki == kj == 1 else w3[kj:kj + 1]
                dw_s[:, ki, kj] = jnp.broadcast_to(w, (LANES, C)).T.reshape(C // 8, 8, LANES)
        qscale = (dh ** -0.5) * math.log2(math.e)
        for kt in range(2):
            wt = wqkv_ref[CW * kt:CW * (kt + 1), :].astype(F32).T
            wq = (wt[0:C] * qscale).astype(BF16).astype(F32)
            words = [(_u32(w[0:CW]) >> 16) | (_u32(w[CW:C]) & hi) for w in (wq, wt[C:2 * C])]
            words = _rows8(_cat(words + [_u32(wt[2 * C:].astype(BF16))]))
            for par in range(2):
                wq_s[par, :, LANES * kt:LANES * kt + CW] = _cat(words[par::2])
        wo = _u32(wo_ref[...])
        for kt, w in enumerate((wo << 16, wo & hi)):
            wo_s[:, LANES * kt:LANES * kt + CW] = _u32(_f32(w.T).astype(BF16))

        def conv0(c2, carry):
            top(c2).wait()

            @pl.when(c2 == 2)
            def _():
                for cp in in_copies(2, 0):
                    cp.start()
            for par in range(2):
                cs = pl.ds(pl.multiple_of(32 * c2 + 16 * par, 16), 16)
                sh = [shifted(_u32(i1_s[r, cs, :])) for r in range(WS + 1)]
                for rho in (WS, WS + 1):
                    stg[par][stg_row(-1, c2, rho)] = sh[rho - 1]
                for hf in range(2):
                    c8 = 4 * c2 + 2 * par + hf
                    w = [dw_s[c8, ki] for ki in range(3)]
                    for t in range(NT):
                        un = [None] + [unpack(row[24 * t:24 * t + 24], hf) for row in sh]
                        for r in range(WS):
                            xbuf[0][r, t, pl.ds(pl.multiple_of(8 * c8, 8), 8), :] = conv_row(un, w, r)
            return carry
        lax.fori_loop(0, NC // 2, conv0, 0)
        for cp in in_copies(0, 1) + in_copies(1, 1):
            cp.start()
        in_wait(2, 0)
        for cp in in_copies(2, 1):
            cp.start()

    def body(subs):
        lane3 = _iota((WS, 8, LANES), 2)
        head = (lane3 < dh, (lane3 >= dh) & (lane3 < 2 * dh))
        zq = jnp.zeros((WS, 8, LANES), F32)
        junk8 = _iota((8, 2 * G), 0) == WS
        ninf8 = jnp.full((8, 2 * G), -jnp.inf, F32)
        key_ok = tuple((_iota((WS + 1, 8, 2 * G), 2) & 8) == 8 * hh for hh in range(2))
        zp = jnp.zeros((WS + 1, 8, 2 * G), F32)
        first_half = (_iota((8, 2 * G), 1) & 8) == 0
        even_head = (_iota((WS, 8, CW), 2) // (dh // 2)) % 2 == 0
        wsp = (HW - 1) // WS

        st = {}
        toks = []
        soft = []
        ticks = []
        j0 = subs[0][0]
        tag = {('qkv', t, r): -1 for t in range(NT) for r in range(WS)}
        tag.update({('o', w): (-1 if w < wsp else None) for w in range(NWIN)})
        dirty = {wsp}
        for b, blk in ((j0 % 3, 0), ((j0 + 2) % 3, -1)):
            tag.update({('x', b, c, t, r): blk for c in range(2 * NC) for t in range(NT) for r in range(WS)})
        tag.update({('s', c % 2, stg_row(j0, c // 2, rho)): (0, c, rho) for c in range(NC) for rho in (0, 1)})

        def gather(ref, w):
            return ref[:, pl.ds(WS * w, 8), :]

        def tick(t):
            c = [x for x in ticks if t <= x[0] <= t + 40]
            if not c:
                return None
            _, res, j = min(c, key=lambda x: x[0])
            return res[8 * j:8 * j + 8, 0:LANES]

        def due(lst, nblk, t0, step):
            inj = {}
            for d, tok in list(lst):
                j = max(0, -(-(d - t0) // step))
                if j < nblk and d >= 0:
                    inj.setdefault(j, []).append(tok)
            lst[:] = [x for x in lst if x[0] > t0 + (nblk - 1) * step]
            return inj

        def lhs(ref, ls, inj, dt):
            nblk = ref.shape[0] // 8
            parts, s = [], 0
            for j in sorted(inj):
                if j > s:
                    parts.append(ref[8 * s:8 * j, ls])
                parts.append(tie(ref[8 * j:8 * j + 8, ls], inj[j]))
                s = j + 1
            if s < nblk:
                parts.append(ref[8 * s:8 * nblk, ls])
            return pltpu.bitcast(_cat(parts), dt)

        def clamp(t, dl, dmin):
            return max(t + dmin, min(t + dl, total - 16))

        def merged(a, b):
            return {j: a.get(j, []) + b.get(j, []) for j in set(a) | set(b)}

        def fence(d, b):
            c = [x for x in ticks if x[0] <= d]
            if c:
                _, res, j = max(c, key=lambda x: x[0])
                xbuf[b][zx + WS, 0, 0:8, :] = res[8 * j:8 * j + 8, 0:LANES]

        def ln1(d, k, t, r):
            b = subs[k][0] % 3
            assert all(tag['x', b, c, t, r] == k for c in range(2 * NC))
            s8 = _sum8(xbuf[b][r, t, 0:C, :])
            soft.append((d, _u32(s8)))
            mean = jnp.sum(s8, axis=0, keepdims=True) * (1.0 / C)
            fence(d + LNG, b)
            st['ln', k, t, r] = [xbuf[b][r, t, 0:C, :] - mean, [], mean]

        def ln3(d, k, t, r):
            b = subs[k][0] % 3
            fence(d, b)
            st['ln', k, t, r][0] = xbuf[b][r, t, 0:C, :] - st['ln', k, t, r][2]

        def ln2(d, n, *key):
            m = C // LNS
            xc = st[('ln',) + key][0][m * n:m * (n + 1)]
            s8 = _sum8(xc * xc)
            soft.append((d, _u32(s8)))
            st[('ln',) + key][1].append(s8)

        def a_dot(t0, k, t, r):
            xc, sq, _ = st.pop(('ln', k, t, r))
            var = jnp.sum(_tree_sum(sq), axis=0, keepdims=True) * (1.0 / C)
            h = xc * lax.rsqrt(var + EPS)
            h = [h[CW * kt:CW * (kt + 1)].astype(BF16) for kt in range(2)]
            inj = due(toks, DA // 16, t0, 16)
            inj0 = merged(inj, due(soft, DA // 16, t0, 16))
            part = [jnp.dot(lhs(wq_s.at[par], slice(LANES * kt, LANES * kt + CW), inj if par or kt else inj0, BF16),
                            h[kt], preferred_element_type=F32)
                    for par in range(2) for kt in range(2)]
            res = [part[0] + part[1], part[2] + part[3]]
            ticks.extend((t0 + MXU_LAT + 8 * j, res[0], j) for j in range(DA // 8))
            qkv = jnp.stack([v.reshape(-1, 16, LANES) for v in res], axis=1).reshape(3 * C, LANES)
            for m in range(3):
                qkv_s[m][r, LANES * t:LANES * (t + 1), 0:CW] = _u32(qkv[C * m:C * (m + 1)].astype(BF16)).T
                toks.append((clamp(t0 + 96 * (m + 1), DL_A, 350), qkv_s[m][zx, 0:8, :]))
            tag['qkv', t, r] = k

        def b_qk(t0, k, p):
            (_, wa), (_, wb) = p
            assert all(tag['qkv', t, r] == k + rel for r in range(WS) for rel, w in p
                       for t in range(WS * w // LANES, min(WS * w + WS, WP - 1) // LANES + 1))
            sts = []
            inj = due(soft, WS, t0, 8)
            for w, swap in ((wa, 0), (wb, 1)):
                qw = gather(q_s, w)
                kw = gather(k_s, w).reshape(G, LANES)
                if not swap and inj:
                    kw = _cat([tie(v, inj.get(r, [])) for r, v in enumerate(_rows8(kw))])
                for tile in range(2):
                    kk = _f32(kw & hi if tile else kw << 16)
                    qq = _f32(qw & hi if tile else qw << 16)
                    qst = jnp.stack([lax.select(head[swap], qq, zq), lax.select(head[1 - swap], qq, zq)], axis=1)
                    sts.append(lax.dot_general(kk, qst.reshape(2 * G, LANES), (((1,), (1,)), ((), ())),
                                               preferred_element_type=F32))
            vw = _cat([gather(v_s, wa), zt[None], gather(v_s, wb), zt[None]]).reshape(LANES, LANES)
            st['nv'] = (st.get('nv', 0) + 1) % len(vts)
            ref = vts[st['nv']]
            assert all(v[1] is not ref for key, v in st.items() if key[0] == 's')
            ref[0] = vw[:, 0:CW].T
            soft.append((tpv[k, p] - VDL, ref[zx + 1, 0:8, :]))
            st['s', p] = (sts, ref)

        def b_pv(t0, tg, k, p):
            (_, wa), (_, wb) = p
            sts, ref = st.pop(('s', p))
            ref[zx + 1, 8:16, :] = zt
            vt = lhs(ref.at[0], slice(0, LANES), due(soft, 3, t0, 16), BF16)
            pts = []
            rinv = []
            for n, s_t in enumerate(sts):
                m8 = _fold7(jnp.maximum, s_t)
                mx = _all8(jnp.maximum, lax.select(junk8, ninf8, m8))
                mv = lax.select(junk8, -ninf8, mx)
                z = tick(tg + SMD * (3 - n))
                if z is not None:
                    mv = tie(mv, [z])
                eg = jnp.exp2(s_t.reshape(WS, 8, 2 * G) - mv)
                rinv.append(_fold7(jnp.add, eg.reshape(G, 2 * G)))
                pts.append(_cat([eg, eg[WS - 1:WS]]))
            for n in range(4):
                den = _all8(jnp.add, rinv[n])
                r0 = pl.reciprocal(den, approx=True)
                rinv[n] = r0 * (2.0 - den * r0)
            rsel = [lax.select(first_half, rinv[n], rinv[(n + 2) % 4]) for n in range(4)]
            outs = []
            for tile in range(2):
                for hh in range(2):
                    h = 2 * tile + hh
                    stn = _cat([lax.select(key_ok[hh], pts[tile], zp), lax.select(key_ok[1 - hh], pts[2 + tile], zp)])
                    ot = jnp.dot(vt[dh * h:dh * (h + 1), :], stn.reshape(-1, 2 * G).astype(BF16),
                                 preferred_element_type=F32)
                    outs.append(ot.reshape(dh // 8, 8, 2 * G) * rsel[2 * hh + tile])
            tw = _u32(_cat(outs).reshape(C, 2 * G).astype(BF16)).T.reshape(WS, 2, 8, CW)
            tw = (tw[:, 0], tw[:, 1])
            o_s[:, pl.ds(WS * wa, 8), 0:CW] = lax.select(even_head, tw[0], tw[1])
            if wb != wa:
                o_s[:, pl.ds(WS * wb, 8), 0:CW] = lax.select(even_head, tw[1], tw[0])
            toks.append((clamp(t0, DL_PV, 480), o_s[zx, 0:8, :]))
            for rel, w in p:
                tag['o', w] = k + rel
                dirty.discard(w)
                dirty.add(w + 1)

        def c_dot(t0, k, h, r):
            b = (subs[k][0] + 2) % 3
            assert all(tag['o', w] == k - 1 and not (w in dirty and WS * w >= HW * h)
                       for w in range(HW * h // WS, min((HW * h + HW - 1) // WS + 1, NWIN)))
            assert all(tag['x', b, c, t, r] == k - 1 for c in range(2 * NC) for t in (2 * h, 2 * h + 1))
            ow = o_s[r, HW * h:HW * (h + 1), :]
            inj = due(toks, DC // 16, t0, 16)
            inj = (merged(inj, due(soft, DC // 16, t0, 16)), inj)
            res = [lax.dot_general(lhs(wo_s, slice(LANES * kt, LANES * (kt + 1)), inj[kt], BF16),
                                   _f32(ow & hi if kt else ow << 16).astype(BF16),
                                   (((1,), (1,)), ((), ())), preferred_element_type=F32) for kt in range(2)]
            res = res[0] + res[1]
            ticks.extend((t0 + MXU_LAT + 8 * j, res, j) for j in range(DC // 8))
            slot = subs[k][2]
            n = min(HW, W - HW * h)
            x0 = _cat([xbuf[b][r, t, 0:C, :] for t in (2 * h, 2 * h + 1)], axis=1)
            xout[slot][row0(slot, g) + r, :, HW * h:HW * h + n] = (x0 + res)[:, 0:n].astype(BF16)
            if h == 1 and not subs[k][3]:
                out_copy(slot, g, r, 1).start()
            elif h == 1 and r == WS - 1:
                start_by(t0 + MXU_LAT + DC + DL_D, [out_copy(slot, g)], xout[slot])

        def start_by(d, copies, ref):
            for cp in copies:
                cp.start()
            spare = ref.shape[0] - 1
            ref[zx + spare, 0:16, 0:LANES] = jnp.zeros((16, LANES), BF16)
            soft.append((d, _u32(ref[zy + spare, 0:16, 0:LANES])))

        def refill(d, slot):
            start_by(d, in_copies(slot, g + 1), xin[slot])

        def stage_row(d, k, c, rho):
            j, slot = subs[k][0:2]
            cs = slice(16 * c, 16 * c + 16)
            u = _u32(xin[slot][row0(slot, g) + rho - 2, cs, :])
            if rho == WS + 1 and slot == 1:
                u = jnp.where(g < ng - 2, u, zero)
            idx = stg_row(j, c // 2, rho)
            stg[c % 2][idx] = shifted(u)
            soft.append((d, stg[c % 2][zx + SPARE, 8:16, 0:LANES]))
            tag['s', c % 2, idx] = (k, c, rho)
            if c == NC - 1 and rho == WS + 1 and slot < NSUB - 1:
                refill(d + DL_D, slot)

        def conv_step(d, k, c, hf, t, r):
            j = subs[k][0]
            if r == 0:
                if t == 0:
                    stg[c % 2][zx + SPARE, 0:8, 0:LANES] = zt
                    st['w'] = [dw_s[2 * c + hf, ki] for ki in range(3)]
                st['un'] = {}
            un = st['un']
            for rho in range(r, r + 3):
                if rho not in un:
                    idx = stg_row(j, c // 2, rho)
                    assert tag['s', c % 2, idx] in ((k, c, rho), (k - 1, c, rho + WS))
                    un[rho] = unpack(stg[c % 2][idx, 24 * t:24 * t + 24, :], hf)
            acc = conv_row(un, st['w'], r)
            xbuf[(j + 1) % 3][r, t, 16 * c + 8 * hf:16 * c + 8 * hf + 8, :] = acc
            soft.append((d, _u32(acc)))
            tag['x', (j + 1) % 3, 2 * c + hf, t, r] = k + 1

        plan, offs = [], [0]
        for k, sub in enumerate(subs):
            pk, tk = _plan(NWIN, wsp - (k == 1), wsp - (k == 0 and len(subs) > 1), NT, sub[3], sub[4])
            plan += [(offs[k] + t, kind, k, idx) for t, kind, idx in pk]
            offs.append(offs[k] + tk)
        total = offs[-1]
        starts = [e[0] for e in plan]
        ev = []

        def at(t, fn, *a):
            ev.append((t, t, len(ev), fn, a))

        def before(d, fn, *a):
            ev.append((max([t for t in starts if t <= d], default=0) - 1, d, len(ev), fn, a))

        load = [0.0] * (total + 1000)
        tqk = {}
        tpv = {(k, idx): t for t, kind, k, idx in plan if kind == 'pv'}

        def add(t0, t1, n):
            for t in range(max(t0, 0), max(t1, 0)):
                load[t] += n / (t1 - t0)

        pend = 0
        for n_op, (t, kind, k, idx) in enumerate(plan):
            tr = t + MXU_LAT
            tp0 = max(starts[n_op - 2] if n_op > 1 else t - 64, pend)
            if kind == 'a':
                if idx == (0, 0) and k > 0:
                    before(t - LN1 - 1, fence, t - LN1 - 40, subs[k][0] % 3)
                before(t - LN1, ln1, t - LN1, k, *idx)
                for n in range(LNS):
                    d = t - LN2 - LND * (LNS - 1 - n)
                    before(d, ln2, d, n, k, *idx)
                    add(d - 16, d, 72 // LNS)
                before(t - LN3, ln3, t - LN3, k, *idx)
                at(t, a_dot, t, k, *idx)
                add(tr, tr + DA, WA * DA // 16)
                pend = t - LN3 + 32
                add(t - LN1 - 16, t - LN1, 32)
                add(t - LN2, t - LN3, 20)
                add(t - LN3, t - LN3 + 32, 60)
            elif kind == 'qk':
                at(t, b_qk, t, k, idx)
                tqk[idx] = t
                add(tp0, tp0 + 60, WQ)
                add(t - 8, t + DQ - 8, 28)
                add(tr, tr + DQ, 24)
                add(tr + DQ, tr + DQ + 16, 36)
                pend = tp0 + 60
            elif kind == 'pv':
                tg = max(tqk[idx] + SM0, t - SMB)
                at(t, b_pv, t, tg, k, idx)
                add(tg, tg + 4 * SMD + 16, 80)
                add(tr - 10, tr + 6, 46)
                add(tr, tr + DP, 36)
                add(t + 400, t + 460, 14)
                pend = tg + 4 * SMD + 16
            else:
                if idx == (0, 0) and k > 0:
                    at(t - 1, fence, t - 100, (subs[k][0] + 2) % 3)
                at(t, c_dot, t, k, *idx)
                add(tr, tr + DC, WC * DC // 16)
                add(tp0, tp0 + 64, 96)
                pend = tp0 + 64
        pre = [0.0]
        for v in load:
            pre.append(pre[-1] + v)
        nstep = NC * 2 * NT * WS
        prev_chunk = 10
        for k, sub in enumerate(subs):
            if not sub[3]:
                continue
            ta = offs[k] + (CVI if k else CV0) - 20
            tb = offs[k + 1] - (CVE if k == len(subs) - 1 else CVX)
            cap = CAP if sub[4] else 64
            free = [max(0.02, cap / 16 - (pre[t + SMO] - pre[max(t - SMO, 0)]) / (2 * SMO)) for t in range(ta, tb)]
            tot_free, acc, tstep = sum(free), 0.0, []
            for t, v in enumerate(free):
                acc += v
                while len(tstep) < nstep and acc >= (len(tstep) + 1) * tot_free / nstep - 1e-6:
                    tstep.append(ta + t)
            for n in range(nstep):
                before(tstep[n], conv_step, tstep[n], k, n // (2 * NT * WS), n // (NT * WS) % 2, n // WS % NT, n % WS)
            for c in range(NC):
                t1 = tstep[c * 2 * NT * WS] - 30
                t0 = prev_chunk + 120
                prev_chunk = t1 + 30
                for rho in range(2, NR):
                    d = t0 + (t1 - t0) * (rho - 2) // (NR - 3)
                    before(d, stage_row, d, k, c, rho)
        if len(subs) > 1:
            at(-10, refill, 200, NSUB - 1)
        ev.sort(key=lambda e: e[:3])
        for e in ev:
            e[3](*e[4])
        if subs[-1][3]:
            n = len(subs)
            assert all(tag['qkv', t, r] == n - 1 for t in range(NT) for r in range(WS))
            assert all(tag['o', w] == n - 1 and w not in dirty for w in range(wsp))

    @pl.when(g == 0)
    def _():
        setup()
        body([(0, 2, 0, True, False)])

    @pl.when(g > 0)
    def _():
        for k in range(NSUB):
            in_wait(k, g)

    @pl.when(g > 1)
    def _():
        for k in range(NSUB - 1):
            out_copy(k, g - 1).wait()

    @pl.when(g > 2)
    def _():
        out_copy(NSUB - 1, g - 2).wait()

    @pl.when((g > 0) & (g < ng - 1))
    def _():
        body([(1 + k, k, k, True, True) for k in range(NSUB)])

    @pl.when(g == ng - 1)
    def _():
        body([(1, 0, 0, False, True)])
        out_copy(NSUB - 1, g - 1).wait()
        for r in range(WS):
            out_copy(0, g, r, 1).wait()


@jax.jit
def pallas_standalone__window_attn_davit__vision_kernel(
    x: jax.Array,
    dw_pe: jax.Array,
    w_qkv: jax.Array,
    w_o: jax.Array,
):
    B, H, W, C = x.shape
    assert B == 1 and H % WS == 0 and W % WS == 0 and C == 192 and x.dtype == BF16
    WP = -(-(W + 1) // (2 * LANES)) * (2 * LANES)
    assert WP == 4 * LANES
    NWIN = W // WS
    NBLK = H // WS
    assert (NBLK - 1) % NSUB == 0
    NM = (NBLK - 1) // NSUB

    xt = jnp.transpose(x[0], (0, 2, 1))

    nstg = WS - 2 + NSUB * (C // 32) * 2 + 1
    kern = functools.partial(_kernel, C=C, H=H, W=W, WP=WP, NWIN=NWIN)
    out = pl.pallas_call(
        kern,
        grid=(NM + 2,),
        in_specs=[pl.BlockSpec(memory_space=pl.ANY)] * 4,
        out_specs=pl.BlockSpec(memory_space=pl.ANY),
        out_shape=jax.ShapeDtypeStruct((H, C, W), x.dtype),
        scratch_shapes=[
            pltpu.VMEM((WS + 1, WP // LANES, C + 8, LANES), F32),
            pltpu.VMEM((WS + 1, WP // LANES, C + 8, LANES), F32),
            pltpu.VMEM((WS + 1, WP // LANES, C + 8, LANES), F32),
            pltpu.VMEM((WS, WP + 8, LANES), U32),
            pltpu.VMEM((WS, WP + 8, LANES), U32),
            pltpu.VMEM((WS, WP + 8, LANES), U32),
            pltpu.VMEM((WS, WP + 8, LANES), U32),
            pltpu.VMEM((2, 3 * C // 4, 2 * LANES), U32),
            pltpu.VMEM((C // 2, 2 * LANES), U32),
            pltpu.VMEM((nstg, WP // LANES * 24, LANES), U32),
            pltpu.VMEM((nstg, WP // LANES * 24, LANES), U32),
            pltpu.VMEM((C // 8, 3, 3, 8, LANES), F32),
            pltpu.VMEM((WS + 1, C, W), BF16),
            pltpu.VMEM((WS + 1, C, W), BF16),
            pltpu.VMEM((2 * WS + 1, C, W), BF16),
            pltpu.VMEM((WS + 1, C, W), BF16),
            pltpu.VMEM((WS + 1, C, W), BF16),
            pltpu.VMEM((2 * WS + 1, C, W), BF16),
            pltpu.VMEM((2, C // 2, LANES), U32),
            pltpu.VMEM((2, C // 2, LANES), U32),
            pltpu.VMEM((2, C // 2, LANES), U32),
            pltpu.VMEM((2, C // 2, LANES), U32),
            pltpu.VMEM(dw_pe.shape, BF16),
            pltpu.VMEM(w_qkv.shape, BF16),
            pltpu.VMEM(w_o.shape, BF16),
            pltpu.SemaphoreType.DMA((NSUB,)),
            pltpu.SemaphoreType.DMA((NSUB + 1,)),
            pltpu.SemaphoreType.DMA((3 + C // 32,)),
        ],
        compiler_params=pltpu.CompilerParams(
            dimension_semantics=("arbitrary",),
            vmem_limit_bytes=96 * 1024 * 1024,
            disable_bounds_checks=True,
        ),
        name="davit_window_attn",
    )(xt, dw_pe, w_qkv, w_o)
    return jnp.transpose(out, (0, 2, 1))[None]
```

```python
import functools
import math

import jax
import jax.numpy as jnp
from jax import lax
import jax.experimental.pallas as pl
import jax.experimental.pallas.tpu as pltpu

WS = 7
NH = 4
EPS = 1e-05
LANES = 128
F32 = jnp.float32
BF16 = jnp.bfloat16
U32 = jnp.uint32
NSUB = 3

DA, DC, DQ, DP = 288, 192, 56, 48
MXU_LAT = 130
DL_A = 500
LAT_QK = 280
DL_PV = 580
PRE_C = 120
TAIL = 1400
LN1 = 200
LN2 = 130
LNS = 3
LND = 16
LN3 = 60
LNG = 16
SM0 = 200
SMD = 16
SMB = 140
VDL = 60
DL_D = 100
CV0 = 450
CVI = 170
CVE = 30
CVX = 180
CAP = 42
SMO = 32
WA = 7
WC = 11
WQ = 40
EC0 = 1500
ECD = 900


def _iota(shape, dim):
    return lax.broadcasted_iota(jnp.int32, shape, dim)


def _plan(nwin, w0, w1, nt, cur, prev):
    a_q = [(t, r) for t in range(nt) for r in range(WS)] if cur else []
    c_q = [(h, r) for h in range(2) for r in range(WS)] if prev else []
    old = [(-1, w) for w in range(w0, nwin)] if prev else []
    new = [(0, w) for w in range(w1)] if cur else []
    ws = old + old[-1:] * ((len(old) + len(new)) % 2) + new
    pairs = list(zip(ws[0::2], ws[1::2]))
    n1 = sum(a[0] < 0 for a, _ in pairs)
    nh = sum(a[0] < 0 and WS * a[1] < nt * LANES // 2 for a, _ in pairs)
    total = len(a_q) * DA + len(c_q) * DC + len(pairs) * (DQ + DP)
    q0 = 0 if prev else total // 5
    t = 0
    ia = ic = iq = ip = 0
    out = []
    tq, tp, ta = {}, {}, {}
    last = None
    while ia < len(a_q) or ic < len(c_q) or ip < len(pairs):
        cands = []
        if ip < iq and t >= tq[ip] + LAT_QK:
            cands.append((-1e6, 'pv'))
        if iq < len(pairs) and (not cur or (iq - ip < 2 and last not in ('qk', 'pv'))):
            ok = iq - ip < 4
            if pairs[iq][1][0] == 0:
                need = (WS * pairs[iq][1][1] + WS) // LANES * WS + WS - 1
                ok = ia > need and t >= ta[need] + DA + DL_A + 60 and ic >= len(c_q) // 2
            if ok:
                pr = q0 + iq * (total - q0 - TAIL) / len(pairs) - t - 200
                cands.append((-2e6 if pr <= 0 else pr, 'qk'))
        if ia < len(a_q):
            cands.append((ia * (total - 700) / len(a_q) - t, 'a'))
        if ic < len(c_q):
            need = nh - 1 if ic < WS else n1 - 1
            if ip > need and t >= tp[need] + DL_PV + PRE_C:
                if cur:
                    tc = 1000 + ic * 900 if ic < WS else total - DC - (2 * WS - 1 - ic) * 950
                else:
                    tc = EC0 + ic * ECD
                cands.append((tc - t, 'c'))
        if not cands:
            t += 8
            last = None
            continue
        last = kind = min(cands)[1]
        if kind == 'pv':
            out.append((t, kind, pairs[ip]))
            tp[ip], ip, t = t, ip + 1, t + DP
        elif kind == 'qk':
            out.append((t, kind, pairs[iq]))
            tq[iq], iq, t = t, iq + 1, t + DQ
        elif kind == 'a':
            out.append((t, kind, a_q[ia]))
            ta[ia], ia, t = t, ia + 1, t + DA
        else:
            out.append((t, kind, c_q[ic]))
            ic, t = ic + 1, t + DC
    return out, t


def _tree_sum(xs):
    while len(xs) > 1:
        xs = [xs[j] + xs[j + 1] if j + 1 < len(xs) else xs[j] for j in range(0, len(xs), 2)]
    return xs[0]


def _sum8(x):
    while x.shape[0] % 16 == 0:
        x = x[:x.shape[0] // 2] + x[x.shape[0] // 2:]
    return _tree_sum(_rows8(x))


def _fold7(op, x):
    t = op(x[0:24], x[24:48])
    return op(op(t[0:8], t[8:16]), op(t[16:24], x[48:56]))


def _all8(op, x):
    for sh in (4, 2, 1):
        x = op(x, pltpu.roll(x, sh, 0))
    return x


def _rows8(x):
    return [x[8 * j:8 * j + 8] for j in range(x.shape[0] // 8)]


def _cat(xs, axis=0):
    return jnp.concatenate(xs, axis=axis) if len(xs) > 1 else xs[0]


def _f32(u):
    return pltpu.bitcast(u, F32)


def _u32(x):
    return pltpu.bitcast(x, U32)


def _kernel(x_hbm, dw_hbm, wqkv_hbm, wo_hbm, o_hbm,
            xa_s, xb_s, xc_s, q_s, k_s, v_s, o_s, wq_s, wo_s, sa_s, sb_s, dw_s,
            i0_s, i1_s, i2_s, o0_s, o1_s, o2_s, va_s, vb_s, vc_s, vd_s,
            dw_ref, wqkv_ref, wo_ref, in_sem, out_sem, w_sem, *, C, H, W, WP, NWIN):
    g = pl.program_id(0)
    ng = pl.num_programs(0)
    dh = C // NH
    CW = C // 2
    NT = WP // LANES
    G = WS * 8
    HW = WP // 2
    NC = C // 16
    NR = WS + 2
    lane8 = _iota((8, LANES), 1)
    last_valid = W - (NT - 1) * LANES
    zero = jnp.uint32(0)
    hi = jnp.uint32(0xFFFF0000)
    qkv_s = (q_s, k_s, v_s)
    xbuf = (xa_s, xb_s, xc_s)
    xin = (i0_s, i1_s, i2_s)
    xout = (o0_s, o1_s, o2_s)

    def row0(k, m):
        return (m & 1) * WS if k == NSUB - 1 else 0

    def in_copies(k, m):
        r = WS * (NSUB * m - 1 + k) + 1
        return [pltpu.make_async_copy(x_hbm.at[pl.ds(jnp.minimum(r + o, H - n), n)],
                                      xin[k].at[pl.ds(row0(k, m) + o, n)], in_sem.at[k])
                for o, n in ((0, WS - 1), (WS - 1, 1))]

    def in_wait(k, m):
        dst = xin[k].at[pl.ds(row0(k, m), WS)]
        pltpu.make_async_copy(dst, dst, in_sem.at[k]).wait()

    def out_copy(k, m, o=0, n=WS):
        return pltpu.make_async_copy(xout[k].at[pl.ds(row0(k, m) + o, n)],
                                     o_hbm.at[pl.ds(WS * (NSUB * (m - 1) + k) + o, n)],
                                     out_sem.at[k + (m & 1) if k == NSUB - 1 else k])

    stg = (sa_s, sb_s)
    vts = (va_s, vb_s, vc_s, vd_s)
    SPARE = sa_s.shape[0] - 1
    zx = g >> 10
    zy = g >> 11
    never = lane8 < zx

    def tie(x, toks):
        if not toks:
            return x
        tok = functools.reduce(lax.bitwise_or, toks)
        n = x.shape[1]
        return lax.select(never[:, 0:n], tok[:, 0:n], x) if n < LANES else lax.select(never, tok, x)

    def stg_row(j, c2, rho):
        if 2 <= rho < WS:
            return rho - 2
        slot = j % NSUB if rho >= WS else (j - 1) % NSUB
        return WS - 2 + (slot * (NC // 2) + c2) * 2 + rho % WS

    zt = jnp.zeros((8, LANES), U32)
    is_first, is_last = lane8 == 0, lane8 == LANES - 1

    def shifted(u):
        tiles = [u[:, LANES * t:LANES * (t + 1)] for t in range(NT)]
        tiles[NT - 1] = _cat([tiles[NT - 1], zt[:, last_valid:]], axis=1)
        left = [pltpu.roll(lax.select(is_last, tiles[t - 1] if t > 0 else zt, tiles[t]), 1, 1)
                for t in range(NT)]
        right = [pltpu.roll(lax.select(is_first, tiles[t + 1], tiles[t]) if t < NT - 1 else tiles[t], LANES - 1, 1)
                 for t in range(NT)]
        return _cat([v[t] for t in range(NT) for v in (left, tiles, right)])

    def unpack(v, hf):
        return pltpu.bitcast(v, BF16).astype(F32).reshape(3, 2, 8, LANES)[:, hf]

    def conv_row(un, w, r):
        return jnp.sum(_tree_sum([un[r + ki] * w[ki] for ki in range(3) if un[r + ki] is not None]), axis=0)

    def setup():
        wcp = [pltpu.make_async_copy(src, dst, w_sem.at[n])
               for n, (src, dst) in enumerate(((dw_hbm, dw_ref), (wqkv_hbm, wqkv_ref), (wo_hbm, wo_ref)))]

        def top(c2):
            cs = pl.ds(pl.multiple_of(32 * c2, 32), 32)
            return pltpu.make_async_copy(x_hbm.at[pl.ds(0, WS + 1), cs], i1_s.at[:, cs], w_sem.at[3 + c2])
        for cp in wcp + [top(c2) for c2 in range(NC // 2)]:
            cp.start()

        def zrow(r, carry):
            for ref in (k_s, o_s):
                ref[r, 0:WP, :] = jnp.zeros((WP, LANES), U32)
            return carry
        lax.fori_loop(0, WS, zrow, 0)
        for ref in (q_s, v_s):
            ref[0, 0:8, :] = zt
        for ref in stg:
            ref[SPARE, 0:16, :] = jnp.zeros((16, LANES), U32)
        for ref in vts:
            ref[1, 0:8, :] = zt
        wo_s[...] = jnp.zeros(wo_s.shape, U32)
        for cp in wcp:
            cp.wait()
        for ki in range(3):
            w3 = dw_ref[ki].astype(F32)
            for kj in range(3):
                w = w3[kj:kj + 1] + 1.0 if ki == kj == 1 else w3[kj:kj + 1]
                dw_s[:, ki, kj] = jnp.broadcast_to(w, (LANES, C)).T.reshape(C // 8, 8, LANES)
        qscale = (dh ** -0.5) * math.log2(math.e)
        for kt in range(2):
            wt = wqkv_ref[CW * kt:CW * (kt + 1), :].astype(F32).T
            wq = (wt[0:C] * qscale).astype(BF16).astype(F32)
            words = [(_u32(w[0:CW]) >> 16) | (_u32(w[CW:C]) & hi) for w in (wq, wt[C:2 * C])]
            words = _rows8(_cat(words + [_u32(wt[2 * C:].astype(BF16))]))
            for par in range(2):
                wq_s[par, :, LANES * kt:LANES * kt + CW] = _cat(words[par::2])
        wo = _u32(wo_ref[...])
        for kt, w in enumerate((wo << 16, wo & hi)):
            wo_s[:, LANES * kt:LANES * kt + CW] = _u32(_f32(w.T).astype(BF16))

        def conv0(c2, carry):
            top(c2).wait()

            @pl.when(c2 == 2)
            def _():
                for cp in in_copies(2, 0):
                    cp.start()
            for par in range(2):
                cs = pl.ds(pl.multiple_of(32 * c2 + 16 * par, 16), 16)
                sh = [shifted(_u32(i1_s[r, cs, :])) for r in range(WS + 1)]
                for rho in (WS, WS + 1):
                    stg[par][stg_row(-1, c2, rho)] = sh[rho - 1]
                for hf in range(2):
                    c8 = 4 * c2 + 2 * par + hf
                    w = [dw_s[c8, ki] for ki in range(3)]
                    for t in range(NT):
                        un = [None] + [unpack(row[24 * t:24 * t + 24], hf) for row in sh]
                        for r in range(WS):
                            xbuf[0][r, t, pl.ds(pl.multiple_of(8 * c8, 8), 8), :] = conv_row(un, w, r)
            return carry
        lax.fori_loop(0, NC // 2, conv0, 0)
        for cp in in_copies(0, 1) + in_copies(1, 1):
            cp.start()
        in_wait(2, 0)
        for cp in in_copies(2, 1):
            cp.start()

    def body(subs):
        lane3 = _iota((WS, 8, LANES), 2)
        head = (lane3 < dh, (lane3 >= dh) & (lane3 < 2 * dh))
        zq = jnp.zeros((WS, 8, LANES), F32)
        junk8 = _iota((8, 2 * G), 0) == WS
        ninf8 = jnp.full((8, 2 * G), -jnp.inf, F32)
        key_ok = tuple((_iota((WS + 1, 8, 2 * G), 2) & 8) == 8 * hh for hh in range(2))
        zp = jnp.zeros((WS + 1, 8, 2 * G), F32)
        first_half = (_iota((8, 2 * G), 1) & 8) == 0
        even_head = (_iota((WS, 8, CW), 2) // (dh // 2)) % 2 == 0
        wsp = (HW - 1) // WS

        st = {}
        toks = []
        soft = []
        ticks = []
        j0 = subs[0][0]
        tag = {('qkv', t, r): -1 for t in range(NT) for r in range(WS)}
        tag.update({('o', w): (-1 if w < wsp else None) for w in range(NWIN)})
        dirty = {wsp}
        for b, blk in ((j0 % 3, 0), ((j0 + 2) % 3, -1)):
            tag.update({('x', b, c, t, r): blk for c in range(2 * NC) for t in range(NT) for r in range(WS)})
        tag.update({('s', c % 2, stg_row(j0, c // 2, rho)): (0, c, rho) for c in range(NC) for rho in (0, 1)})

        def gather(ref, w):
            return ref[:, pl.ds(WS * w, 8), :]

        def tick(t):
            c = [x for x in ticks if t <= x[0] <= t + 40]
            if not c:
                return None
            _, res, j = min(c, key=lambda x: x[0])
            return res[8 * j:8 * j + 8, 0:LANES]

        def tock(t):
            c = [x for x in ticks if x[0] <= t]
            if not c:
                return None
            _, res, j = max(c, key=lambda x: x[0])
            return res[8 * j:8 * j + 8, 0:LANES]

        def due(lst, nblk, t0, step):
            inj = {}
            for d, tok in list(lst):
                j = max(0, -(-(d - t0) // step))
                if j < nblk and d >= 0:
                    inj.setdefault(j, []).append(tok)
            lst[:] = [x for x in lst if x[0] > t0 + (nblk - 1) * step]
            return inj

        def lhs(ref, ls, inj, dt):
            nblk = ref.shape[0] // 8
            parts, s = [], 0
            for j in sorted(inj):
                if j > s:
                    parts.append(ref[8 * s:8 * j, ls])
                parts.append(tie(ref[8 * j:8 * j + 8, ls], inj[j]))
                s = j + 1
            if s < nblk:
                parts.append(ref[8 * s:8 * nblk, ls])
            return pltpu.bitcast(_cat(parts), dt)

        def clamp(t, dl, dmin):
            return max(t + dmin, min(t + dl, total - 16))

        def merged(a, b):
            return {j: a.get(j, []) + b.get(j, []) for j in set(a) | set(b)}

        def fence(d, b):
            z = tock(d)
            if z is not None:
                xbuf[b][zx + WS, 0, 0:8, :] = z

        def ln1(d, k, t, r):
            b = subs[k][0] % 3
            assert all(tag['x', b, c, t, r] == k for c in range(2 * NC))
            s8 = _sum8(xbuf[b][r, t, 0:C, :])
            soft.append((d, _u32(s8)))
            mean = jnp.sum(s8, axis=0, keepdims=True) * (1.0 / C)
            fence(d + LNG, b)
            st['ln', k, t, r] = [xbuf[b][r, t, 0:C, :] - mean, [], mean]

        def ln3(d, k, t, r):
            b = subs[k][0] % 3
            fence(d, b)
            st['ln', k, t, r][0] = xbuf[b][r, t, 0:C, :] - st['ln', k, t, r][2]

        def ln2(d, n, *key):
            m = C // LNS
            xc = st[('ln',) + key][0][m * n:m * (n + 1)]
            s8 = _sum8(xc * xc)
            soft.append((d, _u32(s8)))
            st[('ln',) + key][1].append(s8)

        def a_dot(t0, k, t, r):
            xc, sq, _ = st.pop(('ln', k, t, r))
            var = jnp.sum(_tree_sum(sq), axis=0, keepdims=True) * (1.0 / C)
            h = xc * lax.rsqrt(var + EPS)
            h = [h[CW * kt:CW * (kt + 1)].astype(BF16) for kt in range(2)]
            inj = due(toks, DA // 16, t0, 16)
            inj0 = merged(inj, due(soft, DA // 16, t0, 16))
            part = [jnp.dot(lhs(wq_s.at[par], slice(LANES * kt, LANES * kt + CW), inj if par or kt else inj0, BF16),
                            h[kt], preferred_element_type=F32)
                    for par in range(2) for kt in range(2)]
            res = [part[0] + part[1], part[2] + part[3]]
            ticks.extend((t0 + MXU_LAT + 8 * j, res[0], j) for j in range(DA // 8))
            qkv = jnp.stack([v.reshape(-1, 16, LANES) for v in res], axis=1).reshape(3 * C, LANES)
            for m in range(3):
                qkv_s[m][r, LANES * t:LANES * (t + 1), 0:CW] = _u32(qkv[C * m:C * (m + 1)].astype(BF16)).T
                toks.append((clamp(t0 + 96 * (m + 1), DL_A, 350), qkv_s[m][zx, 0:8, :]))
            tag['qkv', t, r] = k

        def b_qk(t0, k, p):
            (_, wa), (_, wb) = p
            assert all(tag['qkv', t, r] == k + rel for r in range(WS) for rel, w in p
                       for t in range(WS * w // LANES, min(WS * w + WS, WP - 1) // LANES + 1))
            sts = []
            inj = due(soft, WS, t0, 8)
            for w, swap in ((wa, 0), (wb, 1)):
                qw = gather(q_s, w)
                kw = gather(k_s, w).reshape(G, LANES)
                if not swap and inj:
                    kw = _cat([tie(v, inj.get(r, [])) for r, v in enumerate(_rows8(kw))])
                for tile in range(2):
                    kk = _f32(kw & hi if tile else kw << 16)
                    qq = _f32(qw & hi if tile else qw << 16)
                    qst = jnp.stack([lax.select(head[swap], qq, zq), lax.select(head[1 - swap], qq, zq)], axis=1)
                    sts.append(lax.dot_general(kk, qst.reshape(2 * G, LANES).astype(BF16), (((1,), (1,)), ((), ())),
                                               preferred_element_type=F32))
            vw = _cat([gather(v_s, wa), zt[None], gather(v_s, wb), zt[None]]).reshape(LANES, LANES)
            st['nv'] = (st.get('nv', 0) + 1) % len(vts)
            ref = vts[st['nv']]
            assert all(v[1] is not ref for key, v in st.items() if key[0] == 's')
            ref[0] = vw[:, 0:CW].T
            soft.append((tpv[k, p] - VDL, ref[zx + 1, 0:8, :]))
            st['s', p] = (sts, ref)

        def b_pv(t0, tg, k, p):
            (_, wa), (_, wb) = p
            sts, ref = st.pop(('s', p))
            ref[zx + 1, 8:16, :] = zt
            vt = lhs(ref.at[0], slice(0, LANES), due(soft, 3, t0, 16), BF16)
            pts = []
            rinv = []
            for n, s_t in enumerate(sts):
                m8 = _fold7(jnp.maximum, s_t)
                mx = _all8(jnp.maximum, lax.select(junk8, ninf8, m8))
                mv = lax.select(junk8, -ninf8, mx)
                z = tick(tg + SMD * (3 - n))
                if z is not None:
                    mv = tie(mv, [z])
                eg = jnp.exp2(s_t.reshape(WS, 8, 2 * G) - mv)
                rinv.append(_fold7(jnp.add, eg.reshape(G, 2 * G)))
                pts.append(_cat([eg, eg[WS - 1:WS]]))
            for n in range(4):
                den = _all8(jnp.add, rinv[n])
                r0 = pl.reciprocal(den, approx=True)
                rinv[n] = r0 * (2.0 - den * r0)
            rsel = [lax.select(first_half, rinv[n], rinv[(n + 2) % 4]) for n in range(4)]
            outs = []
            for tile in range(2):
                for hh in range(2):
                    h = 2 * tile + hh
                    stn = _cat([lax.select(key_ok[hh], pts[tile], zp), lax.select(key_ok[1 - hh], pts[2 + tile], zp)])
                    ot = jnp.dot(vt[dh * h:dh * (h + 1), :], stn.reshape(-1, 2 * G).astype(BF16),
                                 preferred_element_type=F32)
                    outs.append(ot.reshape(dh // 8, 8, 2 * G) * rsel[2 * hh + tile])
            tw = _u32(_cat(outs).reshape(C, 2 * G).astype(BF16)).T.reshape(WS, 2, 8, CW)
            tw = (tw[:, 0], tw[:, 1])
            o_s[:, pl.ds(WS * wa, 8), 0:CW] = lax.select(even_head, tw[0], tw[1])
            if wb != wa:
                o_s[:, pl.ds(WS * wb, 8), 0:CW] = lax.select(even_head, tw[1], tw[0])
            toks.append((clamp(t0, DL_PV, 480), o_s[zx, 0:8, :]))
            for rel, w in p:
                tag['o', w] = k + rel
                dirty.discard(w)
                dirty.add(w + 1)

        def c_dot(t0, k, h, r):
            b = (subs[k][0] + 2) % 3
            assert all(tag['o', w] == k - 1 and not (w in dirty and WS * w >= HW * h)
                       for w in range(HW * h // WS, min((HW * h + HW - 1) // WS + 1, NWIN)))
            assert all(tag['x', b, c, t, r] == k - 1 for c in range(2 * NC) for t in (2 * h, 2 * h + 1))
            ow = o_s[r, HW * h:HW * (h + 1), :]
            inj = due(toks, DC // 16, t0, 16)
            inj = (merged(inj, due(soft, DC // 16, t0, 16)), inj)
            res = [lax.dot_general(lhs(wo_s, slice(LANES * kt, LANES * (kt + 1)), inj[kt], BF16),
                                   _f32(ow & hi if kt else ow << 16).astype(BF16),
                                   (((1,), (1,)), ((), ())), preferred_element_type=F32) for kt in range(2)]
            res = res[0] + res[1]
            ticks.extend((t0 + MXU_LAT + 8 * j, res, j) for j in range(DC // 8))
            slot = subs[k][2]
            n = min(HW, W - HW * h)
            x0 = _cat([xbuf[b][r, t, 0:C, :] for t in (2 * h, 2 * h + 1)], axis=1)
            xout[slot][row0(slot, g) + r, :, HW * h:HW * h + n] = (x0 + res)[:, 0:n].astype(BF16)
            if h == 1 and not subs[k][3]:
                out_copy(slot, g, r, 1).start()
            elif h == 1 and r == WS - 1:
                start_by(t0 + MXU_LAT + DC + DL_D, [out_copy(slot, g)], xout[slot])

        def start_by(d, copies, ref):
            for cp in copies:
                cp.start()
            spare = ref.shape[0] - 1
            ref[zx + spare, 0:16, 0:LANES] = jnp.zeros((16, LANES), BF16)
            soft.append((d, _u32(ref[zy + spare, 0:16, 0:LANES])))

        def refill(d, slot):
            start_by(d, in_copies(slot, g + 1), xin[slot])

        def stage_row(d, k, c, rho):
            j, slot = subs[k][0:2]
            cs = slice(16 * c, 16 * c + 16)
            u = _u32(xin[slot][row0(slot, g) + rho - 2, cs, :])
            if rho == WS + 1 and slot == 1:
                u = jnp.where(g < ng - 2, u, zero)
            idx = stg_row(j, c // 2, rho)
            stg[c % 2][idx] = shifted(u)
            soft.append((d, stg[c % 2][zx + SPARE, 8:16, 0:LANES]))
            tag['s', c % 2, idx] = (k, c, rho)
            if c == NC - 1 and rho == WS + 1 and slot < NSUB - 1:
                refill(d + DL_D, slot)

        def conv_step(d, k, c, hf, t, r):
            j = subs[k][0]
            if r == 0:
                if t == 0:
                    z = tock(d - 30) if c == hf == 0 else None
                    stg[c % 2][zx + SPARE, 0:8, :] = zt if z is None else _u32(z)
                    st['w'] = [dw_s[2 * c + hf, ki] for ki in range(3)]
                st['un'] = {}
            un = st['un']
            for rho in range(r, r + 3):
                if rho not in un:
                    idx = stg_row(j, c // 2, rho)
                    assert tag['s', c % 2, idx] in ((k, c, rho), (k - 1, c, rho + WS))
                    un[rho] = unpack(stg[c % 2][idx, 24 * t:24 * t + 24, :], hf)
            acc = conv_row(un, st['w'], r)
            xbuf[(j + 1) % 3][r, t, 16 * c + 8 * hf:16 * c + 8 * hf + 8, :] = acc
            soft.append((d, _u32(acc)))
            tag['x', (j + 1) % 3, 2 * c + hf, t, r] = k + 1

        plan, offs = [], [0]
        for k, sub in enumerate(subs):
            pk, tk = _plan(NWIN, wsp - (k == 1), wsp - (k == 0 and len(subs) > 1), NT, sub[3], sub[4])
            plan += [(offs[k] + t, kind, k, idx) for t, kind, idx in pk]
            offs.append(offs[k] + tk)
        total = offs[-1]
        starts = [e[0] for e in plan]
        ev = []

        def at(t, fn, *a):
            ev.append((t, t, len(ev), fn, a))

        def before(d, fn, *a):
            ev.append((max([t for t in starts if t <= d], default=0) - 1, d, len(ev), fn, a))

        load = [0.0] * (total + 1000)
        tqk = {}
        tpv = {(k, idx): t for t, kind, k, idx in plan if kind == 'pv'}

        def add(t0, t1, n):
            for t in range(max(t0, 0), max(t1, 0)):
                load[t] += n / (t1 - t0)

        pend = 0
        for n_op, (t, kind, k, idx) in enumerate(plan):
            tr = t + MXU_LAT
            tp0 = max(starts[n_op - 2] if n_op > 1 else t - 64, pend)
            if kind == 'a':
                if idx == (0, 0) and k > 0:
                    before(t - LN1 - 1, fence, t - LN1 - 40, subs[k][0] % 3)
                before(t - LN1, ln1, t - LN1, k, *idx)
                for n in range(LNS):
                    d = t - LN2 - LND * (LNS - 1 - n)
                    before(d, ln2, d, n, k, *idx)
                    add(d - 16, d, 72 // LNS)
                before(t - LN3, ln3, t - LN3, k, *idx)
                at(t, a_dot, t, k, *idx)
                add(tr, tr + DA, WA * DA // 16)
                pend = t - LN3 + 32
                add(t - LN1 - 16, t - LN1, 32)
                add(t - LN2, t - LN3, 20)
                add(t - LN3, t - LN3 + 32, 60)
            elif kind == 'qk':
                at(t, b_qk, t, k, idx)
                tqk[idx] = t
                add(tp0, tp0 + 60, WQ)
                add(t - 8, t + DQ - 8, 28)
                add(tr, tr + DQ, 24)
                add(tr + DQ, tr + DQ + 16, 36)
                pend = tp0 + 60
            elif kind == 'pv':
                tg = max(tqk[idx] + SM0, t - SMB)
                at(t, b_pv, t, tg, k, idx)
                add(tg, tg + 4 * SMD + 16, 80)
                add(tr - 10, tr + 6, 46)
                add(tr, tr + DP, 36)
                add(t + 400, t + 460, 14)
                pend = tg + 4 * SMD + 16
            else:
                if idx == (0, 0) and k > 0:
                    at(t - 1, fence, t - 100, (subs[k][0] + 2) % 3)
                at(t, c_dot, t, k, *idx)
                add(tr, tr + DC, WC * DC // 16)
                add(tp0, tp0 + 64, 96)
                pend = tp0 + 64
        pre = [0.0]
        for v in load:
            pre.append(pre[-1] + v)
        nstep = NC * 2 * NT * WS
        prev_chunk = 10
        for k, sub in enumerate(subs):
            if not sub[3]:
                continue
            ta = offs[k] + (CVI if k else CV0) - 20
            tb = offs[k + 1] - (CVE if k == len(subs) - 1 else CVX)
            cap = CAP if sub[4] else 64
            free = [max(0.02, cap / 16 - (pre[t + SMO] - pre[max(t - SMO, 0)]) / (2 * SMO)) for t in range(ta, tb)]
            tot_free, acc, tstep = sum(free), 0.0, []
            for t, v in enumerate(free):
                acc += v
                while len(tstep) < nstep and acc >= (len(tstep) + 1) * tot_free / nstep - 1e-6:
                    tstep.append(ta + t)
            for n in range(nstep):
                before(tstep[n], conv_step, tstep[n], k, n // (2 * NT * WS), n // (NT * WS) % 2, n // WS % NT, n % WS)
            for c in range(NC):
                t1 = tstep[c * 2 * NT * WS] - 30
                t0 = prev_chunk + 120
                prev_chunk = t1 + 30
                for rho in range(2, NR):
                    d = t0 + (t1 - t0) * (rho - 2) // (NR - 3)
                    before(d, stage_row, d, k, c, rho)
        if len(subs) > 1:
            at(-10, refill, 200, NSUB - 1)
        ev.sort(key=lambda e: e[:3])
        for e in ev:
            e[3](*e[4])
        if subs[-1][3]:
            n = len(subs)
            assert all(tag['qkv', t, r] == n - 1 for t in range(NT) for r in range(WS))
            assert all(tag['o', w] == n - 1 and w not in dirty for w in range(wsp))

    @pl.when(g == 0)
    def _():
        setup()
        body([(0, 2, 0, True, False)])

    @pl.when(g > 0)
    def _():
        for k in range(NSUB):
            in_wait(k, g)

    @pl.when(g > 1)
    def _():
        for k in range(NSUB - 1):
            out_copy(k, g - 1).wait()

    @pl.when(g > 2)
    def _():
        out_copy(NSUB - 1, g - 2).wait()

    @pl.when((g > 0) & (g < ng - 1))
    def _():
        body([(1 + k, k, k, True, True) for k in range(NSUB)])

    @pl.when(g == ng - 1)
    def _():
        body([(1, 0, 0, False, True)])
        out_copy(NSUB - 1, g - 1).wait()
        for r in range(WS):
            out_copy(0, g, r, 1).wait()


@jax.jit
def pallas_standalone__window_attn_davit__vision_kernel(
    x: jax.Array,
    dw_pe: jax.Array,
    w_qkv: jax.Array,
    w_o: jax.Array,
):
    B, H, W, C = x.shape
    assert B == 1 and H % WS == 0 and W % WS == 0 and C == 192 and x.dtype == BF16
    WP = -(-(W + 1) // (2 * LANES)) * (2 * LANES)
    assert WP == 4 * LANES
    NWIN = W // WS
    NBLK = H // WS
    assert (NBLK - 1) % NSUB == 0
    NM = (NBLK - 1) // NSUB

    xt = jnp.transpose(x[0], (0, 2, 1))

    nstg = WS - 2 + NSUB * (C // 32) * 2 + 1
    kern = functools.partial(_kernel, C=C, H=H, W=W, WP=WP, NWIN=NWIN)
    out = pl.pallas_call(
        kern,
        grid=(NM + 2,),
        in_specs=[pl.BlockSpec(memory_space=pl.ANY)] * 4,
        out_specs=pl.BlockSpec(memory_space=pl.ANY),
        out_shape=jax.ShapeDtypeStruct((H, C, W), x.dtype),
        scratch_shapes=[
            pltpu.VMEM((WS + 1, WP // LANES, C + 8, LANES), F32),
            pltpu.VMEM((WS + 1, WP // LANES, C + 8, LANES), F32),
            pltpu.VMEM((WS + 1, WP // LANES, C + 8, LANES), F32),
            pltpu.VMEM((WS, WP + 8, LANES), U32),
            pltpu.VMEM((WS, WP + 8, LANES), U32),
            pltpu.VMEM((WS, WP + 8, LANES), U32),
            pltpu.VMEM((WS, WP + 8, LANES), U32),
            pltpu.VMEM((2, 3 * C // 4, 2 * LANES), U32),
            pltpu.VMEM((C // 2, 2 * LANES), U32),
            pltpu.VMEM((nstg, WP // LANES * 24, LANES), U32),
            pltpu.VMEM((nstg, WP // LANES * 24, LANES), U32),
            pltpu.VMEM((C // 8, 3, 3, 8, LANES), F32),
            pltpu.VMEM((WS + 1, C, W), BF16),
            pltpu.VMEM((WS + 1, C, W), BF16),
            pltpu.VMEM((2 * WS + 1, C, W), BF16),
            pltpu.VMEM((WS + 1, C, W), BF16),
            pltpu.VMEM((WS + 1, C, W), BF16),
            pltpu.VMEM((2 * WS + 1, C, W), BF16),
            pltpu.VMEM((2, C // 2, LANES), U32),
            pltpu.VMEM((2, C // 2, LANES), U32),
            pltpu.VMEM((2, C // 2, LANES), U32),
            pltpu.VMEM((2, C // 2, LANES), U32),
            pltpu.VMEM(dw_pe.shape, BF16),
            pltpu.VMEM(w_qkv.shape, BF16),
            pltpu.VMEM(w_o.shape, BF16),
            pltpu.SemaphoreType.DMA((NSUB,)),
            pltpu.SemaphoreType.DMA((NSUB + 1,)),
            pltpu.SemaphoreType.DMA((3 + C // 32,)),
        ],
        compiler_params=pltpu.CompilerParams(
            dimension_semantics=("arbitrary",),
            vmem_limit_bytes=96 * 1024 * 1024,
            disable_bounds_checks=True,
        ),
        name="davit_window_attn",
    )(xt, dw_pe, w_qkv, w_o)
    return jnp.transpose(out, (0, 2, 1))[None]
```

```python
import functools
import math

import jax
import jax.numpy as jnp
from jax import lax
import jax.experimental.pallas as pl
import jax.experimental.pallas.tpu as pltpu

WS = 7
NH = 4
EPS = 1e-05
LANES = 128
F32 = jnp.float32
BF16 = jnp.bfloat16
U32 = jnp.uint32
NSUB = 3

DA, DC, DQ, DP = 288, 192, 56, 48
MXU_LAT = 130
DL_A = 500
LAT_QK = 280
DL_PV = 580
PRE_C = 120
TAIL = 1400
LN1 = 200
LN2 = 130
LNS = 3
LND = 16
LN3 = 60
LNG = 16
SM0 = 200
SMD = 16
SMB = 140
VDL = 60
DL_D = 100
CV0 = 450
CVI = 170
CVE = 30
CVX = 180
CAP = 42
SMO = 32
WA = 7
WC = 11
WQ = 40
EC0 = 1500
ECD = 900


def _iota(shape, dim):
    return lax.broadcasted_iota(jnp.int32, shape, dim)


def _plan(nwin, w0, w1, nt, cur, prev):
    a_q = [(t, r) for t in range(nt) for r in range(WS)] if cur else []
    c_q = [(h, r) for h in range(2) for r in range(WS)] if prev else []
    old = [(-1, w) for w in range(w0, nwin)] if prev else []
    new = [(0, w) for w in range(w1)] if cur else []
    ws = old + old[-1:] * ((len(old) + len(new)) % 2) + new
    pairs = list(zip(ws[0::2], ws[1::2]))
    n1 = sum(a[0] < 0 for a, _ in pairs)
    nh = sum(a[0] < 0 and WS * a[1] < nt * LANES // 2 for a, _ in pairs)
    total = len(a_q) * DA + len(c_q) * DC + len(pairs) * (DQ + DP)
    q0 = 0 if prev else total // 5
    t = 0
    ia = ic = iq = ip = 0
    out = []
    tq, tp, ta = {}, {}, {}
    last = None
    while ia < len(a_q) or ic < len(c_q) or ip < len(pairs):
        cands = []
        if ip < iq and t >= tq[ip] + LAT_QK:
            cands.append((-1e6, 'pv'))
        if iq < len(pairs) and (not cur or (iq - ip < 2 and last not in ('qk', 'pv'))):
            ok = iq - ip < 4
            if pairs[iq][1][0] == 0:
                need = (WS * pairs[iq][1][1] + WS) // LANES * WS + WS - 1
                ok = ia > need and t >= ta[need] + DA + DL_A + 60 and ic >= len(c_q) // 2
            if ok:
                pr = q0 + iq * (total - q0 - TAIL) / len(pairs) - t - 200
                cands.append((-2e6 if pr <= 0 else pr, 'qk'))
        if ia < len(a_q):
            cands.append((ia * (total - 700) / len(a_q) - t, 'a'))
        if ic < len(c_q):
            need = nh - 1 if ic < WS else n1 - 1
            if ip > need and t >= tp[need] + DL_PV + PRE_C:
                if cur:
                    tc = 1000 + ic * 900 if ic < WS else total - DC - (2 * WS - 1 - ic) * 950
                else:
                    tc = EC0 + ic * ECD
                cands.append((tc - t, 'c'))
        if not cands:
            t += 8
            last = None
            continue
        last = kind = min(cands)[1]
        if kind == 'pv':
            out.append((t, kind, pairs[ip]))
            tp[ip], ip, t = t, ip + 1, t + DP
        elif kind == 'qk':
            out.append((t, kind, pairs[iq]))
            tq[iq], iq, t = t, iq + 1, t + DQ
        elif kind == 'a':
            out.append((t, kind, a_q[ia]))
            ta[ia], ia, t = t, ia + 1, t + DA
        else:
            out.append((t, kind, c_q[ic]))
            ic, t = ic + 1, t + DC
    return out, t


def _tree_sum(xs):
    while len(xs) > 1:
        xs = [xs[j] + xs[j + 1] if j + 1 < len(xs) else xs[j] for j in range(0, len(xs), 2)]
    return xs[0]


def _sum8(x):
    while x.shape[0] % 16 == 0:
        x = x[:x.shape[0] // 2] + x[x.shape[0] // 2:]
    return _tree_sum(_rows8(x))


def _fold7(op, x):
    t = op(x[0:24], x[24:48])
    return op(op(t[0:8], t[8:16]), op(t[16:24], x[48:56]))


def _all8(op, x):
    for sh in (4, 2, 1):
        x = op(x, pltpu.roll(x, sh, 0))
    return x


def _rows8(x):
    return [x[8 * j:8 * j + 8] for j in range(x.shape[0] // 8)]


def _cat(xs, axis=0):
    return jnp.concatenate(xs, axis=axis) if len(xs) > 1 else xs[0]


def _f32(u):
    return pltpu.bitcast(u, F32)


def _u32(x):
    return pltpu.bitcast(x, U32)


def _kernel(x_hbm, dw_hbm, wqkv_hbm, wo_hbm, o_hbm,
            xa_s, xb_s, xc_s, q_s, k_s, v_s, o_s, wq_s, wo_s, sa_s, sb_s, dw_s,
            i0_s, i1_s, i2_s, o0_s, o1_s, o2_s, va_s, vb_s, vc_s, vd_s,
            dw_ref, wqkv_ref, wo_ref, in_sem, out_sem, w_sem, *, C, H, W, WP, NWIN):
    g = pl.program_id(0)
    ng = pl.num_programs(0)
    dh = C // NH
    CW = C // 2
    NT = WP // LANES
    G = WS * 8
    HW = WP // 2
    NC = C // 16
    NR = WS + 2
    lane8 = _iota((8, LANES), 1)
    last_valid = W - (NT - 1) * LANES
    zero = jnp.uint32(0)
    hi = jnp.uint32(0xFFFF0000)
    qkv_s = (q_s, k_s, v_s)
    xbuf = (xa_s, xb_s, xc_s)
    xin = (i0_s, i1_s, i2_s)
    xout = (o0_s, o1_s, o2_s)

    def row0(k, m):
        return (m & 1) * WS if k == NSUB - 1 else 0

    def in_copies(k, m):
        r = WS * (NSUB * m - 1 + k) + 1
        return [pltpu.make_async_copy(x_hbm.at[pl.ds(jnp.minimum(r + o, H - n), n)],
                                      xin[k].at[pl.ds(row0(k, m) + o, n)], in_sem.at[k])
                for o, n in ((0, WS - 1), (WS - 1, 1))]

    def in_wait(k, m):
        dst = xin[k].at[pl.ds(row0(k, m), WS)]
        pltpu.make_async_copy(dst, dst, in_sem.at[k]).wait()

    def out_copy(k, m, o=0, n=WS):
        return pltpu.make_async_copy(xout[k].at[pl.ds(row0(k, m) + o, n)],
                                     o_hbm.at[pl.ds(WS * (NSUB * (m - 1) + k) + o, n)],
                                     out_sem.at[k + (m & 1) if k == NSUB - 1 else k])

    stg = (sa_s, sb_s)
    vts = (va_s, vb_s, vc_s, vd_s)
    SPARE = sa_s.shape[0] - 1
    zx = g >> 10
    zy = g >> 11
    never = lane8 < zx

    def tie(x, toks):
        if not toks:
            return x
        tok = functools.reduce(lax.bitwise_or, toks)
        n = x.shape[1]
        return lax.select(never[:, 0:n], tok[:, 0:n], x) if n < LANES else lax.select(never, tok, x)

    def stg_row(j, c2, rho):
        if 2 <= rho < WS:
            return rho - 2
        slot = j % NSUB if rho >= WS else (j - 1) % NSUB
        return WS - 2 + (slot * (NC // 2) + c2) * 2 + rho % WS

    zt = jnp.zeros((8, LANES), U32)
    is_first, is_last = lane8 == 0, lane8 == LANES - 1

    def shifted(u):
        tiles = [u[:, LANES * t:LANES * (t + 1)] for t in range(NT)]
        tiles[NT - 1] = _cat([tiles[NT - 1], zt[:, last_valid:]], axis=1)
        left = [pltpu.roll(lax.select(is_last, tiles[t - 1] if t > 0 else zt, tiles[t]), 1, 1)
                for t in range(NT)]
        right = [pltpu.roll(lax.select(is_first, tiles[t + 1], tiles[t]) if t < NT - 1 else tiles[t], LANES - 1, 1)
                 for t in range(NT)]
        return _cat([v[t] for t in range(NT) for v in (left, tiles, right)])

    def unpack(v, hf):
        return pltpu.bitcast(v, BF16).astype(F32).reshape(3, 2, 8, LANES)[:, hf]

    def conv_row(un, w, r):
        return jnp.sum(_tree_sum([un[r + ki] * w[ki] for ki in range(3) if un[r + ki] is not None]), axis=0)

    def setup():
        wcp = [pltpu.make_async_copy(src, dst, w_sem.at[n])
               for n, (src, dst) in enumerate(((dw_hbm, dw_ref), (wqkv_hbm, wqkv_ref), (wo_hbm, wo_ref)))]

        def top(c2):
            cs = pl.ds(pl.multiple_of(32 * c2, 32), 32)
            return pltpu.make_async_copy(x_hbm.at[pl.ds(0, WS + 1), cs], i1_s.at[:, cs], w_sem.at[3 + c2])
        for cp in wcp + [top(c2) for c2 in range(NC // 2)]:
            cp.start()

        def zrow(r, carry):
            for ref in (q_s, k_s, o_s):
                ref[r, 0:WP, :] = jnp.zeros((WP, LANES), U32)
            return carry
        lax.fori_loop(0, WS, zrow, 0)
        v_s[0, 0:8, :] = zt
        for ref in stg:
            ref[SPARE, 0:16, :] = jnp.zeros((16, LANES), U32)
        for ref in vts:
            ref[1, 0:8, :] = zt
        wo_s[...] = jnp.zeros(wo_s.shape, U32)
        for cp in wcp:
            cp.wait()
        for ki in range(3):
            w3 = dw_ref[ki].astype(F32)
            for kj in range(3):
                w = w3[kj:kj + 1] + 1.0 if ki == kj == 1 else w3[kj:kj + 1]
                dw_s[:, ki, kj] = jnp.broadcast_to(w, (LANES, C)).T.reshape(C // 8, 8, LANES)
        qscale = (dh ** -0.5) * math.log2(math.e)
        for kt in range(2):
            wt = wqkv_ref[CW * kt:CW * (kt + 1), :].astype(F32).T
            wq = (wt[0:C] * qscale).astype(BF16).astype(F32)
            words = [(_u32(w[0:CW]) >> 16) | (_u32(w[CW:C]) & hi) for w in (wq, wt[C:2 * C])]
            words = _rows8(_cat(words + [_u32(wt[2 * C:].astype(BF16))]))
            for par in range(2):
                wq_s[par, :, LANES * kt:LANES * kt + CW] = _cat(words[par::2])
        wo = _u32(wo_ref[...])
        for kt, w in enumerate((wo << 16, wo & hi)):
            wo_s[:, LANES * kt:LANES * kt + CW] = _u32(_f32(w.T).astype(BF16))

        def conv0(c2, carry):
            top(c2).wait()

            @pl.when(c2 == 2)
            def _():
                for cp in in_copies(2, 0):
                    cp.start()
            for par in range(2):
                cs = pl.ds(pl.multiple_of(32 * c2 + 16 * par, 16), 16)
                sh = [shifted(_u32(i1_s[r, cs, :])) for r in range(WS + 1)]
                for rho in (WS, WS + 1):
                    stg[par][stg_row(-1, c2, rho)] = sh[rho - 1]
                for hf in range(2):
                    c8 = 4 * c2 + 2 * par + hf
                    w = [dw_s[c8, ki] for ki in range(3)]
                    for t in range(NT):
                        un = [None] + [unpack(row[24 * t:24 * t + 24], hf) for row in sh]
                        for r in range(WS):
                            xbuf[0][r, t, pl.ds(pl.multiple_of(8 * c8, 8), 8), :] = conv_row(un, w, r)
            return carry
        lax.fori_loop(0, NC // 2, conv0, 0)
        for cp in in_copies(0, 1) + in_copies(1, 1):
            cp.start()
        in_wait(2, 0)
        for cp in in_copies(2, 1):
            cp.start()

    def body(subs):
        lane3 = _iota((WS, 8, LANES), 2)
        head = (lane3 < dh, (lane3 >= dh) & (lane3 < 2 * dh))
        zq = jnp.zeros((WS, 8, LANES), F32)
        zv = jnp.zeros((1, 8, CW), U32)
        junk8 = _iota((8, 2 * G), 0) == WS
        ninf8 = jnp.full((8, 2 * G), -jnp.inf, F32)
        key_ok = tuple((_iota((WS + 1, 8, 2 * G), 2) & 8) == 8 * hh for hh in range(2))
        zp = jnp.zeros((WS + 1, 8, 2 * G), F32)
        first_half = (_iota((8, 2 * G), 1) & 8) == 0
        even_head = (_iota((WS, 8, CW), 2) // (dh // 2)) % 2 == 0
        wsp = (HW - 1) // WS

        st = {}
        toks = []
        soft = []
        ticks = []
        j0 = subs[0][0]
        tag = {('qkv', t, r): -1 for t in range(NT) for r in range(WS)}
        tag.update({('o', w): (-1 if w < wsp else None) for w in range(NWIN)})
        dirty = {wsp}
        for b, blk in ((j0 % 3, 0), ((j0 + 2) % 3, -1)):
            tag.update({('x', b, c, t, r): blk for c in range(2 * NC) for t in range(NT) for r in range(WS)})
        tag.update({('s', c % 2, stg_row(j0, c // 2, rho)): (0, c, rho) for c in range(NC) for rho in (0, 1)})

        def gather(ref, w, n=LANES):
            return ref[:, pl.ds(WS * w, 8), 0:n]

        def tick(t):
            c = [x for x in ticks if t <= x[0] <= t + 40]
            if not c:
                return None
            _, res, j = min(c, key=lambda x: x[0])
            return res[8 * j:8 * j + 8, 0:LANES]

        def tock(t):
            c = [x for x in ticks if x[0] <= t]
            if not c:
                return None
            _, res, j = max(c, key=lambda x: x[0])
            return res[8 * j:8 * j + 8, 0:LANES]

        def due(lst, nblk, t0, step):
            inj = {}
            for d, tok in list(lst):
                j = max(0, -(-(d - t0) // step))
                if j < nblk and d >= 0:
                    inj.setdefault(j, []).append(tok)
            lst[:] = [x for x in lst if x[0] > t0 + (nblk - 1) * step]
            return inj

        def lhs(ref, ls, inj, dt):
            nblk = ref.shape[0] // 8
            parts, s = [], 0
            for j in sorted(inj):
                if j > s:
                    parts.append(ref[8 * s:8 * j, ls])
                parts.append(tie(ref[8 * j:8 * j + 8, ls], inj[j]))
                s = j + 1
            if s < nblk:
                parts.append(ref[8 * s:8 * nblk, ls])
            return pltpu.bitcast(_cat(parts), dt)

        def clamp(t, dl, dmin):
            return max(t + dmin, min(t + dl, total - 16))

        def merged(a, b):
            return {j: a.get(j, []) + b.get(j, []) for j in set(a) | set(b)}

        def fence(d, b):
            z = tock(d)
            if z is not None:
                xbuf[b][zx + WS, 0, 0:8, :] = z

        def ln1(d, k, t, r):
            b = subs[k][0] % 3
            assert all(tag['x', b, c, t, r] == k for c in range(2 * NC))
            s8 = _sum8(xbuf[b][r, t, 0:C, :])
            soft.append((d, _u32(s8)))
            mean = jnp.sum(s8, axis=0, keepdims=True) * (1.0 / C)
            fence(d + LNG, b)
            st['ln', k, t, r] = [xbuf[b][r, t, 0:C, :] - mean, [], mean]

        def ln3(d, k, t, r):
            b = subs[k][0] % 3
            fence(d, b)
            st['ln', k, t, r][0] = xbuf[b][r, t, 0:C, :] - st['ln', k, t, r][2]

        def ln2(d, n, *key):
            m = C // LNS
            xc = st[('ln',) + key][0][m * n:m * (n + 1)]
            s8 = _sum8(xc * xc)
            soft.append((d, _u32(s8)))
            st[('ln',) + key][1].append(s8)

        def a_dot(t0, k, t, r):
            xc, sq, _ = st.pop(('ln', k, t, r))
            var = jnp.sum(_tree_sum(sq), axis=0, keepdims=True) * (1.0 / C)
            h = xc * lax.rsqrt(var + EPS)
            h = [h[CW * kt:CW * (kt + 1)].astype(BF16) for kt in range(2)]
            inj = due(toks, DA // 16, t0, 16)
            inj0 = merged(inj, due(soft, DA // 16, t0, 16))
            part = [jnp.dot(lhs(wq_s.at[par], slice(LANES * kt, LANES * kt + CW), inj if par or kt else inj0, BF16),
                            h[kt], preferred_element_type=F32)
                    for par in range(2) for kt in range(2)]
            res = [part[0] + part[1], part[2] + part[3]]
            ticks.extend((t0 + MXU_LAT + 8 * j, res[0], j) for j in range(DA // 8))
            qkv = jnp.stack([v.reshape(-1, 16, LANES) for v in res], axis=1).reshape(3 * C, LANES)
            for m in range(3):
                qkv_s[m][r, LANES * t:LANES * (t + 1), 0:CW] = _u32(qkv[C * m:C * (m + 1)].astype(BF16)).T
                toks.append((clamp(t0 + 96 * (m + 1), DL_A, 350), qkv_s[m][zx, 0:8, :]))
            tag['qkv', t, r] = k

        def b_qk(t0, k, p):
            (_, wa), (_, wb) = p
            assert all(tag['qkv', t, r] == k + rel for r in range(WS) for rel, w in p
                       for t in range(WS * w // LANES, min(WS * w + WS, WP - 1) // LANES + 1))
            sts = []
            inj = due(soft, WS, t0, 8)
            for w, swap in ((wa, 0), (wb, 1)):
                qw = gather(q_s, w)
                kw = gather(k_s, w).reshape(G, LANES)
                if not swap and inj:
                    kw = _cat([tie(v, inj.get(r, [])) for r, v in enumerate(_rows8(kw))])
                for tile in range(2):
                    kk = _f32(kw & hi if tile else kw << 16)
                    qq = _f32(qw & hi if tile else qw << 16)
                    qst = jnp.stack([lax.select(head[swap], qq, zq), lax.select(head[1 - swap], qq, zq)], axis=1)
                    sts.append(lax.dot_general(kk, qst.reshape(2 * G, LANES).astype(BF16), (((1,), (1,)), ((), ())),
                                               preferred_element_type=F32))
            vw = _cat([gather(v_s, wa, CW), zv, gather(v_s, wb, CW), zv]).reshape(LANES, CW)
            st['nv'] = (st.get('nv', 0) + 1) % len(vts)
            ref = vts[st['nv']]
            assert all(v[1] is not ref for key, v in st.items() if key[0] == 's')
            ref[0] = vw.T
            soft.append((tpv[k, p] - VDL, ref[zx + 1, 0:8, :]))
            st['s', p] = (sts, ref)

        def b_pv(t0, tg, k, p):
            (_, wa), (_, wb) = p
            sts, ref = st.pop(('s', p))
            ref[zx + 1, 8:16, :] = zt
            vt = lhs(ref.at[0], slice(0, LANES), due(soft, 3, t0, 16), BF16)
            pts = []
            rinv = []
            for n, s_t in enumerate(sts):
                m8 = _fold7(jnp.maximum, s_t)
                mx = _all8(jnp.maximum, lax.select(junk8, ninf8, m8))
                mv = lax.select(junk8, -ninf8, mx)
                z = tick(tg + SMD * (3 - n))
                if z is not None:
                    mv = tie(mv, [z])
                eg = jnp.exp2(s_t.reshape(WS, 8, 2 * G) - mv)
                rinv.append(_fold7(jnp.add, eg.reshape(G, 2 * G)))
                pts.append(_cat([eg, eg[WS - 1:WS]]))
            for n in range(4):
                den = _all8(jnp.add, rinv[n])
                r0 = pl.reciprocal(den, approx=True)
                rinv[n] = r0 * (2.0 - den * r0)
            rsel = [lax.select(first_half, rinv[n], rinv[(n + 2) % 4]) for n in range(4)]
            outs = []
            for tile in range(2):
                for hh in range(2):
                    h = 2 * tile + hh
                    stn = _cat([lax.select(key_ok[hh], pts[tile], zp), lax.select(key_ok[1 - hh], pts[2 + tile], zp)])
                    ot = jnp.dot(vt[dh * h:dh * (h + 1), :], stn.reshape(-1, 2 * G).astype(BF16),
                                 preferred_element_type=F32)
                    outs.append(ot.reshape(dh // 8, 8, 2 * G) * rsel[2 * hh + tile])
            tw = _u32(_cat(outs).reshape(C, 2 * G).astype(BF16)).T.reshape(WS, 2, 8, CW)
            tw = (tw[:, 0], tw[:, 1])
            o_s[:, pl.ds(WS * wa, 8), 0:CW] = lax.select(even_head, tw[0], tw[1])
            if wb != wa:
                o_s[:, pl.ds(WS * wb, 8), 0:CW] = lax.select(even_head, tw[1], tw[0])
            toks.append((clamp(t0, DL_PV, 480), o_s[zx, 0:8, :]))
            for rel, w in p:
                tag['o', w] = k + rel
                dirty.discard(w)
                dirty.add(w + 1)

        def c_dot(t0, k, h, r):
            b = (subs[k][0] + 2) % 3
            assert all(tag['o', w] == k - 1 and not (w in dirty and WS * w >= HW * h)
                       for w in range(HW * h // WS, min((HW * h + HW - 1) // WS + 1, NWIN)))
            assert all(tag['x', b, c, t, r] == k - 1 for c in range(2 * NC) for t in (2 * h, 2 * h + 1))
            ow = o_s[r, HW * h:HW * (h + 1), :]
            inj = due(toks, DC // 16, t0, 16)
            inj = (merged(inj, due(soft, DC // 16, t0, 16)), inj)
            res = [lax.dot_general(lhs(wo_s, slice(LANES * kt, LANES * (kt + 1)), inj[kt], BF16),
                                   _f32(ow & hi if kt else ow << 16).astype(BF16),
                                   (((1,), (1,)), ((), ())), preferred_element_type=F32) for kt in range(2)]
            res = res[0] + res[1]
            ticks.extend((t0 + MXU_LAT + 8 * j, res, j) for j in range(DC // 8))
            slot = subs[k][2]
            n = min(HW, W - HW * h)
            x0 = _cat([xbuf[b][r, t, 0:C, :] for t in (2 * h, 2 * h + 1)], axis=1)
            xout[slot][row0(slot, g) + r, :, HW * h:HW * h + n] = (x0 + res)[:, 0:n].astype(BF16)
            if h == 1 and not subs[k][3]:
                out_copy(slot, g, r, 1).start()
            elif h == 1 and r == WS - 1:
                start_by(t0 + MXU_LAT + DC + DL_D, [out_copy(slot, g)], xout[slot])

        def start_by(d, copies, ref):
            for cp in copies:
                cp.start()
            spare = ref.shape[0] - 1
            ref[zx + spare, 0:16, 0:LANES] = jnp.zeros((16, LANES), BF16)
            soft.append((d, _u32(ref[zy + spare, 0:16, 0:LANES])))

        def refill(d, slot):
            start_by(d, in_copies(slot, g + 1), xin[slot])

        def stage_row(d, k, c, rho):
            j, slot = subs[k][0:2]
            cs = slice(16 * c, 16 * c + 16)
            u = _u32(xin[slot][row0(slot, g) + rho - 2, cs, :])
            if rho == WS + 1 and slot == 1:
                u = jnp.where(g < ng - 2, u, zero)
            idx = stg_row(j, c // 2, rho)
            stg[c % 2][idx] = shifted(u)
            soft.append((d, stg[c % 2][zx + SPARE, 8:16, 0:LANES]))
            tag['s', c % 2, idx] = (k, c, rho)
            if c == NC - 1 and rho == WS + 1 and slot < NSUB - 1:
                refill(d + DL_D, slot)

        def conv_step(d, k, c, hf, t, r):
            j = subs[k][0]
            if r == 0:
                if t == 0:
                    z = tock(d - 30) if c == hf == 0 else None
                    stg[c % 2][zx + SPARE, 0:8, :] = zt if z is None else _u32(z)
                    st['w'] = [dw_s[2 * c + hf, ki] for ki in range(3)]
                st['un'] = {}
            un = st['un']
            for rho in range(r, r + 3):
                if rho not in un:
                    idx = stg_row(j, c // 2, rho)
                    assert tag['s', c % 2, idx] in ((k, c, rho), (k - 1, c, rho + WS))
                    un[rho] = unpack(stg[c % 2][idx, 24 * t:24 * t + 24, :], hf)
            acc = conv_row(un, st['w'], r)
            xbuf[(j + 1) % 3][r, t, 16 * c + 8 * hf:16 * c + 8 * hf + 8, :] = acc
            soft.append((d, _u32(acc)))
            tag['x', (j + 1) % 3, 2 * c + hf, t, r] = k + 1

        plan, offs = [], [0]
        for k, sub in enumerate(subs):
            pk, tk = _plan(NWIN, wsp - (k == 1), wsp - (k == 0 and len(subs) > 1), NT, sub[3], sub[4])
            plan += [(offs[k] + t, kind, k, idx) for t, kind, idx in pk]
            offs.append(offs[k] + tk)
        total = offs[-1]
        starts = [e[0] for e in plan]
        ev = []

        def at(t, fn, *a):
            ev.append((t, t, len(ev), fn, a))

        def before(d, fn, *a):
            ev.append((max([t for t in starts if t <= d], default=0) - 1, d, len(ev), fn, a))

        load = [0.0] * (total + 1000)
        tqk = {}
        tpv = {(k, idx): t for t, kind, k, idx in plan if kind == 'pv'}

        def add(t0, t1, n):
            for t in range(max(t0, 0), max(t1, 0)):
                load[t] += n / (t1 - t0)

        pend = 0
        for n_op, (t, kind, k, idx) in enumerate(plan):
            tr = t + MXU_LAT
            tp0 = max(starts[n_op - 2] if n_op > 1 else t - 64, pend)
            if kind == 'a':
                if idx == (0, 0) and k > 0:
                    before(t - LN1 - 1, fence, t - LN1 - 40, subs[k][0] % 3)
                before(t - LN1, ln1, t - LN1, k, *idx)
                for n in range(LNS):
                    d = t - LN2 - LND * (LNS - 1 - n)
                    before(d, ln2, d, n, k, *idx)
                    add(d - 16, d, 72 // LNS)
                before(t - LN3, ln3, t - LN3, k, *idx)
                at(t, a_dot, t, k, *idx)
                add(tr, tr + DA, WA * DA // 16)
                pend = t - LN3 + 32
                add(t - LN1 - 16, t - LN1, 32)
                add(t - LN2, t - LN3, 20)
                add(t - LN3, t - LN3 + 32, 60)
            elif kind == 'qk':
                at(t, b_qk, t, k, idx)
                tqk[idx] = t
                add(tp0, tp0 + 60, WQ)
                add(t - 8, t + DQ - 8, 28)
                add(tr, tr + DQ, 24)
                add(tr + DQ, tr + DQ + 16, 36)
                pend = tp0 + 60
            elif kind == 'pv':
                tg = max(tqk[idx] + SM0, t - SMB)
                at(t, b_pv, t, tg, k, idx)
                add(tg, tg + 4 * SMD + 16, 80)
                add(tr - 10, tr + 6, 46)
                add(tr, tr + DP, 36)
                add(t + 400, t + 460, 14)
                pend = tg + 4 * SMD + 16
            else:
                if idx == (0, 0) and k > 0:
                    at(t - 1, fence, t - 100, (subs[k][0] + 2) % 3)
                at(t, c_dot, t, k, *idx)
                add(tr, tr + DC, WC * DC // 16)
                add(tp0, tp0 + 64, 96)
                pend = tp0 + 64
        pre = [0.0]
        for v in load:
            pre.append(pre[-1] + v)
        nstep = NC * 2 * NT * WS
        prev_chunk = 10
        for k, sub in enumerate(subs):
            if not sub[3]:
                continue
            ta = offs[k] + (CVI if k else CV0) - 20
            tb = offs[k + 1] - (CVE if k == len(subs) - 1 else CVX)
            cap = CAP if sub[4] else 64
            free = [max(0.02, cap / 16 - (pre[t + SMO] - pre[max(t - SMO, 0)]) / (2 * SMO)) for t in range(ta, tb)]
            tot_free, acc, tstep = sum(free), 0.0, []
            for t, v in enumerate(free):
                acc += v
                while len(tstep) < nstep and acc >= (len(tstep) + 1) * tot_free / nstep - 1e-6:
                    tstep.append(ta + t)
            for n in range(nstep):
                before(tstep[n], conv_step, tstep[n], k, n // (2 * NT * WS), n // (NT * WS) % 2, n // WS % NT, n % WS)
            for c in range(NC):
                t1 = tstep[c * 2 * NT * WS] - 30
                t0 = prev_chunk + 120
                prev_chunk = t1 + 30
                for rho in range(2, NR):
                    d = t0 + (t1 - t0) * (rho - 2) // (NR - 3)
                    before(d, stage_row, d, k, c, rho)
        if len(subs) > 1:
            at(-10, refill, 200, NSUB - 1)
        ev.sort(key=lambda e: e[:3])
        for e in ev:
            e[3](*e[4])
        if subs[-1][3]:
            n = len(subs)
            assert all(tag['qkv', t, r] == n - 1 for t in range(NT) for r in range(WS))
            assert all(tag['o', w] == n - 1 and w not in dirty for w in range(wsp))

    @pl.when(g == 0)
    def _():
        setup()
        body([(0, 2, 0, True, False)])

    @pl.when(g > 0)
    def _():
        for k in range(NSUB):
            in_wait(k, g)

    @pl.when(g > 1)
    def _():
        for k in range(NSUB - 1):
            out_copy(k, g - 1).wait()

    @pl.when(g > 2)
    def _():
        out_copy(NSUB - 1, g - 2).wait()

    @pl.when((g > 0) & (g < ng - 1))
    def _():
        body([(1 + k, k, k, True, True) for k in range(NSUB)])

    @pl.when(g == ng - 1)
    def _():
        body([(1, 0, 0, False, True)])
        out_copy(NSUB - 1, g - 1).wait()
        for r in range(WS):
            out_copy(0, g, r, 1).wait()


@jax.jit
def pallas_standalone__window_attn_davit__vision_kernel(
    x: jax.Array,
    dw_pe: jax.Array,
    w_qkv: jax.Array,
    w_o: jax.Array,
):
    B, H, W, C = x.shape
    assert B == 1 and H % WS == 0 and W % WS == 0 and C == 192 and x.dtype == BF16
    WP = -(-(W + 1) // (2 * LANES)) * (2 * LANES)
    assert WP == 4 * LANES
    NWIN = W // WS
    NBLK = H // WS
    assert (NBLK - 1) % NSUB == 0
    NM = (NBLK - 1) // NSUB

    xt = jnp.transpose(x[0], (0, 2, 1))

    nstg = WS - 2 + NSUB * (C // 32) * 2 + 1
    kern = functools.partial(_kernel, C=C, H=H, W=W, WP=WP, NWIN=NWIN)
    out = pl.pallas_call(
        kern,
        grid=(NM + 2,),
        in_specs=[pl.BlockSpec(memory_space=pl.ANY)] * 4,
        out_specs=pl.BlockSpec(memory_space=pl.ANY),
        out_shape=jax.ShapeDtypeStruct((H, C, W), x.dtype),
        scratch_shapes=[
            pltpu.VMEM((WS + 1, WP // LANES, C + 8, LANES), F32),
            pltpu.VMEM((WS + 1, WP // LANES, C + 8, LANES), F32),
            pltpu.VMEM((WS + 1, WP // LANES, C + 8, LANES), F32),
            pltpu.VMEM((WS, WP + 8, LANES), U32),
            pltpu.VMEM((WS, WP + 8, LANES), U32),
            pltpu.VMEM((WS, WP + 8, LANES), U32),
            pltpu.VMEM((WS, WP + 8, LANES), U32),
            pltpu.VMEM((2, 3 * C // 4, 2 * LANES), U32),
            pltpu.VMEM((C // 2, 2 * LANES), U32),
            pltpu.VMEM((nstg, WP // LANES * 24, LANES), U32),
            pltpu.VMEM((nstg, WP // LANES * 24, LANES), U32),
            pltpu.VMEM((C // 8, 3, 3, 8, LANES), F32),
            pltpu.VMEM((WS + 1, C, W), BF16),
            pltpu.VMEM((WS + 1, C, W), BF16),
            pltpu.VMEM((2 * WS + 1, C, W), BF16),
            pltpu.VMEM((WS + 1, C, W), BF16),
            pltpu.VMEM((WS + 1, C, W), BF16),
            pltpu.VMEM((2 * WS + 1, C, W), BF16),
            pltpu.VMEM((2, C // 2, LANES), U32),
            pltpu.VMEM((2, C // 2, LANES), U32),
            pltpu.VMEM((2, C // 2, LANES), U32),
            pltpu.VMEM((2, C // 2, LANES), U32),
            pltpu.VMEM(dw_pe.shape, BF16),
            pltpu.VMEM(w_qkv.shape, BF16),
            pltpu.VMEM(w_o.shape, BF16),
            pltpu.SemaphoreType.DMA((NSUB,)),
            pltpu.SemaphoreType.DMA((NSUB + 1,)),
            pltpu.SemaphoreType.DMA((3 + C // 32,)),
        ],
        compiler_params=pltpu.CompilerParams(
            dimension_semantics=("arbitrary",),
            vmem_limit_bytes=64 * 1024 * 1024,
            disable_bounds_checks=True,
        ),
        name="davit_window_attn",
    )(xt, dw_pe, w_qkv, w_o)
    return jnp.transpose(out, (0, 2, 1))[None]
```
